```python
import jax
import jax.numpy as jnp

def _softmax(x, axis=-1):
    return jax.nn.softmax(x, axis=axis)
def _gelu(x):
    return jax.nn.gelu(x, approximate=True)
def _silu(x):
    return jax.nn.silu(x)
def _sigmoid(x):
    return jax.nn.sigmoid(x)
def _layernorm(x, axis=-1, eps=1e-5):
    m = jnp.mean(x, axis=axis, keepdims=True)
    v = jnp.var(x, axis=axis, keepdims=True)
    return (x - m) / jnp.sqrt(v + eps)
def _scatter_add(tgt, idx, src, axis=0):
    return tgt.at[idx].add(src)
def _segment_sum(src, seg, n):
    return jax.ops.segment_sum(src, seg, n)
class _Rng:
    def __init__(self, key):
        self._k = key
    def _next(self):
        self._k, sub = jax.random.split(self._k)
        return sub
    def normal(self, shape):
        return jax.random.normal(self._next(), shape, dtype=jnp.bfloat16)
    def randint(self, lo, hi, shape):
        return jax.random.randint(self._next(), shape, lo, hi, dtype=jnp.int32)
    def uniform(self, shape, lo=0.0, hi=1.0):
        return jax.random.uniform(self._next(), shape, jnp.bfloat16, lo, hi)
    def permutation(self, n):
        return jax.random.permutation(self._next(), n)


kernel_name = 'standalone__modern_conv_block_convnext_v2__vision'

def setup_inputs():
    _rng = _Rng(jax.random.key(int.from_bytes(__import__("os").urandom(4), "little")))
    _w = (lambda a: (lambda t: t.astype(jnp.bfloat16) if jnp.issubdtype(t.dtype, jnp.floating) else t)(jnp.asarray(a)))
    H = W = 512
    C = 96
    K = 3
    return {
        "x": _w((lambda *s: _rng.normal(s) * 0.05)(1, H, W, C)),
        "dw": _w((lambda *s: _rng.normal(s) * 0.05)(K, K, C)),
        "w1": _w((lambda *s: _rng.normal(s) * 0.05)(C, 4 * C)),
        "w2": _w((lambda *s: _rng.normal(s) * 0.05)(4 * C, C)),
        "grn_gamma": _w((lambda *s: _rng.normal(s) * 0.05)(4 * C)),
        "grn_beta": _w((lambda *s: _rng.normal(s) * 0.05)(4 * C)),
    }

def reference(x, dw, w1, w2, grn_gamma, grn_beta):
    B, H, W, C = x.shape
    K = dw.shape[0]
    pad = K // 2
    xp = jnp.pad(x, ((0,0),(pad,pad),(pad,pad),(0,0)))
    out = jnp.zeros_like(x)
    for i in range(K):
        for j in range(K):
            out = out + xp[:, i:i+H, j:j+W, :] * dw[i, j][None, None, None, :]
    h = _layernorm(out, axis=-1)
    h = jnp.einsum('bhwc,ce->bhwe', h, w1)
    h = _gelu(h)
    gx = jnp.sqrt((h * h).sum(axis=(1, 2), keepdims=True) + 1e-6)
    nx = gx / (gx.mean(axis=-1, keepdims=True) + 1e-6)
    h = grn_gamma * (h * nx) + grn_beta + h
    h = jnp.einsum('bhwe,ec->bhwc', h, w2)
    return x + h
```

```python
import functools
import math
import jax
import jax.numpy as jnp
from jax import lax
import jax.experimental.pallas as pl
import jax.experimental.pallas.tpu as pltpu

H = 512; W = 512; C = 96; E = 384
R = 16
NB = H // R
RC0 = 5
NRC = 7
NST = R - NRC

_C1 = math.sqrt(2.0 / math.pi)
_C3 = _C1 * 0.044715
_A = _C3 ** (1.0 / 3.0)
_K = _C1 / _A
_GS = 0.5 / _A

f32 = jnp.float32
bf16 = jnp.bfloat16
u32 = jnp.uint32


def _kernel(x_ref, xp_ref, xn_ref, dw_ref, w1_ref, w2t_ref, g_ref, b_ref, o_ref,
            h_ref, acc_ref, xf_ref, dwb_ref, w1t_ref, w2s_ref, bias_ref, ln_ref):
    p = pl.program_id(0)
    i = pl.program_id(1)

    lane = lax.broadcasted_iota(jnp.int32, (C, W), 1)

    def conv_ln(r):
        x0 = xf_ref[r]; x1 = xf_ref[r + 1]; x2 = xf_ref[r + 2]
        def wv(k):
            w = dwb_ref[k]
            return jnp.concatenate([w] * (W // 128), axis=1)
        a0 = x0 * wv(0) + x1 * wv(3) + x2 * wv(6)
        a1 = x0 * wv(1) + x1 * wv(4) + x2 * wv(7)
        a2 = x0 * wv(2) + x1 * wv(5) + x2 * wv(8)
        l = jnp.where(lane == 0, 0.0, pltpu.roll(a0, 1, 1))
        rr = jnp.where(lane == W - 1, 0.0, pltpu.roll(a2, W - 1, 1))
        cv = a1 + l + rr
        m = jnp.sum(cv, axis=0, keepdims=True) * (1.0 / C)
        d = cv - m
        v = jnp.sum(d * d, axis=0, keepdims=True) * (1.0 / C)
        rs = lax.rsqrt(v + 1e-5) * _A
        return (d * rs).astype(bf16)

    def gelu2(y):
        u = y * (y * y + _K)
        t = jnp.tanh(u)
        return y * t + y

    @pl.when(jnp.logical_and(p == 0, i == 0))
    def _init():
        acc_ref[...] = jnp.zeros_like(acc_ref)
        eye = (lax.broadcasted_iota(jnp.int32, (C, C), 0) == lax.broadcasted_iota(jnp.int32, (C, C), 1))
        dw = dw_ref[...].astype(f32)
        for a in range(3):
            for b in range(3):
                row = dw[a, b:b + 1, :]
                col = jnp.sum(jnp.where(eye, jnp.broadcast_to(row, (C, C)), 0.0), axis=1, keepdims=True)
                dwb_ref[a * 3 + b] = jnp.broadcast_to(col, (C, 128))
        w1 = w1_ref[...].astype(f32)
        w1p = jnp.concatenate([w1, jnp.zeros((128 - C, E), f32)], axis=0)
        w1t_ref[...] = w1p.T[:, :C].astype(bf16)

    @pl.when(p == 0)
    def _phase1():
        xf_ref[0] = jnp.where(i > 0, xp_ref[0].astype(f32), 0.0)
        xf_ref[R + 1] = jnp.where(i < NB - 1, xn_ref[0].astype(f32), 0.0)
        def up(r, c):
            xf_ref[r + 1] = x_ref[r].astype(f32)
            return c
        lax.fori_loop(0, R, up, 0)

        ln_ref[0] = conv_ln(0)
        def body(r, c):
            xn = ln_ref[r % 2]
            y = jnp.dot(w1t_ref[...], xn, preferred_element_type=f32)
            g = gelu2(y)
            sq = g * g
            acc_ref[...] += (sq[:, 0:128] + sq[:, 128:256]) + (sq[:, 256:384] + sq[:, 384:512])
            slot = jnp.where(r < RC0, i * NST + r,
                             jnp.where(r >= RC0 + NRC, i * NST + r - NRC, NB * NST))
            h_ref[slot] = pltpu.bitcast(g.astype(bf16), u32)
            rn = jnp.minimum(r + 1, R - 1)
            ln_ref[(r + 1) % 2] = conv_ln(rn)
            return c
        lax.fori_loop(0, R, body, 0)

    @pl.when(jnp.logical_and(p == 1, i == 0))
    def _grn():
        ss = jnp.sum(acc_ref[...].T, axis=0, keepdims=True) * (_GS * _GS)
        gx = jnp.sqrt(ss + 1e-6)
        nx = gx / (jnp.sum(gx, axis=1, keepdims=True) * (1.0 / E) + 1e-6)
        gam = g_ref[...].astype(f32).reshape(1, E)
        bet = b_ref[...].astype(f32).reshape(1, E)
        s = (gam * nx + 1.0) * _GS
        w2t = w2t_ref[...].astype(f32)
        w2s_ref[...] = (w2t * s).astype(bf16)
        bias_ref[...] = jnp.broadcast_to(jnp.sum(w2t * bet, axis=1, keepdims=True), (C, 128))

    @pl.when(p == 1)
    def _phase2():
        def fin(r, hb):
            o = jnp.dot(w2s_ref[...], hb, preferred_element_type=f32)
            bias = jnp.concatenate([bias_ref[...]] * (W // 128), axis=1)
            o_ref[r] = (o + bias + x_ref[r].astype(f32)).astype(bf16)

        def up(r, c):
            xf_ref[r + 1] = x_ref[r].astype(f32)
            return c
        lax.fori_loop(RC0 - 1, RC0 + NRC + 1, up, 0)

        def st_body(k, c):
            r = jnp.where(k < RC0, k, k + NRC)
            hb = pltpu.bitcast(h_ref[i * NST + k], bf16)
            fin(r, hb)
            return c
        lax.fori_loop(0, NST, st_body, 0)

        def rc_body(k, c):
            r = RC0 + k
            xn = conv_ln(r)
            y = jnp.dot(w1t_ref[...], xn, preferred_element_type=f32)
            g = gelu2(y)
            fin(r, g.astype(bf16))
            return c
        lax.fori_loop(0, NRC, rc_body, 0)


@jax.jit
def pallas_standalone__modern_conv_block_convnext_v2__vision_kernel(x, dw, w1, w2, grn_gamma, grn_beta):
    xt = jnp.transpose(x, (0, 1, 3, 2)).reshape(H, C, W)
    w2t = w2.T
    full = lambda shape: pl.BlockSpec(shape, lambda p, i: (0,) * len(shape))
    out = pl.pallas_call(
        _kernel,
        grid=(2, NB),
        in_specs=[
            pl.BlockSpec((R, C, W), lambda p, i: (i, 0, 0)),
            pl.BlockSpec((1, C, W), lambda p, i: (jnp.maximum(i * R - 1, 0) * (1 - p), 0, 0)),
            pl.BlockSpec((1, C, W), lambda p, i: (jnp.minimum(i * R + R, H - 1) * (1 - p), 0, 0)),
            full((3, 3, C)), full((C, E)), full((C, E)), full((E,)), full((E,)),
        ],
        out_specs=pl.BlockSpec((R, C, W), lambda p, i: (i * p, 0, 0)),
        out_shape=jax.ShapeDtypeStruct((H, C, W), bf16),
        scratch_shapes=[
            pltpu.VMEM((NB * NST + 1, E // 2, W), u32),
            pltpu.VMEM((E, 128), f32),
            pltpu.VMEM((R + 2, C, W), f32),
            pltpu.VMEM((9, C, 128), f32),
            pltpu.VMEM((E, C), bf16),
            pltpu.VMEM((C, E), bf16),
            pltpu.VMEM((C, 128), f32),
            pltpu.VMEM((2, C, W), bf16),
        ],
        compiler_params=pltpu.CompilerParams(
            dimension_semantics=("arbitrary", "arbitrary"),
            vmem_limit_bytes=128 * 1024 * 1024),
    )(xt, xt, xt, dw, w1, w2t, grn_gamma, grn_beta)
    return jnp.transpose(out.reshape(1, H, C, W), (0, 1, 3, 2))
```

```python
import functools
import math
import jax
import jax.numpy as jnp
from jax import lax
import jax.experimental.pallas as pl
import jax.experimental.pallas.tpu as pltpu

H = 512; W = 512; C = 96; E = 384
G = 8
NG = H // G
RC = (2, 3, 4)
ST = tuple(k for k in range(G) if k not in RC)
NST = len(ST)
NV = 4
NX = 4
LEAD = 4

_C1 = math.sqrt(2.0 / math.pi)
_C3 = _C1 * 0.044715
_A = _C3 ** (1.0 / 3.0)
_K = _C1 / _A
_GS = 0.5 / _A

f32 = jnp.float32
bf16 = jnp.bfloat16
u32 = jnp.uint32
i32 = jnp.int32

TAPS = [(i, j) for i in range(3) for j in range(3) if (i, j) != (1, 1)]


def _iota(shape, d):
    return lax.broadcasted_iota(i32, shape, d)


def _perm16(r):
    return (r // 16) * 16 + 2 * (r % 8) + (r % 16) // 8


def _tile4(a):
    return jnp.concatenate([a] * (W // 128), axis=1)


def _pack_pairs(y):
    m = y.shape[0] // 16
    outs = [pltpu.pack_elementwise([y[16 * t:16 * t + 8], y[16 * t + 8:16 * t + 16]], packed_dtype=bf16)
            for t in range(m)]
    o = outs[0] if m == 1 else jnp.concatenate(outs, axis=0)
    return pltpu.bitcast(o, u32) if o.dtype != u32 else o


def _gelu2(y):
    u = y * (y * y + _K)
    t = jnp.tanh(u)
    return y * t + y


def _kernel(x_hbm, dw_ref, w1_ref, w2t_ref, g_ref, b_ref, o_hbm,
            h_ref, acc_ref, xbuf, obuf, ver_ref, xn_ref, ht_ref,
            cl_ref, dwc_ref, dwb_ref, w1p_ref, w1q_ref, w2s_ref, bias_ref,
            xsem, osem):

    def x_copy(row0, nrows, slot):
        return pltpu.make_async_copy(x_hbm.at[pl.ds(row0, nrows)], xbuf.at[slot, pl.ds(0, nrows)], xsem.at[slot])

    def o_copy(row0, slot):
        return pltpu.make_async_copy(obuf.at[slot], o_hbm.at[pl.ds(row0, G)], osem.at[slot])

    x_copy(0, LEAD, 1).start()
    x_copy(LEAD, G, 0).start()

    acc_ref[...] = jnp.zeros_like(acc_ref)
    dw = dw_ref[...].astype(f32)
    r96 = _iota((C, C), 0); c96 = _iota((C, C), 1)
    eye = r96 == c96
    eyep = _perm16(r96) == c96
    for a in range(3):
        for b in range(3):
            row = jnp.broadcast_to(dw[a, b:b + 1, :], (C, C))
            col = jnp.sum(jnp.where(eye, row, 0.0), axis=1, keepdims=True)
            dwb_ref[a * 3 + b] = jnp.broadcast_to(col, (C, 128))
            colp = jnp.sum(jnp.where(eyep, row, 0.0), axis=1, keepdims=True)
            if (a, b) == (1, 1):
                dwc_ref[...] = jnp.broadcast_to(colp, (C, 128))
    rr = _iota((C, 128), 0); cc = _iota((C, 128), 1)
    cl = jnp.zeros((C, 128), f32)
    for t, (a, b) in enumerate(TAPS):
        row = jnp.broadcast_to(dw[a, b:b + 1, :], (C, C))
        colp = jnp.sum(jnp.where(eyep, row, 0.0), axis=1, keepdims=True)
        cl = jnp.where(cc == t * 16 + _perm16(rr) % 16, jnp.broadcast_to(colp, (C, 128)), cl)
    cl_ref[...] = pltpu.bitcast(cl.astype(bf16), u32)
    P = (_perm16(_iota((E, E), 0)) == _iota((E, E), 1))
    Pb = jnp.where(P, 1.0, 0.0).astype(bf16)
    w1p = lax.dot_general(Pb, w1_ref[...], (((1,), (1,)), ((), ())), preferred_element_type=f32)
    w1p_ref[...] = pltpu.bitcast(w1p.astype(bf16), u32)
    Q = jnp.where(r96 == (c96 // 16) * 16 + (c96 % 16) // 2 + 8 * (c96 % 2), 1.0, 0.0).astype(bf16)
    w1q = jnp.dot(w1p.astype(bf16), Q, preferred_element_type=f32)
    w1q_ref[...] = pltpu.bitcast(w1q.astype(bf16), u32)

    lane48 = _iota((C // 2, W), 1)
    lane8 = _iota((8, W), 1)

    def s1(xrow, vslot):
        xu = pltpu.bitcast(xrow, u32)
        z = jnp.zeros_like(xu)
        ver_ref[vslot, 0] = jnp.where(lane48 == 0, z, pltpu.roll(xu, 1, 1))
        ver_ref[vslot, 1] = xu
        ver_ref[vslot, 2] = jnp.where(lane48 == W - 1, z, pltpu.roll(xu, W - 1, 1))

    def conv_group(row, k):
        rhs = jnp.concatenate([ver_ref[(row + i - 1) % NV, j, 8 * k:8 * k + 8, :] for (i, j) in TAPS], axis=0)
        lhs = pltpu.bitcast(cl_ref[8 * k:8 * k + 8, :], bf16)
        cv = jnp.dot(lhs, pltpu.bitcast(rhs, bf16), preferred_element_type=f32)
        xc = ver_ref[row % NV, 1, 8 * k:8 * k + 8, :]
        xe = pltpu.unpack_elementwise(xc, index=0, packed_dtype=bf16, unpacked_dtype=f32)
        xo = pltpu.unpack_elementwise(xc, index=1, packed_dtype=bf16, unpacked_dtype=f32)
        return cv + jnp.concatenate([xe, xo], axis=0) * _tile4(dwc_ref[16 * k:16 * k + 16, :])

    def ln(cv):
        m = jnp.sum(cv, axis=0, keepdims=True) * (1.0 / C)
        d = cv - m
        v = jnp.sum(d * d, axis=0, keepdims=True) * (1.0 / C)
        rs = lax.rsqrt(v + 1e-5) * _A
        return d * rs

    def mm1_chunk(w_ref, xn, c):
        lhs = pltpu.bitcast(w_ref[64 * c:64 * c + 64, :], bf16)
        return _gelu2(jnp.dot(lhs, xn, preferred_element_type=f32))

    def s23(k, hslot):
        cvs = []
        for c in range(3):
            cvs.append(conv_group(k + 2, 2 * c))
            cvs.append(conv_group(k + 2, 2 * c + 1))
            xn = pltpu.bitcast(xn_ref[k % NX], bf16)
            g = mm1_chunk(w1p_ref, xn, c)
            sq = g * g
            acc_ref[128 * c:128 * c + 128, :] += (sq[:, 0:128] + sq[:, 128:256]) + (sq[:, 256:384] + sq[:, 384:512])
            if hslot is not None:
                h_ref[hslot, 64 * c:64 * c + 64, :] = _pack_pairs(g)
        xn_ref[(k + 2) % NX] = _pack_pairs(ln(jnp.concatenate(cvs, axis=0)))

    ver_ref[NV - 1] = jnp.zeros(ver_ref.shape[1:], u32)
    x_copy(0, LEAD, 1).wait()
    for r in range(3):
        s1(xbuf[1, r], r % NV)
    for r in range(2):
        if r == 1:
            pass
        xn_ref[r] = _pack_pairs(ln(jnp.concatenate([conv_group(r, k) for k in range(6)], axis=0)))
    s1(xbuf[1, 3], 3 % NV)

    def p1_body(j, carry):
        slot = j % 2

        @pl.when(j < NG - 1)
        def _():
            x_copy(j * G + LEAD, G, slot).wait()

        @pl.when(j == NG - 1)
        def _():
            x_copy(j * G + LEAD, G - LEAD, slot).wait()
            xbuf[slot, G - LEAD] = jnp.zeros((C, W), bf16)

        @pl.when(j < NG - 2)
        def _():
            x_copy((j + 1) * G + LEAD, G, 1 - slot).start()

        @pl.when(j == NG - 2)
        def _():
            x_copy((j + 1) * G + LEAD, G - LEAD, 1 - slot).start()

        @pl.when(j == NG - 1)
        def _():
            x_copy(0, G, 1 - slot).start()

        for k in range(G):
            hslot = (j * NST + ST.index(k)) if k in ST else None
            s23(k, hslot)
            s1(xbuf[slot, k], (k + LEAD) % NV)
        return carry

    lax.fori_loop(0, NG, p1_body, 0)

    ssc = jnp.sum(acc_ref[...], axis=1, keepdims=True)
    ss = jnp.sum(jnp.where(P, jnp.broadcast_to(ssc, (E, E)), 0.0), axis=0, keepdims=True) * (_GS * _GS)
    gx = jnp.sqrt(ss + 1e-6)
    nx = gx / (jnp.sum(gx, axis=1, keepdims=True) * (1.0 / E) + 1e-6)
    gam = g_ref[...].astype(f32).reshape(1, E)
    bet = b_ref[...].astype(f32).reshape(1, E)
    s = (gam * nx + 1.0) * _GS
    w2t = w2t_ref[...].astype(f32)
    w2s_ref[...] = pltpu.bitcast((w2t * s).astype(bf16), u32)
    bias_ref[...] = jnp.broadcast_to(jnp.sum(w2t * bet, axis=1, keepdims=True), (C, 128))

    def p2_body(j, carry):
        slot = j % 2
        x_copy(j * G, G, slot).wait()

        @pl.when(j < NG - 1)
        def _():
            x_copy((j + 1) * G, G, 1 - slot).start()

        @pl.when(j >= 2)
        def _():
            o_copy((j - 2) * G, slot).wait()

        def fin(k, hu):
            o = jnp.dot(pltpu.bitcast(w2s_ref[...], bf16), pltpu.bitcast(hu, bf16), preferred_element_type=f32)
            obuf[slot, k] = (o + _tile4(bias_ref[...]) + xbuf[slot, k].astype(f32)).astype(bf16)

        def conv_ln_vpu(k, n):
            cvs = []
            for g in range(C // 8):
                sl = slice(8 * g, 8 * g + 8)
                x0 = xbuf[slot, k - 1, sl, :].astype(f32)
                x1 = xbuf[slot, k, sl, :].astype(f32)
                x2 = xbuf[slot, k + 1, sl, :].astype(f32)
                wv = lambda t: _tile4(dwb_ref[t, sl, :])
                a0 = x0 * wv(0) + x1 * wv(3) + x2 * wv(6)
                a1 = x0 * wv(1) + x1 * wv(4) + x2 * wv(7)
                a2 = x0 * wv(2) + x1 * wv(5) + x2 * wv(8)
                l = jnp.where(lane8 == 0, 0.0, pltpu.roll(a0, 1, 1))
                r = jnp.where(lane8 == W - 1, 0.0, pltpu.roll(a2, W - 1, 1))
                cvs.append(a1 + l + r)
            xn_ref[n] = _pack_pairs(ln(jnp.concatenate(cvs, axis=0)))

        def mm1(n):
            for c in range(3):
                xn = pltpu.bitcast(xn_ref[n], bf16)
                ht_ref[n % 2, 64 * c:64 * c + 64, :] = _pack_pairs(mm1_chunk(w1q_ref, xn, c))

        st = lambda q: fin(ST[q], h_ref[j * NST + q])
        conv_ln_vpu(RC[0], 0)
        st(0)
        conv_ln_vpu(RC[1], 1)
        st(1)
        mm1(0)
        conv_ln_vpu(RC[2], 2)
        st(2)
        fin(RC[0], ht_ref[0])
        mm1(1)
        st(3)
        fin(RC[1], ht_ref[1])
        mm1(2)
        st(4)
        fin(RC[2], ht_ref[0])

        o_copy(j * G, slot).start()
        return carry

    lax.fori_loop(0, NG, p2_body, 0)
    o_copy((NG - 2) * G, 0).wait()
    o_copy((NG - 1) * G, 1).wait()


@jax.jit
def pallas_standalone__modern_conv_block_convnext_v2__vision_kernel(x, dw, w1, w2, grn_gamma, grn_beta):
    xt = jnp.transpose(x, (0, 1, 3, 2)).reshape(H, C, W)
    w2t = w2.T
    vm = pl.BlockSpec(memory_space=pltpu.VMEM)
    out = pl.pallas_call(
        _kernel,
        in_specs=[pl.BlockSpec(memory_space=pl.ANY), vm, vm, vm, vm, vm],
        out_specs=pl.BlockSpec(memory_space=pl.ANY),
        out_shape=jax.ShapeDtypeStruct((H, C, W), bf16),
        scratch_shapes=[
            pltpu.VMEM((NG * NST, E // 2, W), u32),
            pltpu.VMEM((E, 128), f32),
            pltpu.VMEM((2, G, C, W), bf16),
            pltpu.VMEM((2, G, C, W), bf16),
            pltpu.VMEM((NV, 3, C // 2, W), u32),
            pltpu.VMEM((NX, C // 2, W), u32),
            pltpu.VMEM((2, E // 2, W), u32),
            pltpu.VMEM((C // 2, 128), u32),
            pltpu.VMEM((C, 128), f32),
            pltpu.VMEM((9, C, 128), f32),
            pltpu.VMEM((E // 2, C), u32),
            pltpu.VMEM((E // 2, C), u32),
            pltpu.VMEM((C // 2, E), u32),
            pltpu.VMEM((C, 128), f32),
            pltpu.SemaphoreType.DMA((2,)),
            pltpu.SemaphoreType.DMA((2,)),
        ],
        compiler_params=pltpu.CompilerParams(vmem_limit_bytes=128 * 1024 * 1024),
    )(xt, dw, w1, w2t, grn_gamma, grn_beta)
    return jnp.transpose(out.reshape(1, H, C, W), (0, 1, 3, 2))
```

```python
import functools
import math
import jax
import jax.numpy as jnp
from jax import lax
import jax.experimental.pallas as pl
import jax.experimental.pallas.tpu as pltpu

H = 512; W = 512; C = 96; E = 384
G = 8
NG = H // G
RC = (1, 3, 5, 7)
ST = tuple(k for k in range(G) if k not in RC)
NST = len(ST)
NRC = len(RC)
NU = 4
NQ = W // 128
XR0 = (NG + 1) * NRC
LN_LAG = 3
NSUB = 3
P2ORD = 'M0,S0,M1,F0,S1,M2,F1,S2,M3,F2,S3,F3'

_C1 = math.sqrt(2.0 / math.pi)
_C3 = _C1 * 0.044715
_A = _C3 ** (1.0 / 3.0)
_K = _C1 / _A
_GS = 0.5 / _A

f32 = jnp.float32
bf16 = jnp.bfloat16
u32 = jnp.uint32
i32 = jnp.int32


def _iota(shape, d):
    return lax.broadcasted_iota(i32, shape, d)


def _perm16(r):
    return (r // 16) * 16 + 2 * (r % 8) + (r % 16) // 8


def _tile4(a):
    return jnp.concatenate([a] * NQ, axis=1)


def _pack_pairs(y):
    m = y.shape[0] // 16
    outs = [pltpu.pack_elementwise([y[16 * t:16 * t + 8], y[16 * t + 8:16 * t + 16]], packed_dtype=bf16)
            for t in range(m)]
    o = outs[0] if m == 1 else jnp.concatenate(outs, axis=0)
    return pltpu.bitcast(o, u32) if o.dtype != u32 else o


def _gelu2(y):
    u = y * (y * y + _K)
    t = jnp.tanh(u)
    return y * t + y


def _tree_sum(xs):
    xs = list(xs)
    while len(xs) > 1:
        xs = [xs[i] + xs[i + 1] for i in range(0, len(xs) - 1, 2)] + ([xs[-1]] if len(xs) % 2 else [])
    return xs[0]


def _xn_slot(j, k):
    jj, kk = k // G, k % G
    if kk in RC:
        return (j + jj) * NRC + RC.index(kk)
    return XR0 + ST.index(kk)


def _kernel(x_hbm, x5_hbm, dw_ref, w1_ref, w2t_ref, g_ref, b_ref, o_hbm,
            h_ref, xn_ref, acc_ref, xbuf, cl_ref, w1q_ref, w2s_ref, bias_ref, zs_ref,
            xsem, osem, psem):

    def x_copy(row0, slot):
        return pltpu.make_async_copy(x_hbm.at[pl.ds(row0, G)], xbuf.at[slot], xsem.at[slot])

    for i in range(2):
        zs_ref[i] = 0
    lane8 = _iota((8, W), 1)

    def phase1(xp, ver_ref):
        def p_copy(u0, n, half, slot, dst0=0):
            src = x5_hbm.at[pl.ds(u0 - 1 + half, n), 1 - half]
            return pltpu.make_async_copy(src, xp.at[slot, pl.ds(dst0, n), :, pl.ds(8 * half, 8), :],
                                         psem.at[slot, half])

        p_copy(1, 2, 0, 1, 1).start()
        p_copy(0, 3, 1, 1).start()
        p_copy(3, 4, 0, 0).start()
        p_copy(3, 4, 1, 0).start()

        acc_ref[...] = jnp.zeros_like(acc_ref)
        dw = dw_ref[...].astype(f32)
        R = _iota((2 * C, C), 0); KK = _iota((2 * C, C), 1)
        chm = KK == 8 * (R // 16) + R % 8
        itap = 2 * (KK // 48) + (KK % 16) // 8 - (R % 16) // 8
        ver = (KK % 48) // 16
        diag = KK % 8 == R % 8
        cl = jnp.zeros((2 * C, C), f32)
        for a in range(3):
            for b in range(3):
                row = jnp.broadcast_to(dw[a, b:b + 1, :], (2 * C, C))
                col = jnp.sum(jnp.where(chm, row, 0.0), axis=1, keepdims=True)
                cl = jnp.where(diag & (itap == a) & (ver == b), jnp.broadcast_to(col, (2 * C, C)), cl)
        cl_ref[...] = pltpu.bitcast(cl.astype(bf16), u32)

        Pb = jnp.where(_perm16(_iota((E, E), 0)) == _iota((E, E), 1), 1.0, 0.0).astype(bf16)
        w1f = w1_ref[...].astype(f32)
        w1c = (w1f - jnp.sum(w1f, axis=0, keepdims=True) * (1.0 / C)).astype(bf16)
        w1p = lax.dot_general(Pb, w1c, (((1,), (1,)), ((), ())), preferred_element_type=f32)
        r96 = _iota((C, C), 0); c96 = _iota((C, C), 1)
        Q = jnp.where(r96 == (c96 // 16) * 16 + (c96 % 16) // 2 + 8 * (c96 % 2), 1.0, 0.0).astype(bf16)
        w1q = jnp.dot(w1p.astype(bf16), Q, preferred_element_type=f32)
        w1q_ref[...] = pltpu.bitcast(w1q.astype(bf16), u32)

        def s1(xu_ref, u):
            for g in range(12):
                m = pltpu.bitcast(xu_ref[g], u32)
                zz = jnp.zeros_like(m)
                ver_ref[u, g, 0:8, :] = jnp.where(lane8 == 0, zz, pltpu.roll(m, 1, 1))
                ver_ref[u, g, 8:16, :] = m
                ver_ref[u, g, 16:24, :] = jnp.where(lane8 == W - 1, zz, pltpu.roll(m, W - 1, 1))

        def conv_round(t, q, gs):
            ls = slice(128 * q, 128 * q + 128)
            cvs = []
            for g in gs:
                rhs = jnp.concatenate([ver_ref[t % NU, g, :, ls], ver_ref[(t + 1) % NU, g, :, ls]], axis=0)
                lhs = pltpu.bitcast(cl_ref[8 * g:8 * g + 8, :], bf16)
                cvs.append(jnp.dot(lhs, pltpu.bitcast(rhs, bf16), preferred_element_type=f32))
            return cvs

        def ln_tile(cvs, q, dsts):
            ls = slice(128 * q, 128 * q + 128)
            for ab in range(2):
                cs = [cv[8 * ab:8 * ab + 8] for cv in cvs]
                s1_ = _tree_sum(cs)
                s2_ = _tree_sum([c * c for c in cs])
                m = jnp.sum(s1_, axis=0, keepdims=True) * (1.0 / C)
                v = jnp.sum(s2_, axis=0, keepdims=True) * (1.0 / C) - m * m
                rs = lax.rsqrt(jnp.maximum(v, 0.0) + 1e-5) * _A
                xn_ref[dsts[ab], :, ls] = _pack_pairs(jnp.concatenate(cs, axis=0) * rs)

        xp[1, 0, :, 0:8, :] = jnp.zeros((12, 8, W), bf16)
        p_copy(1, 2, 0, 1, 1).wait()
        p_copy(0, 3, 1, 1).wait()
        for u in range(3):
            s1(xp.at[1, u], u)
        for q in range(NQ):
            ln_tile(conv_round(0, q, range(12)), q, (_xn_slot(0, 0), _xn_slot(0, 1)))
        for q in range(2):
            ln_tile(conv_round(1, q, range(12)), q, (_xn_slot(0, 2), _xn_slot(0, 3)))

        NP = 2 * NSUB
        RPP = 12 // NP
        MR = E // NSUB

        def body(j, carry):
            slot = j % 2
            z = zs_ref[0]
            z1 = zs_ref[1]
            u0 = 4 * j + 3

            @pl.when(j < NG - 1)
            def _():
                p_copy(u0, 4, 0, slot).wait()
                p_copy(u0, 4, 1, slot).wait()

            @pl.when(j == NG - 1)
            def _():
                p_copy(u0, 2, 0, slot).wait()
                p_copy(u0, 1, 1, slot).wait()
                xp[slot, 1, :, 8:16, :] = jnp.zeros((12, 8, W), bf16)

            @pl.when(j < NG - 2)
            def _():
                p_copy(u0 + 4, 4, 0, 1 - slot).start()
                p_copy(u0 + 4, 4, 1, 1 - slot).start()

            @pl.when(j == NG - 2)
            def _():
                p_copy(u0 + 4, 2, 0, 1 - slot).start()
                p_copy(u0 + 4, 1, 1, 1 - slot).start()

            @pl.when(j == NG - 1)
            def _():
                x_copy(0, 0).start()

            pend = []
            cur = []

            def do_ln(cvs, q, pair):
                ln_tile(cvs, q, (_xn_slot(j, 2 * pair) + z1, _xn_slot(j, 2 * pair + 1) + z1))

            for p in range(G // 2):
                for r in range(NP):
                    gr = p * NP + r
                    ab, c = r // NSUB, r % NSUB
                    k = 2 * p + ab
                    while pend and pend[0][0] <= gr:
                        do_ln(*pend.pop(0)[1:])
                    xn = pltpu.bitcast(xn_ref[_xn_slot(j, k) + z], bf16)
                    lhs = pltpu.bitcast(w1q_ref[MR // 2 * c:MR // 2 * (c + 1), :], bf16)
                    gl = _gelu2(jnp.dot(lhs, xn, preferred_element_type=f32))
                    sq = gl * gl
                    acc_ref[MR * c:MR * (c + 1), :] += (sq[:, 0:128] + sq[:, 128:256]) + (sq[:, 256:384] + sq[:, 384:512])
                    if k in ST:
                        h_ref[j * NST + ST.index(k), MR // 2 * c:MR // 2 * (c + 1), :] = _pack_pairs(gl)
                    if r == NP // 2 - 1:
                        s1(xp.at[slot, p], (p + 3) % NU)
                    for rr in range(r * RPP, (r + 1) * RPP):
                        q = (rr // 3 + 2) % 4
                        pair = p + 1 + (rr >= 6)
                        cur += conv_round(pair, q, range(4 * (rr % 3), 4 * (rr % 3) + 4))
                        if rr % 3 == 2:
                            pend.append((gr + LN_LAG, cur, q, pair))
                            cur = []
            for e in pend:
                do_ln(*e[1:])
            return carry

        with jax.named_scope('loop1'):
            lax.fori_loop(0, NG, body, 0)

    pl.run_scoped(phase1,
                  pltpu.VMEM((2, 4, 12, 16, W), bf16),
                  pltpu.VMEM((NU, 12, 24, W), u32))

    P = _perm16(_iota((E, E), 0)) == _iota((E, E), 1) + zs_ref[0]
    ssc = jnp.sum(acc_ref[...], axis=1, keepdims=True)
    ss = jnp.sum(jnp.where(P, jnp.broadcast_to(ssc, (E, E)), 0.0), axis=0, keepdims=True) * (_GS * _GS)
    gx = jnp.sqrt(ss + 1e-6)
    nx = gx / (jnp.sum(gx, axis=1, keepdims=True) * (1.0 / E) + 1e-6)
    gam = g_ref[...].astype(f32).reshape(1, E)
    bet = b_ref[...].astype(f32).reshape(1, E)
    s = (gam * nx + 1.0) * _GS
    w2t = w2t_ref[...].astype(f32)
    w2s_ref[...] = pltpu.bitcast((w2t * s).astype(bf16), u32)
    bias_ref[...] = jnp.broadcast_to(jnp.sum(w2t * bet, axis=1, keepdims=True), (C, 128))

    def phase2(obuf, ht_ref):
        def o_copy(row0, slot):
            return pltpu.make_async_copy(obuf.at[slot], o_hbm.at[pl.ds(row0, G)], osem.at[slot])

        def body(j, carry):
            slot = j % 2
            z = zs_ref[0]
            x_copy(j * G, slot).wait()

            @pl.when(j < NG - 1)
            def _():
                x_copy((j + 1) * G, 1 - slot).start()

            @pl.when(j >= 2)
            def _():
                o_copy((j - 2) * G, slot).wait()

            def fin(k, hu):
                o = jnp.dot(pltpu.bitcast(w2s_ref[...], bf16), pltpu.bitcast(hu, bf16), preferred_element_type=f32)
                obuf[slot, k] = (o + _tile4(bias_ref[...]) + xbuf[slot, k].astype(f32)).astype(bf16)

            def mm1(n):
                xn = pltpu.bitcast(xn_ref[j * NRC + n], bf16)
                lhs = pltpu.bitcast(w1q_ref[...], bf16)
                ht_ref[n % 2 + z] = _pack_pairs(_gelu2(jnp.dot(lhs, xn, preferred_element_type=f32)))

            for tok in P2ORD.split(','):
                n = int(tok[1])
                if tok[0] == 'M': mm1(n)
                elif tok[0] == 'S': fin(ST[n], h_ref[j * NST + n])
                elif tok[0] == 'F': fin(RC[n], ht_ref[n % 2 + z])

            o_copy(j * G, slot).start()
            return carry

        with jax.named_scope('loop2'):
            lax.fori_loop(0, NG, body, 0)
        o_copy((NG - 2) * G, 0).wait()
        o_copy((NG - 1) * G, 1).wait()

    pl.run_scoped(phase2,
                  pltpu.VMEM((2, G, C, W), bf16),
                  pltpu.VMEM((2, E // 2, W), u32))


@jax.jit
def pallas_standalone__modern_conv_block_convnext_v2__vision_kernel(x, dw, w1, w2, grn_gamma, grn_beta):
    xt = jnp.transpose(x, (0, 1, 3, 2)).reshape(H, C, W)
    x5 = xt.reshape(H // 2, 2, C // 8, 8, W)
    w2t = w2.T
    vm = pl.BlockSpec(memory_space=pltpu.VMEM)
    out = pl.pallas_call(
        _kernel,
        in_specs=[pl.BlockSpec(memory_space=pl.ANY), pl.BlockSpec(memory_space=pl.ANY), vm, vm, vm, vm, vm],
        out_specs=pl.BlockSpec(memory_space=pl.ANY),
        out_shape=jax.ShapeDtypeStruct((H, C, W), bf16),
        scratch_shapes=[
            pltpu.VMEM((NG * NST, E // 2, W), u32),
            pltpu.VMEM((XR0 + NST, C // 2, W), u32),
            pltpu.VMEM((E, 128), f32),
            pltpu.VMEM((2, G, C, W), bf16),
            pltpu.VMEM((C, C), u32),
            pltpu.VMEM((E // 2, C), u32),
            pltpu.VMEM((C // 2, E), u32),
            pltpu.VMEM((C, 128), f32),
            pltpu.SMEM((2,), i32),
            pltpu.SemaphoreType.DMA((2,)),
            pltpu.SemaphoreType.DMA((2,)),
            pltpu.SemaphoreType.DMA((2, 2)),
        ],
        compiler_params=pltpu.CompilerParams(vmem_limit_bytes=128 * 1024 * 1024),
    )(xt, x5, dw, w1, w2t, grn_gamma, grn_beta)
    return jnp.transpose(out.reshape(1, H, C, W), (0, 1, 3, 2))
```

```python
import functools
import math
import jax
import jax.numpy as jnp
from jax import lax
import jax.experimental.pallas as pl
import jax.experimental.pallas.tpu as pltpu

H = 512; W = 512; C = 96; E = 384
G = 8
NG = H // G
RC = tuple(int(c) for c in '0246')
ST = tuple(k for k in range(G) if k not in RC)
NST = len(ST)
NRC = len(RC)
NU = 4
NQ = W // 128
XR0 = (NG + 1) * NRC
LN_LAG = 5
LNM = 1
UN = 2
NB = 4
NB2 = 6
NSUB = 6
P2ORD = 'M0,S0,M1,F0,S1,M2,F1,S2,M3,F2,S3,F3'

_C1 = math.sqrt(2.0 / math.pi)
_C3 = _C1 * 0.044715
_A = _C3 ** (1.0 / 3.0)
_K = _C1 / _A
_GS = 0.5 / _A

f32 = jnp.float32
bf16 = jnp.bfloat16
u32 = jnp.uint32
i32 = jnp.int32


def _iota(shape, d):
    return lax.broadcasted_iota(i32, shape, d)


def _perm16(r):
    return (r // 16) * 16 + 2 * (r % 8) + (r % 16) // 8


def _tile4(a):
    return jnp.concatenate([a] * NQ, axis=1)


def _pack_pairs(y):
    m = y.shape[0] // 16
    outs = [pltpu.pack_elementwise([y[16 * t:16 * t + 8], y[16 * t + 8:16 * t + 16]], packed_dtype=bf16)
            for t in range(m)]
    o = outs[0] if m == 1 else jnp.concatenate(outs, axis=0)
    return pltpu.bitcast(o, u32) if o.dtype != u32 else o


def _gelu2(y):
    u = y * (y * y + _K)
    t = jnp.tanh(u)
    return y * t + y


def _tree_sum(xs):
    xs = list(xs)
    while len(xs) > 1:
        xs = [xs[i] + xs[i + 1] for i in range(0, len(xs) - 1, 2)] + ([xs[-1]] if len(xs) % 2 else [])
    return xs[0]


def _xn_slot(j, k):
    jj, kk = k // G, k % G
    if kk in RC:
        return (j + jj) * NRC + RC.index(kk)
    return XR0 + ST.index(kk)


def _kernel(x_hbm, x5_hbm, dw_ref, w1_ref, w2t_ref, g_ref, b_ref, o_hbm,
            h_ref, xn_ref, w1q_ref, w2s_ref, bias_ref, zs_ref,
            xsem, osem, psem):

    for i in range(2):
        zs_ref[i] = 0
    lane8 = _iota((8, W), 1)

    def phase1(xp, ver_ref, acc_ref, cl_ref):
        def p_copy(u0, n, half, slot, dst0=0):
            src = x5_hbm.at[pl.ds(u0 - 1 + half, n), 1 - half]
            return pltpu.make_async_copy(src, xp.at[slot, pl.ds(dst0, n), :, pl.ds(8 * half, 8), :],
                                         psem.at[slot, half])

        def chunk(j, last):
            return [p_copy(4 * j + 3, 2 if last else 4, 0, j % NB), p_copy(4 * j + 3, 1 if last else 4, 1, j % NB)]

        p_copy(1, 2, 0, 2, 1).start()
        p_copy(0, 3, 1, 2).start()
        for j in range(2):
            for cp in chunk(j, False):
                cp.start()

        acc_ref[...] = jnp.zeros_like(acc_ref)
        dw = dw_ref[...].astype(f32)
        R = _iota((2 * C, C), 0); KK = _iota((2 * C, C), 1)
        chm = KK == 8 * (R // 16) + R % 8
        itap = 2 * (KK // 48) + (KK % 16) // 8 - (R % 16) // 8
        ver = (KK % 48) // 16
        diag = KK % 8 == R % 8
        cl = jnp.zeros((2 * C, C), f32)
        for a in range(3):
            for b in range(3):
                row = jnp.broadcast_to(dw[a, b:b + 1, :], (2 * C, C))
                col = jnp.sum(jnp.where(chm, row, 0.0), axis=1, keepdims=True)
                cl = jnp.where(diag & (itap == a) & (ver == b), jnp.broadcast_to(col, (2 * C, C)), cl)
        cl_ref[...] = pltpu.bitcast(cl.astype(bf16), u32)

        Pb = jnp.where(_perm16(_iota((E, E), 0)) == _iota((E, E), 1), 1.0, 0.0).astype(bf16)
        w1f = w1_ref[...].astype(f32)
        w1c = (w1f - jnp.sum(w1f, axis=0, keepdims=True) * (1.0 / C)).astype(bf16)
        w1p = lax.dot_general(Pb, w1c, (((1,), (1,)), ((), ())), preferred_element_type=f32)
        r96 = _iota((C, C), 0); c96 = _iota((C, C), 1)
        Q = jnp.where(r96 == (c96 // 16) * 16 + (c96 % 16) // 2 + 8 * (c96 % 2), 1.0, 0.0).astype(bf16)
        w1q = jnp.dot(w1p.astype(bf16), Q, preferred_element_type=f32)
        w1q_ref[...] = pltpu.bitcast(w1q.astype(bf16), u32)

        lane = _iota((8, 128), 1)

        def s1(xu_ref, u, kill=None):
            for g in range(12):
                m = pltpu.bitcast(xu_ref[g], u32)
                if kill is not None:
                    m = jnp.where(kill, jnp.zeros_like(m), m)
                mq = [m[:, 128 * q:128 * q + 128] for q in range(NQ)]
                zz = jnp.zeros((8, 128), u32)
                for q in range(NQ):
                    lq = jnp.where(lane == 127, mq[q - 1] if q > 0 else zz, mq[q])
                    rq = jnp.where(lane == 0, mq[q + 1] if q + 1 < NQ else zz, mq[q])
                    ver_ref[u, g, q, 0:8, :] = pltpu.roll(lq, 1, 1)
                    ver_ref[u, g, q, 8:16, :] = mq[q]
                    ver_ref[u, g, q, 16:24, :] = pltpu.roll(rq, 127, 1)

        def conv_round(t, q, gs):
            ls = slice(128 * q, 128 * q + 128)
            cvs = []
            for g in gs:
                rhs = jnp.concatenate([ver_ref[t % NU, g, q], ver_ref[(t + 1) % NU, g, q]], axis=0)
                lhs = pltpu.bitcast(cl_ref[8 * g:8 * g + 8, :], bf16)
                cvs.append(jnp.dot(lhs, pltpu.bitcast(rhs, bf16), preferred_element_type=f32))
            return cvs

        sub = _iota((8, 128), 0)
        m0 = sub % 2 == 0
        m1 = (sub // 2) % 2 == 0
        lnc = jnp.where(m1, 1.0 / (C * _A), 1.0 / (C * _A * _A))

        def merge(a, b, msk, sh):
            return jnp.where(msk, a, b) + pltpu.roll(jnp.where(msk, b, a), 8 - sh, 0)

        def ln_tile(cvs, q, dsts):
            ls = slice(128 * q, 128 * q + 128)
            cs = [[cv[8 * ab:8 * ab + 8] for cv in cvs] for ab in range(2)]
            if not LNM:
                for ab in range(2):
                    s1_ = _tree_sum(cs[ab])
                    s2_ = _tree_sum([c * c for c in cs[ab]])
                    m = jnp.sum(s1_, axis=0, keepdims=True) * (1.0 / C)
                    v = jnp.sum(s2_, axis=0, keepdims=True) * (1.0 / C) - m * m
                    rs = lax.rsqrt(jnp.maximum(v, 0.0) + 1e-5) * _A
                    xn_ref[dsts[ab], :, ls] = _pack_pairs(jnp.concatenate(cs[ab], axis=0) * rs)
                return
            c1 = merge(_tree_sum(cs[0]), _tree_sum(cs[1]), m0, 1)
            c2 = merge(_tree_sum([c * c for c in cs[0]]), _tree_sum([c * c for c in cs[1]]), m0, 1)
            e = merge(c1, c2, m1, 2)
            f = (e + pltpu.roll(e, 4, 0)) * lnc
            v = pltpu.roll(f, 6, 0) - f * f
            rs = lax.rsqrt(jnp.maximum(v, 0.0) + 1e-5 / (_A * _A))
            for ab in range(2):
                xn_ref[dsts[ab], :, ls] = _pack_pairs(jnp.concatenate(cs[ab], axis=0) * rs[ab:ab + 1, :])

        xp[2, 0, :, 0:8, :] = jnp.zeros((12, 8, W), bf16)
        p_copy(1, 2, 0, 2, 1).wait()
        p_copy(0, 3, 1, 2).wait()
        for u in range(3):
            s1(xp.at[2, u], u)
        for q in range(NQ):
            ln_tile(conv_round(0, q, range(12)), q, (_xn_slot(0, 0), _xn_slot(0, 1)))
        for q in range(2):
            ln_tile(conv_round(1, q, range(12)), q, (_xn_slot(0, 2), _xn_slot(0, 3)))

        NP = 2 * NSUB
        RPP = 12 // NP
        MR = E // NSUB

        def body(jj, carry):
            z = zs_ref[0]
            z1 = zs_ref[1]
            pend = []
            cur = []
            NI = NG // UN
            for cp in chunk(2 * jj, False):
                cp.wait()

            @pl.when(jj < NI - 1)
            def _():
                for cp in chunk(2 * jj + 1, False):
                    cp.wait()

            @pl.when(jj == NI - 1)
            def _():
                for cp in chunk(2 * jj + 1, True):
                    cp.wait()

            @pl.when(jj < NI - 1)
            def _():
                for cp in chunk(2 * jj + 2, False):
                    cp.start()

            @pl.when(jj < NI - 2)
            def _():
                for cp in chunk(2 * jj + 3, False):
                    cp.start()

            @pl.when(jj == NI - 2)
            def _():
                for cp in chunk(2 * jj + 3, True):
                    cp.start()

            for hf in range(UN):
                j = jj * UN + hf
                slot = j % NB
                may_last = hf == UN - 1
                for p in range(G // 2):
                    for r in range(NP):
                        gr = (hf * (G // 2) + p) * NP + r
                        ab, c = r // NSUB, r % NSUB
                        k = 2 * p + ab
                        while pend and pend[0][0] <= gr:
                            ln_tile(*pend.pop(0)[1:])
                        xn = pltpu.bitcast(xn_ref[_xn_slot(j, k) + z], bf16)
                        lhs = pltpu.bitcast(w1q_ref[MR // 2 * c:MR // 2 * (c + 1), :], bf16)
                        gl = _gelu2(jnp.dot(lhs, xn, preferred_element_type=f32))
                        sq = gl * gl
                        acc_ref[MR * c:MR * (c + 1), :] += (sq[:, 0:128] + sq[:, 128:256]) + (sq[:, 256:384] + sq[:, 384:512])
                        if k in ST:
                            h_ref[j * NST + ST.index(k), MR // 2 * c:MR // 2 * (c + 1), :] = _pack_pairs(gl)
                        if r == NP // 2 - 1:
                            kill = None
                            if may_last and p == 1:
                                kill = _iota((8, W), 0) >= jnp.where(j == NG - 1, 4, 8)
                            s1(xp.at[slot, p], (p + 3) % NU, kill)
                        for rr in range(r * RPP, (r + 1) * RPP):
                            q = (rr // 3 + 2) % 4
                            pair = p + 1 + (rr >= 6)
                            cur += conv_round(pair, q, range(4 * (rr % 3), 4 * (rr % 3) + 4))
                            if rr % 3 == 2:
                                pend.append((gr + LN_LAG, cur, q,
                                             (_xn_slot(j, 2 * pair) + z1, _xn_slot(j, 2 * pair + 1) + z1)))
                                cur = []
            for e in pend:
                ln_tile(*e[1:])
            return carry

        with jax.named_scope('loop1'):
            lax.fori_loop(0, NG // UN, body, 0)

        P = _perm16(_iota((E, E), 0)) == _iota((E, E), 1) + zs_ref[0]
        ssc = jnp.sum(acc_ref[...], axis=1, keepdims=True)
        ss = jnp.sum(jnp.where(P, jnp.broadcast_to(ssc, (E, E)), 0.0), axis=0, keepdims=True) * (_GS * _GS)
        gx = jnp.sqrt(ss + 1e-6)
        nx = gx / (jnp.sum(gx, axis=1, keepdims=True) * (1.0 / E) + 1e-6)
        gam = g_ref[...].astype(f32).reshape(1, E)
        bet = b_ref[...].astype(f32).reshape(1, E)
        s = (gam * nx + 1.0) * _GS
        w2t = w2t_ref[...].astype(f32)
        w2s_ref[...] = pltpu.bitcast((w2t * s).astype(bf16), u32)
        bias_ref[...] = jnp.broadcast_to(jnp.sum(w2t * bet, axis=1, keepdims=True), (C, 128))

    pl.run_scoped(phase1,
                  pltpu.VMEM((NB, 4, 12, 16, W), bf16),
                  pltpu.VMEM((NU, 12, NQ, 24, 128), u32),
                  pltpu.VMEM((E, 128), f32),
                  pltpu.VMEM((C, C), u32))

    def phase2(xbuf, ht_ref):
        def x_copy(j):
            return pltpu.make_async_copy(x_hbm.at[pl.ds(j * G, G)], xbuf.at[j % NB2], xsem.at[j % NB2])

        def o_copy(j):
            return pltpu.make_async_copy(xbuf.at[j % NB2], o_hbm.at[pl.ds(j * G, G)], osem.at[j % NB2])

        for j in range(2):
            x_copy(j).start()

        def body(jj, carry):
            z = zs_ref[0]
            x_copy(2 * jj).wait()
            x_copy(2 * jj + 1).wait()

            @pl.when(jj >= 2)
            def _():
                o_copy(2 * jj - 4).wait()
                o_copy(2 * jj - 3).wait()

            @pl.when(jj < NG // UN - 1)
            def _():
                x_copy(2 * jj + 2).start()
                x_copy(2 * jj + 3).start()

            for hf in range(UN):
                j = jj * UN + hf
                xs = j % NB2

                def fin(k, hu):
                    o = jnp.dot(pltpu.bitcast(w2s_ref[...], bf16), pltpu.bitcast(hu, bf16), preferred_element_type=f32)
                    xbuf[xs, k] = (o + _tile4(bias_ref[...]) + xbuf[xs, k].astype(f32)).astype(bf16)

                def mm1(n):
                    xn = pltpu.bitcast(xn_ref[j * NRC + n], bf16)
                    lhs = pltpu.bitcast(w1q_ref[...], bf16)
                    ht_ref[n % 2 + z] = _pack_pairs(_gelu2(jnp.dot(lhs, xn, preferred_element_type=f32)))

                for tok in P2ORD.split(','):
                    n = int(tok[1])
                    if tok[0] == 'M': mm1(n)
                    elif tok[0] == 'S': fin(ST[n], h_ref[j * NST + n])
                    elif tok[0] == 'F': fin(RC[n], ht_ref[n % 2 + z])

                o_copy(j).start()
            return carry

        with jax.named_scope('loop2'):
            lax.fori_loop(0, NG // UN, body, 0)
        for j in range(NG - 4, NG):
            o_copy(j).wait()

    pl.run_scoped(phase2,
                  pltpu.VMEM((NB2, G, C, W), bf16),
                  pltpu.VMEM((2, E // 2, W), u32))


@jax.jit
def pallas_standalone__modern_conv_block_convnext_v2__vision_kernel(x, dw, w1, w2, grn_gamma, grn_beta):
    xt = jnp.transpose(x, (0, 1, 3, 2)).reshape(H, C, W)
    x5 = xt.reshape(H // 2, 2, C // 8, 8, W)
    w2t = w2.T
    vm = pl.BlockSpec(memory_space=pltpu.VMEM)
    out = pl.pallas_call(
        _kernel,
        in_specs=[pl.BlockSpec(memory_space=pl.ANY), pl.BlockSpec(memory_space=pl.ANY), vm, vm, vm, vm, vm],
        out_specs=pl.BlockSpec(memory_space=pl.ANY),
        out_shape=jax.ShapeDtypeStruct((H, C, W), bf16),
        scratch_shapes=[
            pltpu.VMEM((NG * NST, E // 2, W), u32),
            pltpu.VMEM((XR0 + NST, C // 2, W), u32),
            pltpu.VMEM((E // 2, C), u32),
            pltpu.VMEM((C // 2, E), u32),
            pltpu.VMEM((C, 128), f32),
            pltpu.SMEM((2,), i32),
            pltpu.SemaphoreType.DMA((NB2,)),
            pltpu.SemaphoreType.DMA((NB2,)),
            pltpu.SemaphoreType.DMA((NB, 2)),
        ],
        compiler_params=pltpu.CompilerParams(vmem_limit_bytes=128 * 1024 * 1024),
    )(xt, x5, dw, w1, w2t, grn_gamma, grn_beta)
    return jnp.transpose(out.reshape(1, H, C, W), (0, 1, 3, 2))
```

```python
import math
import jax
import jax.numpy as jnp
from jax import lax
import jax.experimental.pallas as pl
import jax.experimental.pallas.tpu as pltpu

H = 512; W = 512; C = 96; E = 384
G = 16
NG = H // G
RC = tuple(range(0, G, 2))
ST = tuple(k for k in range(G) if k not in RC)
NST = len(ST)
NRC = len(RC)
NU = 4
NQ = W // 128
NRING = 4
XR0 = NG * NRC + 2
NB2 = 3
LN_LAG = 5
NSUB = 6
OROWS = 4

_C1 = math.sqrt(2.0 / math.pi)
_C3 = _C1 * 0.044715
_A = _C3 ** (1.0 / 3.0)
_K = _C1 / _A
_GS = 0.5 / _A

f32 = jnp.float32
bf16 = jnp.bfloat16
u32 = jnp.uint32
i32 = jnp.int32


def _iota(shape, d):
    return lax.broadcasted_iota(i32, shape, d)


def _perm16(r):
    return (r // 16) * 16 + 2 * (r % 8) + (r % 16) // 8


def _tile4(a):
    return jnp.concatenate([a] * NQ, axis=1)


def _pack_pairs(y):
    m = y.shape[0] // 16
    outs = [pltpu.pack_elementwise([y[16 * t:16 * t + 8], y[16 * t + 8:16 * t + 16]], packed_dtype=bf16)
            for t in range(m)]
    o = outs[0] if m == 1 else jnp.concatenate(outs, axis=0)
    return pltpu.bitcast(o, u32) if o.dtype != u32 else o


def _gelu2(y):
    u = y * (y * y + _K)
    t = jnp.tanh(u)
    return y * t + y


def _tree_sum(xs):
    xs = list(xs)
    while len(xs) > 1:
        xs = [xs[i] + xs[i + 1] for i in range(0, len(xs) - 1, 2)] + ([xs[-1]] if len(xs) % 2 else [])
    return xs[0]


def _xn_slot(j, k):
    jj, kk = k // G, k % G
    if kk in RC:
        return (j + jj) * NRC + RC.index(kk)
    return XR0 + ST.index(kk) % NRING


def _kernel(x_hbm, x5_hbm, dw_ref, w1_ref, w2t_ref, g_ref, b_ref, o_hbm,
            h_ref, xn_ref, w1q_ref, w2s_ref, bias_ref, zs_ref,
            xsem, osem, psem):

    for i in range(2):
        zs_ref[i] = 0

    def phase1(xp, ver_ref, acc_ref, cl_ref):
        def p_copy(u0, n, half, slot, dst0=0):
            src = x5_hbm.at[pl.ds(u0 - 1 + half, n), 1 - half]
            return pltpu.make_async_copy(src, xp.at[slot, pl.ds(dst0, n), :, pl.ds(8 * half, 8), :],
                                         psem.at[slot, half])

        NP2 = G // 2

        def chunk(j, last):
            return [p_copy(NP2 * j + 3, NP2 - 2 if last else NP2, 0, j % 2),
                    p_copy(NP2 * j + 3, NP2 - 3 if last else NP2, 1, j % 2)]

        p_copy(1, 2, 0, 1, 1).start()
        p_copy(0, 3, 1, 1).start()
        for cp in chunk(0, False):
            cp.start()

        acc_ref[...] = jnp.zeros_like(acc_ref)
        dw = dw_ref[...].astype(f32)
        R = _iota((2 * C, C), 0); KK = _iota((2 * C, C), 1)
        chm = KK == 8 * (R // 16) + R % 8
        itap = 2 * (KK // 48) + (KK % 16) // 8 - (R % 16) // 8
        ver = (KK % 48) // 16
        diag = KK % 8 == R % 8
        cl = jnp.zeros((2 * C, C), f32)
        for a in range(3):
            for b in range(3):
                row = jnp.broadcast_to(dw[a, b:b + 1, :], (2 * C, C))
                col = jnp.sum(jnp.where(chm, row, 0.0), axis=1, keepdims=True)
                cl = jnp.where(diag & (itap == a) & (ver == b), jnp.broadcast_to(col, (2 * C, C)), cl)
        cl_ref[...] = pltpu.bitcast(cl.astype(bf16), u32)

        Pb = jnp.where(_perm16(_iota((E, E), 0)) == _iota((E, E), 1), 1.0, 0.0).astype(bf16)
        w1f = w1_ref[...].astype(f32)
        w1c = (w1f - jnp.sum(w1f, axis=0, keepdims=True) * (1.0 / C)).astype(bf16)
        w1p = lax.dot_general(Pb, w1c, (((1,), (1,)), ((), ())), preferred_element_type=f32)
        r96 = _iota((C, C), 0); c96 = _iota((C, C), 1)
        Q = jnp.where(r96 == (c96 // 16) * 16 + (c96 % 16) // 2 + 8 * (c96 % 2), 1.0, 0.0).astype(bf16)
        w1q = jnp.dot(w1p.astype(bf16), Q, preferred_element_type=f32)
        w1q_ref[...] = pltpu.bitcast(w1q.astype(bf16), u32)

        lane = _iota((8, 128), 1)

        def s1(xu_ref, u, kill=None):
            zz = jnp.zeros((8, 128), u32)
            for g in range(12):
                m = pltpu.bitcast(xu_ref[g], u32)
                if kill is not None:
                    m = jnp.where(kill, jnp.zeros_like(m), m)
                mq = [m[:, 128 * q:128 * q + 128] for q in range(NQ)]
                for q in range(NQ):
                    lq = jnp.where(lane == 127, mq[q - 1] if q > 0 else zz, mq[q])
                    rq = jnp.where(lane == 0, mq[q + 1] if q + 1 < NQ else zz, mq[q])
                    ver_ref[u, g, q, 0:8, :] = pltpu.roll(lq, 1, 1)
                    ver_ref[u, g, q, 8:16, :] = mq[q]
                    ver_ref[u, g, q, 16:24, :] = pltpu.roll(rq, 127, 1)

        def conv_round(t, q, gs):
            cvs = []
            for g in gs:
                rhs = jnp.concatenate([ver_ref[t % NU, g, q], ver_ref[(t + 1) % NU, g, q]], axis=0)
                lhs = pltpu.bitcast(cl_ref[8 * g:8 * g + 8, :], bf16)
                cvs.append(jnp.dot(lhs, pltpu.bitcast(rhs, bf16), preferred_element_type=f32))
            return cvs

        sub = _iota((8, 128), 0)
        m0 = sub % 2 == 0
        m1 = (sub // 2) % 2 == 0
        lnc = jnp.where(m1, 1.0 / (C * _A), 1.0 / (C * _A * _A))

        def merge(a, b, msk, sh):
            return jnp.where(msk, a, b) + pltpu.roll(jnp.where(msk, b, a), 8 - sh, 0)

        def ln_tile(cvs, q, dsts):
            ls = slice(128 * q, 128 * q + 128)
            cs = [[cv[8 * ab:8 * ab + 8] for cv in cvs] for ab in range(2)]
            c1 = merge(_tree_sum(cs[0]), _tree_sum(cs[1]), m0, 1)
            c2 = merge(_tree_sum([c * c for c in cs[0]]), _tree_sum([c * c for c in cs[1]]), m0, 1)
            e = merge(c1, c2, m1, 2)
            f = (e + pltpu.roll(e, 4, 0)) * lnc
            v = pltpu.roll(f, 6, 0) - f * f
            rs = lax.rsqrt(jnp.maximum(v, 0.0) + 1e-5 / (_A * _A))
            for ab in range(2):
                xn_ref[dsts[ab], :, ls] = _pack_pairs(jnp.concatenate(cs[ab], axis=0) * rs[ab:ab + 1, :])

        xp[1, 0, :, 0:8, :] = jnp.zeros((12, 8, W), bf16)
        p_copy(1, 2, 0, 1, 1).wait()
        p_copy(0, 3, 1, 1).wait()
        for u in range(3):
            s1(xp.at[1, u], u)
        for q in range(NQ):
            ln_tile(conv_round(0, q, range(12)), q, (_xn_slot(0, 0), _xn_slot(0, 1)))
        for q in range(2):
            ln_tile(conv_round(1, q, range(12)), q, (_xn_slot(0, 2), _xn_slot(0, 3)))

        NP = 2 * NSUB
        RPP = 12 // NP
        MR = E // NSUB

        def body(j, carry):
            z = zs_ref[0]
            z1 = zs_ref[1]
            slot = j % 2

            @pl.when(j < NG - 1)
            def _():
                for cp in chunk(j, False):
                    cp.wait()

            @pl.when(j == NG - 1)
            def _():
                for cp in chunk(j, True):
                    cp.wait()

            @pl.when(j < NG - 2)
            def _():
                for cp in chunk(j + 1, False):
                    cp.start()

            @pl.when(j == NG - 2)
            def _():
                for cp in chunk(j + 1, True):
                    cp.start()

            pend = []
            cur = []
            for p in range(NP2):
                for r in range(NP):
                    gr = p * NP + r
                    ab, c = r // NSUB, r % NSUB
                    k = 2 * p + ab
                    while pend and pend[0][0] <= gr:
                        ln_tile(*pend.pop(0)[1:])
                    xn = pltpu.bitcast(xn_ref[_xn_slot(j, k) + z], bf16)
                    lhs = pltpu.bitcast(w1q_ref[MR // 2 * c:MR // 2 * (c + 1), :], bf16)
                    gl = _gelu2(jnp.dot(lhs, xn, preferred_element_type=f32))
                    sq = gl * gl
                    acc_ref[MR * c:MR * (c + 1), :] += (sq[:, 0:128] + sq[:, 128:256]) + (sq[:, 256:384] + sq[:, 384:512])
                    if k in ST:
                        h_ref[j * NST + ST.index(k), MR // 2 * c:MR // 2 * (c + 1), :] = _pack_pairs(gl)
                    if r == NP // 2 - 1:
                        kill = None
                        if p == NP2 - 3:
                            kill = _iota((8, W), 0) >= jnp.where(j == NG - 1, 4, 8)
                        s1(xp.at[slot, p], (p + 3) % NU, kill)
                    for rr in range(r * RPP, (r + 1) * RPP):
                        q = (rr // 3 + 2) % 4
                        pair = p + 1 + (rr >= 6)
                        cur += conv_round(pair, q, range(4 * (rr % 3), 4 * (rr % 3) + 4))
                        if rr % 3 == 2:
                            pend.append((gr + LN_LAG, cur, q,
                                         (_xn_slot(j, 2 * pair) + z1, _xn_slot(j, 2 * pair + 1) + z1)))
                            cur = []
            for e in pend:
                ln_tile(*e[1:])
            return carry

        with jax.named_scope('loop1'):
            lax.fori_loop(0, NG, body, 0)

        P = _perm16(_iota((E, E), 0)) == _iota((E, E), 1) + zs_ref[0]
        ssc = jnp.sum(acc_ref[...], axis=1, keepdims=True)
        ss = jnp.sum(jnp.where(P, jnp.broadcast_to(ssc, (E, E)), 0.0), axis=0, keepdims=True) * (_GS * _GS)
        gx = jnp.sqrt(ss + 1e-6)
        nx = gx / (jnp.sum(gx, axis=1, keepdims=True) * (1.0 / E) + 1e-6)
        gam = g_ref[...].astype(f32).reshape(1, E)
        bet = b_ref[...].astype(f32).reshape(1, E)
        s = (gam * nx + 1.0) * _GS
        w2t = w2t_ref[...].astype(f32)
        w2s_ref[...] = pltpu.bitcast((w2t * s).astype(bf16), u32)
        bias_ref[...] = jnp.broadcast_to(jnp.sum(w2t * bet, axis=1, keepdims=True), (C, 128))

    pl.run_scoped(phase1,
                  pltpu.VMEM((2, G // 2, 12, 16, W), bf16),
                  pltpu.VMEM((NU, 12, NQ, 24, 128), u32),
                  pltpu.VMEM((E, 128), f32),
                  pltpu.VMEM((C, C), u32))

    def phase2(xbuf, ht_ref):
        def x_copy(j):
            return pltpu.make_async_copy(x_hbm.at[pl.ds(j * G, G)], xbuf.at[j % NB2], xsem.at[j % NB2])

        def o_copy(j, r0, n):
            return pltpu.make_async_copy(xbuf.at[j % NB2, pl.ds(r0, n)], o_hbm.at[pl.ds(j * G + r0, n)],
                                         osem.at[j % NB2])

        x_copy(0).start()

        def body(j, carry):
            z = zs_ref[0]
            xs = j % NB2
            x_copy(j).wait()

            @pl.when(j >= 2)
            def _():
                o_copy(j - 2, 0, G).wait()

            @pl.when(j < NG - 1)
            def _():
                x_copy(j + 1).start()

            def fin(k, hu):
                o = jnp.dot(pltpu.bitcast(w2s_ref[...], bf16), pltpu.bitcast(hu, bf16), preferred_element_type=f32)
                xbuf[xs, k] = (o + _tile4(bias_ref[...]) + xbuf[xs, k].astype(f32)).astype(bf16)

            def mm1(n):
                xn = pltpu.bitcast(xn_ref[j * NRC + n], bf16)
                lhs = pltpu.bitcast(w1q_ref[...], bf16)
                ht_ref[n % 2 + z] = _pack_pairs(_gelu2(jnp.dot(lhs, xn, preferred_element_type=f32)))

            mm1(0)
            for n in range(NRC):
                fin(ST[n], h_ref[j * NST + n])
                if n + 1 < NRC:
                    mm1(n + 1)
                fin(RC[n], ht_ref[n % 2 + z])
                if (2 * n + 2) % OROWS == 0:
                    o_copy(j, 2 * n + 2 - OROWS, OROWS).start()
            return carry

        with jax.named_scope('loop2'):
            lax.fori_loop(0, NG, body, 0)
        for j in range(NG - 2, NG):
            o_copy(j, 0, G).wait()

    pl.run_scoped(phase2,
                  pltpu.VMEM((NB2, G, C, W), bf16),
                  pltpu.VMEM((2, E // 2, W), u32))


@jax.jit
def pallas_standalone__modern_conv_block_convnext_v2__vision_kernel(x, dw, w1, w2, grn_gamma, grn_beta):
    xt = jnp.transpose(x, (0, 1, 3, 2)).reshape(H, C, W)
    x5 = xt.reshape(H // 2, 2, C // 8, 8, W)
    w2t = w2.T
    vm = pl.BlockSpec(memory_space=pltpu.VMEM)
    out = pl.pallas_call(
        _kernel,
        in_specs=[pl.BlockSpec(memory_space=pl.ANY), pl.BlockSpec(memory_space=pl.ANY), vm, vm, vm, vm, vm],
        out_specs=pl.BlockSpec(memory_space=pl.ANY),
        out_shape=jax.ShapeDtypeStruct((H, C, W), bf16),
        scratch_shapes=[
            pltpu.VMEM((NG * NST, E // 2, W), u32),
            pltpu.VMEM((XR0 + NRING, C // 2, W), u32),
            pltpu.VMEM((E // 2, C), u32),
            pltpu.VMEM((C // 2, E), u32),
            pltpu.VMEM((C, 128), f32),
            pltpu.SMEM((2,), i32),
            pltpu.SemaphoreType.DMA((NB2,)),
            pltpu.SemaphoreType.DMA((NB2,)),
            pltpu.SemaphoreType.DMA((2, 2)),
        ],
        compiler_params=pltpu.CompilerParams(vmem_limit_bytes=128 * 1024 * 1024),
    )(xt, x5, dw, w1, w2t, grn_gamma, grn_beta)
    return jnp.transpose(out.reshape(1, H, C, W), (0, 1, 3, 2))
```

```python
import math
import jax
import jax.numpy as jnp
from jax import lax
import jax.experimental.pallas as pl
import jax.experimental.pallas.tpu as pltpu

H = 512; W = 512; C = 96; E = 384
G = 16
NG = H // G
RC = tuple(range(0, G, 2))
ST = tuple(k for k in range(G) if k not in RC)
NST = len(ST)
NRC = len(RC)
NU = 2
NQ = W // 128
NRING = 4
XR0 = NG * NRC + 2
NB2 = 3
LN_LAG = 5
NSUB = 6
OROWS = 2

_C1 = math.sqrt(2.0 / math.pi)
_C3 = _C1 * 0.044715
_A = _C3 ** (1.0 / 3.0)
_K = _C1 / _A
_GS = 0.5 / _A

f32 = jnp.float32
bf16 = jnp.bfloat16
u32 = jnp.uint32
i32 = jnp.int32


def _iota(shape, d):
    return lax.broadcasted_iota(i32, shape, d)


def _perm16(r):
    return (r // 16) * 16 + 2 * (r % 8) + (r % 16) // 8


def _tile4(a):
    return jnp.concatenate([a] * NQ, axis=1)


def _pack_pairs(y):
    m = y.shape[0] // 16
    outs = [pltpu.pack_elementwise([y[16 * t:16 * t + 8], y[16 * t + 8:16 * t + 16]], packed_dtype=bf16)
            for t in range(m)]
    o = outs[0] if m == 1 else jnp.concatenate(outs, axis=0)
    return pltpu.bitcast(o, u32) if o.dtype != u32 else o


def _gelu2(y):
    u = y * (y * y + _K)
    t = jnp.tanh(u)
    return y * t + y


def _tree_sum(xs):
    xs = list(xs)
    while len(xs) > 1:
        xs = [xs[i] + xs[i + 1] for i in range(0, len(xs) - 1, 2)] + ([xs[-1]] if len(xs) % 2 else [])
    return xs[0]


def _xn_slot(j, k):
    jj, kk = k // G, k % G
    if kk in RC:
        return (j + jj) * NRC + RC.index(kk)
    return XR0 + ST.index(kk) % NRING


def _kernel(x_hbm, x5_hbm, dw_ref, w1_ref, w2t_ref, g_ref, b_ref, o_hbm,
            h_ref, xn_ref, xbuf, w1q_ref, w2s_ref, bias_ref, zs_ref,
            xsem, osem, psem):

    for i in range(2):
        zs_ref[i] = 0

    def x_copy(j, sl):
        return pltpu.make_async_copy(x_hbm.at[pl.ds(j * G, G)], xbuf.at[sl], xsem.at[sl])

    def phase1(ver_ref, acc_ref, cl_ref):
        xp = xbuf.reshape(NB2, G // 2, C // 8, 16, W).at[pl.ds(1, 2)]
        def p_copy(u0, n, half, slot, dst0=0):
            src = x5_hbm.at[pl.ds(u0 - 1 + half, n), 1 - half]
            return pltpu.make_async_copy(src, xp.at[slot, pl.ds(dst0, n), :, pl.ds(8 * half, 8), :],
                                         psem.at[slot, half])

        NP2 = G // 2

        def chunk(j, last):
            return [p_copy(NP2 * j + 3, NP2 - 2 if last else NP2, 0, j & 1),
                    p_copy(NP2 * j + 3, NP2 - 3 if last else NP2, 1, j & 1)]

        p_copy(1, 2, 0, 1, 1).start()
        p_copy(0, 3, 1, 1).start()
        for cp in chunk(0, False):
            cp.start()
        x_copy(0, 0).start()

        acc_ref[...] = jnp.zeros_like(acc_ref)
        dw = dw_ref[...].astype(f32)
        R = _iota((2 * C, C), 0); KK = _iota((2 * C, C), 1)
        chm = KK == 8 * (R // 16) + R % 8
        itap = 2 * (KK // 48) + (KK % 16) // 8 - (R % 16) // 8
        ver = (KK % 48) // 16
        diag = KK % 8 == R % 8
        cl = jnp.zeros((2 * C, C), f32)
        for a in range(3):
            for b in range(3):
                row = jnp.broadcast_to(dw[a, b:b + 1, :], (2 * C, C))
                col = jnp.sum(jnp.where(chm, row, 0.0), axis=1, keepdims=True)
                cl = jnp.where(diag & (itap == a) & (ver == b), jnp.broadcast_to(col, (2 * C, C)), cl)
        cl_ref[...] = pltpu.bitcast(cl.astype(bf16), u32)

        Pb = jnp.where(_perm16(_iota((E, E), 0)) == _iota((E, E), 1), 1.0, 0.0).astype(bf16)
        w1f = w1_ref[...].astype(f32)
        w1c = (w1f - jnp.sum(w1f, axis=0, keepdims=True) * (1.0 / C)).astype(bf16)
        w1p = lax.dot_general(Pb, w1c, (((1,), (1,)), ((), ())), preferred_element_type=f32)
        r96 = _iota((C, C), 0); c96 = _iota((C, C), 1)
        Q = jnp.where(r96 == (c96 // 16) * 16 + (c96 % 16) // 2 + 8 * (c96 % 2), 1.0, 0.0).astype(bf16)
        w1q = jnp.dot(w1p.astype(bf16), Q, preferred_element_type=f32)
        w1q_ref[...] = pltpu.bitcast(w1q.astype(bf16), u32)

        lane = _iota((8, 128), 1)

        def s1(xu_ref, u, kill=None):
            zz = jnp.zeros((8, 128), u32)
            for g in range(12):
                m = pltpu.bitcast(xu_ref[g], u32)
                if kill is not None:
                    m = jnp.where(kill, jnp.zeros_like(m), m)
                mq = [m[:, 128 * q:128 * q + 128] for q in range(NQ)]
                for q in range(NQ):
                    lq = jnp.where(lane == 127, mq[q - 1] if q > 0 else zz, mq[q])
                    rq = jnp.where(lane == 0, mq[q + 1] if q + 1 < NQ else zz, mq[q])
                    ver_ref[u, g, q, 0:8, :] = pltpu.roll(lq, 1, 1)
                    ver_ref[u, g, q, 8:16, :] = mq[q]
                    ver_ref[u, g, q, 16:24, :] = pltpu.roll(rq, 127, 1)

        def conv_round(t, q, gs):
            cvs = []
            for g in gs:
                rhs = jnp.concatenate([ver_ref[t % NU, g, q], ver_ref[(t + 1) % NU, g, q]], axis=0)
                lhs = pltpu.bitcast(cl_ref[8 * g:8 * g + 8, :], bf16)
                cvs.append(jnp.dot(lhs, pltpu.bitcast(rhs, bf16), preferred_element_type=f32))
            return cvs

        sub = _iota((8, 128), 0)
        m0 = sub % 2 == 0
        m1 = (sub // 2) % 2 == 0
        lnc = jnp.where(m1, 1.0 / (C * _A), 1.0 / (C * _A * _A))

        def merge(a, b, msk, sh):
            return jnp.where(msk, a, b) + pltpu.roll(jnp.where(msk, b, a), 8 - sh, 0)

        def ln_tile(cvs, q, dsts):
            ls = slice(128 * q, 128 * q + 128)
            cs = [[cv[8 * ab:8 * ab + 8] for cv in cvs] for ab in range(2)]
            c1 = merge(_tree_sum(cs[0]), _tree_sum(cs[1]), m0, 1)
            c2 = merge(_tree_sum([c * c for c in cs[0]]), _tree_sum([c * c for c in cs[1]]), m0, 1)
            e = merge(c1, c2, m1, 2)
            f = (e + pltpu.roll(e, 4, 0)) * lnc
            v = pltpu.roll(f, 6, 0) - f * f
            rs = lax.rsqrt(jnp.maximum(v, 0.0) + 1e-5 / (_A * _A))
            for ab in range(2):
                xn_ref[dsts[ab], :, ls] = _pack_pairs(jnp.concatenate(cs[ab], axis=0) * rs[ab:ab + 1, :])

        xp[1, 0, :, 0:8, :] = jnp.zeros((12, 8, W), bf16)
        p_copy(1, 2, 0, 1, 1).wait()
        p_copy(0, 3, 1, 1).wait()
        for u in range(2):
            s1(xp.at[1, u], u)
        for q in range(NQ):
            ln_tile(conv_round(0, q, range(12)), q, (_xn_slot(0, 0), _xn_slot(0, 1)))
        s1(xp.at[1, 2], 2 % NU)
        for q in range(2):
            ln_tile(conv_round(1, q, range(12)), q, (_xn_slot(0, 2), _xn_slot(0, 3)))

        NP = 2 * NSUB
        RPP = 12 // NP
        MR = E // NSUB

        def body(j, carry):
            z = zs_ref[0]
            z1 = zs_ref[1]
            slot = j & 1

            @pl.when(j < NG - 1)
            def _():
                for cp in chunk(j, False):
                    cp.wait()

            @pl.when(j == NG - 1)
            def _():
                for cp in chunk(j, True):
                    cp.wait()

            @pl.when(j < NG - 2)
            def _():
                for cp in chunk(j + 1, False):
                    cp.start()

            @pl.when(j == NG - 2)
            def _():
                for cp in chunk(j + 1, True):
                    cp.start()

            pend = []
            cur = []
            for p in range(NP2):
                for r in range(NP):
                    gr = p * NP + r
                    ab, c = r // NSUB, r % NSUB
                    k = 2 * p + ab
                    while pend and pend[0][0] <= gr:
                        ln_tile(*pend.pop(0)[1:])
                    xn = pltpu.bitcast(xn_ref[_xn_slot(j, k) + z], bf16)
                    lhs = pltpu.bitcast(w1q_ref[MR // 2 * c:MR // 2 * (c + 1), :], bf16)
                    gl = _gelu2(jnp.dot(lhs, xn, preferred_element_type=f32))
                    sq = gl * gl
                    acc_ref[MR * c:MR * (c + 1), :] += (sq[:, 0:128] + sq[:, 128:256]) + (sq[:, 256:384] + sq[:, 384:512])
                    if k in ST:
                        h_ref[j * NST + ST.index(k), MR // 2 * c:MR // 2 * (c + 1), :] = _pack_pairs(gl)
                    for rr in range(r * RPP, (r + 1) * RPP):
                        q = (rr // 3 + 2) % 4
                        pair = p + 1 + (rr >= 6)
                        cur += conv_round(pair, q, range(4 * (rr % 3), 4 * (rr % 3) + 4))
                        if rr % 3 == 2:
                            pend.append((gr + LN_LAG, cur, q,
                                         (_xn_slot(j, 2 * pair) + z1, _xn_slot(j, 2 * pair + 1) + z1)))
                            cur = []
                    if r == NP // 2 - 1:
                        kill = None
                        if p == NP2 - 3:
                            kill = _iota((8, W), 0) >= jnp.where(j == NG - 1, 4, 8)
                        s1(xp.at[slot, p], (p + 3) % NU, kill)
            for e in pend:
                ln_tile(*e[1:])
            return carry

        with jax.named_scope('loop1'):
            lax.fori_loop(0, NG, body, 0)

        P = _perm16(_iota((E, E), 0)) == _iota((E, E), 1) + zs_ref[0]
        ssc = jnp.sum(acc_ref[...], axis=1, keepdims=True)
        ss = jnp.sum(jnp.where(P, jnp.broadcast_to(ssc, (E, E)), 0.0), axis=0, keepdims=True) * (_GS * _GS)
        gx = jnp.sqrt(ss + 1e-6)
        nx = gx / (jnp.sum(gx, axis=1, keepdims=True) * (1.0 / E) + 1e-6)
        gam = g_ref[...].astype(f32).reshape(1, E)
        bet = b_ref[...].astype(f32).reshape(1, E)
        s = (gam * nx + 1.0) * _GS
        w2t = w2t_ref[...].astype(f32)
        w2s_ref[...] = pltpu.bitcast((w2t * s).astype(bf16), u32)
        bias_ref[...] = jnp.broadcast_to(jnp.sum(w2t * bet, axis=1, keepdims=True), (C, 128))

    pl.run_scoped(phase1,
                  pltpu.VMEM((NU, 12, NQ, 24, 128), u32),
                  pltpu.VMEM((E, 128), f32),
                  pltpu.VMEM((C, C), u32))

    def phase2(ht_ref):
        def o_copy(j, sl, r0, n):
            return pltpu.make_async_copy(xbuf.at[sl, pl.ds(r0, n)], o_hbm.at[pl.ds(j * G + r0, n)], osem.at[sl])

        def body(j, xs):
            z = zs_ref[0]
            xs1 = jnp.where(xs == NB2 - 1, 0, xs + 1)
            x_copy(j, xs).wait()

            @pl.when(j >= 2)
            def _():
                o_copy(j - 2, xs1, 0, G).wait()

            @pl.when(j < NG - 1)
            def _():
                x_copy(j + 1, xs1).start()

            def fin(k, hu):
                o = jnp.dot(pltpu.bitcast(w2s_ref[...], bf16), pltpu.bitcast(hu, bf16), preferred_element_type=f32)
                xbuf[xs, k] = (o + _tile4(bias_ref[...]) + xbuf[xs, k].astype(f32)).astype(bf16)

            def mm1(n):
                xn = pltpu.bitcast(xn_ref[j * NRC + n], bf16)
                lhs = pltpu.bitcast(w1q_ref[...], bf16)
                ht_ref[n % 2 + z] = _pack_pairs(_gelu2(jnp.dot(lhs, xn, preferred_element_type=f32)))

            mm1(0)
            for n in range(NRC):
                fin(ST[n], h_ref[j * NST + n])
                if n + 1 < NRC:
                    mm1(n + 1)
                fin(RC[n], ht_ref[n % 2 + z])
                if (2 * n + 2) % OROWS == 0:
                    o_copy(j, xs, 2 * n + 2 - OROWS, OROWS).start()
            return xs1

        with jax.named_scope('loop2'):
            lax.fori_loop(0, NG, body, jnp.int32(0))
        for j in range(NG - 2, NG):
            o_copy(j, j % NB2, 0, G).wait()

    pl.run_scoped(phase2,
                  pltpu.VMEM((2, E // 2, W), u32))


@jax.jit
def pallas_standalone__modern_conv_block_convnext_v2__vision_kernel(x, dw, w1, w2, grn_gamma, grn_beta):
    xt = jnp.transpose(x, (0, 1, 3, 2)).reshape(H, C, W)
    x5 = xt.reshape(H // 2, 2, C // 8, 8, W)
    w2t = w2.T
    vm = pl.BlockSpec(memory_space=pltpu.VMEM)
    out = pl.pallas_call(
        _kernel,
        in_specs=[pl.BlockSpec(memory_space=pl.ANY), pl.BlockSpec(memory_space=pl.ANY), vm, vm, vm, vm, vm],
        out_specs=pl.BlockSpec(memory_space=pl.ANY),
        out_shape=jax.ShapeDtypeStruct((H, C, W), bf16),
        scratch_shapes=[
            pltpu.VMEM((NG * NST, E // 2, W), u32),
            pltpu.VMEM((XR0 + NRING, C // 2, W), u32),
            pltpu.VMEM((NB2, G, C, W), bf16),
            pltpu.VMEM((E // 2, C), u32),
            pltpu.VMEM((C // 2, E), u32),
            pltpu.VMEM((C, 128), f32),
            pltpu.SMEM((2,), i32),
            pltpu.SemaphoreType.DMA((NB2,)),
            pltpu.SemaphoreType.DMA((NB2,)),
            pltpu.SemaphoreType.DMA((2, 2)),
        ],
        compiler_params=pltpu.CompilerParams(vmem_limit_bytes=128 * 1024 * 1024,
                                             disable_bounds_checks=True),
    )(xt, x5, dw, w1, w2t, grn_gamma, grn_beta)
    return jnp.transpose(out.reshape(1, H, C, W), (0, 1, 3, 2))
```

```python
import math
import jax
import jax.numpy as jnp
from jax import lax
import jax.experimental.pallas as pl
import jax.experimental.pallas.tpu as pltpu

H = 512; W = 512; C = 96; E = 384
G = 16
NG = H // G
RC = tuple(range(0, G, 2))
ST = tuple(k for k in range(G) if k not in RC)
NST = len(ST)
NRC = len(RC)
NU = 2
NQ = W // 128
NRING = 4
XR0 = NG * NRC + 2
NB2 = 3
LN_LAG = 5
NSUB = 6
OROWS = 2

_C1 = math.sqrt(2.0 / math.pi)
_C3 = _C1 * 0.044715
_A = _C3 ** (1.0 / 3.0)
_K = _C1 / _A
_GS = 0.5 / _A

f32 = jnp.float32
bf16 = jnp.bfloat16
u32 = jnp.uint32
i32 = jnp.int32


def _iota(shape, d):
    return lax.broadcasted_iota(i32, shape, d)


def _perm16(r):
    return (r // 16) * 16 + 2 * (r % 8) + (r % 16) // 8


def _tile4(a):
    return jnp.concatenate([a] * NQ, axis=1)


def _pack_pairs(y):
    m = y.shape[0] // 16
    outs = [pltpu.pack_elementwise([y[16 * t:16 * t + 8], y[16 * t + 8:16 * t + 16]], packed_dtype=bf16)
            for t in range(m)]
    o = outs[0] if m == 1 else jnp.concatenate(outs, axis=0)
    return pltpu.bitcast(o, u32) if o.dtype != u32 else o


def _gelu2(y):
    u = y * (y * y + _K)
    t = jnp.tanh(u)
    return y * t + y


def _tree_sum(xs):
    xs = list(xs)
    while len(xs) > 1:
        xs = [xs[i] + xs[i + 1] for i in range(0, len(xs) - 1, 2)] + ([xs[-1]] if len(xs) % 2 else [])
    return xs[0]


def _xn_slot(j, k):
    jj, kk = k // G, k % G
    if kk in RC:
        return (j + jj) * NRC + RC.index(kk)
    return XR0 + ST.index(kk) % NRING


def _kernel(x_hbm, x5_hbm, dw_ref, w1_ref, w2t_ref, g_ref, b_ref, dw2_ref, o_hbm,
            h_ref, xn_ref, xbuf, w1q_ref, w2s_ref, bias_ref, zs_ref,
            xsem, osem, psem):

    for i in range(2):
        zs_ref[i] = 0

    def x_copy(j, sl):
        return pltpu.make_async_copy(x_hbm.at[pl.ds(j * G, G)], xbuf.at[sl], xsem.at[sl])

    def phase1(ver_ref, acc_ref, cl_ref):
        xp = xbuf.reshape(NB2, G // 2, C // 8, 16, W).at[pl.ds(1, 2)]
        def p_copy(u0, n, half, slot, dst0=0):
            src = x5_hbm.at[pl.ds(u0 - 1 + half, n), 1 - half]
            return pltpu.make_async_copy(src, xp.at[slot, pl.ds(dst0, n), :, pl.ds(8 * half, 8), :],
                                         psem.at[slot, half])

        NP2 = G // 2

        def chunk(j, last):
            return [p_copy(NP2 * j + 3, NP2 - 2 if last else NP2, 0, j & 1),
                    p_copy(NP2 * j + 3, NP2 - 3 if last else NP2, 1, j & 1)]

        p_copy(1, 2, 0, 1, 1).start()
        p_copy(0, 3, 1, 1).start()
        for cp in chunk(0, False):
            cp.start()

        acc_ref[...] = jnp.zeros_like(acc_ref)
        dw = jnp.concatenate([dw_ref[0:2].astype(f32), dw2_ref[2:3].astype(f32)], axis=0)
        R = _iota((2 * C, C), 0); KK = _iota((2 * C, C), 1)
        chm = KK == 8 * (R // 16) + R % 8
        itap = 2 * (KK // 48) + (KK % 16) // 8 - (R % 16) // 8
        ver = (KK % 48) // 16
        diag = KK % 8 == R % 8
        cl = jnp.zeros((2 * C, C), f32)
        for a in range(3):
            for b in range(3):
                row = jnp.broadcast_to(dw[a, b:b + 1, :], (2 * C, C))
                col = jnp.sum(jnp.where(chm, row, 0.0), axis=1, keepdims=True)
                cl = jnp.where(diag & (itap == a) & (ver == b), jnp.broadcast_to(col, (2 * C, C)), cl)
        cl_ref[...] = pltpu.bitcast(cl.astype(bf16), u32)

        Pb = jnp.where(_perm16(_iota((E, E), 0)) == _iota((E, E), 1), 1.0, 0.0).astype(bf16)
        w1f = w1_ref[...].astype(f32)
        w1c = (w1f - jnp.sum(w1f, axis=0, keepdims=True) * (1.0 / C)).astype(bf16)
        w1p = lax.dot_general(Pb, w1c, (((1,), (1,)), ((), ())), preferred_element_type=f32)
        r96 = _iota((C, C), 0); c96 = _iota((C, C), 1)
        Q = jnp.where(r96 == (c96 // 16) * 16 + (c96 % 16) // 2 + 8 * (c96 % 2), 1.0, 0.0).astype(bf16)
        w1q = jnp.dot(w1p.astype(bf16), Q, preferred_element_type=f32)
        w1q_ref[...] = pltpu.bitcast(w1q.astype(bf16), u32)

        lane = _iota((8, 128), 1)

        def s1(xu_ref, u, kill=None):
            zz = jnp.zeros((8, 128), u32)
            for g in range(12):
                m = pltpu.bitcast(xu_ref[g], u32)
                if kill is not None:
                    m = jnp.where(kill, jnp.zeros_like(m), m)
                mq = [m[:, 128 * q:128 * q + 128] for q in range(NQ)]
                for q in range(NQ):
                    lq = jnp.where(lane == 127, mq[q - 1] if q > 0 else zz, mq[q])
                    rq = jnp.where(lane == 0, mq[q + 1] if q + 1 < NQ else zz, mq[q])
                    ver_ref[u, g, q, 0:8, :] = pltpu.roll(lq, 1, 1)
                    ver_ref[u, g, q, 8:16, :] = mq[q]
                    ver_ref[u, g, q, 16:24, :] = pltpu.roll(rq, 127, 1)

        def conv_round(t, q, gs):
            cvs = []
            for g in gs:
                rhs = jnp.concatenate([ver_ref[t % NU, g, q], ver_ref[(t + 1) % NU, g, q]], axis=0)
                lhs = pltpu.bitcast(cl_ref[8 * g:8 * g + 8, :], bf16)
                cvs.append(jnp.dot(lhs, pltpu.bitcast(rhs, bf16), preferred_element_type=f32))
            return cvs

        sub = _iota((8, 128), 0)
        m0 = sub % 2 == 0
        m1 = (sub // 2) % 2 == 0
        lnc = jnp.where(m1, 1.0 / (C * _A), 1.0 / (C * _A * _A))

        def merge(a, b, msk, sh):
            return jnp.where(msk, a, b) + pltpu.roll(jnp.where(msk, b, a), 8 - sh, 0)

        def ln_tile(cvs, q, dsts):
            ls = slice(128 * q, 128 * q + 128)
            cs = [[cv[8 * ab:8 * ab + 8] for cv in cvs] for ab in range(2)]
            c1 = merge(_tree_sum(cs[0]), _tree_sum(cs[1]), m0, 1)
            c2 = merge(_tree_sum([c * c for c in cs[0]]), _tree_sum([c * c for c in cs[1]]), m0, 1)
            e = merge(c1, c2, m1, 2)
            f = (e + pltpu.roll(e, 4, 0)) * lnc
            v = pltpu.roll(f, 6, 0) - f * f
            rs = lax.rsqrt(jnp.maximum(v, 0.0) + 1e-5 / (_A * _A))
            for ab in range(2):
                xn_ref[dsts[ab], :, ls] = _pack_pairs(jnp.concatenate(cs[ab], axis=0) * rs[ab:ab + 1, :])

        xp[1, 0, :, 0:8, :] = jnp.zeros((12, 8, W), bf16)
        p_copy(1, 2, 0, 1, 1).wait()
        p_copy(0, 3, 1, 1).wait()
        for u in range(2):
            s1(xp.at[1, u], u)
        for q in range(NQ):
            ln_tile(conv_round(0, q, range(12)), q, (_xn_slot(0, 0), _xn_slot(0, 1)))
        s1(xp.at[1, 2], 2 % NU)
        for q in range(2):
            ln_tile(conv_round(1, q, range(12)), q, (_xn_slot(0, 2), _xn_slot(0, 3)))

        NP = 2 * NSUB
        RPP = 12 // NP
        MR = E // NSUB

        def body(j, carry):
            z = zs_ref[0]
            z1 = zs_ref[1]
            slot = j & 1

            @pl.when(j < NG - 1)
            def _():
                for cp in chunk(j, False):
                    cp.wait()

            @pl.when(j == NG - 1)
            def _():
                for cp in chunk(j, True):
                    cp.wait()
                x_copy(0, 0).start()

            @pl.when(j < NG - 2)
            def _():
                for cp in chunk(j + 1, False):
                    cp.start()

            @pl.when(j == NG - 2)
            def _():
                for cp in chunk(j + 1, True):
                    cp.start()

            pend = []
            cur = []
            for p in range(NP2):
                for r in range(NP):
                    gr = p * NP + r
                    ab, c = r // NSUB, r % NSUB
                    k = 2 * p + ab
                    while pend and pend[0][0] <= gr:
                        ln_tile(*pend.pop(0)[1:])
                    xn = pltpu.bitcast(xn_ref[_xn_slot(j, k) + z], bf16)
                    lhs = pltpu.bitcast(w1q_ref[MR // 2 * c:MR // 2 * (c + 1), :], bf16)
                    gl = _gelu2(jnp.dot(lhs, xn, preferred_element_type=f32))
                    sq = gl * gl
                    acc_ref[MR * c:MR * (c + 1), :] += (sq[:, 0:128] + sq[:, 128:256]) + (sq[:, 256:384] + sq[:, 384:512])
                    if k in ST:
                        h_ref[j * NST + ST.index(k), MR // 2 * c:MR // 2 * (c + 1), :] = _pack_pairs(gl)
                    for rr in range(r * RPP, (r + 1) * RPP):
                        q = (rr // 3 + 2) % 4
                        pair = p + 1 + (rr >= 6)
                        cur += conv_round(pair, q, range(4 * (rr % 3), 4 * (rr % 3) + 4))
                        if rr % 3 == 2:
                            pend.append((gr + LN_LAG, cur, q,
                                         (_xn_slot(j, 2 * pair) + z1, _xn_slot(j, 2 * pair + 1) + z1)))
                            cur = []
                    if r == NP // 2 - 1:
                        kill = None
                        if p == NP2 - 3:
                            kill = _iota((8, W), 0) >= jnp.where(j == NG - 1, 4, 8)
                        s1(xp.at[slot, p], (p + 3) % NU, kill)
            for e in pend:
                ln_tile(*e[1:])
            return carry

        with jax.named_scope('loop1'):
            lax.fori_loop(0, NG, body, 0)

        P = _perm16(_iota((E, E), 0)) == _iota((E, E), 1) + zs_ref[0]
        ssc = jnp.sum(acc_ref[...], axis=1, keepdims=True)
        ss = jnp.sum(jnp.where(P, jnp.broadcast_to(ssc, (E, E)), 0.0), axis=0, keepdims=True) * (_GS * _GS)
        gx = jnp.sqrt(ss + 1e-6)
        nx = gx / (jnp.sum(gx, axis=1, keepdims=True) * (1.0 / E) + 1e-6)
        gam = g_ref[...].astype(f32).reshape(1, E)
        bet = b_ref[...].astype(f32).reshape(1, E)
        s = (gam * nx + 1.0) * _GS
        w2t = w2t_ref[...].astype(f32)
        w2s_ref[...] = pltpu.bitcast((w2t * s).astype(bf16), u32)
        bias_ref[...] = jnp.broadcast_to(jnp.sum(w2t * bet, axis=1, keepdims=True), (C, 128))

    pl.run_scoped(phase1,
                  pltpu.VMEM((NU, 12, NQ, 24, 128), u32),
                  pltpu.VMEM((E, 128), f32),
                  pltpu.VMEM((C, C), u32))

    def phase2(ht_ref):
        def o_copy(j, sl, r0, n):
            return pltpu.make_async_copy(xbuf.at[sl, pl.ds(r0, n)], o_hbm.at[pl.ds(j * G + r0, n)], osem.at[sl])

        def body(j, xs):
            z = zs_ref[0]
            xs1 = jnp.where(xs == NB2 - 1, 0, xs + 1)
            x_copy(j, xs).wait()

            @pl.when(j >= 2)
            def _():
                o_copy(j - 2, xs1, 0, G).wait()

            @pl.when(j < NG - 1)
            def _():
                x_copy(j + 1, xs1).start()

            def fin(k, hu):
                o = jnp.dot(pltpu.bitcast(w2s_ref[...], bf16), pltpu.bitcast(hu, bf16), preferred_element_type=f32)
                xbuf[xs, k] = (o + _tile4(bias_ref[...]) + xbuf[xs, k].astype(f32)).astype(bf16)

            def mm1(n):
                xn = pltpu.bitcast(xn_ref[j * NRC + n], bf16)
                lhs = pltpu.bitcast(w1q_ref[...], bf16)
                ht_ref[n % 2 + z] = _pack_pairs(_gelu2(jnp.dot(lhs, xn, preferred_element_type=f32)))

            mm1(0)
            for n in range(NRC):
                fin(ST[n], h_ref[j * NST + n])
                if n + 1 < NRC:
                    mm1(n + 1)
                fin(RC[n], ht_ref[n % 2 + z])
                if (2 * n + 2) % OROWS == 0:
                    o_copy(j, xs, 2 * n + 2 - OROWS, OROWS).start()
            return xs1

        with jax.named_scope('loop2'):
            lax.fori_loop(0, NG, body, jnp.int32(0))
        for j in range(NG - 2, NG):
            o_copy(j, j % NB2, 0, G).wait()

    pl.run_scoped(phase2,
                  pltpu.VMEM((2, E // 2, W), u32))


@jax.jit
def pallas_standalone__modern_conv_block_convnext_v2__vision_kernel(x, dw, w1, w2, grn_gamma, grn_beta):
    xt = jnp.transpose(x, (0, 1, 3, 2)).reshape(H, C, W)
    x5 = xt.reshape(H // 2, 2, C // 8, 8, W)
    w2t = w2.T
    vm = pl.BlockSpec(memory_space=pltpu.VMEM)
    out = pl.pallas_call(
        _kernel,
        in_specs=[pl.BlockSpec(memory_space=pl.ANY), pl.BlockSpec(memory_space=pl.ANY), vm, vm, vm, vm, vm, vm],
        out_specs=pl.BlockSpec(memory_space=pl.ANY),
        out_shape=jax.ShapeDtypeStruct((H, C, W), bf16),
        scratch_shapes=[
            pltpu.VMEM((NG * NST, E // 2, W), u32),
            pltpu.VMEM((XR0 + NRING, C // 2, W), u32),
            pltpu.VMEM((NB2, G, C, W), bf16),
            pltpu.VMEM((E // 2, C), u32),
            pltpu.VMEM((C // 2, E), u32),
            pltpu.VMEM((C, 128), f32),
            pltpu.SMEM((2,), i32),
            pltpu.SemaphoreType.DMA((NB2,)),
            pltpu.SemaphoreType.DMA((NB2,)),
            pltpu.SemaphoreType.DMA((2, 2)),
        ],
        compiler_params=pltpu.CompilerParams(vmem_limit_bytes=128 * 1024 * 1024,
                                             disable_bounds_checks=True),
    )(xt, x5, dw, w1, w2t, grn_gamma, grn_beta, dw)
    return jnp.transpose(out.reshape(1, H, C, W), (0, 1, 3, 2))
```

```python
import functools
import math
import jax
import jax.numpy as jnp
from jax import lax
import jax.experimental.pallas as pl
import jax.experimental.pallas.tpu as pltpu

H = 512; W = 512; C = 96; E = 384
G = 16
NG = H // G
G2 = 8
NG2 = H // G2
RC = (2, 3, 4)
ST = tuple(k for k in range(G2) if k not in RC)
NST = len(ST)
NR = len(RC)
NU = 2
NQ = W // 128
NVR = NQ * 6 * 3 * (NR + 2)
ACC0 = NU * 12 * NQ * 3
CL0 = ACC0 + E // 8
NB2 = 5
S0 = 4
LN_LAG = 5
NSUB = 6
P2ORD = 'M0,M1,F0,M2,S0,F1,S1,o04,F2,S2,o46,S3,S4,o68'
PLAN = [int(c) for c in ('1' * 48)]
GSET = [int(c) for c in '0,3,6,9,12'.split(',')]
TLAG = 1
TLAG2 = 2
NCV = 2
HCUT = 0

_C1 = math.sqrt(2.0 / math.pi)
_C3 = _C1 * 0.044715
_A = _C3 ** (1.0 / 3.0)
_K = _C1 / _A
_GS = 0.5 / _A

f32 = jnp.float32
bf16 = jnp.bfloat16
u32 = jnp.uint32
i32 = jnp.int32


def _iota(shape, d):
    return lax.broadcasted_iota(i32, shape, d)


def _perm16(r):
    return (r & ~15) + 2 * (r & 7) + ((r >> 3) & 1)


def _tile4(a):
    return jnp.concatenate([a] * NQ, axis=1)


def _pack_pairs(y):
    m = y.shape[0] // 16
    outs = [pltpu.pack_elementwise([y[16 * t:16 * t + 8], y[16 * t + 8:16 * t + 16]], packed_dtype=bf16)
            for t in range(m)]
    o = outs[0] if m == 1 else jnp.concatenate(outs, axis=0)
    return pltpu.bitcast(o, u32) if o.dtype != u32 else o


def _gelu2(y):
    u = y * (y * y + _K)
    t = jnp.tanh(u)
    return y * t + y


def _tree_sum(xs):
    xs = list(xs)
    while len(xs) > 1:
        xs = [xs[i] + xs[i + 1] for i in range(0, len(xs) - 1, 2)] + ([xs[-1]] if len(xs) % 2 else [])
    return xs[0]


def _hslot(j):
    return (j % (NG2 - HCUT) if HCUT else j) * NST


def _merge(a, b, msk, sh):
    return jnp.where(msk, a, b) + pltpu.roll(jnp.where(msk, b, a), 8 - sh, 0)


def _kernel(x_hbm, x5_hbm, dw_ref, w1_ref, w2t_ref, g_ref, b_ref, dw2_ref, o_hbm,
            h_ref, xbuf, big_ref, vr_ref, dwb_ref, cv_ref, xn2_ref, zv_ref, w1q_ref, w2s_ref, bias_ref, zs_ref,
            xsem, osem, psem):

    for i in range(8):
        zs_ref[i] = 0

    def x_copy(j, sl):
        return pltpu.make_async_copy(x_hbm.at[pl.ds(j * G2, G2)], xbuf.at[sl], xsem.at[sl])

    def phase1():
        xn_ref = big_ref
        vi = lambda u, g, q, v: ((u * 12 + g) * NQ + q) * 3 + v
        xp = xbuf.reshape(NB2 * G2 // 2, C // 8, 16, W)
        def p_copy(u0, n, half, slot, dst0=0):
            src = x5_hbm.at[pl.ds(u0 - 1 + half, n), 1 - half]
            return pltpu.make_async_copy(src, xp.at[pl.ds(8 * slot + dst0, n), :, pl.ds(8 * half, 8), :],
                                         psem.at[slot, half])

        NP2 = G // 2

        def chunk(j, last):
            return [p_copy(NP2 * j + 3, NP2 - 2 if last else NP2, 0, j & 1),
                    p_copy(NP2 * j + 3, NP2 - 3 if last else NP2, 1, j & 1)]

        p_copy(1, 2, 0, 1, 1).start()
        p_copy(0, 3, 1, 1).start()
        for cp in chunk(0, False):
            cp.start()

        vr_ref[0, ACC0:CL0] = jnp.zeros((E // 8, 8, 128), u32)
        zv_ref[...] = jnp.zeros(zv_ref.shape, u32)
        dw = jnp.concatenate([dw_ref[0:2].astype(f32), dw2_ref[2:3].astype(f32)], axis=0)
        dif = _iota((8, C), 1) - _iota((8, C), 0)
        R = _iota((16, C), 0); KK = _iota((16, C), 1)
        unit = jnp.where(KK >= 48, 1, 0)
        itap = 2 * unit + ((KK >> 3) & 1) - (R >> 3)
        tapid = jnp.where((KK & 7) == (R & 7), 3 * itap + ((KK - 48 * unit) >> 4), -9)

        def prep_dw(g, c):
            cl = jnp.zeros((16, C), f32)
            for t in range(9):
                row = jnp.broadcast_to(dw[t // 3, t % 3:t % 3 + 1, :], (8, C))
                col = jnp.sum(jnp.where(dif == 8 * g, row, 0.0), axis=1, keepdims=True)
                dwb_ref[0, g, t] = jnp.broadcast_to(col, (8, 128))
                cb = jnp.broadcast_to(col, (8, C))
                cl = jnp.where(tapid == t, jnp.concatenate([cb, cb], axis=0), cl)
            vr_ref[0, CL0 + g, :, 0:C] = pltpu.bitcast(cl.astype(bf16), u32)
            return c
        lax.fori_loop(0, 12, prep_dw, 0, unroll=4)

        w1f = w1_ref[...].astype(f32)
        w1c = (w1f - jnp.sum(w1f, axis=0, keepdims=True) * (1.0 / C)).astype(bf16)
        r96 = _iota((C, C), 0); c96 = _iota((C, C), 1)
        Q = jnp.where(r96 == (c96 & ~15) + ((c96 & 15) >> 1) + 8 * (c96 & 1), 1.0, 0.0).astype(bf16)
        for i in range(6):
            Pb = jnp.where(_perm16(_iota((64, E), 0) + 64 * i) == _iota((64, E), 1), 1.0, 0.0).astype(bf16)
            w1p = lax.dot_general(Pb, w1c, (((1,), (1,)), ((), ())), preferred_element_type=f32)
            w1q = jnp.dot(w1p.astype(bf16), Q, preferred_element_type=f32)
            w1q_ref[32 * i:32 * i + 32, :] = pltpu.bitcast(w1q.astype(bf16), u32)

        lane = _iota((8, 128), 1)

        def s1(xu_ref, u, kill=None):
            zz = jnp.zeros((8, 128), u32)
            for g in range(12):
                m = pltpu.bitcast(xu_ref[g], u32)
                if kill is not None:
                    m = jnp.where(kill, jnp.zeros_like(m), m)
                mq = [m[:, 128 * q:128 * q + 128] for q in range(NQ)]
                for q in range(NQ):
                    lq = jnp.where(lane == 127, mq[q - 1] if q > 0 else zz, mq[q])
                    rq = jnp.where(lane == 0, mq[q + 1] if q + 1 < NQ else zz, mq[q])
                    vr_ref[0, vi(u, g, q, 0)] = pltpu.roll(lq, 1, 1)
                    vr_ref[0, vi(u, g, q, 1)] = mq[q]
                    vr_ref[0, vi(u, g, q, 2)] = pltpu.roll(rq, 127, 1)

        def conv_round(t, q, gs):
            cvs = []
            for g in gs:
                rhs = jnp.concatenate([vr_ref[0, vi(uu % NU, g, q, v)] for uu in (t, t + 1) for v in range(3)], axis=0)
                lhs = pltpu.bitcast(vr_ref[0, CL0 + g, :, 0:C], bf16)
                cvs.append(jnp.dot(lhs, pltpu.bitcast(rhs, bf16), preferred_element_type=f32))
            return cvs

        sub = _iota((8, 128), 0)
        m0 = sub % 2 == 0
        m1 = (sub // 2) % 2 == 0
        lnc = jnp.where(m1, 1.0 / (C * _A), 1.0 / (C * _A * _A))

        merge = _merge

        def ln_tile(cvs, q, dsts):
            ls = slice(128 * q, 128 * q + 128)
            cs = [[cv[8 * ab:8 * ab + 8] for cv in cvs] for ab in range(2)]
            c1 = merge(_tree_sum(cs[0]), _tree_sum(cs[1]), m0, 1)
            c2 = merge(_tree_sum([c * c for c in cs[0]]), _tree_sum([c * c for c in cs[1]]), m0, 1)
            e = merge(c1, c2, m1, 2)
            f = (e + pltpu.roll(e, 4, 0)) * lnc
            v = pltpu.roll(f, 6, 0) - f * f
            rs = lax.rsqrt(jnp.maximum(v, 0.0) + 1e-5 / (_A * _A))
            for ab in range(2):
                xn_ref[dsts[ab], :, ls] = _pack_pairs(jnp.concatenate(cs[ab], axis=0) * rs[ab:ab + 1, :])

        xp[8, :, 0:8, :] = jnp.zeros((12, 8, W), bf16)
        p_copy(1, 2, 0, 1, 1).wait()
        p_copy(0, 3, 1, 1).wait()
        for u in range(2):
            s1(xp.at[8 + u], u)
        for q in range(NQ):
            ln_tile(conv_round(0, q, range(12)), q, (0, 1))
        s1(xp.at[10], 2 % NU)
        for q in range(2):
            ln_tile(conv_round(1, q, range(12)), q, (2, 3))

        NP = 2 * NSUB
        RPP = 12 // NP
        MR = E // NSUB

        def body(j, carry):
            z = zs_ref[0]
            z1 = zs_ref[1]
            slot = j & 1

            @pl.when(j < NG - 1)
            def _():
                for cp in chunk(j, False):
                    cp.wait()

            @pl.when(j == NG - 1)
            def _():
                for cp in chunk(j, True):
                    cp.wait()
                for jn in range(3):
                    x_copy(jn, (S0 + jn) % NB2).start()

            @pl.when(j < NG - 2)
            def _():
                for cp in chunk(j + 1, False):
                    cp.start()

            @pl.when(j == NG - 2)
            def _():
                for cp in chunk(j + 1, True):
                    cp.start()

            pend = []
            cur = []
            for p in range(NP2):
                for r in range(NP):
                    gr = p * NP + r
                    ab, c = r // NSUB, r % NSUB
                    k = 2 * p + ab
                    while pend and pend[0][0] <= gr:
                        ln_tile(*pend.pop(0)[1:])
                    xn = pltpu.bitcast(xn_ref[k % 8 + z], bf16)
                    lhs = pltpu.bitcast(w1q_ref[MR // 2 * c:MR // 2 * (c + 1), :], bf16)
                    gl = _gelu2(jnp.dot(lhs, xn, preferred_element_type=f32))
                    sq = gl * gl
                    s4 = (sq[:, 0:128] + sq[:, 128:256]) + (sq[:, 256:384] + sq[:, 384:512])
                    for i in range(MR // 8):
                        ai = ACC0 + MR // 8 * c + i
                        vr_ref[0, ai] = pltpu.bitcast(pltpu.bitcast(vr_ref[0, ai], f32) + s4[8 * i:8 * i + 8], u32)
                    if k % G2 in ST:
                        h_ref[_hslot(2 * j + k // G2) + ST.index(k % G2), MR // 2 * c:MR // 2 * (c + 1), :] = _pack_pairs(gl)
                    for rr in range(r * RPP, (r + 1) * RPP):
                        q = (rr // 3 + 2) % 4
                        pair = p + 1 + (rr >= 6)
                        cur += conv_round(pair, q, range(4 * (rr % 3), 4 * (rr % 3) + 4))
                        if rr % 3 == 2:
                            pend.append((gr + LN_LAG, cur, q,
                                         (2 * pair % 8 + z1, (2 * pair + 1) % 8 + z1)))
                            cur = []
                    if r == NP // 2 - 1:
                        kill = None
                        if p == NP2 - 3:
                            kill = _iota((8, W), 0) >= jnp.where(j == NG - 1, 4, 8)
                        s1(xp.at[8 * slot + p], (p + 3) % NU, kill)
            for e in pend:
                ln_tile(*e[1:])
            return carry

        with jax.named_scope('loop1'):
            lax.fori_loop(0, NG, body, 0)

        pdif = _iota((8, E), 1) - 2 * _iota((8, E), 0) + zs_ref[0]
        parts = []
        for i in range(E // 8):
            col = jnp.sum(pltpu.bitcast(vr_ref[0, ACC0 + i], f32), axis=1, keepdims=True)
            parts.append(jnp.where(pdif == 16 * (i // 2) + i % 2, jnp.broadcast_to(col, (8, E)), 0.0))
        ss = jnp.sum(_tree_sum(parts), axis=0, keepdims=True) * (_GS * _GS)
        gx = jnp.sqrt(ss + 1e-6)
        nx = gx / (jnp.sum(gx, axis=1, keepdims=True) * (1.0 / E) + 1e-6)
        gam = g_ref[...].astype(f32).reshape(1, E)
        bet = b_ref[...].astype(f32).reshape(1, E)
        s = (gam * nx + 1.0) * _GS
        w2t = w2t_ref[...].astype(f32)
        w2s_ref[...] = pltpu.bitcast((w2t * s).astype(bf16), u32)
        bias_ref[...] = jnp.broadcast_to(jnp.sum(w2t * bet, axis=1, keepdims=True), (C, 128))

    phase1()

    def phase2():
        xn_ref = xn2_ref
        vi = lambda q, k, i: (q * 6 + k) * 3 * (NR + 2) + i
        R0 = RC[0] - 1

        def o_copy(j, sl, r0, n):
            return pltpu.make_async_copy(xbuf.at[sl, pl.ds(r0, n)], o_hbm.at[pl.ds(j * G2 + r0, n)], osem.at[sl])

        z0 = zs_ref[0]
        lane = _iota((8, 128), 1) + z0
        sub = _iota((8, 128), 0) + z0
        m0 = (sub & 1) == 0
        m1 = (sub & 2) == 0
        m2 = sub < 4
        lnc = jnp.where(m2, 1.0 / (C * _A), 1.0 / (C * _A * _A))

        def s1(xs, zv):
            zz = jnp.zeros((8, 128), u32)
            for r in range(NR + 2):
                for k in range(6):
                    m = pltpu.bitcast(xbuf[xs, R0 + r, 16 * k:16 * k + 16, :], u32)
                    mq = [m[:, 128 * q:128 * q + 128] for q in range(NQ)]
                    for q in range(NQ):
                        lq = jnp.where(lane == 127, mq[q - 1] if q > 0 else zz, mq[q])
                        rq = jnp.where(lane == 0, mq[q + 1] if q + 1 < NQ else zz, mq[q])
                        vr_ref[zv, vi(q, k, 3 * r)] = pltpu.roll(lq, 1, 1)
                        vr_ref[zv, vi(q, k, 3 * r + 1)] = mq[q]
                        vr_ref[zv, vi(q, k, 3 * r + 2)] = pltpu.roll(rq, 127, 1)

        def conv_unit(q, zc, zw, zr):
            ls = slice(128 * q, 128 * q + 128)
            st = [None] * NR
            tok = yield None
            for g in range(12):
                w = [dwb_ref[zw, g, t] for t in range(9)]
                acc = [None] * NR
                for r in range(NR + 2):
                    for v in range(3):
                        x = vr_ref[zw, vi(q, g // 2, 3 * r + v)]
                        if tok is not None and 3 * r + v in GSET:
                            x = x | tok
                        xf = pltpu.bitcast(x, bf16).astype(f32)[8 * (g % 2):8 * (g % 2) + 8]
                        for n in range(NR):
                            if 0 <= r - n <= 2:
                                t = xf * w[3 * (r - n) + v]
                                acc[n] = t if acc[n] is None else acc[n] + t
                for n in range(NR):
                    cv = acc[n]
                    st[n] = (cv, cv * cv) if st[n] is None else (st[n][0] + cv, st[n][1] + cv * cv)
                    cv_ref[q % NCV + zc, n, 8 * g:8 * g + 8, :] = cv
                tok = yield pltpu.bitcast((st[0][1] + st[1][1]) + st[2][1], u32)
            half = lambda i: _merge(_merge(st[0][i], st[1][i], m0, 1), st[2][i] + pltpu.roll(st[2][i], 7, 0), m1, 2)
            f = _merge(half(0), half(1), m2, 4) * lnc
            v = pltpu.roll(f, 4, 0) - f * f
            cv_ref[q % NCV + zr, NR, 0:8, :] = lax.rsqrt(jnp.maximum(v, 0.0) + 1e-5 / (_A * _A))
            yield None
            for n in range(NR):
                rs = cv_ref[q % NCV + zc, NR, n:n + 1, :]
                xn_ref[n, :, ls] = _pack_pairs(cv_ref[q % NCV + zc, n] * rs)
            yield None

        x_copy(0, S0).wait()
        s1(S0, zs_ref[0])
        for q in range(NQ):
            for _ in conv_unit(q, zs_ref[0], zs_ref[2 + q], zs_ref[1]):
                pass

        nxt = lambda sl: jnp.where(sl == NB2 - 1, 0, sl + 1)

        def body(j, xs):
            z = zs_ref[0]
            xs1 = nxt(xs)
            xs3 = nxt(nxt(xs1))

            @pl.when(j + 1 < NG2)
            def _():
                x_copy(j + 1, xs1).wait()

            @pl.when(j >= 2)
            def _():
                o_copy(j - 2, xs3, 0, G2).wait()

            @pl.when(j + 3 < NG2)
            def _():
                x_copy(j + 3, xs3).start()

            units = [conv_unit(q, z, zs_ref[2 + q], zs_ref[1]) for q in range(NQ)]
            for u in units:
                next(u)
            s1(xs1, z)
            zv = zv_ref[0:8, :]
            cnt = [0, 0]
            tails = []
            toks = [None]

            def run_pieces(rel):
                tgt = sum(PLAN[:cnt[0] + 1])
                cnt[0] += 1
                res = None
                while cnt[1] < tgt:
                    u = units[cnt[1] // 12]
                    val = u.send(rel)
                    res = val if res is None else res | val
                    cnt[1] += 1
                    if cnt[1] % 12 == 0:
                        tails.append([TLAG, u])
                        tails.append([TLAG + TLAG2, u])
                for t in list(tails):
                    if t[0] == 0:
                        t[1].send(None)
                        tails.remove(t)
                    t[0] -= 1
                return res

            def gate(d):
                if toks[-1] is None:
                    return d
                mr = d.shape[0]
                du = pltpu.bitcast(d[mr - 8:mr, 384:512], u32) | (toks[-1] & zv)
                last = jnp.concatenate([d[mr - 8:mr, 0:384], pltpu.bitcast(du, f32)], axis=1)
                return jnp.concatenate([d[0:mr - 8], last], axis=0)

            def fin(k, hr):
                for mc in range(2):
                    rs_ = slice(48 * mc, 48 * (mc + 1))
                    o = None
                    for kt in range(3):
                        d = jnp.dot(pltpu.bitcast(w2s_ref[24 * mc:24 * (mc + 1), 128 * kt:128 * kt + 128], bf16),
                                    pltpu.bitcast(hr(kt), bf16), preferred_element_type=f32)
                        rel = pltpu.bitcast(d[0:8, 0:128], u32) & zv
                        d = gate(d)
                        o = d if o is None else o + d
                        if kt == 2:
                            xbuf[xs, k, rs_, :] = (o + _tile4(bias_ref[rs_, :]) + xbuf[xs, k, rs_, :].astype(f32)).astype(bf16)
                        toks.append(run_pieces(rel))

            def ht_rows(n, kt):
                return jnp.concatenate([big_ref[4 * (n % 2) + z + r // 48, r % 48:r % 48 + 8, :]
                                        for r in range(64 * kt, 64 * kt + 64, 8)], axis=0)

            def mm1(n):
                xn = pltpu.bitcast(xn_ref[n], bf16)
                lhs = pltpu.bitcast(w1q_ref[...], bf16)
                hp = _pack_pairs(_gelu2(jnp.dot(lhs, xn, preferred_element_type=f32)))
                big_ref[pl.ds(4 * (n % 2) + z, 4)] = hp.reshape(4, C // 2, W)

            for tok in P2ORD.split(','):
                n = int(tok[1])
                if tok[0] == 'M': mm1(n)
                elif tok[0] == 'S': fin(ST[n], lambda kt: h_ref[_hslot(j) + n, 64 * kt:64 * kt + 64, :])
                elif tok[0] == 'F': fin(RC[n], functools.partial(ht_rows, n))
                elif tok[0] == 'o': o_copy(j, xs, n, int(tok[2]) - n).start()
            assert cnt[1] == 48
            for t in tails:
                t[1].send(None)
            return xs1

        with jax.named_scope('loop2'):
            lax.fori_loop(0, NG2, body, jnp.int32(S0))
        for j in range(NG2 - 2, NG2):
            o_copy(j, (j + S0) % NB2, 0, G2).wait()

    phase2()


@jax.jit
def pallas_standalone__modern_conv_block_convnext_v2__vision_kernel(x, dw, w1, w2, grn_gamma, grn_beta):
    xt = jnp.transpose(x, (0, 1, 3, 2)).reshape(H, C, W)
    x5 = xt.reshape(H // 2, 2, C // 8, 8, W)
    w2t = w2.T
    vm = pl.BlockSpec(memory_space=pltpu.VMEM)
    out = pl.pallas_call(
        _kernel,
        in_specs=[pl.BlockSpec(memory_space=pl.ANY), pl.BlockSpec(memory_space=pl.ANY), vm, vm, vm, vm, vm, vm],
        out_specs=pl.BlockSpec(memory_space=pl.ANY),
        out_shape=jax.ShapeDtypeStruct((H, C, W), bf16),
        scratch_shapes=[
            pltpu.VMEM(((NG2 - HCUT) * NST, E // 2, W), u32),
            pltpu.VMEM((NB2, G2, C, W), bf16),
            pltpu.VMEM((8, C // 2, W), u32),
            pltpu.VMEM((1, NVR, 8, 128), u32),
            pltpu.VMEM((1, 12, 9, 8, 128), f32),
            pltpu.VMEM((NCV, NR + 1, C, 128), f32),
            pltpu.VMEM((NR, C // 2, W), u32),
            pltpu.VMEM((32, 128), u32),
            pltpu.VMEM((E // 2, C), u32),
            pltpu.VMEM((C // 2, E), u32),
            pltpu.VMEM((C, 128), f32),
            pltpu.SMEM((8,), i32),
            pltpu.SemaphoreType.DMA((NB2,)),
            pltpu.SemaphoreType.DMA((NB2,)),
            pltpu.SemaphoreType.DMA((2, 2)),
        ],
        compiler_params=pltpu.CompilerParams(vmem_limit_bytes=128 * 1024 * 1024,
                                             disable_bounds_checks=True),
    )(xt, x5, dw, w1, w2t, grn_gamma, grn_beta, dw)
    return jnp.transpose(out.reshape(1, H, C, W), (0, 1, 3, 2))
```

```python
import functools
import math
import jax
import jax.numpy as jnp
from jax import lax
import jax.experimental.pallas as pl
import jax.experimental.pallas.tpu as pltpu

H = 512; W = 512; C = 96; E = 384
G = 16
NG = H // G
G2 = 8
NG2 = H // G2
RC = (2, 3, 4)
ST = tuple(k for k in range(G2) if k not in RC)
NST = len(ST)
NR = len(RC)
NU = 2
NQ = W // 128
NVR = NQ * 6 * 3 * (NR + 2)
ACC0 = NU * 12 * NQ * 3
CL0 = ACC0 + E // 8
NB2 = 5
S0 = 4
LN_LAG = 5
NSUB = 6
P2ORD = 'M0,M1,F0,M2,S0,F1,S1,o04,F2,S2,o46,S3,S4,o68'
PLAN = [int(c) for c in ('22' + '1' * 44 + '00')]
GSET = [int(c) for c in '0,3,6,9,12'.split(',')]
TLAG = 1
TLAG2 = 2
NCV = 2
PU = 12
PRO = 0
HCUT = 0

_C1 = math.sqrt(2.0 / math.pi)
_C3 = _C1 * 0.044715
_A = _C3 ** (1.0 / 3.0)
_K = _C1 / _A
_GS = 0.5 / _A

f32 = jnp.float32
bf16 = jnp.bfloat16
u32 = jnp.uint32
i32 = jnp.int32


def _iota(shape, d):
    return lax.broadcasted_iota(i32, shape, d)


def _perm16(r):
    return (r & ~15) + 2 * (r & 7) + ((r >> 3) & 1)


def _tile4(a):
    return jnp.concatenate([a] * NQ, axis=1)


def _pack_pairs(y):
    m = y.shape[0] // 16
    outs = [pltpu.pack_elementwise([y[16 * t:16 * t + 8], y[16 * t + 8:16 * t + 16]], packed_dtype=bf16)
            for t in range(m)]
    o = outs[0] if m == 1 else jnp.concatenate(outs, axis=0)
    return pltpu.bitcast(o, u32) if o.dtype != u32 else o


def _gelu2(y):
    u = y * (y * y + _K)
    t = jnp.tanh(u)
    return y * t + y


def _tree_sum(xs):
    xs = list(xs)
    while len(xs) > 1:
        xs = [xs[i] + xs[i + 1] for i in range(0, len(xs) - 1, 2)] + ([xs[-1]] if len(xs) % 2 else [])
    return xs[0]


def _hslot(j):
    return (j % (NG2 - HCUT) if HCUT else j) * NST


def _merge(a, b, msk, sh):
    return jnp.where(msk, a, b) + pltpu.roll(jnp.where(msk, b, a), 8 - sh, 0)


def _kernel(x_hbm, x5_hbm, dw_hbm, w1_hbm, w2t_hbm, g_hbm, b_hbm, o_hbm,
            h_ref, xbuf, big_ref, vr_ref, dwb_ref, cv_ref, zv_ref, w1q_ref, w2s_ref, bias_ref, dw_ref, dw2_ref, g_ref, b_ref, zs_ref,
            xsem, osem, psem, wsem):

    for i in range(8):
        zs_ref[i] = 0

    def x_copy(j, sl):
        return pltpu.make_async_copy(x_hbm.at[pl.ds(j * G2, G2)], xbuf.at[sl], xsem.at[sl])

    def phase1():
        xn_ref = big_ref
        vi = lambda u, g, q, v: ((u * 12 + g) * NQ + q) * 3 + v
        xp = xbuf.reshape(NB2 * G2 // 2, C // 8, 16, W)
        def p_copy(u0, n, half, slot, dst0=0):
            src = x5_hbm.at[pl.ds(u0 - 1 + half, n), 1 - half]
            return pltpu.make_async_copy(src, xp.at[pl.ds(8 * slot + dst0, n), :, pl.ds(8 * half, 8), :],
                                         psem.at[slot, half])

        NP2 = G // 2

        def chunk(j, last):
            return [p_copy(NP2 * j + 3, NP2 - 2 if last else NP2, 0, j & 1),
                    p_copy(NP2 * j + 3, NP2 - 3 if last else NP2, 1, j & 1)]

        w1_ref = xbuf.at[4, 0, :, pl.ds(0, E)]
        w2t_ref = xbuf.at[4, 1, :, pl.ds(0, E)]
        small = [pltpu.make_async_copy(a, b, wsem.at[i]) for i, (a, b) in enumerate(
            [(dw_hbm, dw_ref), (dw_hbm, dw2_ref), (w1_hbm, w1_ref), (w2t_hbm, w2t_ref), (g_hbm, g_ref), (b_hbm, b_ref)])]
        for cp in small[:3]:
            cp.start()
        p_copy(1, 3, 0, 1, 1).start()
        p_copy(0, 4, 1, 1).start()
        for cp in small[3:] + chunk(0, False):
            cp.start()
        for cp in small[:2]:
            cp.wait()

        vr_ref[0, ACC0:CL0] = jnp.zeros((E // 8, 8, 128), u32)
        zv_ref[...] = jnp.zeros(zv_ref.shape, u32)
        dw = jnp.concatenate([dw_ref[0:2].astype(f32), dw2_ref[2:3].astype(f32)], axis=0)
        dif = _iota((8, C), 1) - _iota((8, C), 0)
        R = _iota((16, C), 0); KK = _iota((16, C), 1)
        unit = jnp.where(KK >= 48, 1, 0)
        itap = 2 * unit + ((KK >> 3) & 1) - (R >> 3)
        tapid = jnp.where((KK & 7) == (R & 7), 3 * itap + ((KK - 48 * unit) >> 4), -9)

        def prep_dw(g, c):
            cl = jnp.zeros((16, C), f32)
            for t in range(9):
                row = jnp.broadcast_to(dw[t // 3, t % 3:t % 3 + 1, :], (8, C))
                col = jnp.sum(jnp.where(dif == 8 * g, row, 0.0), axis=1, keepdims=True)
                dwb_ref[0, g, t] = jnp.broadcast_to(col, (8, 128))
                cb = jnp.broadcast_to(col, (8, C))
                cl = jnp.where(tapid == t, jnp.concatenate([cb, cb], axis=0), cl)
            vr_ref[0, CL0 + g, :, 0:C] = pltpu.bitcast(cl.astype(bf16), u32)
            return c
        lax.fori_loop(0, 12, prep_dw, 0, unroll=PU)

        for cp in small[2:]:
            cp.wait()
        w1f = w1_ref[...].astype(f32)
        w1k = pltpu.bitcast(_pack_pairs(w1f - jnp.sum(w1f, axis=0, keepdims=True) * (1.0 / C)), bf16)
        for i in range(3):
            Pb = jnp.where(_perm16(_iota((128, E), 0) + 128 * i) == _iota((128, E), 1), 1.0, 0.0).astype(bf16)
            w1q = lax.dot_general(Pb, w1k, (((1,), (1,)), ((), ())), preferred_element_type=f32)
            w1q_ref[64 * i:64 * i + 64, :] = pltpu.bitcast(w1q.astype(bf16), u32)
        w2s_ref[...] = pltpu.bitcast(w2t_ref[...], u32)

        lane = _iota((8, 128), 1)

        def s1(xu_ref, u, kill=None):
            zz = jnp.zeros((8, 128), u32)
            for g in range(12):
                m = pltpu.bitcast(xu_ref[g], u32)
                if kill is not None:
                    m = jnp.where(kill, jnp.zeros_like(m), m)
                mq = [m[:, 128 * q:128 * q + 128] for q in range(NQ)]
                for q in range(NQ):
                    lq = jnp.where(lane == 127, mq[q - 1] if q > 0 else zz, mq[q])
                    rq = jnp.where(lane == 0, mq[q + 1] if q + 1 < NQ else zz, mq[q])
                    vr_ref[0, vi(u, g, q, 0)] = pltpu.roll(lq, 1, 1)
                    vr_ref[0, vi(u, g, q, 1)] = mq[q]
                    vr_ref[0, vi(u, g, q, 2)] = pltpu.roll(rq, 127, 1)

        def conv_round(t, q, gs):
            cvs = []
            for g in gs:
                rhs = jnp.concatenate([vr_ref[0, vi(uu & 1, g, q, v)] for uu in (t, t + 1) for v in range(3)], axis=0)
                lhs = pltpu.bitcast(vr_ref[0, CL0 + g, :, 0:C], bf16)
                cvs.append(jnp.dot(lhs, pltpu.bitcast(rhs, bf16), preferred_element_type=f32))
            return cvs

        sub = _iota((8, 128), 0)
        m0 = sub % 2 == 0
        m1 = (sub // 2) % 2 == 0
        lnc = jnp.where(m1, 1.0 / (C * _A), 1.0 / (C * _A * _A))

        merge = _merge

        def ln_tile(cvs, q, dsts):
            ls = slice(128 * q, 128 * q + 128)
            cs = [[cv[8 * ab:8 * ab + 8] for cv in cvs] for ab in range(2)]
            c1 = merge(_tree_sum(cs[0]), _tree_sum(cs[1]), m0, 1)
            c2 = merge(_tree_sum([c * c for c in cs[0]]), _tree_sum([c * c for c in cs[1]]), m0, 1)
            e = merge(c1, c2, m1, 2)
            f = (e + pltpu.roll(e, 4, 0)) * lnc
            v = pltpu.roll(f, 6, 0) - f * f
            rs = lax.rsqrt(jnp.maximum(v, 0.0) + 1e-5 / (_A * _A))
            for ab in range(2):
                xn_ref[dsts[ab], :, ls] = _pack_pairs(jnp.concatenate(cs[ab], axis=0) * rs[ab:ab + 1, :])

        xp[8, :, 0:8, :] = jnp.zeros((12, 8, W), bf16)
        p_copy(1, 3, 0, 1, 1).wait()
        p_copy(0, 4, 1, 1).wait()
        if PRO == 0:
            s1(xp.at[10], 0)
            s1(xp.at[11], 1)
            for i, (un, da, db) in enumerate([(1, 10, 5), (0, 8, 9), (2, 0, 1)]):
                for q in range(NQ):
                    ln_tile(conv_round(2 - i, q, range(12)), q, (da, db))
                s1(xp.at[8 + un], un & 1)
        else:
            def pro0(i, c):
                s1(xp.at[10 + i], i)
                return c
            lax.fori_loop(0, 2, pro0, 0)

            def pro(i, c):
                da = jnp.where(i == 0, 10, jnp.where(i == 1, 8, 0))
                db = jnp.where(i == 0, 5, jnp.where(i == 1, 9, 1))
                for q in range(NQ):
                    ln_tile(conv_round(2 - i, q, range(12)), q, (da, db))
                un = jnp.where(i == 2, 2, 1 - i)
                s1(xp.at[8 + un], un & 1)
                return c
            lax.fori_loop(0, 3, pro, 0)
        for r in range(2):
            xn_ref[2 + r] = xn_ref[8 + r]

        NP = 2 * NSUB
        RPP = 12 // NP
        MR = E // NSUB

        def body(j, carry):
            z = zs_ref[0]
            z1 = zs_ref[1]
            slot = j & 1

            @pl.when(j < NG - 1)
            def _():
                for cp in chunk(j, False):
                    cp.wait()

            @pl.when(j == NG - 1)
            def _():
                for cp in chunk(j, True):
                    cp.wait()
                for jn in range(3):
                    x_copy(jn, (S0 + jn) % NB2).start()

            @pl.when(j < NG - 2)
            def _():
                for cp in chunk(j + 1, False):
                    cp.start()

            @pl.when(j == NG - 2)
            def _():
                for cp in chunk(j + 1, True):
                    cp.start()


            pend = []
            cur = []
            for p in range(NP2):
                for r in range(NP):
                    gr = p * NP + r
                    ab, c = r // NSUB, r % NSUB
                    k = 2 * p + ab
                    while pend and pend[0][0] <= gr:
                        ln_tile(*pend.pop(0)[1:])
                    xn = pltpu.bitcast(xn_ref[k % 8 + z], bf16)
                    lhs = pltpu.bitcast(w1q_ref[MR // 2 * c:MR // 2 * (c + 1), :], bf16)
                    gl = _gelu2(jnp.dot(lhs, xn, preferred_element_type=f32))
                    sq = gl * gl
                    s4 = (sq[:, 0:128] + sq[:, 128:256]) + (sq[:, 256:384] + sq[:, 384:512])
                    for i in range(MR // 8):
                        ai = ACC0 + MR // 8 * c + i
                        vr_ref[0, ai] = pltpu.bitcast(pltpu.bitcast(vr_ref[0, ai], f32) + s4[8 * i:8 * i + 8], u32)
                    if k % G2 in ST:
                        h_ref[_hslot(2 * j + k // G2) + ST.index(k % G2), MR // 2 * c:MR // 2 * (c + 1), :] = _pack_pairs(gl)
                    for rr in range(r * RPP, (r + 1) * RPP):
                        q = (rr // 3 + 2) % 4
                        pair = p + 1 + (rr >= 6)
                        cur += conv_round(pair, q, range(4 * (rr % 3), 4 * (rr % 3) + 4))
                        if rr % 3 == 2:
                            pend.append((gr + LN_LAG, cur, q,
                                         (2 * pair % 8 + z1, (2 * pair + 1) % 8 + z1)))
                            cur = []
                    if r == NP // 2 - 1:
                        kill = None
                        if p == NP2 - 3:
                            kill = _iota((8, W), 0) >= jnp.where(j == NG - 1, 4, 8)
                        s1(xp.at[8 * slot + p], (p + 3) % NU, kill)
            for e in pend:
                ln_tile(*e[1:])
            return carry

        with jax.named_scope('loop1'):
            lax.fori_loop(0, NG, body, 0)

        pdif = _iota((8, E), 1) - 2 * _iota((8, E), 0) + zs_ref[0]
        parts = []
        for i in range(E // 8):
            col = jnp.sum(pltpu.bitcast(vr_ref[0, ACC0 + i], f32), axis=1, keepdims=True)
            parts.append(jnp.where(pdif == 16 * (i // 2) + i % 2, jnp.broadcast_to(col, (8, E)), 0.0))
        ss = jnp.sum(_tree_sum(parts), axis=0, keepdims=True) * (_GS * _GS)
        gx = jnp.sqrt(ss + 1e-6)
        nx = gx / (jnp.sum(gx, axis=1, keepdims=True) * (1.0 / E) + 1e-6)
        gam = g_ref[...].astype(f32).reshape(1, E)
        bet = b_ref[...].astype(f32).reshape(1, E)
        s = (gam * nx + 1.0) * _GS
        w2t = pltpu.bitcast(w2s_ref[...], bf16).astype(f32)
        w2s_ref[...] = pltpu.bitcast((w2t * s).astype(bf16), u32)
        bias_ref[...] = jnp.broadcast_to(jnp.sum(w2t * bet, axis=1, keepdims=True), (C, 128))

    phase1()

    def phase2():
        vi = lambda q, k, i: (q * 6 + k) * 3 * (NR + 2) + i
        R0 = RC[0] - 1

        def o_copy(j, sl, r0, n):
            return pltpu.make_async_copy(xbuf.at[sl, pl.ds(r0, n)], o_hbm.at[pl.ds(j * G2 + r0, n)], osem.at[sl])

        z0 = zs_ref[0]
        lane = _iota((8, 128), 1) + z0
        sub = _iota((8, 128), 0) + z0
        m0 = (sub & 1) == 0
        m1 = (sub & 2) == 0
        m2 = sub < 4
        lnc = jnp.where(m2, 1.0 / (C * _A), 1.0 / (C * _A * _A))

        def s1(xs, zv):
            zz = jnp.zeros((8, 128), u32)
            for r in range(NR + 2):
                for k in range(6):
                    m = pltpu.bitcast(xbuf[xs, R0 + r, 16 * k:16 * k + 16, :], u32)
                    mq = [m[:, 128 * q:128 * q + 128] for q in range(NQ)]
                    for q in range(NQ):
                        lq = jnp.where(lane == 127, mq[q - 1] if q > 0 else zz, mq[q])
                        rq = jnp.where(lane == 0, mq[q + 1] if q + 1 < NQ else zz, mq[q])
                        vr_ref[zv, vi(q, k, 3 * r)] = pltpu.roll(lq, 1, 1)
                        vr_ref[zv, vi(q, k, 3 * r + 1)] = mq[q]
                        vr_ref[zv, vi(q, k, 3 * r + 2)] = pltpu.roll(rq, 127, 1)

        def conv_unit(q, zc, zw, zr):
            ls = slice(128 * q, 128 * q + 128)
            st = [None] * NR
            tok = yield None
            for g in range(12):
                w = [dwb_ref[zw, g, t] for t in range(9)]
                acc = [None] * NR
                for r in range(NR + 2):
                    for v in range(3):
                        x = vr_ref[zw, vi(q, g // 2, 3 * r + v)]
                        if tok is not None and 3 * r + v in GSET:
                            x = x | tok
                        xf = pltpu.bitcast(x, bf16).astype(f32)[8 * (g % 2):8 * (g % 2) + 8]
                        for n in range(NR):
                            if 0 <= r - n <= 2:
                                t = xf * w[3 * (r - n) + v]
                                acc[n] = t if acc[n] is None else acc[n] + t
                for n in range(NR):
                    cv = acc[n]
                    st[n] = (cv, cv * cv) if st[n] is None else (st[n][0] + cv, st[n][1] + cv * cv)
                    cv_ref[q % NCV + zc, n, 8 * g:8 * g + 8, :] = cv
                tok = yield pltpu.bitcast((st[0][1] + st[1][1]) + st[2][1], u32)
            half = lambda i: _merge(_merge(st[0][i], st[1][i], m0, 1), st[2][i] + pltpu.roll(st[2][i], 7, 0), m1, 2)
            f = _merge(half(0), half(1), m2, 4) * lnc
            v = pltpu.roll(f, 4, 0) - f * f
            cv_ref[q % NCV + zr, NR, 0:8, :] = lax.rsqrt(jnp.maximum(v, 0.0) + 1e-5 / (_A * _A))
            yield None
            for n in range(NR):
                rs = cv_ref[q % NCV + zc, NR, n:n + 1, :]
                big_ref[8 + n + zc, :, ls] = _pack_pairs(cv_ref[q % NCV + zc, n] * rs)
            yield None

        x_copy(0, S0).wait()
        nxt = lambda sl: jnp.where(sl == NB2 - 1, 0, sl + 1)

        def body(j, xs):
            z = zs_ref[0]
            xs1 = nxt(xs)
            xs3 = nxt(nxt(xs1))

            @pl.when(j + 1 < NG2)
            def _():
                x_copy(j + 1, xs1).wait()

            @pl.when(j >= 2)
            def _():
                o_copy(j - 2, xs3, 0, G2).wait()

            @pl.when(j + 3 < NG2)
            def _():
                x_copy(j + 3, xs3).start()

            units = [conv_unit(q, z, zs_ref[2 + q], zs_ref[1]) for q in range(NQ)]
            for u in units:
                next(u)
            s1(xs1, z)
            zv = zv_ref[0:8, :]
            cnt = [0, 0]
            tails = []
            toks = [None]

            def run_pieces(rel):
                tgt = sum(PLAN[:cnt[0] + 1])
                cnt[0] += 1
                res = None
                while cnt[1] < tgt:
                    u = units[cnt[1] // 12]
                    val = u.send(rel)
                    res = val if res is None else res | val
                    cnt[1] += 1
                    if cnt[1] % 12 == 0:
                        tails.append([TLAG, u])
                        tails.append([TLAG + TLAG2, u])
                for t in list(tails):
                    if t[0] == 0:
                        t[1].send(None)
                        tails.remove(t)
                    t[0] -= 1
                return res

            def gate(d):
                if toks[-1] is None:
                    return d
                mr = d.shape[0]
                du = pltpu.bitcast(d[mr - 8:mr, 384:512], u32) | (toks[-1] & zv)
                last = jnp.concatenate([d[mr - 8:mr, 0:384], pltpu.bitcast(du, f32)], axis=1)
                return jnp.concatenate([d[0:mr - 8], last], axis=0)

            def fin(k, hr):
                for mc in range(2):
                    rs_ = slice(48 * mc, 48 * (mc + 1))
                    o = None
                    for kt in range(3):
                        d = jnp.dot(pltpu.bitcast(w2s_ref[24 * mc:24 * (mc + 1), 128 * kt:128 * kt + 128], bf16),
                                    pltpu.bitcast(hr(kt), bf16), preferred_element_type=f32)
                        rel = pltpu.bitcast(d[0:8, 0:128], u32) & zv
                        d = gate(d)
                        o = d if o is None else o + d
                        if kt == 2:
                            xbuf[xs, k, rs_, :] = (o + _tile4(bias_ref[rs_, :]) + xbuf[xs, k, rs_, :].astype(f32)).astype(bf16)
                        toks.append(run_pieces(rel))

            def ht_rows(n, kt):
                return jnp.concatenate([big_ref[4 * (n % 2) + z + r // 48, r % 48:r % 48 + 8, :]
                                        for r in range(64 * kt, 64 * kt + 64, 8)], axis=0)

            def mm1(n):
                xn = pltpu.bitcast(big_ref[8 + n + z], bf16)
                lhs = pltpu.bitcast(w1q_ref[...], bf16)
                hp = _pack_pairs(_gelu2(jnp.dot(lhs, xn, preferred_element_type=f32)))
                big_ref[pl.ds(4 * (n % 2) + z, 4)] = hp.reshape(4, C // 2, W)

            for tok in P2ORD.split(','):
                n = int(tok[1])
                if tok[0] == 'M': mm1(n)
                elif tok[0] == 'S': fin(ST[n], lambda kt: h_ref[_hslot(j) + n, 64 * kt:64 * kt + 64, :])
                elif tok[0] == 'F': fin(RC[n], functools.partial(ht_rows, n))
                elif tok[0] == 'o': o_copy(j, xs, n, int(tok[2]) - n).start()
            assert cnt[1] == 48
            for t in tails:
                t[1].send(None)
            return xs1

        with jax.named_scope('loop2'):
            lax.fori_loop(0, NG2, body, jnp.int32(S0))
        for j in range(NG2 - 2, NG2):
            o_copy(j, (j + S0) % NB2, 0, G2).wait()

    phase2()


@jax.jit
def pallas_standalone__modern_conv_block_convnext_v2__vision_kernel(x, dw, w1, w2, grn_gamma, grn_beta):
    xt = jnp.transpose(x, (0, 1, 3, 2)).reshape(H, C, W)
    x5 = xt.reshape(H // 2, 2, C // 8, 8, W)
    w2t = w2.T
    out = pl.pallas_call(
        _kernel,
        in_specs=[pl.BlockSpec(memory_space=pl.ANY)] * 7,
        out_specs=pl.BlockSpec(memory_space=pl.ANY),
        out_shape=jax.ShapeDtypeStruct((H, C, W), bf16),
        scratch_shapes=[
            pltpu.VMEM(((NG2 - HCUT) * NST, E // 2, W), u32),
            pltpu.VMEM((NB2, G2, C, W), bf16),
            pltpu.VMEM((8 + NR, C // 2, W), u32),
            pltpu.VMEM((1, NVR, 8, 128), u32),
            pltpu.VMEM((1, 12, 9, 8, 128), f32),
            pltpu.VMEM((NCV, NR + 1, C, 128), f32),
            pltpu.VMEM((32, 128), u32),
            pltpu.VMEM((E // 2, C), u32),
            pltpu.VMEM((C // 2, E), u32),
            pltpu.VMEM((C, 128), f32),
            pltpu.VMEM((3, 3, C), bf16),
            pltpu.VMEM((3, 3, C), bf16),
            pltpu.VMEM((E,), bf16),
            pltpu.VMEM((E,), bf16),
            pltpu.SMEM((8,), i32),
            pltpu.SemaphoreType.DMA((NB2,)),
            pltpu.SemaphoreType.DMA((NB2,)),
            pltpu.SemaphoreType.DMA((2, 2)),
            pltpu.SemaphoreType.DMA((6,)),
        ],
        compiler_params=pltpu.CompilerParams(vmem_limit_bytes=128 * 1024 * 1024,
                                             disable_bounds_checks=True),
    )(xt, x5, dw, w1, w2t, grn_gamma, grn_beta)
    return jnp.transpose(out.reshape(1, H, C, W), (0, 1, 3, 2))
```

```python
import functools
import math
import jax
import jax.numpy as jnp
from jax import lax
import jax.experimental.pallas as pl
import jax.experimental.pallas.tpu as pltpu

H = 512; W = 512; C = 96; E = 384
G = 16
NG = H // G
G2 = 8
NG2 = H // G2
RC = (2, 3, 4)
ST = tuple(k for k in range(G2) if k not in RC)
NST = len(ST)
NR = len(RC)
NU = 2
NQ = W // 128
NVR = NQ * 6 * 3 * (NR + 2)
ACC0 = NU * 12 * NQ * 3
CL0 = ACC0 + E // 8
NB2 = 5
S0 = 4
LN_LAG = 5
NSUB = 6
P2ORD = 'M0,M1,F0,M2,S0,F1,S1,o04,F2,S2,o46,S3,S4,o68'
PLAN = [int(c) for c in ('22' + '1' * 44 + '00')]
GSET = [int(c) for c in '2,5,8,11,14'.split(',')]
TLAG = 0
TLAG2 = 0
NCV = 1
PU = 12
PRO = 0
HCUT = 0

_C1 = math.sqrt(2.0 / math.pi)
_C3 = _C1 * 0.044715
_A = _C3 ** (1.0 / 3.0)
_K = _C1 / _A
_GS = 0.5 / _A

f32 = jnp.float32
bf16 = jnp.bfloat16
u32 = jnp.uint32
i32 = jnp.int32


def _iota(shape, d):
    return lax.broadcasted_iota(i32, shape, d)


def _perm16(r):
    return (r & ~15) + 2 * (r & 7) + ((r >> 3) & 1)


def _tile4(a):
    return jnp.concatenate([a] * NQ, axis=1)


def _pack_pairs(y):
    m = y.shape[0] // 16
    outs = [pltpu.pack_elementwise([y[16 * t:16 * t + 8], y[16 * t + 8:16 * t + 16]], packed_dtype=bf16)
            for t in range(m)]
    o = outs[0] if m == 1 else jnp.concatenate(outs, axis=0)
    return pltpu.bitcast(o, u32) if o.dtype != u32 else o


def _gelu2(y):
    u = y * (y * y + _K)
    t = jnp.tanh(u)
    return y * t + y


def _tree_sum(xs):
    xs = list(xs)
    while len(xs) > 1:
        xs = [xs[i] + xs[i + 1] for i in range(0, len(xs) - 1, 2)] + ([xs[-1]] if len(xs) % 2 else [])
    return xs[0]


def _hslot(j):
    return (j % (NG2 - HCUT) if HCUT else j) * NST


def _merge(a, b, msk, sh):
    return jnp.where(msk, a, b) + pltpu.roll(jnp.where(msk, b, a), 8 - sh, 0)


def _kernel(x_hbm, x5_hbm, dw_hbm, w1_hbm, w2t_hbm, g_hbm, b_hbm, o_hbm,
            h_ref, xbuf, big_ref, vr_ref, dwb_ref, cv_ref, w1q_ref, w2s_ref, bias_ref, zv_ref, dw_ref, dw2_ref, g_ref, b_ref, zs_ref,
            xsem, osem, psem, wsem):

    for i in range(8):
        zs_ref[i] = 0

    def x_copy(j, sl):
        return pltpu.make_async_copy(x_hbm.at[pl.ds(j * G2, G2)], xbuf.at[sl], xsem.at[sl])

    def phase1():
        xn_ref = big_ref
        vi = lambda u, g, q, v: ((u * 12 + g) * NQ + q) * 3 + v
        xp = xbuf.reshape(NB2 * G2 // 2, C // 8, 16, W)
        def p_copy(u0, n, half, slot, dst0=0):
            src = x5_hbm.at[pl.ds(u0 - 1 + half, n), 1 - half]
            return pltpu.make_async_copy(src, xp.at[pl.ds(8 * slot + dst0, n), :, pl.ds(8 * half, 8), :],
                                         psem.at[slot, half])

        NP2 = G // 2

        def chunk(j, last):
            return [p_copy(NP2 * j + 3, NP2 - 2 if last else NP2, 0, j & 1),
                    p_copy(NP2 * j + 3, NP2 - 3 if last else NP2, 1, j & 1)]

        w1_ref = xbuf.at[4, 0, :, pl.ds(0, E)]
        w2t_ref = xbuf.at[4, 1, :, pl.ds(0, E)]
        small = [pltpu.make_async_copy(a, b, wsem.at[i]) for i, (a, b) in enumerate(
            [(dw_hbm, dw_ref), (dw_hbm, dw2_ref), (w1_hbm, w1_ref), (w2t_hbm, w2t_ref), (g_hbm, g_ref), (b_hbm, b_ref)])]
        for cp in small[:3]:
            cp.start()
        p_copy(1, 3, 0, 1, 1).start()
        p_copy(0, 4, 1, 1).start()
        for cp in small[3:] + chunk(0, False):
            cp.start()
        for cp in small[:2]:
            cp.wait()

        vr_ref[0, ACC0:CL0] = jnp.zeros((E // 8, 8, 128), u32)
        zv_ref[...] = jnp.zeros(zv_ref.shape, u32)
        dw = jnp.concatenate([dw_ref[0:2].astype(f32), dw2_ref[2:3].astype(f32)], axis=0)
        dif = _iota((8, C), 1) - _iota((8, C), 0)
        R = _iota((16, C), 0); KK = _iota((16, C), 1)
        unit = jnp.where(KK >= 48, 1, 0)
        itap = 2 * unit + ((KK >> 3) & 1) - (R >> 3)
        tapid = jnp.where((KK & 7) == (R & 7), 3 * itap + ((KK - 48 * unit) >> 4), -9)

        def prep_dw(g, c):
            cl = jnp.zeros((16, C), f32)
            for t in range(9):
                row = jnp.broadcast_to(dw[t // 3, t % 3:t % 3 + 1, :], (8, C))
                col = jnp.sum(jnp.where(dif == 8 * g, row, 0.0), axis=1, keepdims=True)
                dwb_ref[0, g, t] = jnp.broadcast_to(col, (8, 128))
                cb = jnp.broadcast_to(col, (8, C))
                cl = jnp.where(tapid == t, jnp.concatenate([cb, cb], axis=0), cl)
            vr_ref[0, CL0 + g, :, 0:C] = pltpu.bitcast(cl.astype(bf16), u32)
            return c
        lax.fori_loop(0, 12, prep_dw, 0, unroll=PU)

        for cp in small[2:]:
            cp.wait()
        w1f = w1_ref[...].astype(f32)
        w1k = pltpu.bitcast(_pack_pairs(w1f - jnp.sum(w1f, axis=0, keepdims=True) * (1.0 / C)), bf16)
        for i in range(3):
            Pb = jnp.where(_perm16(_iota((128, E), 0) + 128 * i) == _iota((128, E), 1), 1.0, 0.0).astype(bf16)
            w1q = lax.dot_general(Pb, w1k, (((1,), (1,)), ((), ())), preferred_element_type=f32)
            w1q_ref[64 * i:64 * i + 64, :] = pltpu.bitcast(w1q.astype(bf16), u32)
        w2s_ref[...] = pltpu.bitcast(w2t_ref[...], u32)

        lane = _iota((8, 128), 1)

        def s1(xu_ref, u, kill=None):
            zz = jnp.zeros((8, 128), u32)
            for g in range(12):
                m = pltpu.bitcast(xu_ref[g], u32)
                if kill is not None:
                    m = jnp.where(kill, jnp.zeros_like(m), m)
                mq = [m[:, 128 * q:128 * q + 128] for q in range(NQ)]
                for q in range(NQ):
                    lq = jnp.where(lane == 127, mq[q - 1] if q > 0 else zz, mq[q])
                    rq = jnp.where(lane == 0, mq[q + 1] if q + 1 < NQ else zz, mq[q])
                    vr_ref[0, vi(u, g, q, 0)] = pltpu.roll(lq, 1, 1)
                    vr_ref[0, vi(u, g, q, 1)] = mq[q]
                    vr_ref[0, vi(u, g, q, 2)] = pltpu.roll(rq, 127, 1)

        def conv_round(t, q, gs):
            cvs = []
            for g in gs:
                rhs = jnp.concatenate([vr_ref[0, vi(uu & 1, g, q, v)] for uu in (t, t + 1) for v in range(3)], axis=0)
                lhs = pltpu.bitcast(vr_ref[0, CL0 + g, :, 0:C], bf16)
                cvs.append(jnp.dot(lhs, pltpu.bitcast(rhs, bf16), preferred_element_type=f32))
            return cvs

        sub = _iota((8, 128), 0)
        m0 = sub % 2 == 0
        m1 = (sub // 2) % 2 == 0
        lnc = jnp.where(m1, 1.0 / (C * _A), 1.0 / (C * _A * _A))

        merge = _merge

        def ln_tile(cvs, q, dsts):
            ls = slice(128 * q, 128 * q + 128)
            cs = [[cv[8 * ab:8 * ab + 8] for cv in cvs] for ab in range(2)]
            c1 = merge(_tree_sum(cs[0]), _tree_sum(cs[1]), m0, 1)
            c2 = merge(_tree_sum([c * c for c in cs[0]]), _tree_sum([c * c for c in cs[1]]), m0, 1)
            e = merge(c1, c2, m1, 2)
            f = (e + pltpu.roll(e, 4, 0)) * lnc
            v = pltpu.roll(f, 6, 0) - f * f
            rs = lax.rsqrt(jnp.maximum(v, 0.0) + 1e-5 / (_A * _A))
            for ab in range(2):
                xn_ref[dsts[ab], :, ls] = _pack_pairs(jnp.concatenate(cs[ab], axis=0) * rs[ab:ab + 1, :])

        xp[8, :, 0:8, :] = jnp.zeros((12, 8, W), bf16)
        p_copy(1, 3, 0, 1, 1).wait()
        p_copy(0, 4, 1, 1).wait()
        if PRO == 0:
            s1(xp.at[10], 0)
            s1(xp.at[11], 1)
            for i, (un, da, db) in enumerate([(1, 10, 5), (0, 8, 9), (2, 0, 1)]):
                for q in range(NQ):
                    ln_tile(conv_round(2 - i, q, range(12)), q, (da, db))
                s1(xp.at[8 + un], un & 1)
        else:
            def pro0(i, c):
                s1(xp.at[10 + i], i)
                return c
            lax.fori_loop(0, 2, pro0, 0)

            def pro(i, c):
                da = jnp.where(i == 0, 10, jnp.where(i == 1, 8, 0))
                db = jnp.where(i == 0, 5, jnp.where(i == 1, 9, 1))
                for q in range(NQ):
                    ln_tile(conv_round(2 - i, q, range(12)), q, (da, db))
                un = jnp.where(i == 2, 2, 1 - i)
                s1(xp.at[8 + un], un & 1)
                return c
            lax.fori_loop(0, 3, pro, 0)
        for r in range(2):
            xn_ref[2 + r] = xn_ref[8 + r]

        NP = 2 * NSUB
        RPP = 12 // NP
        MR = E // NSUB

        def body(j, carry):
            z = zs_ref[0]
            z1 = zs_ref[1]
            slot = j & 1

            @pl.when(j < NG - 1)
            def _():
                for cp in chunk(j, False):
                    cp.wait()

            @pl.when(j == NG - 1)
            def _():
                for cp in chunk(j, True):
                    cp.wait()
                for jn in range(3):
                    x_copy(jn, (S0 + jn) % NB2).start()

            @pl.when(j < NG - 2)
            def _():
                for cp in chunk(j + 1, False):
                    cp.start()

            @pl.when(j == NG - 2)
            def _():
                for cp in chunk(j + 1, True):
                    cp.start()


            pend = []
            cur = []
            for p in range(NP2):
                for r in range(NP):
                    gr = p * NP + r
                    ab, c = r // NSUB, r % NSUB
                    k = 2 * p + ab
                    while pend and pend[0][0] <= gr:
                        ln_tile(*pend.pop(0)[1:])
                    xn = pltpu.bitcast(xn_ref[k % 8 + z], bf16)
                    lhs = pltpu.bitcast(w1q_ref[MR // 2 * c:MR // 2 * (c + 1), :], bf16)
                    gl = _gelu2(jnp.dot(lhs, xn, preferred_element_type=f32))
                    sq = gl * gl
                    s4 = (sq[:, 0:128] + sq[:, 128:256]) + (sq[:, 256:384] + sq[:, 384:512])
                    for i in range(MR // 8):
                        ai = ACC0 + MR // 8 * c + i
                        vr_ref[0, ai] = pltpu.bitcast(pltpu.bitcast(vr_ref[0, ai], f32) + s4[8 * i:8 * i + 8], u32)
                    if k % G2 in ST:
                        h_ref[_hslot(2 * j + k // G2) + ST.index(k % G2), MR // 2 * c:MR // 2 * (c + 1), :] = _pack_pairs(gl)
                    for rr in range(r * RPP, (r + 1) * RPP):
                        q = (rr // 3 + 2) % 4
                        pair = p + 1 + (rr >= 6)
                        cur += conv_round(pair, q, range(4 * (rr % 3), 4 * (rr % 3) + 4))
                        if rr % 3 == 2:
                            pend.append((gr + LN_LAG, cur, q,
                                         (2 * pair % 8 + z1, (2 * pair + 1) % 8 + z1)))
                            cur = []
                    if r == NP // 2 - 1:
                        kill = None
                        if p == NP2 - 3:
                            kill = _iota((8, W), 0) >= jnp.where(j == NG - 1, 4, 8)
                        s1(xp.at[8 * slot + p], (p + 3) % NU, kill)
            for e in pend:
                ln_tile(*e[1:])
            return carry

        with jax.named_scope('loop1'):
            lax.fori_loop(0, NG, body, 0)

        pdif = _iota((8, E), 1) - 2 * _iota((8, E), 0) + zs_ref[0]
        parts = []
        for i in range(E // 8):
            col = jnp.sum(pltpu.bitcast(vr_ref[0, ACC0 + i], f32), axis=1, keepdims=True)
            parts.append(jnp.where(pdif == 16 * (i // 2) + i % 2, jnp.broadcast_to(col, (8, E)), 0.0))
        ss = jnp.sum(_tree_sum(parts), axis=0, keepdims=True) * (_GS * _GS)
        gx = jnp.sqrt(ss + 1e-6)
        nx = gx / (jnp.sum(gx, axis=1, keepdims=True) * (1.0 / E) + 1e-6)
        gam = g_ref[...].astype(f32).reshape(1, E)
        bet = b_ref[...].astype(f32).reshape(1, E)
        s = (gam * nx + 1.0) * _GS
        w2t = pltpu.bitcast(w2s_ref[...], bf16).astype(f32)
        w2s_ref[...] = pltpu.bitcast((w2t * s).astype(bf16), u32)
        bias_ref[...] = jnp.broadcast_to(jnp.sum(w2t * bet, axis=1, keepdims=True), (C, 128))

    pl.run_scoped(lambda: phase1())

    def phase2():
        vi = lambda q, k, i: (q * 6 + k) * 3 * (NR + 2) + i
        R0 = RC[0] - 1

        def o_copy(j, sl, r0, n):
            return pltpu.make_async_copy(xbuf.at[sl, pl.ds(r0, n)], o_hbm.at[pl.ds(j * G2 + r0, n)], osem.at[sl])

        z0 = zs_ref[0]
        lane = _iota((8, 128), 1) + z0
        sub = _iota((8, 128), 0) + z0
        m0 = (sub & 1) == 0
        m1 = (sub & 2) == 0
        m2 = sub < 4
        lnc = jnp.where(m2, 1.0 / (C * _A), 1.0 / (C * _A * _A))

        def s1(xs, zv):
            zz = jnp.zeros((8, 128), u32)
            for r in range(NR + 2):
                for k in range(6):
                    m = pltpu.bitcast(xbuf[xs, R0 + r, 16 * k:16 * k + 16, :], u32)
                    mq = [m[:, 128 * q:128 * q + 128] for q in range(NQ)]
                    for q in range(NQ):
                        lq = jnp.where(lane == 127, mq[q - 1] if q > 0 else zz, mq[q])
                        rq = jnp.where(lane == 0, mq[q + 1] if q + 1 < NQ else zz, mq[q])
                        vr_ref[zv, vi(q, k, 3 * r)] = pltpu.roll(lq, 1, 1)
                        vr_ref[zv, vi(q, k, 3 * r + 1)] = mq[q]
                        vr_ref[zv, vi(q, k, 3 * r + 2)] = pltpu.roll(rq, 127, 1)

        def conv_unit(q, zc, zw, zr):
            ls = slice(128 * q, 128 * q + 128)
            st = [None] * NR
            tok = yield None
            for g in range(12):
                w = [dwb_ref[zw, g, t] for t in range(9)]
                acc = [None] * NR
                for r in range(NR + 2):
                    for v in range(3):
                        x = vr_ref[zw, vi(q, g // 2, 3 * r + v)]
                        if tok is not None and 3 * r + v in GSET:
                            x = x | tok
                        xf = pltpu.bitcast(x, bf16).astype(f32)[8 * (g % 2):8 * (g % 2) + 8]
                        for n in range(NR):
                            if 0 <= r - n <= 2:
                                t = xf * w[3 * (r - n) + v]
                                acc[n] = t if acc[n] is None else acc[n] + t
                for n in range(NR):
                    cv = acc[n]
                    st[n] = (cv, cv * cv) if st[n] is None else (st[n][0] + cv, st[n][1] + cv * cv)
                    cv_ref[q % NCV + zc, 12 * n + g] = cv
                tok = yield pltpu.bitcast((st[0][1] + st[1][1]) + st[2][1], u32)
            half = lambda i: _merge(_merge(st[0][i], st[1][i], m0, 1), st[2][i] + pltpu.roll(st[2][i], 7, 0), m1, 2)
            f = _merge(half(0), half(1), m2, 4) * lnc
            v = pltpu.roll(f, 4, 0) - f * f
            cv_ref[q % NCV + zr, 36] = lax.rsqrt(jnp.maximum(v, 0.0) + 1e-5 / (_A * _A))
            yield None
            for n in range(NR):
                rs = cv_ref[q % NCV + zc, 36, n:n + 1, :]
                big_ref[8 + n + zc, :, ls] = _pack_pairs(cv_ref[q % NCV + zc, 12 * n:12 * n + 12].reshape(C, 128) * rs)
            yield None

        x_copy(0, S0).wait()
        nxt = lambda sl: jnp.where(sl == NB2 - 1, 0, sl + 1)

        def body(j, xs):
            z = zs_ref[0]
            xs1 = nxt(xs)
            xs3 = nxt(nxt(xs1))

            @pl.when(j + 1 < NG2)
            def _():
                x_copy(j + 1, xs1).wait()

            @pl.when(j >= 2)
            def _():
                o_copy(j - 2, xs3, 0, G2).wait()

            @pl.when(j + 3 < NG2)
            def _():
                x_copy(j + 3, xs3).start()

            units = [conv_unit(q, z, zs_ref[2 + q], zs_ref[1]) for q in range(NQ)]
            for u in units:
                next(u)
            s1(xs1, z)
            zv = zv_ref[0:8, :]
            cnt = [0, 0]
            tails = []
            toks = [None]

            def run_pieces(rel):
                tgt = sum(PLAN[:cnt[0] + 1])
                cnt[0] += 1
                res = None
                while cnt[1] < tgt:
                    u = units[cnt[1] // 12]
                    val = u.send(rel)
                    res = val if res is None else res | val
                    cnt[1] += 1
                    if cnt[1] % 12 == 0:
                        tails.append([TLAG, u])
                        tails.append([TLAG + TLAG2, u])
                for t in list(tails):
                    if t[0] == 0:
                        t[1].send(None)
                        tails.remove(t)
                    t[0] -= 1
                return res

            def gate(d):
                if toks[-1] is None:
                    return d
                mr = d.shape[0]
                du = pltpu.bitcast(d[mr - 8:mr, 384:512], u32) | (toks[-1] & zv)
                last = jnp.concatenate([d[mr - 8:mr, 0:384], pltpu.bitcast(du, f32)], axis=1)
                return jnp.concatenate([d[0:mr - 8], last], axis=0)

            def fin(k, hr):
                for mc in range(2):
                    rs_ = slice(48 * mc, 48 * (mc + 1))
                    o = None
                    for kt in range(3):
                        d = jnp.dot(pltpu.bitcast(w2s_ref[24 * mc:24 * (mc + 1), 128 * kt:128 * kt + 128], bf16),
                                    pltpu.bitcast(hr(kt), bf16), preferred_element_type=f32)
                        rel = pltpu.bitcast(d[0:8, 0:128], u32) & zv
                        d = gate(d)
                        o = d if o is None else o + d
                        if kt == 2:
                            xbuf[xs, k, rs_, :] = (o + _tile4(bias_ref[rs_, :]) + xbuf[xs, k, rs_, :].astype(f32)).astype(bf16)
                        toks.append(run_pieces(rel))

            def ht_rows(n, kt):
                return jnp.concatenate([big_ref[4 * (n % 2) + z + r // 48, r % 48:r % 48 + 8, :]
                                        for r in range(64 * kt, 64 * kt + 64, 8)], axis=0)

            def mm1(n):
                xn = pltpu.bitcast(big_ref[8 + n + z], bf16)
                lhs = pltpu.bitcast(w1q_ref[...], bf16)
                hp = _pack_pairs(_gelu2(jnp.dot(lhs, xn, preferred_element_type=f32)))
                big_ref[pl.ds(4 * (n % 2) + z, 4)] = hp.reshape(4, C // 2, W)

            for tok in P2ORD.split(','):
                n = int(tok[1])
                if tok[0] == 'M': mm1(n)
                elif tok[0] == 'S': fin(ST[n], lambda kt: h_ref[_hslot(j) + n, 64 * kt:64 * kt + 64, :])
                elif tok[0] == 'F': fin(RC[n], functools.partial(ht_rows, n))
                elif tok[0] == 'o': o_copy(j, xs, n, int(tok[2]) - n).start()
            assert cnt[1] == 48
            for t in tails:
                t[1].send(None)
            return xs1

        with jax.named_scope('loop2'):
            lax.fori_loop(0, NG2, body, jnp.int32(S0))
        for j in range(NG2 - 2, NG2):
            o_copy(j, (j + S0) % NB2, 0, G2).wait()

    pl.run_scoped(lambda: phase2())


@jax.jit
def pallas_standalone__modern_conv_block_convnext_v2__vision_kernel(x, dw, w1, w2, grn_gamma, grn_beta):
    xt = jnp.transpose(x, (0, 1, 3, 2)).reshape(H, C, W)
    x5 = xt.reshape(H // 2, 2, C // 8, 8, W)
    w2t = w2.T
    out = pl.pallas_call(
        _kernel,
        in_specs=[pl.BlockSpec(memory_space=pl.ANY)] * 7,
        out_specs=pl.BlockSpec(memory_space=pl.ANY),
        out_shape=jax.ShapeDtypeStruct((H, C, W), bf16),
        scratch_shapes=[
            pltpu.VMEM(((NG2 - HCUT) * NST, E // 2, W), u32),
            pltpu.VMEM((NB2, G2, C, W), bf16),
            pltpu.VMEM((8 + NR, C // 2, W), u32),
            pltpu.VMEM((1, NVR, 8, 128), u32),
            pltpu.VMEM((1, 12, 9, 8, 128), f32),
            pltpu.VMEM((NCV, 40, 8, 128), f32),
            pltpu.VMEM((E // 2, C), u32),
            pltpu.VMEM((C // 2, E), u32),
            pltpu.VMEM((C, 128), f32),
            pltpu.VMEM((8, 128), u32),
            pltpu.VMEM((3, 3, C), bf16),
            pltpu.VMEM((3, 3, C), bf16),
            pltpu.VMEM((E,), bf16),
            pltpu.VMEM((E,), bf16),
            pltpu.SMEM((8,), i32),
            pltpu.SemaphoreType.DMA((NB2,)),
            pltpu.SemaphoreType.DMA((NB2,)),
            pltpu.SemaphoreType.DMA((2, 2)),
            pltpu.SemaphoreType.DMA((6,)),
        ],
        compiler_params=pltpu.CompilerParams(vmem_limit_bytes=128 * 1024 * 1024,
                                             disable_bounds_checks=True),
    )(xt, x5, dw, w1, w2t, grn_gamma, grn_beta)
    return jnp.transpose(out.reshape(1, H, C, W), (0, 1, 3, 2))
```

```python
import functools
import math
import jax
import jax.numpy as jnp
from jax import lax
import jax.experimental.pallas as pl
import jax.experimental.pallas.tpu as pltpu

H = 512; W = 512; C = 96; E = 384
G = 16
NG = H // G
G2 = 8
NG2 = H // G2
RC = (2, 3, 4)
ST = tuple(k for k in range(G2) if k not in RC)
NST = len(ST)
NR = len(RC)
NU = 2
NQ = W // 128
NVR = NQ * 6 * 3 * (NR + 2)
ACC0 = NU * 12 * NQ * 3
CL0 = ACC0 + E // 8
NB2 = 5
S0 = 4
LN_LAG = 5
NSUB = 6
P2ORD = 'M0,M1,F0,M2,S0,F1,S1,o04,F2,S2,o46,S3,S4,o68'
PLAN = [int(c) for c in ('22' + '1' * 44 + '00')]
GSET = [int(c) for c in '2,5,8,11,14'.split(',')]
TLAG = 0
TLAG2 = 0
NCV = 1
PU = 12
PRO = 0
CFIRST = 0
PFAT = 3
HCUT = 0

_C1 = math.sqrt(2.0 / math.pi)
_C3 = _C1 * 0.044715
_A = _C3 ** (1.0 / 3.0)
_K = _C1 / _A
_GS = 0.5 / _A

f32 = jnp.float32
bf16 = jnp.bfloat16
u32 = jnp.uint32
i32 = jnp.int32


def _iota(shape, d):
    return lax.broadcasted_iota(i32, shape, d)


def _perm16(r):
    return (r & ~15) + 2 * (r & 7) + ((r >> 3) & 1)


def _tile4(a):
    return jnp.concatenate([a] * NQ, axis=1)


def _pack_pairs(y):
    m = y.shape[0] // 16
    outs = [pltpu.pack_elementwise([y[16 * t:16 * t + 8], y[16 * t + 8:16 * t + 16]], packed_dtype=bf16)
            for t in range(m)]
    o = outs[0] if m == 1 else jnp.concatenate(outs, axis=0)
    return pltpu.bitcast(o, u32) if o.dtype != u32 else o


def _gelu2(y):
    u = y * (y * y + _K)
    t = jnp.tanh(u)
    return y * t + y


def _tree_sum(xs):
    xs = list(xs)
    while len(xs) > 1:
        xs = [xs[i] + xs[i + 1] for i in range(0, len(xs) - 1, 2)] + ([xs[-1]] if len(xs) % 2 else [])
    return xs[0]


def _hslot(j):
    return (j % (NG2 - HCUT) if HCUT else j) * NST


def _merge(a, b, msk, sh):
    return jnp.where(msk, a, b) + pltpu.roll(jnp.where(msk, b, a), 8 - sh, 0)


def _kernel(x_hbm, x5_hbm, dw_hbm, w1_hbm, w2t_hbm, g_hbm, b_hbm, o_hbm,
            h_ref, xbuf, big_ref, vr_ref, dwb_ref, cv_ref, w1q_ref, w2s_ref, bias_ref, zv_ref, dw_ref, dw2_ref, g_ref, b_ref, zs_ref,
            xsem, osem, psem, wsem):

    for i in range(8):
        zs_ref[i] = 0

    def x_copy(j, sl):
        return pltpu.make_async_copy(x_hbm.at[pl.ds(j * G2, G2)], xbuf.at[sl], xsem.at[sl])

    def phase1():
        xn_ref = big_ref
        vi = lambda u, g, q, v: ((u * 12 + g) * NQ + q) * 3 + v
        xp = xbuf.reshape(NB2 * G2 // 2, C // 8, 16, W)
        NP2 = G // 2

        def row_copy(u, half, slot, i):
            return pltpu.make_async_copy(x5_hbm.at[u - 1 + half, 1 - half],
                                         xp.at[NP2 * slot + i, :, pl.ds(8 * half, 8), :], psem.at[slot])

        def rows_copy(u, n, half, slot, i):
            return pltpu.make_async_copy(x5_hbm.at[pl.ds(u - 1 + half, n), 1 - half],
                                         xp.at[pl.ds(NP2 * slot + i, n), :, pl.ds(8 * half, 8), :], psem.at[slot])

        def start_rows(j, inner):
            for i in range(NP2):
                for half in range(2):
                    if (i < NP2 - 2 - half) == inner:
                        row_copy(NP2 * j + 3 + i, half, j & 1, i).start()

        def wait_rows(slot, last):
            if last:
                bufs = [xbuf.at[2 * slot], xbuf.at[2 * slot + 1, pl.ds(0, G - 5 - G2)]]
            else:
                bufs = [xbuf.at[pl.ds(2 * slot, 2)]]
            for buf in bufs:
                pltpu.make_async_copy(buf, buf, psem.at[slot]).wait()

        w1_ref = xbuf.at[4, 0, :, pl.ds(0, E)]
        w2t_ref = xbuf.at[4, 1, :, pl.ds(0, E)]
        small = [pltpu.make_async_copy(a, b, wsem.at[i]) for i, (a, b) in enumerate(
            [(dw_hbm, dw_ref), (dw_hbm, dw2_ref), (w1_hbm, w1_ref), (w2t_hbm, w2t_ref), (g_hbm, g_ref), (b_hbm, b_ref)])]
        for cp in small[:3]:
            cp.start()
        rows_copy(1, 3, 0, 1, 1).start()
        rows_copy(0, 4, 1, 1, 0).start()
        for cp in small[3:]:
            cp.start()
        rows_copy(3, NP2, 0, 0, 0).start()
        rows_copy(3, NP2, 1, 0, 0).start()
        for cp in small[:2]:
            cp.wait()

        vr_ref[0, ACC0:CL0] = jnp.zeros((E // 8, 8, 128), u32)
        zv_ref[...] = jnp.zeros(zv_ref.shape, u32)
        dw = jnp.concatenate([dw_ref[0:2].astype(f32), dw2_ref[2:3].astype(f32)], axis=0)
        dif = _iota((8, C), 1) - _iota((8, C), 0)
        R = _iota((16, C), 0); KK = _iota((16, C), 1)
        unit = jnp.where(KK >= 48, 1, 0)
        itap = 2 * unit + ((KK >> 3) & 1) - (R >> 3)
        tapid = jnp.where((KK & 7) == (R & 7), 3 * itap + ((KK - 48 * unit) >> 4), -9)

        def prep_dw(g, c):
            cl = jnp.zeros((16, C), f32)
            for t in range(9):
                row = jnp.broadcast_to(dw[t // 3, t % 3:t % 3 + 1, :], (8, C))
                col = jnp.sum(jnp.where(dif == 8 * g, row, 0.0), axis=1, keepdims=True)
                dwb_ref[0, g, t] = jnp.broadcast_to(col, (8, 128))
                cb = jnp.broadcast_to(col, (8, C))
                cl = jnp.where(tapid == t, jnp.concatenate([cb, cb], axis=0), cl)
            vr_ref[0, CL0 + g, :, 0:C] = pltpu.bitcast(cl.astype(bf16), u32)
            return c
        lax.fori_loop(0, 12, prep_dw, 0, unroll=PU)

        for cp in small[2:]:
            cp.wait()
        w1f = w1_ref[...].astype(f32)
        w1k = pltpu.bitcast(_pack_pairs(w1f - jnp.sum(w1f, axis=0, keepdims=True) * (1.0 / C)), bf16)
        for i in range(3):
            Pb = jnp.where(_perm16(_iota((128, E), 0) + 128 * i) == _iota((128, E), 1), 1.0, 0.0).astype(bf16)
            w1q = lax.dot_general(Pb, w1k, (((1,), (1,)), ((), ())), preferred_element_type=f32)
            w1q_ref[64 * i:64 * i + 64, :] = pltpu.bitcast(w1q.astype(bf16), u32)
        w2s_ref[...] = pltpu.bitcast(w2t_ref[...], u32)

        lane = _iota((8, 128), 1)

        def s1(xu_ref, u, kill=None):
            zz = jnp.zeros((8, 128), u32)
            for g in range(12):
                m = pltpu.bitcast(xu_ref[g], u32)
                if kill is not None:
                    m = jnp.where(kill, jnp.zeros_like(m), m)
                mq = [m[:, 128 * q:128 * q + 128] for q in range(NQ)]
                for q in range(NQ):
                    lq = jnp.where(lane == 127, mq[q - 1] if q > 0 else zz, mq[q])
                    rq = jnp.where(lane == 0, mq[q + 1] if q + 1 < NQ else zz, mq[q])
                    vr_ref[0, vi(u, g, q, 0)] = pltpu.roll(lq, 1, 1)
                    vr_ref[0, vi(u, g, q, 1)] = mq[q]
                    vr_ref[0, vi(u, g, q, 2)] = pltpu.roll(rq, 127, 1)

        def conv_round(t, q, gs):
            cvs = []
            for g in gs:
                rhs = jnp.concatenate([vr_ref[0, vi(uu & 1, g, q, v)] for uu in (t, t + 1) for v in range(3)], axis=0)
                lhs = pltpu.bitcast(vr_ref[0, CL0 + g, :, 0:C], bf16)
                cvs.append(jnp.dot(lhs, pltpu.bitcast(rhs, bf16), preferred_element_type=f32))
            return cvs

        sub = _iota((8, 128), 0)
        m0 = sub % 2 == 0
        m1 = (sub // 2) % 2 == 0
        lnc = jnp.where(m1, 1.0 / (C * _A), 1.0 / (C * _A * _A))

        merge = _merge

        def ln_tile(cvs, q, dsts):
            ls = slice(128 * q, 128 * q + 128)
            cs = [[cv[8 * ab:8 * ab + 8] for cv in cvs] for ab in range(2)]
            c1 = merge(_tree_sum(cs[0]), _tree_sum(cs[1]), m0, 1)
            c2 = merge(_tree_sum([c * c for c in cs[0]]), _tree_sum([c * c for c in cs[1]]), m0, 1)
            e = merge(c1, c2, m1, 2)
            f = (e + pltpu.roll(e, 4, 0)) * lnc
            v = pltpu.roll(f, 6, 0) - f * f
            rs = lax.rsqrt(jnp.maximum(v, 0.0) + 1e-5 / (_A * _A))
            for ab in range(2):
                xn_ref[dsts[ab], :, ls] = _pack_pairs(jnp.concatenate(cs[ab], axis=0) * rs[ab:ab + 1, :])

        xp[8, :, 0:8, :] = jnp.zeros((12, 8, W), bf16)
        rows_copy(1, 3, 0, 1, 1).wait()
        rows_copy(0, 4, 1, 1, 0).wait()
        if PRO == 0:
            s1(xp.at[10], 0)
            s1(xp.at[11], 1)
            for i, (un, da, db) in enumerate([(1, 10, 5), (0, 8, 9), (2, 0, 1)]):
                for q in range(NQ):
                    ln_tile(conv_round(2 - i, q, range(12)), q, (da, db))
                s1(xp.at[8 + un], un & 1)
        else:
            def pro0(i, c):
                s1(xp.at[10 + i], i)
                return c
            lax.fori_loop(0, 2, pro0, 0)

            def pro(i, c):
                da = jnp.where(i == 0, 10, jnp.where(i == 1, 8, 0))
                db = jnp.where(i == 0, 5, jnp.where(i == 1, 9, 1))
                for q in range(NQ):
                    ln_tile(conv_round(2 - i, q, range(12)), q, (da, db))
                un = jnp.where(i == 2, 2, 1 - i)
                s1(xp.at[8 + un], un & 1)
                return c
            lax.fori_loop(0, 3, pro, 0)
        for r in range(2):
            xn_ref[2 + r] = xn_ref[8 + r]

        NP = 2 * NSUB
        RPP = 12 // NP
        MR = E // NSUB

        def body(j, carry):
            z = zs_ref[0]
            z1 = zs_ref[1]
            slot = j & 1

            @pl.when(j < NG - 1)
            def _():
                wait_rows(slot, False)

            @pl.when(j == NG - 1)
            def _():
                wait_rows(slot, True)

            def prefetch():
                @pl.when(j < NG - 1)
                def _():
                    start_rows(j + 1, True)

                @pl.when(j < NG - 2)
                def _():
                    start_rows(j + 1, False)

                @pl.when(j == NG - 1)
                def _():
                    for jn in range(3):
                        x_copy(jn, (S0 + jn) % NB2).start()

            pend = []
            cur = []
            for p in range(NP2):
                for r in range(NP):
                    gr = p * NP + r
                    ab, c = r // NSUB, r % NSUB
                    k = 2 * p + ab
                    def mm_part():
                        while pend and pend[0][0] <= gr:
                            ln_tile(*pend.pop(0)[1:])
                        xn = pltpu.bitcast(xn_ref[k % 8 + z], bf16)
                        lhs = pltpu.bitcast(w1q_ref[MR // 2 * c:MR // 2 * (c + 1), :], bf16)
                        gl = _gelu2(jnp.dot(lhs, xn, preferred_element_type=f32))
                        sq = gl * gl
                        s4 = (sq[:, 0:128] + sq[:, 128:256]) + (sq[:, 256:384] + sq[:, 384:512])
                        for i in range(MR // 8):
                            ai = ACC0 + MR // 8 * c + i
                            vr_ref[0, ai] = pltpu.bitcast(pltpu.bitcast(vr_ref[0, ai], f32) + s4[8 * i:8 * i + 8], u32)
                        if k % G2 in ST:
                            h_ref[_hslot(2 * j + k // G2) + ST.index(k % G2), MR // 2 * c:MR // 2 * (c + 1), :] = _pack_pairs(gl)
                    def cv_part():
                        nonlocal cur
                        for rr in range(r * RPP, (r + 1) * RPP):
                            q = (rr // 3 + 2) % 4
                            pair = p + 1 + (rr >= 6)
                            cur += conv_round(pair, q, range(4 * (rr % 3), 4 * (rr % 3) + 4))
                            if rr % 3 == 2:
                                pend.append((gr + LN_LAG, cur, q,
                                             (2 * pair % 8 + z1, (2 * pair + 1) % 8 + z1)))
                                cur = []
                    if gr == PFAT:
                        prefetch()
                    if CFIRST:
                        cv_part(); mm_part()
                    else:
                        mm_part(); cv_part()
                    if r == NP // 2 - 1:
                        kill = None
                        if p == NP2 - 3:
                            kill = _iota((8, W), 0) >= jnp.where(j == NG - 1, 4, 8)
                        s1(xp.at[8 * slot + p], (p + 3) % NU, kill)
            for e in pend:
                ln_tile(*e[1:])
            return carry

        with jax.named_scope('loop1'):
            lax.fori_loop(0, NG, body, 0)

        pdif = _iota((8, E), 1) - 2 * _iota((8, E), 0) + zs_ref[0]
        parts = []
        for i in range(E // 8):
            col = jnp.sum(pltpu.bitcast(vr_ref[0, ACC0 + i], f32), axis=1, keepdims=True)
            parts.append(jnp.where(pdif == 16 * (i // 2) + i % 2, jnp.broadcast_to(col, (8, E)), 0.0))
        ss = jnp.sum(_tree_sum(parts), axis=0, keepdims=True) * (_GS * _GS)
        gx = jnp.sqrt(ss + 1e-6)
        nx = gx / (jnp.sum(gx, axis=1, keepdims=True) * (1.0 / E) + 1e-6)
        gam = g_ref[...].astype(f32).reshape(1, E)
        bet = b_ref[...].astype(f32).reshape(1, E)
        s = (gam * nx + 1.0) * _GS
        w2t = pltpu.bitcast(w2s_ref[...], bf16).astype(f32)
        w2s_ref[...] = pltpu.bitcast((w2t * s).astype(bf16), u32)
        bias_ref[...] = jnp.broadcast_to(jnp.sum(w2t * bet, axis=1, keepdims=True), (C, 128))

    pl.run_scoped(lambda: phase1())

    def phase2():
        vi = lambda q, k, i: (q * 6 + k) * 3 * (NR + 2) + i
        R0 = RC[0] - 1

        def o_copy(j, sl, r0, n):
            return pltpu.make_async_copy(xbuf.at[sl, pl.ds(r0, n)], o_hbm.at[pl.ds(j * G2 + r0, n)], osem.at[sl])

        z0 = zs_ref[0]
        lane = _iota((8, 128), 1) + z0
        sub = _iota((8, 128), 0) + z0
        m0 = (sub & 1) == 0
        m1 = (sub & 2) == 0
        m2 = sub < 4
        lnc = jnp.where(m2, 1.0 / (C * _A), 1.0 / (C * _A * _A))

        def s1(xs, zv):
            zz = jnp.zeros((8, 128), u32)
            for r in range(NR + 2):
                for k in range(6):
                    m = pltpu.bitcast(xbuf[xs, R0 + r, 16 * k:16 * k + 16, :], u32)
                    mq = [m[:, 128 * q:128 * q + 128] for q in range(NQ)]
                    for q in range(NQ):
                        lq = jnp.where(lane == 127, mq[q - 1] if q > 0 else zz, mq[q])
                        rq = jnp.where(lane == 0, mq[q + 1] if q + 1 < NQ else zz, mq[q])
                        vr_ref[zv, vi(q, k, 3 * r)] = pltpu.roll(lq, 1, 1)
                        vr_ref[zv, vi(q, k, 3 * r + 1)] = mq[q]
                        vr_ref[zv, vi(q, k, 3 * r + 2)] = pltpu.roll(rq, 127, 1)

        def conv_unit(q, zc, zw, zr):
            ls = slice(128 * q, 128 * q + 128)
            st = [None] * NR
            tok = yield None
            for g in range(12):
                w = [dwb_ref[zw, g, t] for t in range(9)]
                acc = [None] * NR
                for r in range(NR + 2):
                    for v in range(3):
                        x = vr_ref[zw, vi(q, g // 2, 3 * r + v)]
                        if tok is not None and 3 * r + v in GSET:
                            x = x | tok
                        xf = pltpu.bitcast(x, bf16).astype(f32)[8 * (g % 2):8 * (g % 2) + 8]
                        for n in range(NR):
                            if 0 <= r - n <= 2:
                                t = xf * w[3 * (r - n) + v]
                                acc[n] = t if acc[n] is None else acc[n] + t
                for n in range(NR):
                    cv = acc[n]
                    st[n] = (cv, cv * cv) if st[n] is None else (st[n][0] + cv, st[n][1] + cv * cv)
                    cv_ref[q % NCV + zc, 12 * n + g] = cv
                tok = yield pltpu.bitcast((st[0][1] + st[1][1]) + st[2][1], u32)
            half = lambda i: _merge(_merge(st[0][i], st[1][i], m0, 1), st[2][i] + pltpu.roll(st[2][i], 7, 0), m1, 2)
            f = _merge(half(0), half(1), m2, 4) * lnc
            v = pltpu.roll(f, 4, 0) - f * f
            cv_ref[q % NCV + zr, 36] = lax.rsqrt(jnp.maximum(v, 0.0) + 1e-5 / (_A * _A))
            yield None
            for n in range(NR):
                rs = cv_ref[q % NCV + zc, 36, n:n + 1, :]
                big_ref[8 + n + zc, :, ls] = _pack_pairs(cv_ref[q % NCV + zc, 12 * n:12 * n + 12].reshape(C, 128) * rs)
            yield None

        x_copy(0, S0).wait()
        nxt = lambda sl: jnp.where(sl == NB2 - 1, 0, sl + 1)

        def body(j, xs):
            z = zs_ref[0]
            xs1 = nxt(xs)
            xs3 = nxt(nxt(xs1))

            @pl.when(j + 1 < NG2)
            def _():
                x_copy(j + 1, xs1).wait()

            @pl.when(j >= 2)
            def _():
                o_copy(j - 2, xs3, 0, G2).wait()

            @pl.when(j + 3 < NG2)
            def _():
                x_copy(j + 3, xs3).start()

            units = [conv_unit(q, z, zs_ref[2 + q], zs_ref[1]) for q in range(NQ)]
            for u in units:
                next(u)
            s1(xs1, z)
            zv = zv_ref[0:8, :]
            cnt = [0, 0]
            tails = []
            toks = [None]

            def run_pieces(rel):
                tgt = sum(PLAN[:cnt[0] + 1])
                cnt[0] += 1
                res = None
                while cnt[1] < tgt:
                    u = units[cnt[1] // 12]
                    val = u.send(rel)
                    res = val if res is None else res | val
                    cnt[1] += 1
                    if cnt[1] % 12 == 0:
                        tails.append([TLAG, u])
                        tails.append([TLAG + TLAG2, u])
                for t in list(tails):
                    if t[0] == 0:
                        t[1].send(None)
                        tails.remove(t)
                    t[0] -= 1
                return res

            def gate(d):
                if toks[-1] is None:
                    return d
                mr = d.shape[0]
                du = pltpu.bitcast(d[mr - 8:mr, 384:512], u32) | (toks[-1] & zv)
                last = jnp.concatenate([d[mr - 8:mr, 0:384], pltpu.bitcast(du, f32)], axis=1)
                return jnp.concatenate([d[0:mr - 8], last], axis=0)

            def fin(k, hr):
                for mc in range(2):
                    rs_ = slice(48 * mc, 48 * (mc + 1))
                    o = None
                    for kt in range(3):
                        d = jnp.dot(pltpu.bitcast(w2s_ref[24 * mc:24 * (mc + 1), 128 * kt:128 * kt + 128], bf16),
                                    pltpu.bitcast(hr(kt), bf16), preferred_element_type=f32)
                        rel = pltpu.bitcast(d[0:8, 0:128], u32) & zv
                        d = gate(d)
                        o = d if o is None else o + d
                        if kt == 2:
                            xbuf[xs, k, rs_, :] = (o + _tile4(bias_ref[rs_, :]) + xbuf[xs, k, rs_, :].astype(f32)).astype(bf16)
                        toks.append(run_pieces(rel))

            def ht_rows(n, kt):
                return jnp.concatenate([big_ref[4 * (n % 2) + z + r // 48, r % 48:r % 48 + 8, :]
                                        for r in range(64 * kt, 64 * kt + 64, 8)], axis=0)

            def mm1(n):
                xn = pltpu.bitcast(big_ref[8 + n + z], bf16)
                lhs = pltpu.bitcast(w1q_ref[...], bf16)
                hp = _pack_pairs(_gelu2(jnp.dot(lhs, xn, preferred_element_type=f32)))
                big_ref[pl.ds(4 * (n % 2) + z, 4)] = hp.reshape(4, C // 2, W)

            for tok in P2ORD.split(','):
                n = int(tok[1])
                if tok[0] == 'M': mm1(n)
                elif tok[0] == 'S': fin(ST[n], lambda kt: h_ref[_hslot(j) + n, 64 * kt:64 * kt + 64, :])
                elif tok[0] == 'F': fin(RC[n], functools.partial(ht_rows, n))
                elif tok[0] == 'o': o_copy(j, xs, n, int(tok[2]) - n).start()
            assert cnt[1] == 48
            for t in tails:
                t[1].send(None)
            return xs1

        with jax.named_scope('loop2'):
            lax.fori_loop(0, NG2, body, jnp.int32(S0))
        for j in range(NG2 - 2, NG2):
            o_copy(j, (j + S0) % NB2, 0, G2).wait()

    pl.run_scoped(lambda: phase2())


@jax.jit
def pallas_standalone__modern_conv_block_convnext_v2__vision_kernel(x, dw, w1, w2, grn_gamma, grn_beta):
    xt = jnp.transpose(x, (0, 1, 3, 2)).reshape(H, C, W)
    x5 = xt.reshape(H // 2, 2, C // 8, 8, W)
    w2t = w2.T
    out = pl.pallas_call(
        _kernel,
        in_specs=[pl.BlockSpec(memory_space=pl.ANY)] * 7,
        out_specs=pl.BlockSpec(memory_space=pl.ANY),
        out_shape=jax.ShapeDtypeStruct((H, C, W), bf16),
        scratch_shapes=[
            pltpu.VMEM(((NG2 - HCUT) * NST, E // 2, W), u32),
            pltpu.VMEM((NB2, G2, C, W), bf16),
            pltpu.VMEM((8 + NR, C // 2, W), u32),
            pltpu.VMEM((1, NVR, 8, 128), u32),
            pltpu.VMEM((1, 12, 9, 8, 128), f32),
            pltpu.VMEM((NCV, 40, 8, 128), f32),
            pltpu.VMEM((E // 2, C), u32),
            pltpu.VMEM((C // 2, E), u32),
            pltpu.VMEM((C, 128), f32),
            pltpu.VMEM((8, 128), u32),
            pltpu.VMEM((3, 3, C), bf16),
            pltpu.VMEM((3, 3, C), bf16),
            pltpu.VMEM((E,), bf16),
            pltpu.VMEM((E,), bf16),
            pltpu.SMEM((8,), i32),
            pltpu.SemaphoreType.DMA((NB2,)),
            pltpu.SemaphoreType.DMA((NB2,)),
            pltpu.SemaphoreType.DMA((2,)),
            pltpu.SemaphoreType.DMA((6,)),
        ],
        compiler_params=pltpu.CompilerParams(vmem_limit_bytes=128 * 1024 * 1024,
                                             disable_bounds_checks=True),
    )(xt, x5, dw, w1, w2t, grn_gamma, grn_beta)
    return jnp.transpose(out.reshape(1, H, C, W), (0, 1, 3, 2))
```

```python
import functools
import math
import jax
import jax.numpy as jnp
from jax import lax
import jax.experimental.pallas as pl
import jax.experimental.pallas.tpu as pltpu

H = 512; W = 512; C = 96; E = 384
G = 16
NG = H // G
G2 = 8
NG2 = H // G2
RC = (2, 3, 4)
ST = tuple(k for k in range(G2) if k not in RC)
NST = len(ST)
NR = len(RC)
NU = 2
NQ = W // 128
NVR = NQ * 6 * 3 * (NR + 2)
ACC0 = NU * 12 * NQ * 3
CL0 = ACC0 + E // 8
NB2 = 5
S0 = 4
LN_LAG = 5
NSUB = 6
P2ORD = 'M0,M1,F0,M2,S0,F1,S1,o04,F2,S2,o46,S3,S4,o68'
PLAN = [int(c) for c in ('22' + '1' * 44 + '00')]
GSET = [int(c) for c in '2,5,8,11,14'.split(',')]
TLAG = 0
TLAG2 = 0
NCV = 1
PU = 12
PRO = 0
CFIRST = 0
PFAT = 3
HCUT = 0

_C1 = math.sqrt(2.0 / math.pi)
_C3 = _C1 * 0.044715
_A = _C3 ** (1.0 / 3.0)
_K = _C1 / _A
_GS = 0.5 / _A

f32 = jnp.float32
bf16 = jnp.bfloat16
u32 = jnp.uint32
i32 = jnp.int32


def _iota(shape, d):
    return lax.broadcasted_iota(i32, shape, d)


def _tile4(a):
    return jnp.concatenate([a] * NQ, axis=1)


def _pack(y, n=1):
    return pltpu.bitcast(y.reshape(n, y.shape[0] // n, y.shape[1]).astype(bf16), u32)


def _gelu2(y):
    u = y * (y * y + _K)
    t = jnp.tanh(u)
    return y * t + y


def _tree_sum(xs):
    xs = list(xs)
    while len(xs) > 1:
        xs = [xs[i] + xs[i + 1] for i in range(0, len(xs) - 1, 2)] + ([xs[-1]] if len(xs) % 2 else [])
    return xs[0]


def _hslot(j):
    return (j % (NG2 - HCUT) if HCUT else j) * NST


def _merge(a, b, msk, sh):
    return jnp.where(msk, a, b) + pltpu.roll(jnp.where(msk, b, a), 8 - sh, 0)


def _kernel(x_hbm, x5_hbm, dw_hbm, w1_hbm, w2t_hbm, g_hbm, b_hbm, o_hbm,
            h_ref, xbuf, big_ref, vr_ref, dwb_ref, cv_ref, w1q_ref, w2s_ref, bias_ref, zv_ref, dw_ref, dw2_ref, g_ref, b_ref, zs_ref,
            xsem, osem, psem, wsem):

    for i in range(8):
        zs_ref[i] = 0

    def x_copy(j, sl):
        return pltpu.make_async_copy(x_hbm.at[pl.ds(j * G2, G2)], xbuf.at[sl], xsem.at[sl])

    def phase1():
        xn_ref = big_ref
        vi = lambda u, g, q, v: ((u * 12 + g) * NQ + q) * 3 + v
        xp = xbuf.reshape(NB2 * G2 // 2, C // 8, 16, W)
        NP2 = G // 2

        def row_copy(u, half, slot, i):
            return pltpu.make_async_copy(x5_hbm.at[u - 1 + half, 1 - half],
                                         xp.at[NP2 * slot + i, :, pl.ds(8 * half, 8), :], psem.at[slot])

        def rows_copy(u, n, half, slot, i):
            return pltpu.make_async_copy(x5_hbm.at[pl.ds(u - 1 + half, n), 1 - half],
                                         xp.at[pl.ds(NP2 * slot + i, n), :, pl.ds(8 * half, 8), :], psem.at[slot])

        def start_rows(j, inner):
            for i in range(NP2):
                for half in range(2):
                    if (i < NP2 - 2 - half) == inner:
                        row_copy(NP2 * j + 3 + i, half, j & 1, i).start()

        def wait_rows(slot, last):
            if last:
                bufs = [xbuf.at[2 * slot], xbuf.at[2 * slot + 1, pl.ds(0, G - 5 - G2)]]
            else:
                bufs = [xbuf.at[pl.ds(2 * slot, 2)]]
            for buf in bufs:
                pltpu.make_async_copy(buf, buf, psem.at[slot]).wait()

        w1_ref = xbuf.at[4, 0, :, pl.ds(0, E)]
        w2t_ref = xbuf.at[4, 1, :, pl.ds(0, E)]
        small = [pltpu.make_async_copy(a, b, wsem.at[i]) for i, (a, b) in enumerate(
            [(dw_hbm, dw_ref), (dw_hbm, dw2_ref), (w1_hbm, w1_ref), (w2t_hbm, w2t_ref), (g_hbm, g_ref), (b_hbm, b_ref)])]
        for cp in small[:3]:
            cp.start()
        rows_copy(1, 3, 0, 1, 1).start()
        rows_copy(0, 4, 1, 1, 0).start()
        for cp in small[3:]:
            cp.start()
        rows_copy(3, NP2, 0, 0, 0).start()
        rows_copy(3, NP2, 1, 0, 0).start()
        for cp in small[:2]:
            cp.wait()

        vr_ref[0, ACC0:CL0] = jnp.zeros((E // 8, 8, 128), u32)
        zv_ref[...] = jnp.zeros(zv_ref.shape, u32)
        dw = jnp.concatenate([dw_ref[0:2].astype(f32), dw2_ref[2:3].astype(f32)], axis=0)
        dif = _iota((8, C), 1) - _iota((8, C), 0)
        R = _iota((16, C), 0); KK = _iota((16, C), 1)
        unit = jnp.where(KK >= 48, 1, 0)
        itap = 2 * unit + ((KK >> 3) & 1) - (R >> 3)
        tapid = jnp.where((KK & 7) == (R & 7), 3 * itap + ((KK - 48 * unit) >> 4), -9)

        def prep_dw(g, c):
            cl = jnp.zeros((16, C), f32)
            for t in range(9):
                row = jnp.broadcast_to(dw[t // 3, t % 3:t % 3 + 1, :], (8, C))
                col = jnp.sum(jnp.where(dif == 8 * g, row, 0.0), axis=1, keepdims=True)
                dwb_ref[0, g, t] = jnp.broadcast_to(col, (8, 128))
                cb = jnp.broadcast_to(col, (8, C))
                cl = jnp.where(tapid == t, jnp.concatenate([cb, cb], axis=0), cl)
            vr_ref[0, CL0 + g, :, 0:C] = pltpu.bitcast(cl.astype(bf16), u32)
            return c
        lax.fori_loop(0, 12, prep_dw, 0, unroll=PU)

        for cp in small[2:]:
            cp.wait()
        w1f = w1_ref[...].astype(f32)
        w1k = (w1f - jnp.sum(w1f, axis=0, keepdims=True) * (1.0 / C)).astype(bf16)
        for i in range(3):
            Pb = jnp.where(_iota((128, E), 0) + 128 * i == _iota((128, E), 1), 1.0, 0.0).astype(bf16)
            w1q = lax.dot_general(Pb, w1k, (((1,), (1,)), ((), ())), preferred_element_type=f32)
            w1q_ref[64 * i:64 * i + 64, :] = pltpu.bitcast(w1q.astype(bf16), u32)
        w2s_ref[...] = pltpu.bitcast(w2t_ref[...], u32)

        lane = _iota((8, 128), 1)

        def s1(xu_ref, u, kill=None):
            zz = jnp.zeros((8, 128), u32)
            for g in range(12):
                m = pltpu.bitcast(xu_ref[g], u32)
                if kill is not None:
                    m = jnp.where(kill, jnp.zeros_like(m), m)
                mq = [m[:, 128 * q:128 * q + 128] for q in range(NQ)]
                for q in range(NQ):
                    lq = jnp.where(lane == 127, mq[q - 1] if q > 0 else zz, mq[q])
                    rq = jnp.where(lane == 0, mq[q + 1] if q + 1 < NQ else zz, mq[q])
                    vr_ref[0, vi(u, g, q, 0)] = pltpu.roll(lq, 1, 1)
                    vr_ref[0, vi(u, g, q, 1)] = mq[q]
                    vr_ref[0, vi(u, g, q, 2)] = pltpu.roll(rq, 127, 1)

        def conv_round(t, q, gs):
            cvs = []
            for g in gs:
                rhs = jnp.concatenate([vr_ref[0, vi(uu & 1, g, q, v)] for uu in (t, t + 1) for v in range(3)], axis=0)
                lhs = pltpu.bitcast(vr_ref[0, CL0 + g, :, 0:C], bf16)
                cvs.append(jnp.dot(lhs, pltpu.bitcast(rhs, bf16), preferred_element_type=f32))
            return cvs

        sub = _iota((8, 128), 0)
        m0 = sub % 2 == 0
        m1 = (sub // 2) % 2 == 0
        lnc = jnp.where(m1, 1.0 / (C * _A), 1.0 / (C * _A * _A))

        merge = _merge

        def ln_tile(cvs, q, dsts):
            ls = slice(128 * q, 128 * q + 128)
            cs = [[cv[8 * ab:8 * ab + 8] for cv in cvs] for ab in range(2)]
            c1 = merge(_tree_sum(cs[0]), _tree_sum(cs[1]), m0, 1)
            c2 = merge(_tree_sum([c * c for c in cs[0]]), _tree_sum([c * c for c in cs[1]]), m0, 1)
            e = merge(c1, c2, m1, 2)
            f = (e + pltpu.roll(e, 4, 0)) * lnc
            v = pltpu.roll(f, 6, 0) - f * f
            rs = lax.rsqrt(jnp.maximum(v, 0.0) + 1e-5 / (_A * _A))
            for ab in range(2):
                xn_ref[pl.ds(dsts[ab], 1), :, ls] = _pack(jnp.concatenate(cs[ab], axis=0) * rs[ab:ab + 1, :])

        xp[8, :, 0:8, :] = jnp.zeros((12, 8, W), bf16)
        rows_copy(1, 3, 0, 1, 1).wait()
        rows_copy(0, 4, 1, 1, 0).wait()
        if PRO == 0:
            s1(xp.at[10], 0)
            s1(xp.at[11], 1)
            for i, (un, da, db) in enumerate([(1, 10, 5), (0, 8, 9), (2, 0, 1)]):
                for q in range(NQ):
                    ln_tile(conv_round(2 - i, q, range(12)), q, (da, db))
                s1(xp.at[8 + un], un & 1)
        else:
            def pro0(i, c):
                s1(xp.at[10 + i], i)
                return c
            lax.fori_loop(0, 2, pro0, 0)

            def pro(i, c):
                da = jnp.where(i == 0, 10, jnp.where(i == 1, 8, 0))
                db = jnp.where(i == 0, 5, jnp.where(i == 1, 9, 1))
                for q in range(NQ):
                    ln_tile(conv_round(2 - i, q, range(12)), q, (da, db))
                un = jnp.where(i == 2, 2, 1 - i)
                s1(xp.at[8 + un], un & 1)
                return c
            lax.fori_loop(0, 3, pro, 0)
        for r in range(2):
            xn_ref[2 + r] = xn_ref[8 + r]

        NP = 2 * NSUB
        RPP = 12 // NP
        MR = E // NSUB

        def body(j, carry):
            z = zs_ref[0]
            z1 = zs_ref[1]
            slot = j & 1

            @pl.when(j < NG - 1)
            def _():
                wait_rows(slot, False)

            @pl.when(j == NG - 1)
            def _():
                wait_rows(slot, True)

            def prefetch():
                @pl.when(j < NG - 1)
                def _():
                    start_rows(j + 1, True)

                @pl.when(j < NG - 2)
                def _():
                    start_rows(j + 1, False)

                @pl.when(j == NG - 1)
                def _():
                    for jn in range(3):
                        x_copy(jn, (S0 + jn) % NB2).start()

            pend = []
            cur = []
            for p in range(NP2):
                for r in range(NP):
                    gr = p * NP + r
                    ab, c = r // NSUB, r % NSUB
                    k = 2 * p + ab
                    def mm_part():
                        while pend and pend[0][0] <= gr:
                            ln_tile(*pend.pop(0)[1:])
                        xn = pltpu.bitcast(xn_ref[k % 8 + z], bf16)
                        lhs = pltpu.bitcast(w1q_ref[MR // 2 * c:MR // 2 * (c + 1), :], bf16)
                        gl = _gelu2(jnp.dot(lhs, xn, preferred_element_type=f32))
                        sq = gl * gl
                        s4 = (sq[:, 0:128] + sq[:, 128:256]) + (sq[:, 256:384] + sq[:, 384:512])
                        for i in range(MR // 8):
                            ai = ACC0 + MR // 8 * c + i
                            vr_ref[0, ai] = pltpu.bitcast(pltpu.bitcast(vr_ref[0, ai], f32) + s4[8 * i:8 * i + 8], u32)
                        if k % G2 in ST:
                            h_ref[pl.ds(_hslot(2 * j + k // G2) + ST.index(k % G2), 1), MR // 2 * c:MR // 2 * (c + 1), :] = _pack(gl)
                    def cv_part():
                        nonlocal cur
                        for rr in range(r * RPP, (r + 1) * RPP):
                            q = (rr // 3 + 2) % 4
                            pair = p + 1 + (rr >= 6)
                            cur += conv_round(pair, q, range(4 * (rr % 3), 4 * (rr % 3) + 4))
                            if rr % 3 == 2:
                                pend.append((gr + LN_LAG, cur, q,
                                             (2 * pair % 8 + z1, (2 * pair + 1) % 8 + z1)))
                                cur = []
                    if gr == PFAT:
                        prefetch()
                    if CFIRST:
                        cv_part(); mm_part()
                    else:
                        mm_part(); cv_part()
                    if r == NP // 2 - 1:
                        kill = None
                        if p == NP2 - 3:
                            kill = _iota((8, W), 0) >= jnp.where(j == NG - 1, 4, 8)
                        s1(xp.at[8 * slot + p], (p + 3) % NU, kill)
            for e in pend:
                ln_tile(*e[1:])
            return carry

        with jax.named_scope('loop1'):
            lax.fori_loop(0, NG, body, 0)

        pdif = _iota((8, E), 1) - _iota((8, E), 0) + zs_ref[0]
        parts = []
        for i in range(E // 8):
            col = jnp.sum(pltpu.bitcast(vr_ref[0, ACC0 + i], f32), axis=1, keepdims=True)
            parts.append(jnp.where(pdif == 8 * i, jnp.broadcast_to(col, (8, E)), 0.0))
        ss = jnp.sum(_tree_sum(parts), axis=0, keepdims=True) * (_GS * _GS)
        gx = jnp.sqrt(ss + 1e-6)
        nx = gx / (jnp.sum(gx, axis=1, keepdims=True) * (1.0 / E) + 1e-6)
        gam = g_ref[...].astype(f32).reshape(1, E)
        bet = b_ref[...].astype(f32).reshape(1, E)
        s = (gam * nx + 1.0) * _GS
        w2t = pltpu.bitcast(w2s_ref[...], bf16).astype(f32)
        w2s_ref[...] = pltpu.bitcast((w2t * s).astype(bf16), u32)
        bias_ref[...] = jnp.broadcast_to(jnp.sum(w2t * bet, axis=1, keepdims=True), (C, 128))

    pl.run_scoped(lambda: phase1())

    def phase2():
        vi = lambda q, k, i: (q * 6 + k) * 3 * (NR + 2) + i
        R0 = RC[0] - 1

        def o_copy(j, sl, r0, n):
            return pltpu.make_async_copy(xbuf.at[sl, pl.ds(r0, n)], o_hbm.at[pl.ds(j * G2 + r0, n)], osem.at[sl])

        z0 = zs_ref[0]
        lane = _iota((8, 128), 1) + z0
        sub = _iota((8, 128), 0) + z0
        m0 = (sub & 1) == 0
        m1 = (sub & 2) == 0
        m2 = sub < 4
        lnc = jnp.where(m2, 1.0 / (C * _A), 1.0 / (C * _A * _A))

        def s1(xs, zv):
            zz = jnp.zeros((8, 128), u32)
            for r in range(NR + 2):
                for k in range(6):
                    m = pltpu.bitcast(xbuf[xs, R0 + r, 16 * k:16 * k + 16, :], u32)
                    mq = [m[:, 128 * q:128 * q + 128] for q in range(NQ)]
                    for q in range(NQ):
                        lq = jnp.where(lane == 127, mq[q - 1] if q > 0 else zz, mq[q])
                        rq = jnp.where(lane == 0, mq[q + 1] if q + 1 < NQ else zz, mq[q])
                        vr_ref[zv, vi(q, k, 3 * r)] = pltpu.roll(lq, 1, 1)
                        vr_ref[zv, vi(q, k, 3 * r + 1)] = mq[q]
                        vr_ref[zv, vi(q, k, 3 * r + 2)] = pltpu.roll(rq, 127, 1)

        def conv_unit(q, zc, zw, zr):
            ls = slice(128 * q, 128 * q + 128)
            st = [None] * NR
            tok = yield None
            for g in range(12):
                w = [dwb_ref[zw, g, t] for t in range(9)]
                acc = [None] * NR
                for r in range(NR + 2):
                    for v in range(3):
                        x = vr_ref[zw, vi(q, g // 2, 3 * r + v)]
                        if tok is not None and 3 * r + v in GSET:
                            x = x | tok
                        xf = pltpu.bitcast(x, bf16).astype(f32)[8 * (g % 2):8 * (g % 2) + 8]
                        for n in range(NR):
                            if 0 <= r - n <= 2:
                                t = xf * w[3 * (r - n) + v]
                                acc[n] = t if acc[n] is None else acc[n] + t
                for n in range(NR):
                    cv = acc[n]
                    st[n] = (cv, cv * cv) if st[n] is None else (st[n][0] + cv, st[n][1] + cv * cv)
                    cv_ref[q % NCV + zc, 12 * n + g] = cv
                tok = yield pltpu.bitcast((st[0][1] + st[1][1]) + st[2][1], u32)
            half = lambda i: _merge(_merge(st[0][i], st[1][i], m0, 1), st[2][i] + pltpu.roll(st[2][i], 7, 0), m1, 2)
            f = _merge(half(0), half(1), m2, 4) * lnc
            v = pltpu.roll(f, 4, 0) - f * f
            cv_ref[q % NCV + zr, 36] = lax.rsqrt(jnp.maximum(v, 0.0) + 1e-5 / (_A * _A))
            yield None
            for n in range(NR):
                rs = cv_ref[q % NCV + zc, 36, n:n + 1, :]
                big_ref[pl.ds(8 + n + zc, 1), :, ls] = _pack(cv_ref[q % NCV + zc, 12 * n:12 * n + 12].reshape(C, 128) * rs)
            yield None

        x_copy(0, S0).wait()
        nxt = lambda sl: jnp.where(sl == NB2 - 1, 0, sl + 1)

        def body(j, xs):
            z = zs_ref[0]
            xs1 = nxt(xs)
            xs3 = nxt(nxt(xs1))

            @pl.when(j + 1 < NG2)
            def _():
                x_copy(j + 1, xs1).wait()

            @pl.when(j >= 2)
            def _():
                o_copy(j - 2, xs3, 0, G2).wait()

            @pl.when(j + 3 < NG2)
            def _():
                x_copy(j + 3, xs3).start()

            units = [conv_unit(q, z, zs_ref[2 + q], zs_ref[1]) for q in range(NQ)]
            for u in units:
                next(u)
            s1(xs1, z)
            zv = zv_ref[0:8, :]
            cnt = [0, 0]
            tails = []
            toks = [None]

            def run_pieces(rel):
                tgt = sum(PLAN[:cnt[0] + 1])
                cnt[0] += 1
                res = None
                while cnt[1] < tgt:
                    u = units[cnt[1] // 12]
                    val = u.send(rel)
                    res = val if res is None else res | val
                    cnt[1] += 1
                    if cnt[1] % 12 == 0:
                        tails.append([TLAG, u])
                        tails.append([TLAG + TLAG2, u])
                for t in list(tails):
                    if t[0] == 0:
                        t[1].send(None)
                        tails.remove(t)
                    t[0] -= 1
                return res

            def gate(d):
                if toks[-1] is None:
                    return d
                mr = d.shape[0]
                du = pltpu.bitcast(d[mr - 8:mr, 384:512], u32) | (toks[-1] & zv)
                last = jnp.concatenate([d[mr - 8:mr, 0:384], pltpu.bitcast(du, f32)], axis=1)
                return jnp.concatenate([d[0:mr - 8], last], axis=0)

            def fin(k, hr):
                for mc in range(2):
                    rs_ = slice(48 * mc, 48 * (mc + 1))
                    o = None
                    for kt in range(3):
                        d = jnp.dot(pltpu.bitcast(w2s_ref[24 * mc:24 * (mc + 1), 128 * kt:128 * kt + 128], bf16),
                                    pltpu.bitcast(hr(kt), bf16), preferred_element_type=f32)
                        rel = pltpu.bitcast(d[0:8, 0:128], u32) & zv
                        d = gate(d)
                        o = d if o is None else o + d
                        if kt == 2:
                            xbuf[xs, k, rs_, :] = (o + _tile4(bias_ref[rs_, :]) + xbuf[xs, k, rs_, :].astype(f32)).astype(bf16)
                        toks.append(run_pieces(rel))

            def ht_rows(n, kt):
                return jnp.concatenate([big_ref[4 * (n % 2) + z + r // 48, r % 48:r % 48 + 8, :]
                                        for r in range(64 * kt, 64 * kt + 64, 8)], axis=0)

            def mm1(n):
                xn = pltpu.bitcast(big_ref[8 + n + z], bf16)
                lhs = pltpu.bitcast(w1q_ref[...], bf16)
                big_ref[pl.ds(4 * (n % 2) + z, 4)] = _pack(_gelu2(jnp.dot(lhs, xn, preferred_element_type=f32)), 4)

            for tok in P2ORD.split(','):
                n = int(tok[1])
                if tok[0] == 'M': mm1(n)
                elif tok[0] == 'S': fin(ST[n], lambda kt: h_ref[_hslot(j) + n, 64 * kt:64 * kt + 64, :])
                elif tok[0] == 'F': fin(RC[n], functools.partial(ht_rows, n))
                elif tok[0] == 'o': o_copy(j, xs, n, int(tok[2]) - n).start()
            assert cnt[1] == 48
            for t in tails:
                t[1].send(None)
            return xs1

        with jax.named_scope('loop2'):
            lax.fori_loop(0, NG2, body, jnp.int32(S0))
        for j in range(NG2 - 2, NG2):
            o_copy(j, (j + S0) % NB2, 0, G2).wait()

    pl.run_scoped(lambda: phase2())


@jax.jit
def pallas_standalone__modern_conv_block_convnext_v2__vision_kernel(x, dw, w1, w2, grn_gamma, grn_beta):
    xt = jnp.transpose(x, (0, 1, 3, 2)).reshape(H, C, W)
    x5 = xt.reshape(H // 2, 2, C // 8, 8, W)
    w2t = w2.T
    out = pl.pallas_call(
        _kernel,
        in_specs=[pl.BlockSpec(memory_space=pl.ANY)] * 7,
        out_specs=pl.BlockSpec(memory_space=pl.ANY),
        out_shape=jax.ShapeDtypeStruct((H, C, W), bf16),
        scratch_shapes=[
            pltpu.VMEM(((NG2 - HCUT) * NST, E // 2, W), u32),
            pltpu.VMEM((NB2, G2, C, W), bf16),
            pltpu.VMEM((8 + NR, C // 2, W), u32),
            pltpu.VMEM((1, NVR, 8, 128), u32),
            pltpu.VMEM((1, 12, 9, 8, 128), f32),
            pltpu.VMEM((NCV, 40, 8, 128), f32),
            pltpu.VMEM((E // 2, C), u32),
            pltpu.VMEM((C // 2, E), u32),
            pltpu.VMEM((C, 128), f32),
            pltpu.VMEM((8, 128), u32),
            pltpu.VMEM((3, 3, C), bf16),
            pltpu.VMEM((3, 3, C), bf16),
            pltpu.VMEM((E,), bf16),
            pltpu.VMEM((E,), bf16),
            pltpu.SMEM((8,), i32),
            pltpu.SemaphoreType.DMA((NB2,)),
            pltpu.SemaphoreType.DMA((NB2,)),
            pltpu.SemaphoreType.DMA((2,)),
            pltpu.SemaphoreType.DMA((6,)),
        ],
        compiler_params=pltpu.CompilerParams(vmem_limit_bytes=128 * 1024 * 1024,
                                             disable_bounds_checks=True),
    )(xt, x5, dw, w1, w2t, grn_gamma, grn_beta)
    return jnp.transpose(out.reshape(1, H, C, W), (0, 1, 3, 2))
```

```python
import functools
import math
import jax
import jax.numpy as jnp
from jax import lax
import jax.experimental.pallas as pl
import jax.experimental.pallas.tpu as pltpu

H = 512; W = 512; C = 96; E = 384
G = 16
NG = H // G
G2 = 8
NG2 = H // G2
RC = (2, 3, 4)
ST = tuple(k for k in range(G2) if k not in RC)
NST = len(ST)
NR = len(RC)
NU = 2
NQ = W // 128
NVR = NQ * 6 * 3 * (NR + 2)
ACC0 = NU * 12 * NQ * 3
CL0 = ACC0 + E // 8
NB2 = 5
S0 = 4
LN_LAG = 5
NSUB = 6
P2ORD = 'M0,M1,F0,M2,S0,F1,S1,o04,F2,S2,o46,S3,S4,o68'
PLAN = [int(c) for c in ('22' + '1' * 44 + '00')]
GSET = [int(c) for c in '2,5,8,11,14'.split(',')]
TLAG = 0
TLAG2 = 0
NCV = 1
PU = 12
CFIRST = 0
PFAT = 3
HCUT = 0

_C1 = math.sqrt(2.0 / math.pi)
_C3 = _C1 * 0.044715
_A = _C3 ** (1.0 / 3.0)
_K = _C1 / _A
_GS = 0.5 / _A

f32 = jnp.float32
bf16 = jnp.bfloat16
u32 = jnp.uint32
i32 = jnp.int32


def _iota(shape, d):
    return lax.broadcasted_iota(i32, shape, d)


def _tile4(a):
    return jnp.concatenate([a] * NQ, axis=1)


def _pack(y, n=1):
    return pltpu.bitcast(y.reshape(n, y.shape[0] // n, y.shape[1]).astype(bf16), u32)


def _gelu2(y):
    u = y * (y * y + _K)
    t = jnp.tanh(u)
    return y * t + y


def _tree_sum(xs):
    xs = list(xs)
    while len(xs) > 1:
        xs = [xs[i] + xs[i + 1] for i in range(0, len(xs) - 1, 2)] + ([xs[-1]] if len(xs) % 2 else [])
    return xs[0]


def _hslot(j):
    return (j % (NG2 - HCUT) if HCUT else j) * NST


def _merge(a, b, msk, sh):
    return jnp.where(msk, a, b) + pltpu.roll(jnp.where(msk, b, a), 8 - sh, 0)


def _kernel(x_hbm, x5_hbm, dw_hbm, w1_hbm, w2t_hbm, g_hbm, b_hbm, o_hbm,
            h_ref, xbuf, big_ref, vr_ref, dwb_ref, cv_ref, w1q_ref, w2s_ref, bias_ref, zs_ref,
            xsem, osem, psem, wsem):

    for i in range(8):
        zs_ref[i] = 0

    def x_copy(j, sl):
        return pltpu.make_async_copy(x_hbm.at[pl.ds(j * G2, G2)], xbuf.at[sl], xsem.at[sl])

    def phase1(gb_ref):
        xn_ref = big_ref
        vi = lambda u, g, q, v: ((u * 12 + g) * NQ + q) * 3 + v
        xp = xbuf.reshape(NB2 * G2 // 2, C // 8, 16, W)
        NP2 = G // 2

        def row_copy(u, half, slot, i):
            return pltpu.make_async_copy(x5_hbm.at[u - 1 + half, 1 - half],
                                         xp.at[NP2 * slot + i, :, pl.ds(8 * half, 8), :], psem.at[slot])

        def rows_copy(u, n, half, slot, i):
            return pltpu.make_async_copy(x5_hbm.at[pl.ds(u - 1 + half, n), 1 - half],
                                         xp.at[pl.ds(NP2 * slot + i, n), :, pl.ds(8 * half, 8), :], psem.at[slot])

        def start_rows(j, inner):
            for i in range(NP2):
                for half in range(2):
                    if (i < NP2 - 2 - half) == inner:
                        row_copy(NP2 * j + 3 + i, half, j & 1, i).start()

        def wait_rows(slot, last):
            if last:
                bufs = [xbuf.at[2 * slot], xbuf.at[2 * slot + 1, pl.ds(0, G - 5 - G2)]]
            else:
                bufs = [xbuf.at[pl.ds(2 * slot, 2)]]
            for buf in bufs:
                pltpu.make_async_copy(buf, buf, psem.at[slot]).wait()

        lane = _iota((8, 128), 1)

        def s1(xu_ref, u, kill=None):
            zz = jnp.zeros((8, 128), u32)
            for g in range(12):
                m = pltpu.bitcast(xu_ref[g], u32)
                if kill is not None:
                    m = jnp.where(kill, jnp.zeros_like(m), m)
                mq = [m[:, 128 * q:128 * q + 128] for q in range(NQ)]
                for q in range(NQ):
                    lq = jnp.where(lane == 127, mq[q - 1] if q > 0 else zz, mq[q])
                    rq = jnp.where(lane == 0, mq[q + 1] if q + 1 < NQ else zz, mq[q])
                    vr_ref[0, vi(u, g, q, 0)] = pltpu.roll(lq, 1, 1)
                    vr_ref[0, vi(u, g, q, 1)] = mq[q]
                    vr_ref[0, vi(u, g, q, 2)] = pltpu.roll(rq, 127, 1)

        def conv_round(t, q, gs):
            cvs = []
            for g in gs:
                rhs = jnp.concatenate([vr_ref[0, vi(uu & 1, g, q, v)] for uu in (t, t + 1) for v in range(3)], axis=0)
                lhs = pltpu.bitcast(vr_ref[0, CL0 + g, :, 0:C], bf16)
                cvs.append(jnp.dot(lhs, pltpu.bitcast(rhs, bf16), preferred_element_type=f32))
            return cvs

        sub = _iota((8, 128), 0)
        m0 = sub % 2 == 0
        m1 = (sub // 2) % 2 == 0
        lnc = jnp.where(m1, 1.0 / (C * _A), 1.0 / (C * _A * _A))

        merge = _merge

        def ln_tile(cvs, q, dsts, dsts2=None):
            ls = slice(128 * q, 128 * q + 128)
            cs = [[cv[8 * ab:8 * ab + 8] for cv in cvs] for ab in range(2)]
            c1 = merge(_tree_sum(cs[0]), _tree_sum(cs[1]), m0, 1)
            c2 = merge(_tree_sum([c * c for c in cs[0]]), _tree_sum([c * c for c in cs[1]]), m0, 1)
            e = merge(c1, c2, m1, 2)
            f = (e + pltpu.roll(e, 4, 0)) * lnc
            v = pltpu.roll(f, 6, 0) - f * f
            rs = lax.rsqrt(jnp.maximum(v, 0.0) + 1e-5 / (_A * _A))
            for ab in range(2):
                xn = _pack(jnp.concatenate(cs[ab], axis=0) * rs[ab:ab + 1, :])
                xn_ref[pl.ds(dsts[ab], 1), :, ls] = xn
                if dsts2 is not None:
                    xn_ref[pl.ds(dsts2[ab], 1), :, ls] = xn

        def setup(dw_ref, g_ref, b_ref):
            w1_ref = xbuf.at[4, 0, :, pl.ds(0, E)]
            w2t_ref = xbuf.at[4, 1, :, pl.ds(0, E)]
            small = [pltpu.make_async_copy(a, b, wsem.at[i]) for i, (a, b) in enumerate(
                [(dw_hbm, dw_ref), (w1_hbm, w1_ref), (w2t_hbm, w2t_ref), (g_hbm, g_ref), (b_hbm, b_ref)])]
            for cp in small[:2]:
                cp.start()
            rows_copy(1, 3, 0, 1, 1).start()
            rows_copy(0, 4, 1, 1, 0).start()
            for cp in small[2:]:
                cp.start()
            rows_copy(3, NP2, 0, 0, 0).start()
            rows_copy(3, NP2, 1, 0, 0).start()
            small[0].wait()

            vr_ref[0, ACC0:CL0] = jnp.zeros((E // 8, 8, 128), u32)
            dw = dw_ref[...].astype(f32)
            dif = _iota((8, C), 1) - _iota((8, C), 0)
            R = _iota((16, C), 0); KK = _iota((16, C), 1)
            unit = jnp.where(KK >= 48, 1, 0)
            itap = 2 * unit + ((KK >> 3) & 1) - (R >> 3)
            tapid = jnp.where((KK & 7) == (R & 7), 3 * itap + ((KK - 48 * unit) >> 4), -9)

            def prep_dw(g, c):
                cl = jnp.zeros((16, C), f32)
                for t in range(9):
                    row = jnp.broadcast_to(dw[t // 3, t % 3:t % 3 + 1, :], (8, C))
                    col = jnp.sum(jnp.where(dif == 8 * g, row, 0.0), axis=1, keepdims=True)
                    dwb_ref[0, g, t] = jnp.broadcast_to(col, (8, 128))
                    cb = jnp.broadcast_to(col, (8, C))
                    cl = jnp.where(tapid == t, jnp.concatenate([cb, cb], axis=0), cl)
                vr_ref[0, CL0 + g, :, 0:C] = pltpu.bitcast(cl.astype(bf16), u32)
                return c
            lax.fori_loop(0, 12, prep_dw, 0, unroll=PU)

            for cp in small[1:]:
                cp.wait()
            w1f = w1_ref[...].astype(f32)
            w1k = (w1f - jnp.sum(w1f, axis=0, keepdims=True) * (1.0 / C)).astype(bf16)
            for i in range(3):
                Pb = jnp.where(_iota((128, E), 0) + 128 * i == _iota((128, E), 1), 1.0, 0.0).astype(bf16)
                w1q = lax.dot_general(Pb, w1k, (((1,), (1,)), ((), ())), preferred_element_type=f32)
                w1q_ref[64 * i:64 * i + 64, :] = pltpu.bitcast(w1q.astype(bf16), u32)
            w2s_ref[...] = pltpu.bitcast(w2t_ref[...], u32)
            gb_ref[0:1, :] = g_ref[...].astype(f32).reshape(1, E)
            gb_ref[1:2, :] = b_ref[...].astype(f32).reshape(1, E)

            xp[8, :, 0:8, :] = jnp.zeros((12, 8, W), bf16)
            rows_copy(1, 3, 0, 1, 1).wait()
            rows_copy(0, 4, 1, 1, 0).wait()
            s1(xp.at[10], 0)
            s1(xp.at[11], 1)
            for i, (un, da, db) in enumerate([(1, 10, 5), (0, 8, 9), (2, 0, 1)]):
                for q in range(NQ):
                    ln_tile(conv_round(2 - i, q, range(12)), q, (da, db), (2, 3) if i == 1 and q < 2 else None)
                s1(xp.at[8 + un], un & 1)

        pl.run_scoped(setup, pltpu.VMEM((3, 3, C), bf16), pltpu.VMEM((E,), bf16), pltpu.VMEM((E,), bf16))

        NP = 2 * NSUB
        RPP = 12 // NP
        MR = E // NSUB

        def body(j, carry):
            z = zs_ref[0]
            z1 = zs_ref[1]
            slot = j & 1

            @pl.when(j < NG - 1)
            def _():
                wait_rows(slot, False)

            @pl.when(j == NG - 1)
            def _():
                wait_rows(slot, True)

            def prefetch():
                @pl.when(j < NG - 1)
                def _():
                    start_rows(j + 1, True)

                @pl.when(j < NG - 2)
                def _():
                    start_rows(j + 1, False)

                @pl.when(j == NG - 1)
                def _():
                    for jn in range(3):
                        x_copy(jn, (S0 + jn) % NB2).start()

            pend = []
            cur = []
            for p in range(NP2):
                for r in range(NP):
                    gr = p * NP + r
                    ab, c = r // NSUB, r % NSUB
                    k = 2 * p + ab
                    def mm_part():
                        while pend and pend[0][0] <= gr:
                            ln_tile(*pend.pop(0)[1:])
                        xn = pltpu.bitcast(xn_ref[k % 8 + z], bf16)
                        lhs = pltpu.bitcast(w1q_ref[MR // 2 * c:MR // 2 * (c + 1), :], bf16)
                        gl = _gelu2(jnp.dot(lhs, xn, preferred_element_type=f32))
                        sq = gl * gl
                        s4 = (sq[:, 0:128] + sq[:, 128:256]) + (sq[:, 256:384] + sq[:, 384:512])
                        for i in range(MR // 8):
                            ai = ACC0 + MR // 8 * c + i
                            vr_ref[0, ai] = pltpu.bitcast(pltpu.bitcast(vr_ref[0, ai], f32) + s4[8 * i:8 * i + 8], u32)
                        if k % G2 in ST:
                            h_ref[pl.ds(_hslot(2 * j + k // G2) + ST.index(k % G2), 1), MR // 2 * c:MR // 2 * (c + 1), :] = _pack(gl)
                    def cv_part():
                        nonlocal cur
                        for rr in range(r * RPP, (r + 1) * RPP):
                            q = (rr // 3 + 2) % 4
                            pair = p + 1 + (rr >= 6)
                            cur += conv_round(pair, q, range(4 * (rr % 3), 4 * (rr % 3) + 4))
                            if rr % 3 == 2:
                                pend.append((gr + LN_LAG, cur, q,
                                             (2 * pair % 8 + z1, (2 * pair + 1) % 8 + z1)))
                                cur = []
                    if gr == PFAT:
                        prefetch()
                    if CFIRST:
                        cv_part(); mm_part()
                    else:
                        mm_part(); cv_part()
                    if r == NP // 2 - 1:
                        kill = None
                        if p == NP2 - 3:
                            kill = _iota((8, W), 0) >= jnp.where(j == NG - 1, 4, 8)
                        s1(xp.at[8 * slot + p], (p + 3) % NU, kill)
            for e in pend:
                ln_tile(*e[1:])
            return carry

        with jax.named_scope('loop1'):
            lax.fori_loop(0, NG, body, 0)

        pdif = _iota((8, E), 1) - _iota((8, E), 0) + zs_ref[0]
        parts = []
        for i in range(E // 8):
            col = jnp.sum(pltpu.bitcast(vr_ref[0, ACC0 + i], f32), axis=1, keepdims=True)
            parts.append(jnp.where(pdif == 8 * i, jnp.broadcast_to(col, (8, E)), 0.0))
        ss = jnp.sum(_tree_sum(parts), axis=0, keepdims=True) * (_GS * _GS)
        gx = jnp.sqrt(ss + 1e-6)
        nx = gx / (jnp.sum(gx, axis=1, keepdims=True) * (1.0 / E) + 1e-6)
        gam = gb_ref[0:1, :]
        bet = gb_ref[1:2, :]
        s = (gam * nx + 1.0) * _GS
        w2t = pltpu.bitcast(w2s_ref[...], bf16).astype(f32)
        w2s_ref[...] = pltpu.bitcast((w2t * s).astype(bf16), u32)
        bias_ref[...] = jnp.broadcast_to(jnp.sum(w2t * bet, axis=1, keepdims=True), (C, 128))

    pl.run_scoped(phase1, pltpu.VMEM((8, E), f32))

    def phase2(zv_ref):
        zv_ref[...] = jnp.zeros(zv_ref.shape, u32)
        vi = lambda q, k, i: (q * 6 + k) * 3 * (NR + 2) + i
        R0 = RC[0] - 1

        def o_copy(j, sl, r0, n):
            return pltpu.make_async_copy(xbuf.at[sl, pl.ds(r0, n)], o_hbm.at[pl.ds(j * G2 + r0, n)], osem.at[sl])

        z0 = zs_ref[0]
        lane = _iota((8, 128), 1) + z0
        sub = _iota((8, 128), 0) + z0
        m0 = (sub & 1) == 0
        m1 = (sub & 2) == 0
        m2 = sub < 4
        lnc = jnp.where(m2, 1.0 / (C * _A), 1.0 / (C * _A * _A))

        def s1(xs, zv):
            zz = jnp.zeros((8, 128), u32)
            for r in range(NR + 2):
                for k in range(6):
                    m = pltpu.bitcast(xbuf[xs, R0 + r, 16 * k:16 * k + 16, :], u32)
                    mq = [m[:, 128 * q:128 * q + 128] for q in range(NQ)]
                    for q in range(NQ):
                        lq = jnp.where(lane == 127, mq[q - 1] if q > 0 else zz, mq[q])
                        rq = jnp.where(lane == 0, mq[q + 1] if q + 1 < NQ else zz, mq[q])
                        vr_ref[zv, vi(q, k, 3 * r)] = pltpu.roll(lq, 1, 1)
                        vr_ref[zv, vi(q, k, 3 * r + 1)] = mq[q]
                        vr_ref[zv, vi(q, k, 3 * r + 2)] = pltpu.roll(rq, 127, 1)

        def conv_unit(q, zc, zw, zr):
            ls = slice(128 * q, 128 * q + 128)
            st = [None] * NR
            tok = yield None
            for g in range(12):
                w = [dwb_ref[zw, g, t] for t in range(9)]
                acc = [None] * NR
                for r in range(NR + 2):
                    for v in range(3):
                        x = vr_ref[zw, vi(q, g // 2, 3 * r + v)]
                        if tok is not None and 3 * r + v in GSET:
                            x = x | tok
                        xf = pltpu.bitcast(x, bf16).astype(f32)[8 * (g % 2):8 * (g % 2) + 8]
                        for n in range(NR):
                            if 0 <= r - n <= 2:
                                t = xf * w[3 * (r - n) + v]
                                acc[n] = t if acc[n] is None else acc[n] + t
                for n in range(NR):
                    cv = acc[n]
                    st[n] = (cv, cv * cv) if st[n] is None else (st[n][0] + cv, st[n][1] + cv * cv)
                    cv_ref[q % NCV + zc, 12 * n + g] = cv
                tok = yield pltpu.bitcast((st[0][1] + st[1][1]) + st[2][1], u32)
            half = lambda i: _merge(_merge(st[0][i], st[1][i], m0, 1), st[2][i] + pltpu.roll(st[2][i], 7, 0), m1, 2)
            f = _merge(half(0), half(1), m2, 4) * lnc
            v = pltpu.roll(f, 4, 0) - f * f
            cv_ref[q % NCV + zr, 36] = lax.rsqrt(jnp.maximum(v, 0.0) + 1e-5 / (_A * _A))
            yield None
            for n in range(NR):
                rs = cv_ref[q % NCV + zc, 36, n:n + 1, :]
                big_ref[pl.ds(8 + n + zc, 1), :, ls] = _pack(cv_ref[q % NCV + zc, 12 * n:12 * n + 12].reshape(C, 128) * rs)
            yield None

        x_copy(0, S0).wait()
        nxt = lambda sl: jnp.where(sl == NB2 - 1, 0, sl + 1)

        def body(j, xs):
            z = zs_ref[0]
            xs1 = nxt(xs)
            xs3 = nxt(nxt(xs1))

            @pl.when(j + 1 < NG2)
            def _():
                x_copy(j + 1, xs1).wait()

            @pl.when(j >= 2)
            def _():
                o_copy(j - 2, xs3, 0, G2).wait()

            @pl.when(j + 3 < NG2)
            def _():
                x_copy(j + 3, xs3).start()

            units = [conv_unit(q, z, zs_ref[2 + q], zs_ref[1]) for q in range(NQ)]
            for u in units:
                next(u)
            s1(xs1, z)
            zv = zv_ref[0:8, :]
            cnt = [0, 0]
            tails = []
            toks = [None]

            def run_pieces(rel):
                tgt = sum(PLAN[:cnt[0] + 1])
                cnt[0] += 1
                res = None
                while cnt[1] < tgt:
                    u = units[cnt[1] // 12]
                    val = u.send(rel)
                    res = val if res is None else res | val
                    cnt[1] += 1
                    if cnt[1] % 12 == 0:
                        tails.append([TLAG, u])
                        tails.append([TLAG + TLAG2, u])
                for t in list(tails):
                    if t[0] == 0:
                        t[1].send(None)
                        tails.remove(t)
                    t[0] -= 1
                return res

            def gate(d):
                if toks[-1] is None:
                    return d
                mr = d.shape[0]
                du = pltpu.bitcast(d[mr - 8:mr, 384:512], u32) | (toks[-1] & zv)
                last = jnp.concatenate([d[mr - 8:mr, 0:384], pltpu.bitcast(du, f32)], axis=1)
                return jnp.concatenate([d[0:mr - 8], last], axis=0)

            def fin(k, hr):
                for mc in range(2):
                    rs_ = slice(48 * mc, 48 * (mc + 1))
                    o = None
                    for kt in range(3):
                        d = jnp.dot(pltpu.bitcast(w2s_ref[24 * mc:24 * (mc + 1), 128 * kt:128 * kt + 128], bf16),
                                    pltpu.bitcast(hr(kt), bf16), preferred_element_type=f32)
                        rel = pltpu.bitcast(d[0:8, 0:128], u32) & zv
                        d = gate(d)
                        o = d if o is None else o + d
                        if kt == 2:
                            xbuf[xs, k, rs_, :] = (o + _tile4(bias_ref[rs_, :]) + xbuf[xs, k, rs_, :].astype(f32)).astype(bf16)
                        toks.append(run_pieces(rel))

            def ht_rows(n, kt):
                return jnp.concatenate([big_ref[4 * (n % 2) + z + r // 48, r % 48:r % 48 + 8, :]
                                        for r in range(64 * kt, 64 * kt + 64, 8)], axis=0)

            def mm1(n):
                xn = pltpu.bitcast(big_ref[8 + n + z], bf16)
                lhs = pltpu.bitcast(w1q_ref[...], bf16)
                big_ref[pl.ds(4 * (n % 2) + z, 4)] = _pack(_gelu2(jnp.dot(lhs, xn, preferred_element_type=f32)), 4)

            for tok in P2ORD.split(','):
                n = int(tok[1])
                if tok[0] == 'M': mm1(n)
                elif tok[0] == 'S': fin(ST[n], lambda kt: h_ref[_hslot(j) + n, 64 * kt:64 * kt + 64, :])
                elif tok[0] == 'F': fin(RC[n], functools.partial(ht_rows, n))
                elif tok[0] == 'o': o_copy(j, xs, n, int(tok[2]) - n).start()
            assert cnt[1] == 48
            for t in tails:
                t[1].send(None)
            return xs1

        with jax.named_scope('loop2'):
            lax.fori_loop(0, NG2, body, jnp.int32(S0))
        for j in range(NG2 - 2, NG2):
            o_copy(j, (j + S0) % NB2, 0, G2).wait()

    pl.run_scoped(phase2, pltpu.VMEM((8, 128), u32))


@jax.jit
def pallas_standalone__modern_conv_block_convnext_v2__vision_kernel(x, dw, w1, w2, grn_gamma, grn_beta):
    xt = jnp.transpose(x, (0, 1, 3, 2)).reshape(H, C, W)
    x5 = xt.reshape(H // 2, 2, C // 8, 8, W)
    w2t = w2.T
    out = pl.pallas_call(
        _kernel,
        in_specs=[pl.BlockSpec(memory_space=pl.ANY)] * 7,
        out_specs=pl.BlockSpec(memory_space=pl.ANY),
        out_shape=jax.ShapeDtypeStruct((H, C, W), bf16),
        scratch_shapes=[
            pltpu.VMEM(((NG2 - HCUT) * NST, E // 2, W), u32),
            pltpu.VMEM((NB2, G2, C, W), bf16),
            pltpu.VMEM((8 + NR, C // 2, W), u32),
            pltpu.VMEM((1, NVR, 8, 128), u32),
            pltpu.VMEM((1, 12, 9, 8, 128), f32),
            pltpu.VMEM((NCV, 40, 8, 128), f32),
            pltpu.VMEM((E // 2, C), u32),
            pltpu.VMEM((C // 2, E), u32),
            pltpu.VMEM((C, 128), f32),
            pltpu.SMEM((8,), i32),
            pltpu.SemaphoreType.DMA((NB2,)),
            pltpu.SemaphoreType.DMA((NB2,)),
            pltpu.SemaphoreType.DMA((2,)),
            pltpu.SemaphoreType.DMA((5,)),
        ],
        compiler_params=pltpu.CompilerParams(vmem_limit_bytes=128 * 1024 * 1024,
                                             disable_bounds_checks=True),
    )(xt, x5, dw, w1, w2t, grn_gamma, grn_beta)
    return jnp.transpose(out.reshape(1, H, C, W), (0, 1, 3, 2))
```

```python
import functools
import math

import jax
import jax.numpy as jnp
from jax import lax
import jax.experimental.pallas as pl
import jax.experimental.pallas.tpu as pltpu

H, W, C, E = 512, 512, 96, 384
NQ = W // 128
G = 16
NG = H // G
NP2 = G // 2
G2 = 8
NG2 = H // G2
RC = (2, 3, 4)
ST = tuple(k for k in range(G2) if k not in RC)
NST = len(ST)
NR = len(RC)
NVR = NQ * 6 * 3 * (NR + 2)
ACC0 = 2 * 12 * NQ * 3
CL0 = ACC0 + E // 8
NB = 5
S0 = 4
NSUB = 6
MR = E // NSUB
NP = 2 * NSUB
LN_LAG = 5
P2ORD = 'M0,M1,F0,M2,S0,F1,S1,o04,F2,S2,o46,S3,S4,o68'.split(',')
PLAN = [2, 2] + [1] * 44 + [0, 0]

_C1 = math.sqrt(2.0 / math.pi)
_A = (_C1 * 0.044715) ** (1.0 / 3.0)
_K = _C1 / _A
_GS = 0.5 / _A
_EPS = 1e-5 / (_A * _A)

f32 = jnp.float32
bf16 = jnp.bfloat16
u32 = jnp.uint32
i32 = jnp.int32


def _iota(shape, d):
    return lax.broadcasted_iota(i32, shape, d)


def _pack(y, n=1):
    return pltpu.bitcast(y.reshape(n, y.shape[0] // n, y.shape[1]).astype(bf16), u32)


def _gelu2(y):
    u = y * (y * y + _K)
    t = jnp.tanh(u)
    return y * t + y


def _tree_sum(xs):
    xs = list(xs)
    while len(xs) > 1:
        xs = [xs[i] + xs[i + 1] for i in range(0, len(xs) - 1, 2)] + ([xs[-1]] if len(xs) % 2 else [])
    return xs[0]


def _merge(a, b, msk, sh):
    return jnp.where(msk, a, b) + pltpu.roll(jnp.where(msk, b, a), 8 - sh, 0)


def _shifted(m, lane):
    zz = jnp.zeros((8, 128), u32)
    mq = [m[:, 128 * q:128 * q + 128] for q in range(NQ)]
    for q in range(NQ):
        lq = jnp.where(lane == 127, mq[q - 1] if q > 0 else zz, mq[q])
        rq = jnp.where(lane == 0, mq[q + 1] if q + 1 < NQ else zz, mq[q])
        yield q, (pltpu.roll(lq, 1, 1), mq[q], pltpu.roll(rq, 127, 1))


def _kernel(x_hbm, x5_hbm, dw_hbm, w1_hbm, w2t_hbm, g_hbm, b_hbm, o_hbm,
            h_ref, xbuf, big_ref, vr_ref, dwb_ref, cv_ref, w1t_ref, w2s_ref, bias_ref, zs_ref,
            xsem, osem, psem, wsem):

    for i in range(6):
        zs_ref[i] = 0

    def x_copy(j, sl):
        return pltpu.make_async_copy(x_hbm.at[pl.ds(j * G2, G2)], xbuf.at[sl], xsem.at[sl])

    def phase1(gb_ref):
        xn_ref = big_ref
        vi = lambda u, g, q, v: ((u * 12 + g) * NQ + q) * 3 + v
        xp = xbuf.reshape(NB * G2 // 2, C // 8, 16, W)

        def row_copy(u, half, slot, i):
            return pltpu.make_async_copy(x5_hbm.at[u - 1 + half, 1 - half],
                                         xp.at[NP2 * slot + i, :, pl.ds(8 * half, 8), :], psem.at[slot])

        def rows_copy(u, n, half, slot, i):
            return pltpu.make_async_copy(x5_hbm.at[pl.ds(u - 1 + half, n), 1 - half],
                                         xp.at[pl.ds(NP2 * slot + i, n), :, pl.ds(8 * half, 8), :], psem.at[slot])

        def start_rows(j, inner):
            for i in range(NP2):
                for half in range(2):
                    if (i < NP2 - 2 - half) == inner:
                        row_copy(NP2 * j + 3 + i, half, j & 1, i).start()

        def wait_units(slot, n):
            buf = xp.at[pl.ds(NP2 * slot, n)]
            pltpu.make_async_copy(buf, buf, psem.at[slot]).wait()

        lane = _iota((8, 128), 1)

        def shift_unit(xu_ref, u):
            for g in range(12):
                for q, vs in _shifted(pltpu.bitcast(xu_ref[g], u32), lane):
                    for v in range(3):
                        vr_ref[0, vi(u, g, q, v)] = vs[v]

        def conv_round(t, q, gs):
            cvs = []
            for g in gs:
                rhs = jnp.concatenate([vr_ref[0, vi(uu & 1, g, q, v)] for uu in (t, t + 1) for v in range(3)], axis=0)
                lhs = pltpu.bitcast(vr_ref[0, CL0 + g, :, 0:C], bf16)
                cvs.append(jnp.dot(lhs, pltpu.bitcast(rhs, bf16), preferred_element_type=f32))
            return cvs

        sub = _iota((8, 128), 0)
        m0 = sub % 2 == 0
        m1 = (sub // 2) % 2 == 0
        lnc = jnp.where(m1, 1.0 / (C * _A), 1.0 / (C * _A * _A))

        def ln_tile(cvs, q, dsts, dsts2=None):
            ls = slice(128 * q, 128 * q + 128)
            cs = [[cv[8 * ab:8 * ab + 8] for cv in cvs] for ab in range(2)]
            c1 = _merge(_tree_sum(cs[0]), _tree_sum(cs[1]), m0, 1)
            c2 = _merge(_tree_sum([c * c for c in cs[0]]), _tree_sum([c * c for c in cs[1]]), m0, 1)
            e = _merge(c1, c2, m1, 2)
            f = (e + pltpu.roll(e, 4, 0)) * lnc
            v = pltpu.roll(f, 6, 0) - f * f
            rs = lax.rsqrt(jnp.maximum(v, 0.0) + _EPS)
            for ab in range(2):
                xn = _pack(jnp.concatenate(cs[ab], axis=0) * rs[ab:ab + 1, :])
                xn_ref[pl.ds(dsts[ab], 1), :, ls] = xn
                if dsts2 is not None:
                    xn_ref[pl.ds(dsts2[ab], 1), :, ls] = xn

        def setup(dw_ref, g_ref, b_ref):
            w1_ref = xbuf.at[4, 0, :, pl.ds(0, E)]
            w2t_ref = xbuf.at[4, 1, :, pl.ds(0, E)]
            small = [pltpu.make_async_copy(a, b, wsem.at[i]) for i, (a, b) in enumerate(
                [(dw_hbm, dw_ref), (w1_hbm, w1_ref), (w2t_hbm, w2t_ref), (g_hbm, g_ref), (b_hbm, b_ref)])]
            for cp in small[:2]:
                cp.start()
            rows_copy(1, 3, 0, 1, 1).start()
            rows_copy(0, 4, 1, 1, 0).start()
            for cp in small[2:]:
                cp.start()
            rows_copy(3, NP2, 0, 0, 0).start()
            rows_copy(3, NP2, 1, 0, 0).start()
            small[0].wait()

            vr_ref[0, ACC0:CL0] = jnp.zeros((E // 8, 8, 128), u32)
            dw = dw_ref[...].astype(f32)
            dif = _iota((8, C), 1) - _iota((8, C), 0)
            row = _iota((16, C), 0)
            col = _iota((16, C), 1)
            unit = jnp.where(col >= 48, 1, 0)
            itap = 2 * unit + ((col >> 3) & 1) - (row >> 3)
            tapid = jnp.where((col & 7) == (row & 7), 3 * itap + ((col - 48 * unit) >> 4), -9)
            for g in range(12):
                cl = jnp.zeros((16, C), f32)
                for t in range(9):
                    dwt = jnp.broadcast_to(dw[t // 3, t % 3:t % 3 + 1, :], (8, C))
                    dwc = jnp.sum(jnp.where(dif == 8 * g, dwt, 0.0), axis=1, keepdims=True)
                    dwb_ref[0, g, t] = jnp.broadcast_to(dwc, (8, 128))
                    cb = jnp.broadcast_to(dwc, (8, C))
                    cl = jnp.where(tapid == t, jnp.concatenate([cb, cb], axis=0), cl)
                vr_ref[0, CL0 + g, :, 0:C] = pltpu.bitcast(cl.astype(bf16), u32)

            for cp in small[1:]:
                cp.wait()
            w1f = w1_ref[...].astype(f32)
            w1c = (w1f - jnp.sum(w1f, axis=0, keepdims=True) * (1.0 / C)).astype(bf16)
            for i in range(3):
                eye = jnp.where(_iota((128, E), 0) + 128 * i == _iota((128, E), 1), 1.0, 0.0).astype(bf16)
                w1t = lax.dot_general(eye, w1c, (((1,), (1,)), ((), ())), preferred_element_type=f32)
                w1t_ref[64 * i:64 * i + 64, :] = pltpu.bitcast(w1t.astype(bf16), u32)
            w2s_ref[...] = pltpu.bitcast(w2t_ref[...], u32)
            gb_ref[0:1, :] = g_ref[...].astype(f32).reshape(1, E)
            gb_ref[1:2, :] = b_ref[...].astype(f32).reshape(1, E)

            xp[8, :, 0:8, :] = jnp.zeros((12, 8, W), bf16)
            xp[17, :, 0:8, :] = jnp.zeros((12, 8, W), bf16)
            rows_copy(1, 3, 0, 1, 1).wait()
            rows_copy(0, 4, 1, 1, 0).wait()
            shift_unit(xp.at[10], 0)
            shift_unit(xp.at[11], 1)
            for i, (un, da, db) in enumerate([(1, 10, 5), (0, 8, 9), (2, 0, 1)]):
                for q in range(NQ):
                    ln_tile(conv_round(2 - i, q, range(12)), q, (da, db), (2, 3) if i == 1 and q < 2 else None)
                shift_unit(xp.at[8 + un], un & 1)

        pl.run_scoped(setup, pltpu.VMEM((3, 3, C), bf16), pltpu.VMEM((E,), bf16), pltpu.VMEM((E,), bf16))

        def body(j, carry):
            z = zs_ref[0]
            z1 = zs_ref[1]
            slot = j & 1

            @pl.when(j < NG - 1)
            def _():
                wait_units(slot, NP2)

            @pl.when(j == NG - 1)
            def _():
                wait_units(slot, NP2 - 2)

            @pl.when(j == NG - 2)
            def _():
                pltpu.make_async_copy(xp.at[17, :, pl.ds(0, 8), :],
                                      xp.at[NP2 * (1 - slot) + NP2 - 3, :, pl.ds(8, 8), :],
                                      psem.at[1 - slot]).start()

            def prefetch():
                @pl.when(j < NG - 1)
                def _():
                    start_rows(j + 1, True)

                @pl.when(j < NG - 2)
                def _():
                    start_rows(j + 1, False)

                @pl.when(j == NG - 1)
                def _():
                    for jn in range(3):
                        x_copy(jn, (S0 + jn) % NB).start()

            pend = []
            cur = []
            for p in range(NP2):
                for r in range(NP):
                    gr = p * NP + r
                    c = r % NSUB
                    k = 2 * p + r // NSUB
                    if gr == 3:
                        prefetch()
                    while pend and pend[0][0] <= gr:
                        ln_tile(*pend.pop(0)[1:])
                    xn = pltpu.bitcast(xn_ref[k % 8 + z], bf16)
                    lhs = pltpu.bitcast(w1t_ref[MR // 2 * c:MR // 2 * (c + 1), :], bf16)
                    gl = _gelu2(jnp.dot(lhs, xn, preferred_element_type=f32))
                    sq = gl * gl
                    s4 = (sq[:, 0:128] + sq[:, 128:256]) + (sq[:, 256:384] + sq[:, 384:512])
                    for i in range(MR // 8):
                        ai = ACC0 + MR // 8 * c + i
                        vr_ref[0, ai] = pltpu.bitcast(pltpu.bitcast(vr_ref[0, ai], f32) + s4[8 * i:8 * i + 8], u32)
                    if k % G2 in ST:
                        hs = (2 * j + k // G2) * NST + ST.index(k % G2)
                        h_ref[pl.ds(hs, 1), MR // 2 * c:MR // 2 * (c + 1), :] = _pack(gl)
                    q = (r // 3 + 2) % 4
                    pair = p + 1 + (r >= 6)
                    cur += conv_round(pair, q, range(4 * (r % 3), 4 * (r % 3) + 4))
                    if r % 3 == 2:
                        pend.append((gr + LN_LAG, cur, q, (2 * pair % 8 + z1, (2 * pair + 1) % 8 + z1)))
                        cur = []
                    if r == NP // 2 - 1:
                        shift_unit(xp.at[8 * slot + p], (p + 3) % 2)
            for e in pend:
                ln_tile(*e[1:])
            return carry

        lax.fori_loop(0, NG, body, 0)

        pdif = _iota((8, E), 1) - _iota((8, E), 0) + zs_ref[0]
        parts = []
        for i in range(E // 8):
            col = jnp.sum(pltpu.bitcast(vr_ref[0, ACC0 + i], f32), axis=1, keepdims=True)
            parts.append(jnp.where(pdif == 8 * i, jnp.broadcast_to(col, (8, E)), 0.0))
        ss = jnp.sum(_tree_sum(parts), axis=0, keepdims=True) * (_GS * _GS)
        gx = jnp.sqrt(ss + 1e-6)
        nx = gx / (jnp.sum(gx, axis=1, keepdims=True) * (1.0 / E) + 1e-6)
        s = (gb_ref[0:1, :] * nx + 1.0) * _GS
        w2t = pltpu.bitcast(w2s_ref[...], bf16).astype(f32)
        w2s_ref[...] = pltpu.bitcast((w2t * s).astype(bf16), u32)
        bias_ref[...] = jnp.broadcast_to(jnp.sum(w2t * gb_ref[1:2, :], axis=1, keepdims=True), (C, 128))

    pl.run_scoped(phase1, pltpu.VMEM((8, E), f32))

    def phase2(zv_ref):
        zv_ref[...] = jnp.zeros(zv_ref.shape, u32)
        vi = lambda q, k, i: (q * 6 + k) * 3 * (NR + 2) + i

        def o_copy(j, sl, r0, n):
            return pltpu.make_async_copy(xbuf.at[sl, pl.ds(r0, n)], o_hbm.at[pl.ds(j * G2 + r0, n)], osem.at[sl])

        z0 = zs_ref[0]
        lane = _iota((8, 128), 1) + z0
        sub = _iota((8, 128), 0) + z0
        m0 = (sub & 1) == 0
        m1 = (sub & 2) == 0
        m2 = sub < 4
        lnc = jnp.where(m2, 1.0 / (C * _A), 1.0 / (C * _A * _A))

        def shift_rows(xs, zv):
            for r in range(NR + 2):
                for k in range(6):
                    m = pltpu.bitcast(xbuf[xs, RC[0] - 1 + r, 16 * k:16 * k + 16, :], u32)
                    for q, vs in _shifted(m, lane):
                        for v in range(3):
                            vr_ref[zv, vi(q, k, 3 * r + v)] = vs[v]

        def conv_tile(q, zc, zw, zr):
            st = [None] * NR
            tok = yield None
            for g in range(12):
                w = [dwb_ref[zw, g, t] for t in range(9)]
                acc = [None] * NR
                for r in range(NR + 2):
                    for v in range(3):
                        x = vr_ref[zw, vi(q, g // 2, 3 * r + v)]
                        if v == 2:
                            x = x | tok
                        xf = pltpu.bitcast(x, bf16).astype(f32)[8 * (g % 2):8 * (g % 2) + 8]
                        for n in range(NR):
                            if 0 <= r - n <= 2:
                                t = xf * w[3 * (r - n) + v]
                                acc[n] = t if acc[n] is None else acc[n] + t
                for n in range(NR):
                    cv = acc[n]
                    st[n] = (cv, cv * cv) if st[n] is None else (st[n][0] + cv, st[n][1] + cv * cv)
                    cv_ref[zc, 12 * n + g] = cv
                tok = yield pltpu.bitcast((st[0][1] + st[1][1]) + st[2][1], u32)
            half = lambda i: _merge(_merge(st[0][i], st[1][i], m0, 1), st[2][i] + pltpu.roll(st[2][i], 7, 0), m1, 2)
            f = _merge(half(0), half(1), m2, 4) * lnc
            v = pltpu.roll(f, 4, 0) - f * f
            cv_ref[zr, 36] = lax.rsqrt(jnp.maximum(v, 0.0) + _EPS)
            for n in range(NR):
                rs = cv_ref[zc, 36, n:n + 1, :]
                big_ref[pl.ds(8 + n + zc, 1), :, 128 * q:128 * q + 128] = _pack(
                    cv_ref[zc, 12 * n:12 * n + 12].reshape(C, 128) * rs)
            yield None

        x_copy(0, S0).wait()
        nxt = lambda sl: jnp.where(sl == NB - 1, 0, sl + 1)

        def body(j, xs):
            z = zs_ref[0]
            xs1 = nxt(xs)
            xs3 = nxt(nxt(xs1))

            @pl.when(j + 1 < NG2)
            def _():
                x_copy(j + 1, xs1).wait()

            @pl.when(j >= 2)
            def _():
                o_copy(j - 2, xs3, 0, G2).wait()

            @pl.when(j + 3 < NG2)
            def _():
                x_copy(j + 3, xs3).start()

            tiles = [conv_tile(q, z, zs_ref[2 + q], zs_ref[1]) for q in range(NQ)]
            for t in tiles:
                next(t)
            shift_rows(xs1, z)
            zv = zv_ref[...]
            state = dict(slot=0, piece=0, tok=None)

            def run_pieces(rel):
                res = None
                for _ in range(PLAN[state['slot']]):
                    t = tiles[state['piece'] // 12]
                    val = t.send(rel)
                    res = val if res is None else res | val
                    state['piece'] += 1
                    if state['piece'] % 12 == 0:
                        t.send(None)
                state['slot'] += 1
                state['tok'] = res

            def gate(d):
                if state['tok'] is None:
                    return d
                du = pltpu.bitcast(d[40:48, 384:512], u32) | (state['tok'] & zv)
                last = jnp.concatenate([d[40:48, 0:384], pltpu.bitcast(du, f32)], axis=1)
                return jnp.concatenate([d[0:40], last], axis=0)

            def fin(k, hr):
                for mc in range(2):
                    rs_ = slice(48 * mc, 48 * (mc + 1))
                    o = None
                    for kt in range(3):
                        d = jnp.dot(pltpu.bitcast(w2s_ref[24 * mc:24 * (mc + 1), 128 * kt:128 * kt + 128], bf16),
                                    pltpu.bitcast(hr(kt), bf16), preferred_element_type=f32)
                        rel = pltpu.bitcast(d[0:8, 0:128], u32) & zv
                        d = gate(d)
                        o = d if o is None else o + d
                        if kt == 2:
                            bias = jnp.concatenate([bias_ref[rs_, :]] * NQ, axis=1)
                            xbuf[xs, k, rs_, :] = (o + bias + xbuf[xs, k, rs_, :].astype(f32)).astype(bf16)
                        run_pieces(rel)

            def kept_rows(n, kt):
                return h_ref[j * NST + n, 64 * kt:64 * kt + 64, :]

            def temp_rows(n, kt):
                return jnp.concatenate([big_ref[4 * (n % 2) + z + r // 48, r % 48:r % 48 + 8, :]
                                        for r in range(64 * kt, 64 * kt + 64, 8)], axis=0)

            for op in P2ORD:
                n = int(op[1])
                if op[0] == 'M':
                    assert state['piece'] < 12
                    xn = pltpu.bitcast(big_ref[8 + n + z], bf16)
                    y = jnp.dot(pltpu.bitcast(w1t_ref[...], bf16), xn, preferred_element_type=f32)
                    big_ref[pl.ds(4 * (n % 2) + z, 4)] = _pack(_gelu2(y), 4)
                elif op[0] == 'S':
                    fin(ST[n], functools.partial(kept_rows, n))
                elif op[0] == 'F':
                    fin(RC[n], functools.partial(temp_rows, n))
                else:
                    o_copy(j, xs, n, int(op[2]) - n).start()
            assert state['piece'] == 12 * NQ
            return xs1

        lax.fori_loop(0, NG2, body, jnp.int32(S0))
        for j in range(NG2 - 2, NG2):
            o_copy(j, (j + S0) % NB, 0, G2).wait()

    pl.run_scoped(phase2, pltpu.VMEM((8, 128), u32))


@jax.jit
def pallas_standalone__modern_conv_block_convnext_v2__vision_kernel(x, dw, w1, w2, grn_gamma, grn_beta):
    xt = jnp.transpose(x, (0, 1, 3, 2)).reshape(H, C, W)
    x5 = xt.reshape(H // 2, 2, C // 8, 8, W)
    out = pl.pallas_call(
        _kernel,
        in_specs=[pl.BlockSpec(memory_space=pl.ANY)] * 7,
        out_specs=pl.BlockSpec(memory_space=pl.ANY),
        out_shape=jax.ShapeDtypeStruct((H, C, W), bf16),
        scratch_shapes=[
            pltpu.VMEM((NG2 * NST, E // 2, W), u32),
            pltpu.VMEM((NB, G2, C, W), bf16),
            pltpu.VMEM((8 + NR, C // 2, W), u32),
            pltpu.VMEM((1, NVR, 8, 128), u32),
            pltpu.VMEM((1, 12, 9, 8, 128), f32),
            pltpu.VMEM((1, 40, 8, 128), f32),
            pltpu.VMEM((E // 2, C), u32),
            pltpu.VMEM((C // 2, E), u32),
            pltpu.VMEM((C, 128), f32),
            pltpu.SMEM((6,), i32),
            pltpu.SemaphoreType.DMA((NB,)),
            pltpu.SemaphoreType.DMA((NB,)),
            pltpu.SemaphoreType.DMA((2,)),
            pltpu.SemaphoreType.DMA((5,)),
        ],
        compiler_params=pltpu.CompilerParams(vmem_limit_bytes=128 * 1024 * 1024,
                                             disable_bounds_checks=True),
    )(xt, x5, dw, w1, w2.T, grn_gamma, grn_beta)
    return jnp.transpose(out.reshape(1, H, C, W), (0, 1, 3, 2))
```

```python
import functools
import math

import jax
import jax.numpy as jnp
from jax import lax
import jax.experimental.pallas as pl
import jax.experimental.pallas.tpu as pltpu

H, W, C, E = 512, 512, 96, 384
NQ = W // 128
G = 16
NG = H // G
NP2 = G // 2
G2 = 8
NG2 = H // G2
RC = (2, 3, 4)
ST = tuple(k for k in range(G2) if k not in RC)
NST = len(ST)
NR = len(RC)
NVR = NQ * 6 * 3 * (NR + 2)
ACC0 = 2 * 12 * NQ * 3
CL0 = ACC0 + E // 8
NB = 5
S0 = 4
NSUB = 6
MR = E // NSUB
NP = 2 * NSUB
LN_LAG = 5
P2ORD = 'M0,M1,F0,M2,S0,F1,S1,o04,F2,S2,o46,S3,S4,o68'.split(',')
PLAN = [2, 2] + [1] * 44 + [0, 0]

_C1 = math.sqrt(2.0 / math.pi)
_A = (_C1 * 0.044715) ** (1.0 / 3.0)
_K = _C1 / _A
_GS = 0.5 / _A
_EPS = 1e-5 / (_A * _A)

f32 = jnp.float32
bf16 = jnp.bfloat16
u32 = jnp.uint32
i32 = jnp.int32


def _iota(shape, d):
    return lax.broadcasted_iota(i32, shape, d)


def _pack(y, n=1):
    return pltpu.bitcast(y.reshape(n, y.shape[0] // n, y.shape[1]).astype(bf16), u32)


def _gelu2(y):
    return y * (jnp.tanh(y * (y * y + _K)) + 1.0)


def _tree_sum(xs):
    xs = list(xs)
    while len(xs) > 1:
        xs = [xs[i] + xs[i + 1] for i in range(0, len(xs) - 1, 2)] + ([xs[-1]] if len(xs) % 2 else [])
    return xs[0]


def _merge(a, b, msk, sh):
    return jnp.where(msk, a, b) + pltpu.roll(jnp.where(msk, b, a), 8 - sh, 0)


def _shifted(m, lane):
    zz = jnp.zeros((8, 128), u32)
    mq = [m[:, 128 * q:128 * q + 128] for q in range(NQ)]
    for q in range(NQ):
        lq = jnp.where(lane == 127, mq[q - 1] if q > 0 else zz, mq[q])
        rq = jnp.where(lane == 0, mq[q + 1] if q + 1 < NQ else zz, mq[q])
        yield q, (pltpu.roll(lq, 1, 1), mq[q], pltpu.roll(rq, 127, 1))


def _kernel(x_hbm, x5_hbm, dw_hbm, w1_hbm, w2t_hbm, g_hbm, b_hbm, o_hbm,
            h_ref, xbuf, big_ref, vr_ref, dwb_ref, cv_ref, w1t_ref, w2s_ref, bias_ref, zs_ref,
            xsem, osem, psem, wsem):

    for i in range(6):
        zs_ref[i] = 0

    def x_copy(j, sl):
        return pltpu.make_async_copy(x_hbm.at[pl.ds(j * G2, G2)], xbuf.at[sl], xsem.at[sl])

    def phase1(gb_ref):
        xn_ref = big_ref
        vi = lambda u, g, q, v: ((u * 12 + g) * NQ + q) * 3 + v
        xp = xbuf.reshape(NB * G2 // 2, C // 8, 16, W)

        def row_copy(u, half, slot, i):
            return pltpu.make_async_copy(x5_hbm.at[u - 1 + half, 1 - half],
                                         xp.at[NP2 * slot + i, :, pl.ds(8 * half, 8), :], psem.at[slot])

        def rows_copy(u, n, half, slot, i):
            return pltpu.make_async_copy(x5_hbm.at[pl.ds(u - 1 + half, n), 1 - half],
                                         xp.at[pl.ds(NP2 * slot + i, n), :, pl.ds(8 * half, 8), :], psem.at[slot])

        def start_rows(j, inner):
            for i in range(NP2):
                for half in range(2):
                    if (i < NP2 - 2 - half) == inner:
                        row_copy(NP2 * j + 3 + i, half, j & 1, i).start()

        def wait_units(slot, n):
            buf = xp.at[pl.ds(NP2 * slot, n)]
            pltpu.make_async_copy(buf, buf, psem.at[slot]).wait()

        lane = _iota((8, 128), 1)

        def shift_unit(xu_ref, u):
            for g in range(12):
                for q, vs in _shifted(pltpu.bitcast(xu_ref[g], u32), lane):
                    for v in range(3):
                        vr_ref[0, vi(u, g, q, v)] = vs[v]

        def conv_round(t, q, gs):
            cvs = []
            for g in gs:
                rhs = jnp.concatenate([vr_ref[0, vi(uu & 1, g, q, v)] for uu in (t, t + 1) for v in range(3)], axis=0)
                lhs = pltpu.bitcast(vr_ref[0, CL0 + g, :, 0:C], bf16)
                cvs.append(jnp.dot(lhs, pltpu.bitcast(rhs, bf16), preferred_element_type=f32))
            return cvs

        sub = _iota((8, 128), 0)
        m0 = sub % 2 == 0
        m1 = (sub // 2) % 2 == 0
        lnc = jnp.where(m1, 1.0 / (C * _A), 1.0 / (C * _A * _A))

        def ln_tile(cvs, q, dsts, dsts2=None):
            ls = slice(128 * q, 128 * q + 128)
            cs = [[cv[8 * ab:8 * ab + 8] for cv in cvs] for ab in range(2)]
            c1 = _merge(_tree_sum(cs[0]), _tree_sum(cs[1]), m0, 1)
            c2 = _merge(_tree_sum([c * c for c in cs[0]]), _tree_sum([c * c for c in cs[1]]), m0, 1)
            e = _merge(c1, c2, m1, 2)
            f = (e + pltpu.roll(e, 4, 0)) * lnc
            v = pltpu.roll(f, 6, 0) - f * f
            rs = lax.rsqrt(jnp.maximum(v, 0.0) + _EPS)
            for ab in range(2):
                xn = _pack(jnp.concatenate(cs[ab], axis=0) * rs[ab:ab + 1, :])
                xn_ref[pl.ds(dsts[ab], 1), :, ls] = xn
                if dsts2 is not None:
                    xn_ref[pl.ds(dsts2[ab], 1), :, ls] = xn

        def setup(dw_ref, g_ref, b_ref):
            w1_ref = xbuf.at[4, 0, :, pl.ds(0, E)]
            w2t_ref = xbuf.at[4, 1, :, pl.ds(0, E)]
            small = [pltpu.make_async_copy(a, b, wsem.at[i]) for i, (a, b) in enumerate(
                [(dw_hbm, dw_ref), (w1_hbm, w1_ref), (w2t_hbm, w2t_ref), (g_hbm, g_ref), (b_hbm, b_ref)])]
            for cp in small[:2]:
                cp.start()
            rows_copy(1, 3, 0, 1, 1).start()
            rows_copy(0, 4, 1, 1, 0).start()
            for cp in small[2:]:
                cp.start()
            rows_copy(3, NP2, 0, 0, 0).start()
            rows_copy(3, NP2, 1, 0, 0).start()
            small[0].wait()

            vr_ref[0, ACC0:CL0] = jnp.zeros((E // 8, 8, 128), u32)
            dw = dw_ref[...].astype(f32)
            dif = _iota((8, C), 1) - _iota((8, C), 0)
            row = _iota((16, C), 0)
            col = _iota((16, C), 1)
            unit = jnp.where(col >= 48, 1, 0)
            itap = 2 * unit + ((col >> 3) & 1) - (row >> 3)
            tapid = jnp.where((col & 7) == (row & 7), 3 * itap + ((col - 48 * unit) >> 4), -9)
            for g in range(12):
                cl = jnp.zeros((16, C), f32)
                for t in range(9):
                    dwt = jnp.broadcast_to(dw[t // 3, t % 3:t % 3 + 1, :], (8, C))
                    dwc = jnp.sum(jnp.where(dif == 8 * g, dwt, 0.0), axis=1, keepdims=True)
                    dwb_ref[0, g, t] = jnp.broadcast_to(dwc, (8, 128))
                    cb = jnp.broadcast_to(dwc, (8, C))
                    cl = jnp.where(tapid == t, jnp.concatenate([cb, cb], axis=0), cl)
                vr_ref[0, CL0 + g, :, 0:C] = pltpu.bitcast(cl.astype(bf16), u32)

            for cp in small[1:]:
                cp.wait()
            w1f = w1_ref[...].astype(f32)
            w1c = (w1f - jnp.sum(w1f, axis=0, keepdims=True) * (1.0 / C)).astype(bf16)
            for i in range(3):
                eye = jnp.where(_iota((128, E), 0) + 128 * i == _iota((128, E), 1), 1.0, 0.0).astype(bf16)
                w1t = lax.dot_general(eye, w1c, (((1,), (1,)), ((), ())), preferred_element_type=f32)
                w1t_ref[64 * i:64 * i + 64, :] = pltpu.bitcast(w1t.astype(bf16), u32)
            w2s_ref[...] = pltpu.bitcast(w2t_ref[...], u32)
            gb_ref[0:1, :] = g_ref[...].astype(f32).reshape(1, E)
            gb_ref[1:2, :] = b_ref[...].astype(f32).reshape(1, E)

            xp[8, :, 0:8, :] = jnp.zeros((12, 8, W), bf16)
            xp[17, :, 0:8, :] = jnp.zeros((12, 8, W), bf16)
            rows_copy(1, 3, 0, 1, 1).wait()
            rows_copy(0, 4, 1, 1, 0).wait()
            shift_unit(xp.at[10], 0)
            shift_unit(xp.at[11], 1)
            for i, (un, da, db) in enumerate([(1, 10, 5), (0, 8, 9), (2, 0, 1)]):
                for q in range(NQ):
                    ln_tile(conv_round(2 - i, q, range(12)), q, (da, db), (2, 3) if i == 1 and q < 2 else None)
                shift_unit(xp.at[8 + un], un & 1)

        pl.run_scoped(setup, pltpu.VMEM((3, 3, C), bf16), pltpu.VMEM((E,), bf16), pltpu.VMEM((E,), bf16))

        def body(j, carry):
            z = zs_ref[0]
            z1 = zs_ref[1]
            slot = j & 1

            @pl.when(j < NG - 1)
            def _():
                wait_units(slot, NP2)

            @pl.when(j == NG - 1)
            def _():
                wait_units(slot, NP2 - 2)

            @pl.when(j == NG - 2)
            def _():
                pltpu.make_async_copy(xp.at[17, :, pl.ds(0, 8), :],
                                      xp.at[NP2 * (1 - slot) + NP2 - 3, :, pl.ds(8, 8), :],
                                      psem.at[1 - slot]).start()

            def prefetch():
                @pl.when(j < NG - 1)
                def _():
                    start_rows(j + 1, True)

                @pl.when(j < NG - 2)
                def _():
                    start_rows(j + 1, False)

                @pl.when(j == NG - 1)
                def _():
                    for jn in range(3):
                        x_copy(jn, (S0 + jn) % NB).start()

            pend = []
            cur = []
            for p in range(NP2):
                for r in range(NP):
                    gr = p * NP + r
                    c = r % NSUB
                    k = 2 * p + r // NSUB
                    if gr == 3:
                        prefetch()
                    while pend and pend[0][0] <= gr:
                        ln_tile(*pend.pop(0)[1:])
                    xn = pltpu.bitcast(xn_ref[k % 8 + z], bf16)
                    lhs = pltpu.bitcast(w1t_ref[MR // 2 * c:MR // 2 * (c + 1), :], bf16)
                    gl = _gelu2(jnp.dot(lhs, xn, preferred_element_type=f32))
                    if k % G2 in ST:
                        hs = (2 * j + k // G2) * NST + ST.index(k % G2)
                        h_ref[pl.ds(hs, 1), MR // 2 * c:MR // 2 * (c + 1), :] = _pack(gl)
                    sq = gl * gl
                    for i in range(MR // 8):
                        ai = ACC0 + MR // 8 * c + i
                        sr = [sq[8 * i:8 * i + 8, 128 * q:128 * q + 128] for q in range(NQ)]
                        acc = ((pltpu.bitcast(vr_ref[0, ai], f32) + sr[0]) + sr[1]) + (sr[2] + sr[3])
                        vr_ref[0, ai] = pltpu.bitcast(acc, u32)
                    q = (r // 3 + 2) % 4
                    pair = p + 1 + (r >= 6)
                    cur += conv_round(pair, q, range(4 * (r % 3), 4 * (r % 3) + 4))
                    if r % 3 == 2:
                        pend.append((gr + LN_LAG, cur, q, (2 * pair % 8 + z1, (2 * pair + 1) % 8 + z1)))
                        cur = []
                    if r == NP // 2 - 1:
                        shift_unit(xp.at[8 * slot + p], (p + 3) % 2)
            for e in pend:
                ln_tile(*e[1:])
            return carry

        lax.fori_loop(0, NG, body, 0)

        pdif = _iota((8, E), 1) - _iota((8, E), 0) + zs_ref[0]
        parts = []
        for i in range(E // 8):
            col = jnp.sum(pltpu.bitcast(vr_ref[0, ACC0 + i], f32), axis=1, keepdims=True)
            parts.append(jnp.where(pdif == 8 * i, jnp.broadcast_to(col, (8, E)), 0.0))
        ss = jnp.sum(_tree_sum(parts), axis=0, keepdims=True) * (_GS * _GS)
        gx = jnp.sqrt(ss + 1e-6)
        nx = gx / (jnp.sum(gx, axis=1, keepdims=True) * (1.0 / E) + 1e-6)
        s = (gb_ref[0:1, :] * nx + 1.0) * _GS
        w2t = pltpu.bitcast(w2s_ref[...], bf16).astype(f32)
        w2s_ref[...] = pltpu.bitcast((w2t * s).astype(bf16), u32)
        bias_ref[...] = jnp.broadcast_to(jnp.sum(w2t * gb_ref[1:2, :], axis=1, keepdims=True), (C, 128))

    pl.run_scoped(phase1, pltpu.VMEM((8, E), f32))

    def phase2(zv_ref):
        zv_ref[...] = jnp.zeros(zv_ref.shape, u32)
        vi = lambda q, k, i: (q * 6 + k) * 3 * (NR + 2) + i

        def o_copy(j, sl, r0, n):
            return pltpu.make_async_copy(xbuf.at[sl, pl.ds(r0, n)], o_hbm.at[pl.ds(j * G2 + r0, n)], osem.at[sl])

        z0 = zs_ref[0]
        lane = _iota((8, 128), 1) + z0
        sub = _iota((8, 128), 0) + z0
        m0 = (sub & 1) == 0
        m1 = (sub & 2) == 0
        m2 = sub < 4
        lnc = jnp.where(m2, 1.0 / (C * _A), 1.0 / (C * _A * _A))

        def shift_rows(xs, zv):
            for r in range(NR + 2):
                for k in range(6):
                    m = pltpu.bitcast(xbuf[xs, RC[0] - 1 + r, 16 * k:16 * k + 16, :], u32)
                    for q, vs in _shifted(m, lane):
                        for v in range(3):
                            vr_ref[zv, vi(q, k, 3 * r + v)] = vs[v]

        def conv_tile(q, zc, zw, zr):
            st = [None] * NR
            tok = yield None
            for g in range(12):
                w = [dwb_ref[zw, g, t] for t in range(9)]
                acc = [None] * NR
                for r in range(NR + 2):
                    for v in range(3):
                        x = vr_ref[zw, vi(q, g // 2, 3 * r + v)]
                        if v == 2:
                            x = x | tok
                        xf = pltpu.bitcast(x, bf16).astype(f32)[8 * (g % 2):8 * (g % 2) + 8]
                        for n in range(NR):
                            if 0 <= r - n <= 2:
                                t = xf * w[3 * (r - n) + v]
                                acc[n] = t if acc[n] is None else acc[n] + t
                for n in range(NR):
                    cv = acc[n]
                    st[n] = (cv, cv * cv) if st[n] is None else (st[n][0] + cv, st[n][1] + cv * cv)
                    cv_ref[zc, 12 * n + g] = cv
                tok = yield pltpu.bitcast((st[0][1] + st[1][1]) + st[2][1], u32)
            half = lambda i: _merge(_merge(st[0][i], st[1][i], m0, 1), st[2][i] + pltpu.roll(st[2][i], 7, 0), m1, 2)
            f = _merge(half(0), half(1), m2, 4) * lnc
            v = pltpu.roll(f, 4, 0) - f * f
            cv_ref[zr, 36] = lax.rsqrt(jnp.maximum(v, 0.0) + _EPS)
            for n in range(NR):
                rs = cv_ref[zc, 36, n:n + 1, :]
                big_ref[pl.ds(8 + n + zc, 1), :, 128 * q:128 * q + 128] = _pack(
                    cv_ref[zc, 12 * n:12 * n + 12].reshape(C, 128) * rs)
            yield None

        x_copy(0, S0).wait()
        nxt = lambda sl: jnp.where(sl == NB - 1, 0, sl + 1)

        def body(j, xs):
            z = zs_ref[0]
            xs1 = nxt(xs)
            xs3 = nxt(nxt(xs1))

            @pl.when(j + 1 < NG2)
            def _():
                x_copy(j + 1, xs1).wait()

            @pl.when(j >= 2)
            def _():
                o_copy(j - 2, xs3, 0, G2).wait()

            @pl.when(j + 3 < NG2)
            def _():
                x_copy(j + 3, xs3).start()

            tiles = [conv_tile(q, z, zs_ref[2 + q], zs_ref[1]) for q in range(NQ)]
            for t in tiles:
                next(t)
            shift_rows(xs1, z)
            zv = zv_ref[...]
            state = dict(slot=0, piece=0, tok=None)

            def run_pieces(rel):
                res = None
                for _ in range(PLAN[state['slot']]):
                    t = tiles[state['piece'] // 12]
                    val = t.send(rel)
                    res = val if res is None else res | val
                    state['piece'] += 1
                    if state['piece'] % 12 == 0:
                        t.send(None)
                state['slot'] += 1
                state['tok'] = res

            def gate(d):
                if state['tok'] is None:
                    return d
                du = pltpu.bitcast(d[40:48, 384:512], u32) | (state['tok'] & zv)
                last = jnp.concatenate([d[40:48, 0:384], pltpu.bitcast(du, f32)], axis=1)
                return jnp.concatenate([d[0:40], last], axis=0)

            def fin(k, hr):
                for mc in range(2):
                    rs_ = slice(48 * mc, 48 * (mc + 1))
                    o = None
                    for kt in range(3):
                        d = jnp.dot(pltpu.bitcast(w2s_ref[24 * mc:24 * (mc + 1), 128 * kt:128 * kt + 128], bf16),
                                    pltpu.bitcast(hr(kt), bf16), preferred_element_type=f32)
                        rel = pltpu.bitcast(d[0:8, 0:128], u32) & zv
                        d = gate(d)
                        o = d if o is None else o + d
                        if kt == 2:
                            bias = jnp.concatenate([bias_ref[rs_, :]] * NQ, axis=1)
                            xbuf[xs, k, rs_, :] = (o + bias + xbuf[xs, k, rs_, :].astype(f32)).astype(bf16)
                        run_pieces(rel)

            def kept_rows(n, kt):
                return h_ref[j * NST + n, 64 * kt:64 * kt + 64, :]

            def temp_rows(n, kt):
                return jnp.concatenate([big_ref[4 * (n % 2) + z + r // 48, r % 48:r % 48 + 8, :]
                                        for r in range(64 * kt, 64 * kt + 64, 8)], axis=0)

            for op in P2ORD:
                n = int(op[1])
                if op[0] == 'M':
                    assert state['piece'] < 12
                    xn = pltpu.bitcast(big_ref[8 + n + z], bf16)
                    y = jnp.dot(pltpu.bitcast(w1t_ref[...], bf16), xn, preferred_element_type=f32)
                    big_ref[pl.ds(4 * (n % 2) + z, 4)] = _pack(_gelu2(y), 4)
                elif op[0] == 'S':
                    fin(ST[n], functools.partial(kept_rows, n))
                elif op[0] == 'F':
                    fin(RC[n], functools.partial(temp_rows, n))
                else:
                    o_copy(j, xs, n, int(op[2]) - n).start()
            assert state['piece'] == 12 * NQ
            return xs1

        lax.fori_loop(0, NG2, body, jnp.int32(S0))
        for j in range(NG2 - 2, NG2):
            o_copy(j, (j + S0) % NB, 0, G2).wait()

    pl.run_scoped(phase2, pltpu.VMEM((8, 128), u32))


@jax.jit
def pallas_standalone__modern_conv_block_convnext_v2__vision_kernel(x, dw, w1, w2, grn_gamma, grn_beta):
    xt = jnp.transpose(x, (0, 1, 3, 2)).reshape(H, C, W)
    x5 = xt.reshape(H // 2, 2, C // 8, 8, W)
    out = pl.pallas_call(
        _kernel,
        in_specs=[pl.BlockSpec(memory_space=pl.ANY)] * 7,
        out_specs=pl.BlockSpec(memory_space=pl.ANY),
        out_shape=jax.ShapeDtypeStruct((H, C, W), bf16),
        scratch_shapes=[
            pltpu.VMEM((NG2 * NST, E // 2, W), u32),
            pltpu.VMEM((NB, G2, C, W), bf16),
            pltpu.VMEM((8 + NR, C // 2, W), u32),
            pltpu.VMEM((1, NVR, 8, 128), u32),
            pltpu.VMEM((1, 12, 9, 8, 128), f32),
            pltpu.VMEM((1, 40, 8, 128), f32),
            pltpu.VMEM((E // 2, C), u32),
            pltpu.VMEM((C // 2, E), u32),
            pltpu.VMEM((C, 128), f32),
            pltpu.SMEM((6,), i32),
            pltpu.SemaphoreType.DMA((NB,)),
            pltpu.SemaphoreType.DMA((NB,)),
            pltpu.SemaphoreType.DMA((2,)),
            pltpu.SemaphoreType.DMA((5,)),
        ],
        compiler_params=pltpu.CompilerParams(vmem_limit_bytes=128 * 1024 * 1024,
                                             disable_bounds_checks=True),
    )(xt, x5, dw, w1, w2.T, grn_gamma, grn_beta)
    return jnp.transpose(out.reshape(1, H, C, W), (0, 1, 3, 2))
```

```python
import functools
import math

import jax
import jax.numpy as jnp
from jax import lax
import jax.experimental.pallas as pl
import jax.experimental.pallas.tpu as pltpu

H, W, C, E = 512, 512, 96, 384
NQ = W // 128
G = 16
NG = H // G
NP2 = G // 2
G2 = 8
NG2 = H // G2
RC = (2, 3, 4)
ST = tuple(k for k in range(G2) if k not in RC)
NST = len(ST)
NR = len(RC)
NVR = NQ * 6 * 3 * (NR + 2)
ACC0 = 2 * 12 * NQ * 3
CL0 = ACC0 + E // 8
NB = 5
S0 = 4
NSUB = 6
MR = E // NSUB
NP = 2 * NSUB
LN_LAG = 5
P2ORD = 'M0,M1,F0,M2,S0,F1,S1,o04,F2,S2,o46,S3,S4,o68'.split(',')
PLAN = [2, 2] + [1] * 44 + [0, 0]

_C1 = math.sqrt(2.0 / math.pi)
_A = (_C1 * 0.044715) ** (1.0 / 3.0)
_K = _C1 / _A
_GS = 0.5 / _A
_EPS = 1e-5 / (_A * _A)

f32 = jnp.float32
bf16 = jnp.bfloat16
u32 = jnp.uint32
i32 = jnp.int32


def _iota(shape, d):
    return lax.broadcasted_iota(i32, shape, d)


def _pack(y, n=1):
    return pltpu.bitcast(y.reshape(n, y.shape[0] // n, y.shape[1]).astype(bf16), u32)


def _gelu2(y):
    return y * (jnp.tanh(y * (y * y + _K)) + 1.0)


def _tree_sum(xs):
    xs = list(xs)
    while len(xs) > 1:
        xs = [xs[i] + xs[i + 1] for i in range(0, len(xs) - 1, 2)] + ([xs[-1]] if len(xs) % 2 else [])
    return xs[0]


def _merge(a, b, msk, sh):
    return jnp.where(msk, a, b) + pltpu.roll(jnp.where(msk, b, a), 8 - sh, 0)


def _shifted(m, lane):
    zz = jnp.zeros((8, 128), u32)
    mq = [m[:, 128 * q:128 * q + 128] for q in range(NQ)]
    for q in range(NQ):
        lq = jnp.where(lane == 127, mq[q - 1] if q > 0 else zz, mq[q])
        rq = jnp.where(lane == 0, mq[q + 1] if q + 1 < NQ else zz, mq[q])
        yield q, (pltpu.roll(lq, 1, 1), mq[q], pltpu.roll(rq, 127, 1))


def _kernel(x_hbm, x5_hbm, dw_hbm, w1_hbm, w2t_hbm, g_hbm, b_hbm, o_hbm,
            h_ref, xbuf, big_ref, vr_ref, dwb_ref, cv_ref, w1t_ref, w2s_ref, bias_ref, zs_ref,
            xsem, osem, psem, wsem):

    for i in range(6):
        zs_ref[i] = 0

    def x_copy(j, sl):
        return pltpu.make_async_copy(x_hbm.at[pl.ds(j * G2, G2)], xbuf.at[sl], xsem.at[sl])

    def phase1(gb_ref):
        xn_ref = big_ref
        vi = lambda u, g, q, v: ((u * 12 + g) * NQ + q) * 3 + v
        xp = xbuf.reshape(NB * G2 // 2, C // 8, 16, W)

        def row_copy(u, half, slot, i):
            return pltpu.make_async_copy(x5_hbm.at[u - 1 + half, 1 - half],
                                         xp.at[NP2 * slot + i, :, pl.ds(8 * half, 8), :], psem.at[slot])

        def rows_copy(u, n, half, slot, i):
            return pltpu.make_async_copy(x5_hbm.at[pl.ds(u - 1 + half, n), 1 - half],
                                         xp.at[pl.ds(NP2 * slot + i, n), :, pl.ds(8 * half, 8), :], psem.at[slot])

        def start_rows(j, inner):
            for i in range(NP2):
                for half in range(2):
                    if (i < NP2 - 2 - half) == inner:
                        row_copy(NP2 * j + 3 + i, half, j & 1, i).start()

        def wait_units(slot, n):
            buf = xp.at[pl.ds(NP2 * slot, n)]
            pltpu.make_async_copy(buf, buf, psem.at[slot]).wait()

        lane = _iota((8, 128), 1)

        def shift_unit(xu_ref, u):
            for g in range(12):
                for q, vs in _shifted(pltpu.bitcast(xu_ref[g], u32), lane):
                    for v in range(3):
                        vr_ref[0, vi(u, g, q, v)] = vs[v]

        def conv_round(t, q, gs):
            cvs = []
            for g in gs:
                rhs = jnp.concatenate([vr_ref[0, vi(uu & 1, g, q, v)] for uu in (t, t + 1) for v in range(3)], axis=0)
                lhs = pltpu.bitcast(vr_ref[0, CL0 + g, :, 0:C], bf16)
                cvs.append(jnp.dot(lhs, pltpu.bitcast(rhs, bf16), preferred_element_type=f32))
            return cvs

        sub = _iota((8, 128), 0)
        m0 = sub % 2 == 0
        m1 = (sub // 2) % 2 == 0
        lnc = jnp.where(m1, 1.0 / (C * _A), 1.0 / (C * _A * _A))

        def ln_tile(cvs, q, dsts, dsts2=None):
            ls = slice(128 * q, 128 * q + 128)
            cs = [[cv[8 * ab:8 * ab + 8] for cv in cvs] for ab in range(2)]
            c1 = _merge(_tree_sum(cs[0]), _tree_sum(cs[1]), m0, 1)
            c2 = _merge(_tree_sum([c * c for c in cs[0]]), _tree_sum([c * c for c in cs[1]]), m0, 1)
            e = _merge(c1, c2, m1, 2)
            f = (e + pltpu.roll(e, 4, 0)) * lnc
            v = pltpu.roll(f, 6, 0) - f * f
            rs = lax.rsqrt(jnp.maximum(v, 0.0) + _EPS)
            for ab in range(2):
                xn = _pack(jnp.concatenate(cs[ab], axis=0) * rs[ab:ab + 1, :])
                xn_ref[pl.ds(dsts[ab], 1), :, ls] = xn
                if dsts2 is not None:
                    xn_ref[pl.ds(dsts2[ab], 1), :, ls] = xn

        def setup(dw_ref, g_ref, b_ref):
            w1_ref = xbuf.at[4, 0, :, pl.ds(0, E)]
            w2t_ref = xbuf.at[4, 1, :, pl.ds(0, E)]
            small = [pltpu.make_async_copy(a, b, wsem.at[i]) for i, (a, b) in enumerate(
                [(dw_hbm, dw_ref), (w1_hbm, w1_ref), (w2t_hbm, w2t_ref), (g_hbm, g_ref), (b_hbm, b_ref)])]
            for cp in small[:2]:
                cp.start()
            rows_copy(1, 3, 0, 1, 1).start()
            rows_copy(0, 4, 1, 1, 0).start()
            for cp in small[2:]:
                cp.start()
            rows_copy(3, NP2, 0, 0, 0).start()
            rows_copy(3, NP2, 1, 0, 0).start()
            small[0].wait()

            vr_ref[0, ACC0:CL0] = jnp.zeros((E // 8, 8, 128), u32)
            dw = dw_ref[...].astype(f32)
            dif = _iota((8, C), 1) - _iota((8, C), 0)
            row = _iota((16, C), 0)
            col = _iota((16, C), 1)
            unit = jnp.where(col >= 48, 1, 0)
            itap = 2 * unit + ((col >> 3) & 1) - (row >> 3)
            tapid = jnp.where((col & 7) == (row & 7), 3 * itap + ((col - 48 * unit) >> 4), -9)
            for g in range(12):
                cl = jnp.zeros((16, C), f32)
                for t in range(9):
                    dwt = jnp.broadcast_to(dw[t // 3, t % 3:t % 3 + 1, :], (8, C))
                    dwc = jnp.sum(jnp.where(dif == 8 * g, dwt, 0.0), axis=1, keepdims=True)
                    dwb_ref[0, g, t] = jnp.broadcast_to(dwc, (8, 128))
                    cb = jnp.broadcast_to(dwc, (8, C))
                    cl = jnp.where(tapid == t, jnp.concatenate([cb, cb], axis=0), cl)
                vr_ref[0, CL0 + g, :, 0:C] = pltpu.bitcast(cl.astype(bf16), u32)

            for cp in small[1:]:
                cp.wait()
            w1f = w1_ref[...].astype(f32)
            w1c = (w1f - jnp.sum(w1f, axis=0, keepdims=True) * (1.0 / C)).astype(bf16)
            for i in range(3):
                eye = jnp.where(_iota((128, E), 0) + 128 * i == _iota((128, E), 1), 1.0, 0.0).astype(bf16)
                w1t = lax.dot_general(eye, w1c, (((1,), (1,)), ((), ())), preferred_element_type=f32)
                w1t_ref[64 * i:64 * i + 64, :] = pltpu.bitcast(w1t.astype(bf16), u32)
            w2s_ref[...] = pltpu.bitcast(w2t_ref[...], u32)
            gb_ref[0:1, :] = g_ref[...].astype(f32).reshape(1, E)
            gb_ref[1:2, :] = b_ref[...].astype(f32).reshape(1, E)

            xp[8, :, 0:8, :] = jnp.zeros((12, 8, W), bf16)
            xp[17, :, 0:8, :] = jnp.zeros((12, 8, W), bf16)
            rows_copy(1, 3, 0, 1, 1).wait()
            rows_copy(0, 4, 1, 1, 0).wait()
            shift_unit(xp.at[10], 0)
            shift_unit(xp.at[11], 1)
            for i, (un, da, db) in enumerate([(1, 10, 5), (0, 8, 9), (2, 0, 1)]):
                for q in range(NQ):
                    ln_tile(conv_round(2 - i, q, range(12)), q, (da, db), (2, 3) if i == 1 and q < 2 else None)
                shift_unit(xp.at[8 + un], un & 1)

        pl.run_scoped(setup, pltpu.VMEM((3, 3, C), bf16), pltpu.VMEM((E,), bf16), pltpu.VMEM((E,), bf16))

        def body(j, carry):
            z = zs_ref[0]
            z1 = zs_ref[1]
            slot = j & 1

            @pl.when(j < NG - 1)
            def _():
                wait_units(slot, NP2)

            @pl.when(j == NG - 1)
            def _():
                wait_units(slot, NP2 - 2)

            @pl.when(j == NG - 2)
            def _():
                pltpu.make_async_copy(xp.at[17, :, pl.ds(0, 8), :],
                                      xp.at[NP2 * (1 - slot) + NP2 - 3, :, pl.ds(8, 8), :],
                                      psem.at[1 - slot]).start()

            def prefetch():
                @pl.when(j < NG - 1)
                def _():
                    start_rows(j + 1, True)

                @pl.when(j < NG - 2)
                def _():
                    start_rows(j + 1, False)

                @pl.when(j == NG - 1)
                def _():
                    for jn in range(3):
                        x_copy(jn, (S0 + jn) % NB).start()

            pend = []
            cur = []

            def conv_step(p, r):
                q = (r // 3 + 2) % 4
                pair = p + 1 + (r >= 6)
                cur.extend(conv_round(pair, q, range(4 * (r % 3), 4 * (r % 3) + 4)))
                if r % 3 == 2:
                    pend.append((p * NP + r + LN_LAG, list(cur), q, (2 * pair % 8 + z1, (2 * pair + 1) % 8 + z1)))
                    cur.clear()

            for p in range(NP2):
                for r in range(NP):
                    gr = p * NP + r
                    c = r % NSUB
                    k = 2 * p + r // NSUB
                    last = gr == NP2 * NP - 1
                    if last:
                        conv_step(p, r)
                    if gr == 3:
                        prefetch()
                    while pend and pend[0][0] <= gr:
                        ln_tile(*pend.pop(0)[1:])
                    xn = pltpu.bitcast(xn_ref[k % 8 + z], bf16)
                    lhs = pltpu.bitcast(w1t_ref[MR // 2 * c:MR // 2 * (c + 1), :], bf16)
                    gl = _gelu2(jnp.dot(lhs, xn, preferred_element_type=f32))
                    if k % G2 in ST:
                        hs = (2 * j + k // G2) * NST + ST.index(k % G2)
                        h_ref[pl.ds(hs, 1), MR // 2 * c:MR // 2 * (c + 1), :] = _pack(gl)
                    sq = gl * gl
                    for i in range(MR // 8):
                        ai = ACC0 + MR // 8 * c + i
                        sr = [sq[8 * i:8 * i + 8, 128 * q:128 * q + 128] for q in range(NQ)]
                        acc = ((pltpu.bitcast(vr_ref[0, ai], f32) + sr[0]) + sr[1]) + (sr[2] + sr[3])
                        vr_ref[0, ai] = pltpu.bitcast(acc, u32)
                    if not last:
                        conv_step(p, r)
                    if r == NP // 2 - 1:
                        shift_unit(xp.at[8 * slot + p], (p + 3) % 2)
            for e in pend:
                ln_tile(*e[1:])
            return carry

        lax.fori_loop(0, NG, body, 0)

        pdif = _iota((8, E), 1) - _iota((8, E), 0) + zs_ref[0]
        parts = []
        for i in range(E // 8):
            col = jnp.sum(pltpu.bitcast(vr_ref[0, ACC0 + i], f32), axis=1, keepdims=True)
            parts.append(jnp.where(pdif == 8 * i, jnp.broadcast_to(col, (8, E)), 0.0))
        ss = jnp.sum(_tree_sum(parts), axis=0, keepdims=True) * (_GS * _GS)
        gx = jnp.sqrt(ss + 1e-6)
        nx = gx / (jnp.sum(gx, axis=1, keepdims=True) * (1.0 / E) + 1e-6)
        s = (gb_ref[0:1, :] * nx + 1.0) * _GS
        w2t = pltpu.bitcast(w2s_ref[...], bf16).astype(f32)
        w2s_ref[...] = pltpu.bitcast((w2t * s).astype(bf16), u32)
        bias_ref[...] = jnp.broadcast_to(jnp.sum(w2t * gb_ref[1:2, :], axis=1, keepdims=True), (C, 128))

    pl.run_scoped(phase1, pltpu.VMEM((8, E), f32))

    def phase2(zv_ref):
        zv_ref[...] = jnp.zeros(zv_ref.shape, u32)
        vi = lambda q, k, i: (q * 6 + k) * 3 * (NR + 2) + i

        def o_copy(j, sl, r0, n):
            return pltpu.make_async_copy(xbuf.at[sl, pl.ds(r0, n)], o_hbm.at[pl.ds(j * G2 + r0, n)], osem.at[sl])

        z0 = zs_ref[0]
        lane = _iota((8, 128), 1) + z0
        sub = _iota((8, 128), 0) + z0
        m0 = (sub & 1) == 0
        m1 = (sub & 2) == 0
        m2 = sub < 4
        lnc = jnp.where(m2, 1.0 / (C * _A), 1.0 / (C * _A * _A))

        def shift_rows(xs, zv):
            for r in range(NR + 2):
                for k in range(6):
                    m = pltpu.bitcast(xbuf[xs, RC[0] - 1 + r, 16 * k:16 * k + 16, :], u32)
                    for q, vs in _shifted(m, lane):
                        for v in range(3):
                            vr_ref[zv, vi(q, k, 3 * r + v)] = vs[v]

        def conv_tile(q, zc, zw, zr):
            st = [None] * NR
            tok = yield None
            for g in range(12):
                w = [dwb_ref[zw, g, t] for t in range(9)]
                acc = [None] * NR
                for r in range(NR + 2):
                    for v in range(3):
                        x = vr_ref[zw, vi(q, g // 2, 3 * r + v)]
                        if v == 2:
                            x = x | tok
                        xf = pltpu.bitcast(x, bf16).astype(f32)[8 * (g % 2):8 * (g % 2) + 8]
                        for n in range(NR):
                            if 0 <= r - n <= 2:
                                t = xf * w[3 * (r - n) + v]
                                acc[n] = t if acc[n] is None else acc[n] + t
                for n in range(NR):
                    cv = acc[n]
                    st[n] = (cv, cv * cv) if st[n] is None else (st[n][0] + cv, st[n][1] + cv * cv)
                    cv_ref[zc, 12 * n + g] = cv
                tok = yield pltpu.bitcast((acc[0] + acc[1]) + acc[2], u32)
            half = lambda i: _merge(_merge(st[0][i], st[1][i], m0, 1), st[2][i] + pltpu.roll(st[2][i], 7, 0), m1, 2)
            f = _merge(half(0), half(1), m2, 4) * lnc
            v = pltpu.roll(f, 4, 0) - f * f
            cv_ref[zr, 36] = lax.rsqrt(jnp.maximum(v, 0.0) + _EPS)
            for n in range(NR):
                rs = cv_ref[zc, 36, n:n + 1, :]
                big_ref[pl.ds(8 + n + zc, 1), :, 128 * q:128 * q + 128] = _pack(
                    cv_ref[zc, 12 * n:12 * n + 12].reshape(C, 128) * rs)
            yield None

        x_copy(0, S0).wait()
        nxt = lambda sl: jnp.where(sl == NB - 1, 0, sl + 1)

        def body(j, xs):
            z = zs_ref[0]
            xs1 = nxt(xs)
            xs3 = nxt(nxt(xs1))

            @pl.when(j + 1 < NG2)
            def _():
                x_copy(j + 1, xs1).wait()

            @pl.when(j >= 2)
            def _():
                o_copy(j - 2, xs3, 0, G2).wait()

            @pl.when(j + 3 < NG2)
            def _():
                x_copy(j + 3, xs3).start()

            tiles = [conv_tile(q, z, zs_ref[2 + q], zs_ref[1]) for q in range(NQ)]
            for t in tiles:
                next(t)
            shift_rows(xs1, z)
            zv = zv_ref[...]
            state = dict(slot=0, piece=0, tok=None)

            def run_pieces(rel):
                res = None
                for _ in range(PLAN[state['slot']]):
                    t = tiles[state['piece'] // 12]
                    val = t.send(rel)
                    res = val if res is None else res | val
                    state['piece'] += 1
                    if state['piece'] % 12 == 0:
                        t.send(None)
                state['slot'] += 1
                state['tok'] = res

            def gate(d):
                if state['tok'] is None:
                    return d
                du = pltpu.bitcast(d[40:48, 384:512], u32) | (state['tok'] & zv)
                last = jnp.concatenate([d[40:48, 0:384], pltpu.bitcast(du, f32)], axis=1)
                return jnp.concatenate([d[0:40], last], axis=0)

            def fin(k, hr):
                for mc in range(2):
                    rs_ = slice(48 * mc, 48 * (mc + 1))
                    o = None
                    for kt in range(3):
                        d = jnp.dot(pltpu.bitcast(w2s_ref[24 * mc:24 * (mc + 1), 128 * kt:128 * kt + 128], bf16),
                                    pltpu.bitcast(hr(kt), bf16), preferred_element_type=f32)
                        rel = pltpu.bitcast(d[0:8, 0:128], u32) & zv
                        d = gate(d)
                        o = d if o is None else o + d
                        if kt == 2:
                            bias = jnp.concatenate([bias_ref[rs_, :]] * NQ, axis=1)
                            xbuf[xs, k, rs_, :] = (o + bias + xbuf[xs, k, rs_, :].astype(f32)).astype(bf16)
                        run_pieces(rel)

            def kept_rows(n, kt):
                return h_ref[j * NST + n, 64 * kt:64 * kt + 64, :]

            def temp_rows(n, kt):
                return jnp.concatenate([big_ref[4 * (n % 2) + z + r // 48, r % 48:r % 48 + 8, :]
                                        for r in range(64 * kt, 64 * kt + 64, 8)], axis=0)

            for op in P2ORD:
                n = int(op[1])
                if op[0] == 'M':
                    assert state['piece'] < 12
                    xn = pltpu.bitcast(big_ref[8 + n + z], bf16)
                    y = jnp.dot(pltpu.bitcast(w1t_ref[...], bf16), xn, preferred_element_type=f32)
                    big_ref[pl.ds(4 * (n % 2) + z, 4)] = _pack(_gelu2(y), 4)
                elif op[0] == 'S':
                    fin(ST[n], functools.partial(kept_rows, n))
                elif op[0] == 'F':
                    fin(RC[n], functools.partial(temp_rows, n))
                else:
                    o_copy(j, xs, n, int(op[2]) - n).start()
            assert state['piece'] == 12 * NQ
            return xs1

        lax.fori_loop(0, NG2, body, jnp.int32(S0))
        for j in range(NG2 - 2, NG2):
            o_copy(j, (j + S0) % NB, 0, G2).wait()

    pl.run_scoped(phase2, pltpu.VMEM((8, 128), u32))


@jax.jit
def pallas_standalone__modern_conv_block_convnext_v2__vision_kernel(x, dw, w1, w2, grn_gamma, grn_beta):
    xt = jnp.transpose(x, (0, 1, 3, 2)).reshape(H, C, W)
    x5 = xt.reshape(H // 2, 2, C // 8, 8, W)
    out = pl.pallas_call(
        _kernel,
        in_specs=[pl.BlockSpec(memory_space=pl.ANY)] * 7,
        out_specs=pl.BlockSpec(memory_space=pl.ANY),
        out_shape=jax.ShapeDtypeStruct((H, C, W), bf16),
        scratch_shapes=[
            pltpu.VMEM((NG2 * NST, E // 2, W), u32),
            pltpu.VMEM((NB, G2, C, W), bf16),
            pltpu.VMEM((8 + NR, C // 2, W), u32),
            pltpu.VMEM((1, NVR, 8, 128), u32),
            pltpu.VMEM((1, 12, 9, 8, 128), f32),
            pltpu.VMEM((1, 40, 8, 128), f32),
            pltpu.VMEM((E // 2, C), u32),
            pltpu.VMEM((C // 2, E), u32),
            pltpu.VMEM((C, 128), f32),
            pltpu.SMEM((6,), i32),
            pltpu.SemaphoreType.DMA((NB,)),
            pltpu.SemaphoreType.DMA((NB,)),
            pltpu.SemaphoreType.DMA((2,)),
            pltpu.SemaphoreType.DMA((5,)),
        ],
        compiler_params=pltpu.CompilerParams(vmem_limit_bytes=128 * 1024 * 1024,
                                             disable_bounds_checks=True),
    )(xt, x5, dw, w1, w2.T, grn_gamma, grn_beta)
    return jnp.transpose(out.reshape(1, H, C, W), (0, 1, 3, 2))
```

```python
import functools
import math

import jax
import jax.numpy as jnp
from jax import lax
import jax.experimental.pallas as pl
import jax.experimental.pallas.tpu as pltpu

H, W, C, E = 512, 512, 96, 384
NQ = W // 128
G = 16
NG = H // G
NP2 = G // 2
G2 = 8
NG2 = H // G2
RC = (2, 3, 4)
ST = tuple(k for k in range(G2) if k not in RC)
NST = len(ST)
NR = len(RC)
NVR = NQ * 6 * 3 * (NR + 2)
ACC0 = 2 * 12 * NQ * 3
CL0 = ACC0 + E // 8
NB = 5
S0 = 4
NSUB = 6
MR = E // NSUB
NP = 2 * NSUB
LN_LAG = 5
P2ORD = 'M0,M1,F0,M2,S0,F1,S1,o04,F2,S2,o46,S3,S4,o68'.split(',')
PLAN = [2, 2] + [1] * 44 + [0, 0]

_C1 = math.sqrt(2.0 / math.pi)
_A = (_C1 * 0.044715) ** (1.0 / 3.0)
_K = _C1 / _A
_GS = 0.5 / _A
_EPS = 1e-5 / (_A * _A)

f32 = jnp.float32
bf16 = jnp.bfloat16
u32 = jnp.uint32
i32 = jnp.int32


def _iota(shape, d):
    return lax.broadcasted_iota(i32, shape, d)


def _pack(y, n=1):
    return pltpu.bitcast(y.reshape(n, y.shape[0] // n, y.shape[1]).astype(bf16), u32)


def _gelu2(y):
    return y * (jnp.tanh(y * (y * y + _K)) + 1.0)


def _tree_sum(xs):
    xs = list(xs)
    while len(xs) > 1:
        xs = [xs[i] + xs[i + 1] for i in range(0, len(xs) - 1, 2)] + ([xs[-1]] if len(xs) % 2 else [])
    return xs[0]


def _merge(a, b, msk, sh):
    return jnp.where(msk, a, b) + pltpu.roll(jnp.where(msk, b, a), 8 - sh, 0)


def _shifted(m, lane):
    zz = jnp.zeros((8, 128), u32)
    mq = [m[:, 128 * q:128 * q + 128] for q in range(NQ)]
    for q in range(NQ):
        lq = jnp.where(lane == 127, mq[q - 1] if q > 0 else zz, mq[q])
        rq = jnp.where(lane == 0, mq[q + 1] if q + 1 < NQ else zz, mq[q])
        yield q, (pltpu.roll(lq, 1, 1), mq[q], pltpu.roll(rq, 127, 1))


def _kernel(x_hbm, x5_hbm, dw_hbm, w1_hbm, w2t_hbm, g_hbm, b_hbm, o_hbm,
            h_ref, xbuf, big_ref, vr_ref, dwb_ref, cv_ref, w1t_ref, w2s_ref, bias_ref, zs_ref,
            xsem, osem, psem, wsem):

    for i in range(6):
        zs_ref[i] = 0

    def x_copy(j, sl):
        return pltpu.make_async_copy(x_hbm.at[pl.ds(j * G2, G2)], xbuf.at[sl], xsem.at[sl])

    def phase1(gb_ref):
        xn_ref = big_ref
        vi = lambda u, g, q, v: ((u * 12 + g) * NQ + q) * 3 + v
        xp = xbuf.reshape(NB * 4, C // 8, 16, W)

        def rows_copy(u, n, half, i, sem):
            return pltpu.make_async_copy(x5_hbm.at[pl.ds(u - 1 + half, n), 1 - half],
                                         xp.at[pl.ds(i, n), :, pl.ds(8 * half, 8), :], psem.at[sem])

        def start_slot(u, sl, sem, rows=range(8)):
            for i in rows:
                pltpu.make_async_copy(x5_hbm.at[u + i // 2 - 1 + i % 2, 1 - i % 2],
                                      xp.at[4 * sl + i // 2, :, pl.ds(8 * (i % 2), 8), :], psem.at[sem]).start()

        def wait_for(buf, sem):
            pltpu.make_async_copy(buf, buf, psem.at[sem]).wait()

        lane = _iota((8, 128), 1)

        def shift_unit(xu_ref, u):
            for g in range(12):
                for q, vs in _shifted(pltpu.bitcast(xu_ref[g], u32), lane):
                    for v in range(3):
                        vr_ref[0, vi(u, g, q, v)] = vs[v]

        def conv_round(t, q, gs):
            cvs = []
            for g in gs:
                rhs = jnp.concatenate([vr_ref[0, vi(uu & 1, g, q, v)] for uu in (t, t + 1) for v in range(3)], axis=0)
                lhs = pltpu.bitcast(vr_ref[0, CL0 + g, :, 0:C], bf16)
                cvs.append(jnp.dot(lhs, pltpu.bitcast(rhs, bf16), preferred_element_type=f32))
            return cvs

        sub = _iota((8, 128), 0)
        m0 = sub % 2 == 0
        m1 = (sub // 2) % 2 == 0
        lnc = jnp.where(m1, 1.0 / (C * _A), 1.0 / (C * _A * _A))

        def ln_tile(cvs, q, dsts, dsts2=None):
            ls = slice(128 * q, 128 * q + 128)
            cs = [[cv[8 * ab:8 * ab + 8] for cv in cvs] for ab in range(2)]
            c1 = _merge(_tree_sum(cs[0]), _tree_sum(cs[1]), m0, 1)
            c2 = _merge(_tree_sum([c * c for c in cs[0]]), _tree_sum([c * c for c in cs[1]]), m0, 1)
            e = _merge(c1, c2, m1, 2)
            f = (e + pltpu.roll(e, 4, 0)) * lnc
            v = pltpu.roll(f, 6, 0) - f * f
            rs = lax.rsqrt(jnp.maximum(v, 0.0) + _EPS)
            for ab in range(2):
                xn = _pack(jnp.concatenate(cs[ab], axis=0) * rs[ab:ab + 1, :])
                xn_ref[pl.ds(dsts[ab], 1), :, ls] = xn
                if dsts2 is not None:
                    xn_ref[pl.ds(dsts2[ab], 1), :, ls] = xn

        def setup(dw_ref, g_ref, b_ref):
            w1_ref = xbuf.at[3, 0, :, pl.ds(0, E)]
            w2t_ref = xbuf.at[3, 1, :, pl.ds(0, E)]
            small = [pltpu.make_async_copy(a, b, wsem.at[i]) for i, (a, b) in enumerate(
                [(dw_hbm, dw_ref), (w1_hbm, w1_ref), (w2t_hbm, w2t_ref), (g_hbm, g_ref), (b_hbm, b_ref)])]
            for cp in small[:2]:
                cp.start()
            rows_copy(1, 3, 0, 17, 1).start()
            rows_copy(0, 4, 1, 16, 1).start()
            for cp in small[2:]:
                cp.start()
            rows_copy(3, NP2, 0, 0, 0).start()
            rows_copy(3, NP2, 1, 0, 0).start()
            small[0].wait()

            vr_ref[0, ACC0:CL0] = jnp.zeros((E // 8, 8, 128), u32)
            dw = dw_ref[...].astype(f32)
            dif = _iota((8, C), 1) - _iota((8, C), 0)
            row = _iota((16, C), 0)
            col = _iota((16, C), 1)
            unit = jnp.where(col >= 48, 1, 0)
            itap = 2 * unit + ((col >> 3) & 1) - (row >> 3)
            tapid = jnp.where((col & 7) == (row & 7), 3 * itap + ((col - 48 * unit) >> 4), -9)
            for g in range(12):
                cl = jnp.zeros((16, C), f32)
                for t in range(9):
                    dwt = jnp.broadcast_to(dw[t // 3, t % 3:t % 3 + 1, :], (8, C))
                    dwc = jnp.sum(jnp.where(dif == 8 * g, dwt, 0.0), axis=1, keepdims=True)
                    dwb_ref[0, g, t] = jnp.broadcast_to(dwc, (8, 128))
                    cb = jnp.broadcast_to(dwc, (8, C))
                    cl = jnp.where(tapid == t, jnp.concatenate([cb, cb], axis=0), cl)
                vr_ref[0, CL0 + g, :, 0:C] = pltpu.bitcast(cl.astype(bf16), u32)

            for cp in small[1:]:
                cp.wait()
            w1f = w1_ref[...].astype(f32)
            w1c = (w1f - jnp.sum(w1f, axis=0, keepdims=True) * (1.0 / C)).astype(bf16)
            for i in range(3):
                eye = jnp.where(_iota((128, E), 0) + 128 * i == _iota((128, E), 1), 1.0, 0.0).astype(bf16)
                w1t = lax.dot_general(eye, w1c, (((1,), (1,)), ((), ())), preferred_element_type=f32)
                w1t_ref[64 * i:64 * i + 64, :] = pltpu.bitcast(w1t.astype(bf16), u32)
            w2s_ref[...] = pltpu.bitcast(w2t_ref[...], u32)
            gb_ref[0:1, :] = g_ref[...].astype(f32).reshape(1, E)
            gb_ref[1:2, :] = b_ref[...].astype(f32).reshape(1, E)

            xp[16, :, 0:8, :] = jnp.zeros((12, 8, W), bf16)
            rows_copy(1, 3, 0, 17, 1).wait()
            rows_copy(0, 4, 1, 16, 1).wait()
            shift_unit(xp.at[18], 0)
            shift_unit(xp.at[19], 1)
            for i, (un, da, db) in enumerate([(1, 10, 5), (0, 8, 9), (2, 0, 1)]):
                for q in range(NQ):
                    ln_tile(conv_round(2 - i, q, range(12)), q, (da, db), (2, 3) if i == 1 and q < 2 else None)
                shift_unit(xp.at[16 + un], un & 1)

        pl.run_scoped(setup, pltpu.VMEM((3, 3, C), bf16), pltpu.VMEM((E,), bf16), pltpu.VMEM((E,), bf16))

        nxt = lambda sl: jnp.where(sl == NB - 1, 0, sl + 1)
        NI = H // 32

        def block(g0, slots, prefetch):
            z = zs_ref[0]
            z1 = zs_ref[1]
            pend = []
            cur = []

            def conv_step(p, r):
                q = (r // 3 + 2) % 4
                pair = p + 1 + (r >= 6)
                cur.extend(conv_round(pair, q, range(4 * (r % 3), 4 * (r % 3) + 4)))
                if r % 3 == 2:
                    pend.append((p * NP + r + LN_LAG, list(cur), q, (2 * pair % 8 + z1, (2 * pair + 1) % 8 + z1)))
                    cur.clear()

            npair = 4 * len(slots)
            for p in range(npair):
                for r in range(NP):
                    gr = p * NP + r
                    c = r % NSUB
                    k = 2 * p + r // NSUB
                    last = gr == npair * NP - 1
                    if last:
                        conv_step(p, r)
                    if p % 4 == 0 and r == 3:
                        prefetch(p // 4)
                    while pend and pend[0][0] <= gr:
                        ln_tile(*pend.pop(0)[1:])
                    xn = pltpu.bitcast(xn_ref[k % 8 + z], bf16)
                    lhs = pltpu.bitcast(w1t_ref[MR // 2 * c:MR // 2 * (c + 1), :], bf16)
                    gl = _gelu2(jnp.dot(lhs, xn, preferred_element_type=f32))
                    if k % G2 in ST:
                        hs = (g0 + k // G2) * NST + ST.index(k % G2)
                        h_ref[pl.ds(hs, 1), MR // 2 * c:MR // 2 * (c + 1), :] = _pack(gl)
                    sq = gl * gl
                    for i in range(MR // 8):
                        ai = ACC0 + MR // 8 * c + i
                        sr = [sq[8 * i:8 * i + 8, 128 * q:128 * q + 128] for q in range(NQ)]
                        acc = ((pltpu.bitcast(vr_ref[0, ai], f32) + sr[0]) + sr[1]) + (sr[2] + sr[3])
                        vr_ref[0, ai] = pltpu.bitcast(acc, u32)
                    if not last:
                        conv_step(p, r)
                    if r == NP // 2 - 1:
                        shift_unit(xp.at[4 * slots[p // 4] + p % 4], (p + 3) % 2)
            for e in pend:
                ln_tile(*e[1:])


        def body_a(j, carry):
            wait_for(xp.at[pl.ds(8 * j, 8)], j)

            def prefetch(n):
                if n == 0:
                    start_slot(11 + 12 * j, 2 - 2 * j, 1 - j)
                    start_slot(15 + 12 * j, 3 - 2 * j, 1 - j)
                else:
                    start_slot(19 + 12 * j, 4 - 2 * j, 0)

            block(2 * j, [2 * j, 2 * j + 1], prefetch)
            return carry

        def body_b(jj, s0):
            slots = [s0]
            for _ in range(4):
                slots.append(nxt(slots[-1]))
            sem = 1 - (jj & 1)

            @pl.when(jj < NI - 1)
            def _():
                wait_for(xp.at[pl.ds(0, 16)], sem)

            @pl.when(jj == NI - 1)
            def _():
                wait_for(xp.at[pl.ds(0, 13)], sem)
                wait_for(xp.at[13, :, pl.ds(0, 8), :], sem)
                xp[4 * slots[3] + 1, :, 8:16, :] = jnp.zeros((12, 8, W), bf16)

            def prefetch(n):
                dst = slots[(n + 4) % 5]

                @pl.when(jj < NI - 1)
                def _():
                    start_slot(16 * jj + 19 + 4 * n, dst, 1 - sem, range(3) if n == 3 else range(8))

                if n == 3:
                    @pl.when(jj < NI - 2)
                    def _():
                        start_slot(16 * jj + 19 + 4 * n, dst, 1 - sem, range(3, 8))
                else:
                    @pl.when(jj == NI - 1)
                    def _():
                        x_copy(n, (S0 + n) % NB).start()

            block(4 * jj, slots[:4], prefetch)
            return slots[4]

        lax.fori_loop(0, 2, body_a, 0)
        lax.fori_loop(1, NI, body_b, jnp.int32(4))

        pdif = _iota((8, E), 1) - _iota((8, E), 0) + zs_ref[0]
        parts = []
        for i in range(E // 8):
            col = jnp.sum(pltpu.bitcast(vr_ref[0, ACC0 + i], f32), axis=1, keepdims=True)
            parts.append(jnp.where(pdif == 8 * i, jnp.broadcast_to(col, (8, E)), 0.0))
        ss = jnp.sum(_tree_sum(parts), axis=0, keepdims=True) * (_GS * _GS)
        gx = jnp.sqrt(ss + 1e-6)
        nx = gx / (jnp.sum(gx, axis=1, keepdims=True) * (1.0 / E) + 1e-6)
        s = (gb_ref[0:1, :] * nx + 1.0) * _GS
        w2t = pltpu.bitcast(w2s_ref[...], bf16).astype(f32)
        w2s_ref[...] = pltpu.bitcast((w2t * s).astype(bf16), u32)
        bias_ref[...] = jnp.broadcast_to(jnp.sum(w2t * gb_ref[1:2, :], axis=1, keepdims=True), (C, 128))

    pl.run_scoped(phase1, pltpu.VMEM((8, E), f32))

    def phase2(zv_ref):
        zv_ref[...] = jnp.zeros(zv_ref.shape, u32)
        vi = lambda q, k, i: (q * 6 + k) * 3 * (NR + 2) + i

        def o_copy(j, sl, r0, n):
            return pltpu.make_async_copy(xbuf.at[sl, pl.ds(r0, n)], o_hbm.at[pl.ds(j * G2 + r0, n)], osem.at[sl])

        z0 = zs_ref[0]
        lane = _iota((8, 128), 1) + z0
        sub = _iota((8, 128), 0) + z0
        m0 = (sub & 1) == 0
        m1 = (sub & 2) == 0
        m2 = sub < 4
        lnc = jnp.where(m2, 1.0 / (C * _A), 1.0 / (C * _A * _A))

        def shift_rows(xs, zv):
            for r in range(NR + 2):
                for k in range(6):
                    m = pltpu.bitcast(xbuf[xs, RC[0] - 1 + r, 16 * k:16 * k + 16, :], u32)
                    for q, vs in _shifted(m, lane):
                        for v in range(3):
                            vr_ref[zv, vi(q, k, 3 * r + v)] = vs[v]

        def conv_tile(q, zc, zw, zr):
            st = [None] * NR
            tok = yield None
            for g in range(12):
                w = [dwb_ref[zw, g, t] for t in range(9)]
                acc = [None] * NR
                for r in range(NR + 2):
                    for v in range(3):
                        x = vr_ref[zw, vi(q, g // 2, 3 * r + v)]
                        if v == 2:
                            x = x | tok
                        xf = pltpu.bitcast(x, bf16).astype(f32)[8 * (g % 2):8 * (g % 2) + 8]
                        for n in range(NR):
                            if 0 <= r - n <= 2:
                                t = xf * w[3 * (r - n) + v]
                                acc[n] = t if acc[n] is None else acc[n] + t
                for n in range(NR):
                    cv = acc[n]
                    st[n] = (cv, cv * cv) if st[n] is None else (st[n][0] + cv, st[n][1] + cv * cv)
                    cv_ref[zc, 12 * n + g] = cv
                tok = yield pltpu.bitcast((acc[0] + acc[1]) + acc[2], u32)
            half = lambda i: _merge(_merge(st[0][i], st[1][i], m0, 1), st[2][i] + pltpu.roll(st[2][i], 7, 0), m1, 2)
            f = _merge(half(0), half(1), m2, 4) * lnc
            v = pltpu.roll(f, 4, 0) - f * f
            cv_ref[zr, 36] = lax.rsqrt(jnp.maximum(v, 0.0) + _EPS)
            for n in range(NR):
                rs = cv_ref[zc, 36, n:n + 1, :]
                big_ref[pl.ds(8 + n + zc, 1), :, 128 * q:128 * q + 128] = _pack(
                    cv_ref[zc, 12 * n:12 * n + 12].reshape(C, 128) * rs)
            yield None

        x_copy(0, S0).wait()
        nxt = lambda sl: jnp.where(sl == NB - 1, 0, sl + 1)

        def body(j, xs):
            z = zs_ref[0]
            xs1 = nxt(xs)
            xs3 = nxt(nxt(xs1))

            @pl.when(j + 1 < NG2)
            def _():
                x_copy(j + 1, xs1).wait()

            @pl.when(j >= 2)
            def _():
                o_copy(j - 2, xs3, 0, G2).wait()

            @pl.when(j + 3 < NG2)
            def _():
                x_copy(j + 3, xs3).start()

            tiles = [conv_tile(q, z, zs_ref[2 + q], zs_ref[1]) for q in range(NQ)]
            for t in tiles:
                next(t)
            shift_rows(xs1, z)
            zv = zv_ref[...]
            state = dict(slot=0, piece=0, tok=None)

            def run_pieces(rel):
                res = None
                for _ in range(PLAN[state['slot']]):
                    t = tiles[state['piece'] // 12]
                    val = t.send(rel)
                    res = val if res is None else res | val
                    state['piece'] += 1
                    if state['piece'] % 12 == 0:
                        t.send(None)
                state['slot'] += 1
                state['tok'] = res

            def gate(d):
                if state['tok'] is None:
                    return d
                du = pltpu.bitcast(d[40:48, 384:512], u32) | (state['tok'] & zv)
                last = jnp.concatenate([d[40:48, 0:384], pltpu.bitcast(du, f32)], axis=1)
                return jnp.concatenate([d[0:40], last], axis=0)

            def fin(k, hr):
                for mc in range(2):
                    rs_ = slice(48 * mc, 48 * (mc + 1))
                    o = None
                    for kt in range(3):
                        d = jnp.dot(pltpu.bitcast(w2s_ref[24 * mc:24 * (mc + 1), 128 * kt:128 * kt + 128], bf16),
                                    pltpu.bitcast(hr(kt), bf16), preferred_element_type=f32)
                        rel = pltpu.bitcast(d[0:8, 0:128], u32) & zv
                        d = gate(d)
                        o = d if o is None else o + d
                        if kt == 2:
                            bias = jnp.concatenate([bias_ref[rs_, :]] * NQ, axis=1)
                            xbuf[xs, k, rs_, :] = (o + bias + xbuf[xs, k, rs_, :].astype(f32)).astype(bf16)
                        run_pieces(rel)

            def kept_rows(n, kt):
                return h_ref[j * NST + n, 64 * kt:64 * kt + 64, :]

            def temp_rows(n, kt):
                return jnp.concatenate([big_ref[4 * (n % 2) + z + r // 48, r % 48:r % 48 + 8, :]
                                        for r in range(64 * kt, 64 * kt + 64, 8)], axis=0)

            for op in P2ORD:
                n = int(op[1])
                if op[0] == 'M':
                    assert state['piece'] < 12
                    xn = pltpu.bitcast(big_ref[8 + n + z], bf16)
                    y = jnp.dot(pltpu.bitcast(w1t_ref[...], bf16), xn, preferred_element_type=f32)
                    big_ref[pl.ds(4 * (n % 2) + z, 4)] = _pack(_gelu2(y), 4)
                elif op[0] == 'S':
                    fin(ST[n], functools.partial(kept_rows, n))
                elif op[0] == 'F':
                    fin(RC[n], functools.partial(temp_rows, n))
                else:
                    o_copy(j, xs, n, int(op[2]) - n).start()
            assert state['piece'] == 12 * NQ
            return xs1

        lax.fori_loop(0, NG2, body, jnp.int32(S0))
        for j in range(NG2 - 2, NG2):
            o_copy(j, (j + S0) % NB, 0, G2).wait()

    pl.run_scoped(phase2, pltpu.VMEM((8, 128), u32))


@jax.jit
def pallas_standalone__modern_conv_block_convnext_v2__vision_kernel(x, dw, w1, w2, grn_gamma, grn_beta):
    xt = jnp.transpose(x, (0, 1, 3, 2)).reshape(H, C, W)
    x5 = xt.reshape(H // 2, 2, C // 8, 8, W)
    out = pl.pallas_call(
        _kernel,
        in_specs=[pl.BlockSpec(memory_space=pl.ANY)] * 7,
        out_specs=pl.BlockSpec(memory_space=pl.ANY),
        out_shape=jax.ShapeDtypeStruct((H, C, W), bf16),
        scratch_shapes=[
            pltpu.VMEM((NG2 * NST, E // 2, W), u32),
            pltpu.VMEM((NB, G2, C, W), bf16),
            pltpu.VMEM((8 + NR, C // 2, W), u32),
            pltpu.VMEM((1, NVR, 8, 128), u32),
            pltpu.VMEM((1, 12, 9, 8, 128), f32),
            pltpu.VMEM((1, 40, 8, 128), f32),
            pltpu.VMEM((E // 2, C), u32),
            pltpu.VMEM((C // 2, E), u32),
            pltpu.VMEM((C, 128), f32),
            pltpu.SMEM((6,), i32),
            pltpu.SemaphoreType.DMA((NB,)),
            pltpu.SemaphoreType.DMA((NB,)),
            pltpu.SemaphoreType.DMA((2,)),
            pltpu.SemaphoreType.DMA((5,)),
        ],
        compiler_params=pltpu.CompilerParams(vmem_limit_bytes=128 * 1024 * 1024,
                                             disable_bounds_checks=True),
    )(xt, x5, dw, w1, w2.T, grn_gamma, grn_beta)
    return jnp.transpose(out.reshape(1, H, C, W), (0, 1, 3, 2))
```

```python
import functools
import math

import jax
import jax.numpy as jnp
from jax import lax
import jax.experimental.pallas as pl
import jax.experimental.pallas.tpu as pltpu

H, W, C, E = 512, 512, 96, 384
NQ = W // 128
G2 = 8
NG2 = H // G2
RC = (2, 3, 4)
ST = tuple(k for k in range(G2) if k not in RC)
NST = len(ST)
NR = len(RC)
NVR = NQ * 6 * 3 * (NR + 2)
ACC0 = 2 * 12 * NQ * 3
CL0 = ACC0 + E // 8
NB = 5
S0 = 4
NSUB = 6
MR = E // NSUB
NP = 2 * NSUB
LN_LAG = 5
P2ORD = 'M0,M1,F0,M2,S0,F1,S1,o04,F2,S2,o46,S3,S4,o68'.split(',')
PLAN = [2, 2] + [1] * 44 + [0, 0]

_C1 = math.sqrt(2.0 / math.pi)
_A = (_C1 * 0.044715) ** (1.0 / 3.0)
_K = _C1 / _A
_GS = 0.5 / _A
_EPS = 1e-5 / (_A * _A)

f32 = jnp.float32
bf16 = jnp.bfloat16
u32 = jnp.uint32
i32 = jnp.int32


def _iota(shape, d):
    return lax.broadcasted_iota(i32, shape, d)


def _pack(y, n=1):
    return pltpu.bitcast(y.reshape(n, y.shape[0] // n, y.shape[1]).astype(bf16), u32)


def _gelu2(y):
    return y * (jnp.tanh(y * (y * y + _K)) + 1.0)


def _tree_sum(xs):
    xs = list(xs)
    while len(xs) > 1:
        xs = [xs[i] + xs[i + 1] for i in range(0, len(xs) - 1, 2)] + ([xs[-1]] if len(xs) % 2 else [])
    return xs[0]


def _merge(a, b, msk, sh):
    return jnp.where(msk, a, b) + pltpu.roll(jnp.where(msk, b, a), 8 - sh, 0)


def _shifted(m, lane):
    zz = jnp.zeros((8, 128), u32)
    mq = [m[:, 128 * q:128 * q + 128] for q in range(NQ)]
    for q in range(NQ):
        lq = jnp.where(lane == 127, mq[q - 1] if q > 0 else zz, mq[q])
        rq = jnp.where(lane == 0, mq[q + 1] if q + 1 < NQ else zz, mq[q])
        yield q, (pltpu.roll(lq, 1, 1), mq[q], pltpu.roll(rq, 127, 1))


def _kernel(x_hbm, x5_hbm, dw_hbm, w1_hbm, w2t_hbm, g_hbm, b_hbm, o_hbm,
            h_ref, xbuf, big_ref, vr_ref, dwb_ref, cv_ref, w1t_ref, w2s_ref, bias_ref, zs_ref,
            xsem, osem, psem, wsem):

    for i in range(6):
        zs_ref[i] = 0

    def x_copy(j, sl):
        return pltpu.make_async_copy(x_hbm.at[pl.ds(j * G2, G2)], xbuf.at[sl], xsem.at[sl])

    def phase1(gb_ref):
        xn_ref = big_ref
        vi = lambda u, g, q, v: ((u * 12 + g) * NQ + q) * 3 + v
        xp = xbuf.reshape(NB * 4, C // 8, 16, W)

        def rows_copy(u, n, half, i, sem):
            return pltpu.make_async_copy(x5_hbm.at[pl.ds(u - 1 + half, n), 1 - half],
                                         xp.at[pl.ds(i, n), :, pl.ds(8 * half, 8), :], psem.at[sem])

        def start_slot(u, sl, sem, rows=range(8)):
            for i in rows:
                pltpu.make_async_copy(x5_hbm.at[u + i // 2 - 1 + i % 2, 1 - i % 2],
                                      xp.at[4 * sl + i // 2, :, pl.ds(8 * (i % 2), 8), :], psem.at[sem]).start()

        def wait_for(buf, sem):
            pltpu.make_async_copy(buf, buf, psem.at[sem]).wait()

        lane = _iota((8, 128), 1)

        def shift_unit(xu_ref, u):
            for g in range(12):
                for q, vs in _shifted(pltpu.bitcast(xu_ref[g], u32), lane):
                    for v in range(3):
                        vr_ref[0, vi(u, g, q, v)] = vs[v]

        def conv_round(t, q, gs):
            cvs = []
            for g in gs:
                rhs = jnp.concatenate([vr_ref[0, vi(uu & 1, g, q, v)] for uu in (t, t + 1) for v in range(3)], axis=0)
                lhs = pltpu.bitcast(vr_ref[0, CL0 + g, :, 0:C], bf16)
                cvs.append(jnp.dot(lhs, pltpu.bitcast(rhs, bf16), preferred_element_type=f32))
            return cvs

        sub = _iota((8, 128), 0)
        m0 = sub % 2 == 0
        m1 = (sub // 2) % 2 == 0
        lnc = jnp.where(m1, 1.0 / (C * _A), 1.0 / (C * _A * _A))

        def ln_tile(cvs, q, dsts):
            ls = slice(128 * q, 128 * q + 128)
            cs = [[cv[8 * ab:8 * ab + 8] for cv in cvs] for ab in range(2)]
            c1 = _merge(_tree_sum(cs[0]), _tree_sum(cs[1]), m0, 1)
            c2 = _merge(_tree_sum([c * c for c in cs[0]]), _tree_sum([c * c for c in cs[1]]), m0, 1)
            e = _merge(c1, c2, m1, 2)
            f = (e + pltpu.roll(e, 4, 0)) * lnc
            v = pltpu.roll(f, 6, 0) - f * f
            rs = lax.rsqrt(jnp.maximum(v, 0.0) + _EPS)
            for ab in range(2):
                xn_ref[pl.ds(dsts[ab], 1), :, ls] = _pack(jnp.concatenate(cs[ab], axis=0) * rs[ab:ab + 1, :])

        def setup(dw_ref, g_ref, b_ref):
            w1_ref = xbuf.at[3, 0, :, pl.ds(0, E)]
            w2t_ref = xbuf.at[3, 1, :, pl.ds(0, E)]
            small = [pltpu.make_async_copy(a, b, wsem.at[i]) for i, (a, b) in enumerate(
                [(dw_hbm, dw_ref), (w1_hbm, w1_ref), (w2t_hbm, w2t_ref), (g_hbm, g_ref), (b_hbm, b_ref)])]
            for cp in small[:2]:
                cp.start()
            rows_copy(1, 2, 0, 17, 1).start()
            rows_copy(0, 3, 1, 16, 1).start()
            rows_copy(3, 4, 0, 0, 0).start()
            rows_copy(3, 4, 1, 0, 0).start()
            for cp in small[2:]:
                cp.start()
            small[0].wait()

            vr_ref[0, ACC0:CL0] = jnp.zeros((E // 8, 8, 128), u32)
            dw = dw_ref[...].astype(f32)
            dif = _iota((8, C), 1) - _iota((8, C), 0)
            row = _iota((16, C), 0)
            col = _iota((16, C), 1)
            unit = jnp.where(col >= 48, 1, 0)
            itap = 2 * unit + ((col >> 3) & 1) - (row >> 3)
            tapid = jnp.where((col & 7) == (row & 7), 3 * itap + ((col - 48 * unit) >> 4), -9)
            for g in range(12):
                cl = jnp.zeros((16, C), f32)
                for t in range(9):
                    dwt = jnp.broadcast_to(dw[t // 3, t % 3:t % 3 + 1, :], (8, C))
                    dwc = jnp.sum(jnp.where(dif == 8 * g, dwt, 0.0), axis=1, keepdims=True)
                    dwb_ref[0, g, t] = jnp.broadcast_to(dwc, (8, 128))
                    cb = jnp.broadcast_to(dwc, (8, C))
                    cl = jnp.where(tapid == t, jnp.concatenate([cb, cb], axis=0), cl)
                vr_ref[0, CL0 + g, :, 0:C] = pltpu.bitcast(cl.astype(bf16), u32)

            small[1].wait()
            w1f = w1_ref[...].astype(f32)
            w1c = (w1f - jnp.sum(w1f, axis=0, keepdims=True) * (1.0 / C)).astype(bf16)
            for i in range(3):
                eye = jnp.where(_iota((128, E), 0) + 128 * i == _iota((128, E), 1), 1.0, 0.0).astype(bf16)
                w1t = lax.dot_general(eye, w1c, (((1,), (1,)), ((), ())), preferred_element_type=f32)
                w1t_ref[64 * i:64 * i + 64, :] = pltpu.bitcast(w1t.astype(bf16), u32)

            xp[16, :, 0:8, :] = jnp.zeros((12, 8, W), bf16)
            rows_copy(1, 2, 0, 17, 1).wait()
            rows_copy(0, 3, 1, 16, 1).wait()
            shift_unit(xp.at[16], 0)
            shift_unit(xp.at[17], 1)
            for q in range(NQ):
                ln_tile(conv_round(0, q, range(12)), q, (0, 1))
            shift_unit(xp.at[18], 0)
            for q in range(2):
                ln_tile(conv_round(1, q, range(12)), q, (8, 9))

            for cp in small[2:]:
                cp.wait()
            w2s_ref[...] = pltpu.bitcast(w2t_ref[...], u32)
            gb_ref[0:1, :] = g_ref[...].astype(f32).reshape(1, E)
            gb_ref[1:2, :] = b_ref[...].astype(f32).reshape(1, E)

        pl.run_scoped(setup, pltpu.VMEM((3, 3, C), bf16), pltpu.VMEM((E,), bf16), pltpu.VMEM((E,), bf16))

        nxt = lambda sl: jnp.where(sl == NB - 1, 0, sl + 1)
        NI = H // 32

        def block(g0, slots, prefetch, keep=0):
            z = zs_ref[0]
            z1 = zs_ref[1]
            xslot = lambda k: k + keep if k in RC else k % 8
            pend = []
            cur = []

            def conv_step(p, r):
                q = (r // 3 + 2) % 4
                pair = p + 1 + (r >= 6)
                cur.extend(conv_round(pair, q, range(4 * (r % 3), 4 * (r % 3) + 4)))
                if r % 3 == 2:
                    pend.append((p * NP + r + LN_LAG, list(cur), q, (xslot(2 * pair) + z1, xslot(2 * pair + 1) + z1)))
                    cur.clear()

            npair = 4 * len(slots)
            for p in range(npair):
                for r in range(NP):
                    gr = p * NP + r
                    c = r % NSUB
                    k = 2 * p + r // NSUB
                    last = gr == npair * NP - 1
                    if last:
                        conv_step(p, r)
                    if p % 4 == 0 and r == 3:
                        prefetch(p // 4)
                    while pend and pend[0][0] <= gr:
                        ln_tile(*pend.pop(0)[1:])
                    xn = pltpu.bitcast(xn_ref[xslot(k) + z], bf16)
                    lhs = pltpu.bitcast(w1t_ref[MR // 2 * c:MR // 2 * (c + 1), :], bf16)
                    gl = _gelu2(jnp.dot(lhs, xn, preferred_element_type=f32))
                    if k % G2 in ST:
                        hs = (g0 + k // G2) * NST + ST.index(k % G2)
                        h_ref[pl.ds(hs, 1), MR // 2 * c:MR // 2 * (c + 1), :] = _pack(gl)
                    sq = gl * gl
                    for i in range(MR // 8):
                        ai = ACC0 + MR // 8 * c + i
                        sr = [sq[8 * i:8 * i + 8, 128 * q:128 * q + 128] for q in range(NQ)]
                        acc = ((pltpu.bitcast(vr_ref[0, ai], f32) + sr[0]) + sr[1]) + (sr[2] + sr[3])
                        vr_ref[0, ai] = pltpu.bitcast(acc, u32)
                    if not last:
                        conv_step(p, r)
                    if r == NP // 2 - 1:
                        shift_unit(xp.at[4 * slots[p // 4] + p % 4], (p + 3) % 2)
            for e in pend:
                ln_tile(*e[1:])

        def body_a(j, carry):
            wait_for(xp.at[pl.ds(4 * j, 4)], j & 1)

            def prefetch(n):
                @pl.when(j < 3)
                def _():
                    start_slot(7 + 4 * j, j + 1, 1 - (j & 1))
                start_slot(19 + 4 * j, jnp.where(j == 0, 4, j - 1), 2)

            block(j, [j], prefetch, jnp.where(j == 0, 8 - RC[0], 0))
            return carry

        def body_b(jj, s0):
            slots = [s0]
            for _ in range(4):
                slots.append(nxt(slots[-1]))
            sem = 2 * (jj & 1)

            @pl.when(jj < NI - 1)
            def _():
                wait_for(xp.at[pl.ds(0, 16)], sem)

            @pl.when(jj == NI - 1)
            def _():
                wait_for(xp.at[pl.ds(0, 13)], sem)
                wait_for(xp.at[13, :, pl.ds(0, 8), :], sem)
                xp[4 * slots[3] + 1, :, 8:16, :] = jnp.zeros((12, 8, W), bf16)

            def prefetch(n):
                dst = slots[(n + 4) % 5]

                @pl.when(jj < NI - 1)
                def _():
                    start_slot(16 * jj + 19 + 4 * n, dst, 2 - sem, range(3) if n == 3 else range(8))

                if n == 3:
                    @pl.when(jj < NI - 2)
                    def _():
                        start_slot(16 * jj + 19 + 4 * n, dst, 2 - sem, range(3, 8))
                else:
                    @pl.when(jj == NI - 1)
                    def _():
                        x_copy(n, (S0 + n) % NB).start()

            block(4 * jj, slots[:4], prefetch)
            return slots[4]

        lax.fori_loop(0, 4, body_a, 0)
        lax.fori_loop(1, NI, body_b, jnp.int32(4))

        pdif = _iota((8, E), 1) - _iota((8, E), 0) + zs_ref[0]
        parts = []
        for i in range(E // 8):
            col = jnp.sum(pltpu.bitcast(vr_ref[0, ACC0 + i], f32), axis=1, keepdims=True)
            parts.append(jnp.where(pdif == 8 * i, jnp.broadcast_to(col, (8, E)), 0.0))
        ss = jnp.sum(_tree_sum(parts), axis=0, keepdims=True) * (_GS * _GS)
        gx = jnp.sqrt(ss + 1e-6)
        nx = gx / (jnp.sum(gx, axis=1, keepdims=True) * (1.0 / E) + 1e-6)
        s = (gb_ref[0:1, :] * nx + 1.0) * _GS
        w2t = pltpu.bitcast(w2s_ref[...], bf16).astype(f32)
        w2s_ref[...] = pltpu.bitcast((w2t * s).astype(bf16), u32)
        bias_ref[...] = jnp.broadcast_to(jnp.sum(w2t * gb_ref[1:2, :], axis=1, keepdims=True), (C, 128))

    pl.run_scoped(phase1, pltpu.VMEM((8, E), f32))

    def phase2(zv_ref):
        zv_ref[...] = jnp.zeros(zv_ref.shape, u32)
        vi = lambda q, k, i: (q * 6 + k) * 3 * (NR + 2) + i

        def o_copy(j, sl, r0, n):
            return pltpu.make_async_copy(xbuf.at[sl, pl.ds(r0, n)], o_hbm.at[pl.ds(j * G2 + r0, n)], osem.at[sl])

        z0 = zs_ref[0]
        lane = _iota((8, 128), 1) + z0
        sub = _iota((8, 128), 0) + z0
        m0 = (sub & 1) == 0
        m1 = (sub & 2) == 0
        m2 = sub < 4
        lnc = jnp.where(m2, 1.0 / (C * _A), 1.0 / (C * _A * _A))

        def shift_rows(xs, zv):
            for r in range(NR + 2):
                for k in range(6):
                    m = pltpu.bitcast(xbuf[xs, RC[0] - 1 + r, 16 * k:16 * k + 16, :], u32)
                    for q, vs in _shifted(m, lane):
                        for v in range(3):
                            vr_ref[zv, vi(q, k, 3 * r + v)] = vs[v]

        def conv_tile(q, zc, zw, zr):
            st = [None] * NR
            tok = yield None
            for g in range(12):
                w = [dwb_ref[zw, g, t] for t in range(9)]
                acc = [None] * NR
                for r in range(NR + 2):
                    for v in range(3):
                        x = vr_ref[zw, vi(q, g // 2, 3 * r + v)]
                        if v == 2:
                            x = x | tok
                        xf = pltpu.bitcast(x, bf16).astype(f32)[8 * (g % 2):8 * (g % 2) + 8]
                        for n in range(NR):
                            if 0 <= r - n <= 2:
                                t = xf * w[3 * (r - n) + v]
                                acc[n] = t if acc[n] is None else acc[n] + t
                for n in range(NR):
                    cv = acc[n]
                    st[n] = (cv, cv * cv) if st[n] is None else (st[n][0] + cv, st[n][1] + cv * cv)
                    cv_ref[zc, 12 * n + g] = cv
                tok = yield pltpu.bitcast((acc[0] + acc[1]) + acc[2], u32)
            half = lambda i: _merge(_merge(st[0][i], st[1][i], m0, 1), st[2][i] + pltpu.roll(st[2][i], 7, 0), m1, 2)
            f = _merge(half(0), half(1), m2, 4) * lnc
            v = pltpu.roll(f, 4, 0) - f * f
            cv_ref[zr, 36] = lax.rsqrt(jnp.maximum(v, 0.0) + _EPS)
            for n in range(NR):
                rs = cv_ref[zc, 36, n:n + 1, :]
                big_ref[pl.ds(8 + n + zc, 1), :, 128 * q:128 * q + 128] = _pack(
                    cv_ref[zc, 12 * n:12 * n + 12].reshape(C, 128) * rs)
            yield None

        x_copy(0, S0).wait()
        nxt = lambda sl: jnp.where(sl == NB - 1, 0, sl + 1)

        def body(j, xs):
            z = zs_ref[0]
            xs1 = nxt(xs)
            xs3 = nxt(nxt(xs1))

            @pl.when(j + 1 < NG2)
            def _():
                x_copy(j + 1, xs1).wait()

            @pl.when(j >= 2)
            def _():
                o_copy(j - 2, xs3, 0, G2).wait()

            @pl.when(j + 3 < NG2)
            def _():
                x_copy(j + 3, xs3).start()

            tiles = [conv_tile(q, z, zs_ref[2 + q], zs_ref[1]) for q in range(NQ)]
            for t in tiles:
                next(t)
            shift_rows(xs1, z)
            zv = zv_ref[...]
            state = dict(slot=0, piece=0, tok=None)

            def run_pieces(rel):
                res = None
                for _ in range(PLAN[state['slot']]):
                    t = tiles[state['piece'] // 12]
                    val = t.send(rel)
                    res = val if res is None else res | val
                    state['piece'] += 1
                    if state['piece'] % 12 == 0:
                        t.send(None)
                state['slot'] += 1
                state['tok'] = res

            def gate(d):
                if state['tok'] is None:
                    return d
                du = pltpu.bitcast(d[40:48, 384:512], u32) | (state['tok'] & zv)
                last = jnp.concatenate([d[40:48, 0:384], pltpu.bitcast(du, f32)], axis=1)
                return jnp.concatenate([d[0:40], last], axis=0)

            def fin(k, hr):
                for mc in range(2):
                    rs_ = slice(48 * mc, 48 * (mc + 1))
                    o = None
                    for kt in range(3):
                        d = jnp.dot(pltpu.bitcast(w2s_ref[24 * mc:24 * (mc + 1), 128 * kt:128 * kt + 128], bf16),
                                    pltpu.bitcast(hr(kt), bf16), preferred_element_type=f32)
                        rel = pltpu.bitcast(d[0:8, 0:128], u32) & zv
                        d = gate(d)
                        o = d if o is None else o + d
                        if kt == 2:
                            bias = jnp.concatenate([bias_ref[rs_, :]] * NQ, axis=1)
                            xbuf[xs, k, rs_, :] = (o + bias + xbuf[xs, k, rs_, :].astype(f32)).astype(bf16)
                        run_pieces(rel)

            def kept_rows(n, kt):
                return h_ref[j * NST + n, 64 * kt:64 * kt + 64, :]

            def temp_rows(n, kt):
                return jnp.concatenate([big_ref[4 * (n % 2) + z + r // 48, r % 48:r % 48 + 8, :]
                                        for r in range(64 * kt, 64 * kt + 64, 8)], axis=0)

            for op in P2ORD:
                n = int(op[1])
                if op[0] == 'M':
                    assert state['piece'] < 12
                    xn = pltpu.bitcast(big_ref[8 + n + z], bf16)
                    y = jnp.dot(pltpu.bitcast(w1t_ref[...], bf16), xn, preferred_element_type=f32)
                    big_ref[pl.ds(4 * (n % 2) + z, 4)] = _pack(_gelu2(y), 4)
                elif op[0] == 'S':
                    fin(ST[n], functools.partial(kept_rows, n))
                elif op[0] == 'F':
                    fin(RC[n], functools.partial(temp_rows, n))
                else:
                    o_copy(j, xs, n, int(op[2]) - n).start()
            assert state['piece'] == 12 * NQ
            return xs1

        lax.fori_loop(0, NG2, body, jnp.int32(S0))
        for j in range(NG2 - 2, NG2):
            o_copy(j, (j + S0) % NB, 0, G2).wait()

    pl.run_scoped(phase2, pltpu.VMEM((8, 128), u32))


@jax.jit
def pallas_standalone__modern_conv_block_convnext_v2__vision_kernel(x, dw, w1, w2, grn_gamma, grn_beta):
    xt = jnp.transpose(x, (0, 1, 3, 2)).reshape(H, C, W)
    x5 = xt.reshape(H // 2, 2, C // 8, 8, W)
    out = pl.pallas_call(
        _kernel,
        in_specs=[pl.BlockSpec(memory_space=pl.ANY)] * 7,
        out_specs=pl.BlockSpec(memory_space=pl.ANY),
        out_shape=jax.ShapeDtypeStruct((H, C, W), bf16),
        scratch_shapes=[
            pltpu.VMEM((NG2 * NST, E // 2, W), u32),
            pltpu.VMEM((NB, G2, C, W), bf16),
            pltpu.VMEM((8 + NR, C // 2, W), u32),
            pltpu.VMEM((1, NVR, 8, 128), u32),
            pltpu.VMEM((1, 12, 9, 8, 128), f32),
            pltpu.VMEM((1, 40, 8, 128), f32),
            pltpu.VMEM((E // 2, C), u32),
            pltpu.VMEM((C // 2, E), u32),
            pltpu.VMEM((C, 128), f32),
            pltpu.SMEM((6,), i32),
            pltpu.SemaphoreType.DMA((NB,)),
            pltpu.SemaphoreType.DMA((NB,)),
            pltpu.SemaphoreType.DMA((3,)),
            pltpu.SemaphoreType.DMA((5,)),
        ],
        compiler_params=pltpu.CompilerParams(vmem_limit_bytes=128 * 1024 * 1024,
                                             disable_bounds_checks=True),
    )(xt, x5, dw, w1, w2.T, grn_gamma, grn_beta)
    return jnp.transpose(out.reshape(1, H, C, W), (0, 1, 3, 2))
```

```python
import functools
import math

import jax
import jax.numpy as jnp
from jax import lax
import jax.experimental.pallas as pl
import jax.experimental.pallas.tpu as pltpu

H, W, C, E = 512, 512, 96, 384
NQ = W // 128
G2 = 8
NG2 = H // G2
RC = (2, 3, 4)
ST = tuple(k for k in range(G2) if k not in RC)
NST = len(ST)
NR = len(RC)
NVR = NQ * 6 * 3 * (NR + 2)
ACC0 = 2 * 12 * NQ * 3
CL0 = ACC0 + E // 8
NB = 5
S0 = 4
NSUB = 4
MR = E // NSUB
NP = 2 * NSUB
LN_LAG = 3
P2ORD = 'M0,M1,F0,M2,S0,F1,S1,o04,F2,S2,o46,S3,S4,o68'.split(',')
PLAN = [2, 2] + [1] * 44 + [0, 0]

_C1 = math.sqrt(2.0 / math.pi)
_A = (_C1 * 0.044715) ** (1.0 / 3.0)
_K = _C1 / _A
_GS = 0.5 / _A
_EPS = 1e-5 / (_A * _A)

f32 = jnp.float32
bf16 = jnp.bfloat16
u32 = jnp.uint32
i32 = jnp.int32


def _iota(shape, d):
    return lax.broadcasted_iota(i32, shape, d)


def _pack(y, n=1):
    return pltpu.bitcast(y.reshape(n, y.shape[0] // n, y.shape[1]).astype(bf16), u32)


def _gelu2(y):
    return y * (jnp.tanh(y * (y * y + _K)) + 1.0)


def _tree_sum(xs):
    xs = list(xs)
    while len(xs) > 1:
        xs = [xs[i] + xs[i + 1] for i in range(0, len(xs) - 1, 2)] + ([xs[-1]] if len(xs) % 2 else [])
    return xs[0]


def _merge(a, b, msk, sh):
    return jnp.where(msk, a, b) + pltpu.roll(jnp.where(msk, b, a), 8 - sh, 0)


def _shifted(m, lane):
    zz = jnp.zeros((8, 128), u32)
    mq = [m[:, 128 * q:128 * q + 128] for q in range(NQ)]
    for q in range(NQ):
        lq = jnp.where(lane == 127, mq[q - 1] if q > 0 else zz, mq[q])
        rq = jnp.where(lane == 0, mq[q + 1] if q + 1 < NQ else zz, mq[q])
        yield q, (pltpu.roll(lq, 1, 1), mq[q], pltpu.roll(rq, 127, 1))


def _kernel(x_hbm, x5_hbm, dw_hbm, w1_hbm, w2t_hbm, g_hbm, b_hbm, o_hbm,
            h_ref, xbuf, big_ref, vr_ref, dwb_ref, cv_ref, w1t_ref, w2s_ref, bias_ref, zs_ref,
            xsem, osem, psem, wsem):

    for i in range(6):
        zs_ref[i] = 0

    def x_copy(j, sl):
        return pltpu.make_async_copy(x_hbm.at[pl.ds(j * G2, G2)], xbuf.at[sl], xsem.at[sl])

    def phase1(gb_ref):
        xn_ref = big_ref
        vi = lambda u, g, q, v: ((u * 12 + g) * NQ + q) * 3 + v
        xp = xbuf.reshape(NB * 4, C // 8, 16, W)

        def rows_copy(u, n, half, i, sem):
            return pltpu.make_async_copy(x5_hbm.at[pl.ds(u - 1 + half, n), 1 - half],
                                         xp.at[pl.ds(i, n), :, pl.ds(8 * half, 8), :], psem.at[sem])

        def start_slot(u, sl, sem, rows=range(8)):
            for i in rows:
                pltpu.make_async_copy(x5_hbm.at[u + i // 2 - 1 + i % 2, 1 - i % 2],
                                      xp.at[4 * sl + i // 2, :, pl.ds(8 * (i % 2), 8), :], psem.at[sem]).start()

        def wait_for(buf, sem):
            pltpu.make_async_copy(buf, buf, psem.at[sem]).wait()

        lane = _iota((8, 128), 1)

        def shift_unit(xu_ref, u):
            for g in range(12):
                for q, vs in _shifted(pltpu.bitcast(xu_ref[g], u32), lane):
                    for v in range(3):
                        vr_ref[0, vi(u, g, q, v)] = vs[v]

        def conv_round(t, q, gs):
            cvs = []
            for g in gs:
                rhs = jnp.concatenate([vr_ref[0, vi(uu & 1, g, q, v)] for uu in (t, t + 1) for v in range(3)], axis=0)
                lhs = pltpu.bitcast(vr_ref[0, CL0 + g, :, 0:C], bf16)
                cvs.append(jnp.dot(lhs, pltpu.bitcast(rhs, bf16), preferred_element_type=f32))
            return cvs

        sub = _iota((8, 128), 0)
        m0 = sub % 2 == 0
        m1 = (sub // 2) % 2 == 0
        lnc = jnp.where(m1, 1.0 / (C * _A), 1.0 / (C * _A * _A))

        def ln_tile(cvs, q, dsts):
            ls = slice(128 * q, 128 * q + 128)
            cs = [[cv[8 * ab:8 * ab + 8] for cv in cvs] for ab in range(2)]
            c1 = _merge(_tree_sum(cs[0]), _tree_sum(cs[1]), m0, 1)
            c2 = _merge(_tree_sum([c * c for c in cs[0]]), _tree_sum([c * c for c in cs[1]]), m0, 1)
            e = _merge(c1, c2, m1, 2)
            f = (e + pltpu.roll(e, 4, 0)) * lnc
            v = pltpu.roll(f, 6, 0) - f * f
            rs = lax.rsqrt(jnp.maximum(v, 0.0) + _EPS)
            for ab in range(2):
                xn_ref[pl.ds(dsts[ab], 1), :, ls] = _pack(jnp.concatenate(cs[ab], axis=0) * rs[ab:ab + 1, :])

        def setup(dw_ref, g_ref, b_ref):
            w1_ref = xbuf.at[3, 0, :, pl.ds(0, E)]
            w2t_ref = xbuf.at[3, 1, :, pl.ds(0, E)]
            small = [pltpu.make_async_copy(a, b, wsem.at[i]) for i, (a, b) in enumerate(
                [(dw_hbm, dw_ref), (w1_hbm, w1_ref), (w2t_hbm, w2t_ref), (g_hbm, g_ref), (b_hbm, b_ref)])]
            for cp in small[:2]:
                cp.start()
            rows_copy(1, 2, 0, 17, 1).start()
            rows_copy(0, 3, 1, 16, 1).start()
            rows_copy(3, 4, 0, 0, 0).start()
            rows_copy(3, 4, 1, 0, 0).start()
            for cp in small[2:]:
                cp.start()
            small[0].wait()

            vr_ref[0, ACC0:CL0] = jnp.zeros((E // 8, 8, 128), u32)
            dw = dw_ref[...].astype(f32)
            dif = _iota((8, C), 1) - _iota((8, C), 0)
            row = _iota((16, C), 0)
            col = _iota((16, C), 1)
            unit = jnp.where(col >= 48, 1, 0)
            itap = 2 * unit + ((col >> 3) & 1) - (row >> 3)
            tapid = jnp.where((col & 7) == (row & 7), 3 * itap + ((col - 48 * unit) >> 4), -9)
            for g in range(12):
                cl = jnp.zeros((16, C), f32)
                for t in range(9):
                    dwt = jnp.broadcast_to(dw[t // 3, t % 3:t % 3 + 1, :], (8, C))
                    dwc = jnp.sum(jnp.where(dif == 8 * g, dwt, 0.0), axis=1, keepdims=True)
                    dwb_ref[0, g, t] = jnp.broadcast_to(dwc, (8, 128))
                    cb = jnp.broadcast_to(dwc, (8, C))
                    cl = jnp.where(tapid == t, jnp.concatenate([cb, cb], axis=0), cl)
                vr_ref[0, CL0 + g, :, 0:C] = pltpu.bitcast(cl.astype(bf16), u32)

            small[1].wait()
            w1f = w1_ref[...].astype(f32)
            w1c = (w1f - jnp.sum(w1f, axis=0, keepdims=True) * (1.0 / C)).astype(bf16)
            for i in range(3):
                eye = jnp.where(_iota((128, E), 0) + 128 * i == _iota((128, E), 1), 1.0, 0.0).astype(bf16)
                w1t = lax.dot_general(eye, w1c, (((1,), (1,)), ((), ())), preferred_element_type=f32)
                w1t_ref[64 * i:64 * i + 64, :] = pltpu.bitcast(w1t.astype(bf16), u32)

            xp[16, :, 0:8, :] = jnp.zeros((12, 8, W), bf16)
            rows_copy(1, 2, 0, 17, 1).wait()
            rows_copy(0, 3, 1, 16, 1).wait()
            shift_unit(xp.at[16], 0)
            shift_unit(xp.at[17], 1)
            for q in range(NQ):
                ln_tile(conv_round(0, q, range(12)), q, (0, 1))
            shift_unit(xp.at[18], 0)
            for q in range(2):
                ln_tile(conv_round(1, q, range(12)), q, (8, 9))

            for cp in small[2:]:
                cp.wait()
            w2s_ref[...] = pltpu.bitcast(w2t_ref[...], u32)
            gb_ref[0:1, :] = g_ref[...].astype(f32).reshape(1, E)
            gb_ref[1:2, :] = b_ref[...].astype(f32).reshape(1, E)

        pl.run_scoped(setup, pltpu.VMEM((3, 3, C), bf16), pltpu.VMEM((E,), bf16), pltpu.VMEM((E,), bf16))

        nxt = lambda sl: jnp.where(sl == NB - 1, 0, sl + 1)
        NI = H // 32

        def block(g0, slots, prefetch, keep=0):
            z = zs_ref[0]
            z1 = zs_ref[1]
            xslot = lambda k: k + keep if k in RC else k % 8
            pend = []
            cur = []

            def conv_step(p, r):
                for rr in range(12):
                    if rr * NP // 12 != r:
                        continue
                    q = (rr // 3 + 2) % 4
                    pair = p + 1 + (rr >= 6)
                    cur.extend(conv_round(pair, q, range(4 * (rr % 3), 4 * (rr % 3) + 4)))
                    if rr % 3 == 2:
                        pend.append((p * NP + r + LN_LAG, list(cur), q, (xslot(2 * pair) + z1, xslot(2 * pair + 1) + z1)))
                        cur.clear()

            npair = 4 * len(slots)
            for p in range(npair):
                for r in range(NP):
                    gr = p * NP + r
                    c = r % NSUB
                    k = 2 * p + r // NSUB
                    last = gr == npair * NP - 1
                    if last:
                        conv_step(p, r)
                    if p % 4 == 0 and r == 2:
                        prefetch(p // 4)
                    while pend and pend[0][0] <= gr:
                        ln_tile(*pend.pop(0)[1:])
                    xn = pltpu.bitcast(xn_ref[xslot(k) + z], bf16)
                    lhs = pltpu.bitcast(w1t_ref[MR // 2 * c:MR // 2 * (c + 1), :], bf16)
                    gl = _gelu2(jnp.dot(lhs, xn, preferred_element_type=f32))
                    if k % G2 in ST:
                        hs = (g0 + k // G2) * NST + ST.index(k % G2)
                        h_ref[pl.ds(hs, 1), MR // 2 * c:MR // 2 * (c + 1), :] = _pack(gl)
                    sq = gl * gl
                    for i in range(MR // 8):
                        ai = ACC0 + MR // 8 * c + i
                        sr = [sq[8 * i:8 * i + 8, 128 * q:128 * q + 128] for q in range(NQ)]
                        acc = ((pltpu.bitcast(vr_ref[0, ai], f32) + sr[0]) + sr[1]) + (sr[2] + sr[3])
                        vr_ref[0, ai] = pltpu.bitcast(acc, u32)
                    if not last:
                        conv_step(p, r)
                    if r == NP // 2 - 1:
                        shift_unit(xp.at[4 * slots[p // 4] + p % 4], (p + 3) % 2)
            for e in pend:
                ln_tile(*e[1:])

        def body_a(j, carry):
            wait_for(xp.at[pl.ds(4 * j, 4)], j & 1)

            def prefetch(n):
                @pl.when(j < 3)
                def _():
                    start_slot(7 + 4 * j, j + 1, 1 - (j & 1))
                start_slot(19 + 4 * j, jnp.where(j == 0, 4, j - 1), 2)

            block(j, [j], prefetch, jnp.where(j == 0, 8 - RC[0], 0))
            return carry

        def body_b(jj, s0):
            slots = [s0]
            for _ in range(4):
                slots.append(nxt(slots[-1]))
            sem = 2 * (jj & 1)

            @pl.when(jj < NI - 1)
            def _():
                wait_for(xp.at[pl.ds(0, 16)], sem)

            @pl.when(jj == NI - 1)
            def _():
                wait_for(xp.at[pl.ds(0, 13)], sem)
                wait_for(xp.at[13, :, pl.ds(0, 8), :], sem)
                xp[4 * slots[3] + 1, :, 8:16, :] = jnp.zeros((12, 8, W), bf16)

            def prefetch(n):
                dst = slots[(n + 4) % 5]

                @pl.when(jj < NI - 1)
                def _():
                    start_slot(16 * jj + 19 + 4 * n, dst, 2 - sem, range(3) if n == 3 else range(8))

                if n == 3:
                    @pl.when(jj < NI - 2)
                    def _():
                        start_slot(16 * jj + 19 + 4 * n, dst, 2 - sem, range(3, 8))
                else:
                    @pl.when(jj == NI - 1)
                    def _():
                        x_copy(n, (S0 + n) % NB).start()

            block(4 * jj, slots[:4], prefetch)
            return slots[4]

        lax.fori_loop(0, 4, body_a, 0)
        lax.fori_loop(1, NI, body_b, jnp.int32(4))

        pdif = _iota((8, E), 1) - _iota((8, E), 0) + zs_ref[0]
        parts = []
        for i in range(E // 8):
            col = jnp.sum(pltpu.bitcast(vr_ref[0, ACC0 + i], f32), axis=1, keepdims=True)
            parts.append(jnp.where(pdif == 8 * i, jnp.broadcast_to(col, (8, E)), 0.0))
        ss = jnp.sum(_tree_sum(parts), axis=0, keepdims=True) * (_GS * _GS)
        gx = jnp.sqrt(ss + 1e-6)
        nx = gx / (jnp.sum(gx, axis=1, keepdims=True) * (1.0 / E) + 1e-6)
        s = (gb_ref[0:1, :] * nx + 1.0) * _GS
        w2t = pltpu.bitcast(w2s_ref[...], bf16).astype(f32)
        w2s_ref[...] = pltpu.bitcast((w2t * s).astype(bf16), u32)
        bias_ref[...] = jnp.broadcast_to(jnp.sum(w2t * gb_ref[1:2, :], axis=1, keepdims=True), (C, 128))

    pl.run_scoped(phase1, pltpu.VMEM((8, E), f32))

    def phase2(zv_ref):
        zv_ref[...] = jnp.zeros(zv_ref.shape, u32)
        vi = lambda q, k, i: (q * 6 + k) * 3 * (NR + 2) + i

        def o_copy(j, sl, r0, n):
            return pltpu.make_async_copy(xbuf.at[sl, pl.ds(r0, n)], o_hbm.at[pl.ds(j * G2 + r0, n)], osem.at[sl])

        z0 = zs_ref[0]
        lane = _iota((8, 128), 1) + z0
        sub = _iota((8, 128), 0) + z0
        m0 = (sub & 1) == 0
        m1 = (sub & 2) == 0
        m2 = sub < 4
        lnc = jnp.where(m2, 1.0 / (C * _A), 1.0 / (C * _A * _A))

        def shift_rows(xs, zv):
            for r in range(NR + 2):
                for k in range(6):
                    m = pltpu.bitcast(xbuf[xs, RC[0] - 1 + r, 16 * k:16 * k + 16, :], u32)
                    for q, vs in _shifted(m, lane):
                        for v in range(3):
                            vr_ref[zv, vi(q, k, 3 * r + v)] = vs[v]

        def conv_tile(q, zc, zw, zr):
            st = [None] * NR
            tok = yield None
            for g in range(12):
                w = [dwb_ref[zw, g, t] for t in range(9)]
                acc = [None] * NR
                for r in range(NR + 2):
                    for v in range(3):
                        x = vr_ref[zw, vi(q, g // 2, 3 * r + v)]
                        if v == 2:
                            x = x | tok
                        xf = pltpu.bitcast(x, bf16).astype(f32)[8 * (g % 2):8 * (g % 2) + 8]
                        for n in range(NR):
                            if 0 <= r - n <= 2:
                                t = xf * w[3 * (r - n) + v]
                                acc[n] = t if acc[n] is None else acc[n] + t
                for n in range(NR):
                    cv = acc[n]
                    st[n] = (cv, cv * cv) if st[n] is None else (st[n][0] + cv, st[n][1] + cv * cv)
                    cv_ref[zc, 12 * n + g] = cv
                tok = yield pltpu.bitcast((acc[0] + acc[1]) + acc[2], u32)
            half = lambda i: _merge(_merge(st[0][i], st[1][i], m0, 1), st[2][i] + pltpu.roll(st[2][i], 7, 0), m1, 2)
            f = _merge(half(0), half(1), m2, 4) * lnc
            v = pltpu.roll(f, 4, 0) - f * f
            cv_ref[zr, 36] = lax.rsqrt(jnp.maximum(v, 0.0) + _EPS)
            for n in range(NR):
                rs = cv_ref[zc, 36, n:n + 1, :]
                big_ref[pl.ds(8 + n + zc, 1), :, 128 * q:128 * q + 128] = _pack(
                    cv_ref[zc, 12 * n:12 * n + 12].reshape(C, 128) * rs)
            yield None

        x_copy(0, S0).wait()
        nxt = lambda sl: jnp.where(sl == NB - 1, 0, sl + 1)

        def body(j, xs):
            z = zs_ref[0]
            xs1 = nxt(xs)
            xs3 = nxt(nxt(xs1))

            @pl.when(j + 1 < NG2)
            def _():
                x_copy(j + 1, xs1).wait()

            @pl.when(j >= 2)
            def _():
                o_copy(j - 2, xs3, 0, G2).wait()

            @pl.when(j + 3 < NG2)
            def _():
                x_copy(j + 3, xs3).start()

            tiles = [conv_tile(q, z, zs_ref[2 + q], zs_ref[1]) for q in range(NQ)]
            for t in tiles:
                next(t)
            shift_rows(xs1, z)
            zv = zv_ref[...]
            state = dict(slot=0, piece=0, tok=None)

            def run_pieces(rel):
                res = None
                for _ in range(PLAN[state['slot']]):
                    t = tiles[state['piece'] // 12]
                    val = t.send(rel)
                    res = val if res is None else res | val
                    state['piece'] += 1
                    if state['piece'] % 12 == 0:
                        t.send(None)
                state['slot'] += 1
                state['tok'] = res

            def gate(d):
                if state['tok'] is None:
                    return d
                du = pltpu.bitcast(d[40:48, 384:512], u32) | (state['tok'] & zv)
                last = jnp.concatenate([d[40:48, 0:384], pltpu.bitcast(du, f32)], axis=1)
                return jnp.concatenate([d[0:40], last], axis=0)

            def fin(k, hr):
                for mc in range(2):
                    rs_ = slice(48 * mc, 48 * (mc + 1))
                    o = None
                    for kt in range(3):
                        d = jnp.dot(pltpu.bitcast(w2s_ref[24 * mc:24 * (mc + 1), 128 * kt:128 * kt + 128], bf16),
                                    pltpu.bitcast(hr(kt), bf16), preferred_element_type=f32)
                        rel = pltpu.bitcast(d[0:8, 0:128], u32) & zv
                        d = gate(d)
                        o = d if o is None else o + d
                        if kt == 2:
                            bias = jnp.concatenate([bias_ref[rs_, :]] * NQ, axis=1)
                            xbuf[xs, k, rs_, :] = (o + bias + xbuf[xs, k, rs_, :].astype(f32)).astype(bf16)
                        run_pieces(rel)

            def kept_rows(n, kt):
                return h_ref[j * NST + n, 64 * kt:64 * kt + 64, :]

            def temp_rows(n, kt):
                return jnp.concatenate([big_ref[4 * (n % 2) + z + r // 48, r % 48:r % 48 + 8, :]
                                        for r in range(64 * kt, 64 * kt + 64, 8)], axis=0)

            for op in P2ORD:
                n = int(op[1])
                if op[0] == 'M':
                    assert state['piece'] < 12
                    xn = pltpu.bitcast(big_ref[8 + n + z], bf16)
                    y = jnp.dot(pltpu.bitcast(w1t_ref[...], bf16), xn, preferred_element_type=f32)
                    big_ref[pl.ds(4 * (n % 2) + z, 4)] = _pack(_gelu2(y), 4)
                elif op[0] == 'S':
                    fin(ST[n], functools.partial(kept_rows, n))
                elif op[0] == 'F':
                    fin(RC[n], functools.partial(temp_rows, n))
                else:
                    o_copy(j, xs, n, int(op[2]) - n).start()
            assert state['piece'] == 12 * NQ
            return xs1

        lax.fori_loop(0, NG2, body, jnp.int32(S0))
        for j in range(NG2 - 2, NG2):
            o_copy(j, (j + S0) % NB, 0, G2).wait()

    pl.run_scoped(phase2, pltpu.VMEM((8, 128), u32))


@jax.jit
def pallas_standalone__modern_conv_block_convnext_v2__vision_kernel(x, dw, w1, w2, grn_gamma, grn_beta):
    xt = jnp.transpose(x, (0, 1, 3, 2)).reshape(H, C, W)
    x5 = xt.reshape(H // 2, 2, C // 8, 8, W)
    out = pl.pallas_call(
        _kernel,
        in_specs=[pl.BlockSpec(memory_space=pl.ANY)] * 7,
        out_specs=pl.BlockSpec(memory_space=pl.ANY),
        out_shape=jax.ShapeDtypeStruct((H, C, W), bf16),
        scratch_shapes=[
            pltpu.VMEM((NG2 * NST, E // 2, W), u32),
            pltpu.VMEM((NB, G2, C, W), bf16),
            pltpu.VMEM((8 + NR, C // 2, W), u32),
            pltpu.VMEM((1, NVR, 8, 128), u32),
            pltpu.VMEM((1, 12, 9, 8, 128), f32),
            pltpu.VMEM((1, 40, 8, 128), f32),
            pltpu.VMEM((E // 2, C), u32),
            pltpu.VMEM((C // 2, E), u32),
            pltpu.VMEM((C, 128), f32),
            pltpu.SMEM((6,), i32),
            pltpu.SemaphoreType.DMA((NB,)),
            pltpu.SemaphoreType.DMA((NB,)),
            pltpu.SemaphoreType.DMA((3,)),
            pltpu.SemaphoreType.DMA((5,)),
        ],
        compiler_params=pltpu.CompilerParams(vmem_limit_bytes=128 * 1024 * 1024,
                                             disable_bounds_checks=True),
    )(xt, x5, dw, w1, w2.T, grn_gamma, grn_beta)
    return jnp.transpose(out.reshape(1, H, C, W), (0, 1, 3, 2))
```

```python
import functools
import math

import jax
import jax.numpy as jnp
from jax import lax
import jax.experimental.pallas as pl
import jax.experimental.pallas.tpu as pltpu

H, W, C, E = 512, 512, 96, 384
NQ = W // 128
G2 = 8
NG2 = H // G2
RC = (2, 3, 4)
ST = tuple(k for k in range(G2) if k not in RC)
NST = len(ST)
NR = len(RC)
NVR = NQ * 6 * 3 * (NR + 2)
ACC0 = 2 * 12 * NQ * 3
CL0 = ACC0 + E // 8
NB = 5
S0 = 4
CH = (128, 64, 128, 64)
RD = (2, 1, 2, 1) * 2
NSUB = len(CH)
NP = 2 * NSUB
LN_LAG = 3
P2ORD = 'M0,M1,F0,M2,S0,F1,S1,o04,F2,S2,o46,S3,S4,o68'.split(',')
PLAN = [2, 2] + [1] * 44 + [0, 0]

_C1 = math.sqrt(2.0 / math.pi)
_A = (_C1 * 0.044715) ** (1.0 / 3.0)
_K = _C1 / _A
_GS = 0.5 / _A
_EPS = 1e-5 / (_A * _A)

f32 = jnp.float32
bf16 = jnp.bfloat16
u32 = jnp.uint32
i32 = jnp.int32


def _iota(shape, d):
    return lax.broadcasted_iota(i32, shape, d)


def _pack(y, n=1):
    return pltpu.bitcast(y.reshape(n, y.shape[0] // n, y.shape[1]).astype(bf16), u32)


def _gelu2(y):
    return y * (jnp.tanh(y * (y * y + _K)) + 1.0)


def _tree_sum(xs):
    xs = list(xs)
    while len(xs) > 1:
        xs = [xs[i] + xs[i + 1] for i in range(0, len(xs) - 1, 2)] + ([xs[-1]] if len(xs) % 2 else [])
    return xs[0]


def _merge(a, b, msk, sh):
    return jnp.where(msk, a, b) + pltpu.roll(jnp.where(msk, b, a), 8 - sh, 0)


def _shifted(m, lane):
    zz = jnp.zeros((8, 128), u32)
    mq = [m[:, 128 * q:128 * q + 128] for q in range(NQ)]
    for q in range(NQ):
        lq = jnp.where(lane == 127, mq[q - 1] if q > 0 else zz, mq[q])
        rq = jnp.where(lane == 0, mq[q + 1] if q + 1 < NQ else zz, mq[q])
        yield q, (pltpu.roll(lq, 1, 1), mq[q], pltpu.roll(rq, 127, 1))


def _kernel(x_hbm, x5_hbm, dw_hbm, w1_hbm, w2t_hbm, g_hbm, b_hbm, o_hbm,
            h_ref, xbuf, big_ref, vr_ref, dwb_ref, cv_ref, w1t_ref, w2s_ref, bias_ref, zs_ref,
            xsem, osem, psem, wsem):

    for i in range(6):
        zs_ref[i] = 0

    def x_copy(j, sl):
        return pltpu.make_async_copy(x_hbm.at[pl.ds(j * G2, G2)], xbuf.at[sl], xsem.at[sl])

    def phase1(gb_ref):
        xn_ref = big_ref
        vi = lambda u, g, q, v: ((u * 12 + g) * NQ + q) * 3 + v
        xp = xbuf.reshape(NB * 4, C // 8, 16, W)

        def rows_copy(u, n, half, i, sem):
            return pltpu.make_async_copy(x5_hbm.at[pl.ds(u - 1 + half, n), 1 - half],
                                         xp.at[pl.ds(i, n), :, pl.ds(8 * half, 8), :], psem.at[sem])

        def start_slot(u, sl, sem, rows=range(8)):
            for i in rows:
                pltpu.make_async_copy(x5_hbm.at[u + i // 2 - 1 + i % 2, 1 - i % 2],
                                      xp.at[4 * sl + i // 2, :, pl.ds(8 * (i % 2), 8), :], psem.at[sem]).start()

        def wait_for(buf, sem):
            pltpu.make_async_copy(buf, buf, psem.at[sem]).wait()

        lane = _iota((8, 128), 1)

        def shift_unit(xu_ref, u):
            for g in range(12):
                for q, vs in _shifted(pltpu.bitcast(xu_ref[g], u32), lane):
                    for v in range(3):
                        vr_ref[0, vi(u, g, q, v)] = vs[v]

        def conv_round(t, q, gs):
            cvs = []
            for g in gs:
                rhs = jnp.concatenate([vr_ref[0, vi(uu & 1, g, q, v)] for uu in (t, t + 1) for v in range(3)], axis=0)
                lhs = pltpu.bitcast(vr_ref[0, CL0 + g, :, 0:C], bf16)
                cvs.append(jnp.dot(lhs, pltpu.bitcast(rhs, bf16), preferred_element_type=f32))
            return cvs

        sub = _iota((8, 128), 0)
        m0 = sub % 2 == 0
        m1 = (sub // 2) % 2 == 0
        lnc = jnp.where(m1, 1.0 / (C * _A), 1.0 / (C * _A * _A))

        def ln_tile(cvs, q, dsts):
            ls = slice(128 * q, 128 * q + 128)
            cs = [[cv[8 * ab:8 * ab + 8] for cv in cvs] for ab in range(2)]
            c1 = _merge(_tree_sum(cs[0]), _tree_sum(cs[1]), m0, 1)
            c2 = _merge(_tree_sum([c * c for c in cs[0]]), _tree_sum([c * c for c in cs[1]]), m0, 1)
            e = _merge(c1, c2, m1, 2)
            f = (e + pltpu.roll(e, 4, 0)) * lnc
            v = pltpu.roll(f, 6, 0) - f * f
            rs = lax.rsqrt(jnp.maximum(v, 0.0) + _EPS)
            for ab in range(2):
                xn_ref[pl.ds(dsts[ab], 1), :, ls] = _pack(jnp.concatenate(cs[ab], axis=0) * rs[ab:ab + 1, :])

        def setup(dw_ref, g_ref, b_ref):
            w1_ref = xbuf.at[3, 0, :, pl.ds(0, E)]
            w2t_ref = xbuf.at[3, 1, :, pl.ds(0, E)]
            small = [pltpu.make_async_copy(a, b, wsem.at[i]) for i, (a, b) in enumerate(
                [(dw_hbm, dw_ref), (w1_hbm, w1_ref), (w2t_hbm, w2t_ref), (g_hbm, g_ref), (b_hbm, b_ref)])]
            for cp in small[:2]:
                cp.start()
            rows_copy(1, 2, 0, 17, 1).start()
            rows_copy(0, 3, 1, 16, 1).start()
            rows_copy(3, 4, 0, 0, 0).start()
            rows_copy(3, 4, 1, 0, 0).start()
            for cp in small[2:]:
                cp.start()
            small[0].wait()

            vr_ref[0, ACC0:CL0] = jnp.zeros((E // 8, 8, 128), u32)
            dw = dw_ref[...].astype(f32)
            dif = _iota((8, C), 1) - _iota((8, C), 0)
            row = _iota((16, C), 0)
            col = _iota((16, C), 1)
            unit = jnp.where(col >= 48, 1, 0)
            itap = 2 * unit + ((col >> 3) & 1) - (row >> 3)
            tapid = jnp.where((col & 7) == (row & 7), 3 * itap + ((col - 48 * unit) >> 4), -9)
            for g in range(12):
                cl = jnp.zeros((16, C), f32)
                for t in range(9):
                    dwt = jnp.broadcast_to(dw[t // 3, t % 3:t % 3 + 1, :], (8, C))
                    dwc = jnp.sum(jnp.where(dif == 8 * g, dwt, 0.0), axis=1, keepdims=True)
                    dwb_ref[0, g, t] = jnp.broadcast_to(dwc, (8, 128))
                    cb = jnp.broadcast_to(dwc, (8, C))
                    cl = jnp.where(tapid == t, jnp.concatenate([cb, cb], axis=0), cl)
                vr_ref[0, CL0 + g, :, 0:C] = pltpu.bitcast(cl.astype(bf16), u32)

            small[1].wait()
            w1f = w1_ref[...].astype(f32)
            w1c = (w1f - jnp.sum(w1f, axis=0, keepdims=True) * (1.0 / C)).astype(bf16)
            for i in range(3):
                eye = jnp.where(_iota((128, E), 0) + 128 * i == _iota((128, E), 1), 1.0, 0.0).astype(bf16)
                w1t = lax.dot_general(eye, w1c, (((1,), (1,)), ((), ())), preferred_element_type=f32)
                w1t_ref[64 * i:64 * i + 64, :] = pltpu.bitcast(w1t.astype(bf16), u32)

            xp[16, :, 0:8, :] = jnp.zeros((12, 8, W), bf16)
            rows_copy(1, 2, 0, 17, 1).wait()
            rows_copy(0, 3, 1, 16, 1).wait()
            shift_unit(xp.at[16], 0)
            shift_unit(xp.at[17], 1)
            for q in range(NQ):
                ln_tile(conv_round(0, q, range(12)), q, (0, 1))
            shift_unit(xp.at[18], 0)
            for q in range(2):
                ln_tile(conv_round(1, q, range(12)), q, (8, 9))

            for cp in small[2:]:
                cp.wait()
            w2s_ref[...] = pltpu.bitcast(w2t_ref[...], u32)
            gb_ref[0:1, :] = g_ref[...].astype(f32).reshape(1, E)
            gb_ref[1:2, :] = b_ref[...].astype(f32).reshape(1, E)

        pl.run_scoped(setup, pltpu.VMEM((3, 3, C), bf16), pltpu.VMEM((E,), bf16), pltpu.VMEM((E,), bf16))

        nxt = lambda sl: jnp.where(sl == NB - 1, 0, sl + 1)
        NI = H // 32

        def block(g0, slots, prefetch, keep=0):
            z = zs_ref[0]
            z1 = zs_ref[1]
            xslot = lambda k: k + keep if k in RC else k % 8
            pend = []
            cur = []

            def conv_step(p, r):
                for rr in range(12):
                    if not sum(RD[:r]) <= rr < sum(RD[:r + 1]):
                        continue
                    q = (rr // 3 + 2) % 4
                    pair = p + 1 + (rr >= 6)
                    cur.extend(conv_round(pair, q, range(4 * (rr % 3), 4 * (rr % 3) + 4)))
                    if rr % 3 == 2:
                        pend.append((p * NP + r + LN_LAG, list(cur), q, (xslot(2 * pair) + z1, xslot(2 * pair + 1) + z1)))
                        cur.clear()

            npair = 4 * len(slots)
            for p in range(npair):
                for r in range(NP):
                    gr = p * NP + r
                    c = r % NSUB
                    M0, MR = sum(CH[:c]), CH[c]
                    k = 2 * p + r // NSUB
                    last = gr == npair * NP - 1
                    if last:
                        conv_step(p, r)
                    if p % 4 == 0 and r == 1:
                        prefetch(p // 4)
                    while pend and pend[0][0] <= gr:
                        ln_tile(*pend.pop(0)[1:])
                    xn = pltpu.bitcast(xn_ref[xslot(k) + z], bf16)
                    lhs = pltpu.bitcast(w1t_ref[M0 // 2:(M0 + MR) // 2, :], bf16)
                    gl = _gelu2(jnp.dot(lhs, xn, preferred_element_type=f32))
                    if k % G2 in ST:
                        hs = (g0 + k // G2) * NST + ST.index(k % G2)
                        h_ref[pl.ds(hs, 1), M0 // 2:(M0 + MR) // 2, :] = _pack(gl)
                    sq = gl * gl
                    for i in range(MR // 8):
                        ai = ACC0 + M0 // 8 + i
                        sr = [sq[8 * i:8 * i + 8, 128 * q:128 * q + 128] for q in range(NQ)]
                        acc = (pltpu.bitcast(vr_ref[0, ai], f32) + sr[0]) + ((sr[1] + sr[2]) + sr[3])
                        vr_ref[0, ai] = pltpu.bitcast(acc, u32)
                    if not last:
                        conv_step(p, r)
                    if r == NP // 2 - 1:
                        shift_unit(xp.at[4 * slots[p // 4] + p % 4], (p + 3) % 2)
            for e in pend:
                ln_tile(*e[1:])

        def body_a(j, carry):
            wait_for(xp.at[pl.ds(4 * j, 4)], j & 1)

            def prefetch(n):
                @pl.when(j < 3)
                def _():
                    start_slot(7 + 4 * j, j + 1, 1 - (j & 1))
                start_slot(19 + 4 * j, jnp.where(j == 0, 4, j - 1), 2)

            block(j, [j], prefetch, jnp.where(j == 0, 8 - RC[0], 0))
            return carry

        def body_b(jj, s0):
            slots = [s0]
            for _ in range(4):
                slots.append(nxt(slots[-1]))
            sem = 2 * (jj & 1)

            @pl.when(jj < NI - 1)
            def _():
                wait_for(xp.at[pl.ds(0, 16)], sem)

            @pl.when(jj == NI - 1)
            def _():
                wait_for(xp.at[pl.ds(0, 13)], sem)
                wait_for(xp.at[13, :, pl.ds(0, 8), :], sem)
                xp[4 * slots[3] + 1, :, 8:16, :] = jnp.zeros((12, 8, W), bf16)

            def prefetch(n):
                dst = slots[(n + 4) % 5]

                @pl.when(jj < NI - 1)
                def _():
                    start_slot(16 * jj + 19 + 4 * n, dst, 2 - sem, range(3) if n == 3 else range(8))

                if n == 3:
                    @pl.when(jj < NI - 2)
                    def _():
                        start_slot(16 * jj + 19 + 4 * n, dst, 2 - sem, range(3, 8))
                else:
                    @pl.when(jj == NI - 1)
                    def _():
                        x_copy(n, (S0 + n) % NB).start()

            block(4 * jj, slots[:4], prefetch)
            return slots[4]

        lax.fori_loop(0, 4, body_a, 0)
        lax.fori_loop(1, NI, body_b, jnp.int32(4))

        pdif = _iota((8, E), 1) - _iota((8, E), 0) + zs_ref[0]
        parts = []
        for i in range(E // 8):
            col = jnp.sum(pltpu.bitcast(vr_ref[0, ACC0 + i], f32), axis=1, keepdims=True)
            parts.append(jnp.where(pdif == 8 * i, jnp.broadcast_to(col, (8, E)), 0.0))
        ss = jnp.sum(_tree_sum(parts), axis=0, keepdims=True) * (_GS * _GS)
        gx = jnp.sqrt(ss + 1e-6)
        nx = gx / (jnp.sum(gx, axis=1, keepdims=True) * (1.0 / E) + 1e-6)
        s = (gb_ref[0:1, :] * nx + 1.0) * _GS
        w2t = pltpu.bitcast(w2s_ref[...], bf16).astype(f32)
        w2s_ref[...] = pltpu.bitcast((w2t * s).astype(bf16), u32)
        bias_ref[...] = jnp.broadcast_to(jnp.sum(w2t * gb_ref[1:2, :], axis=1, keepdims=True), (C, 128))

    pl.run_scoped(phase1, pltpu.VMEM((8, E), f32))

    def phase2(zv_ref):
        zv_ref[...] = jnp.zeros(zv_ref.shape, u32)
        vi = lambda q, k, i: (q * 6 + k) * 3 * (NR + 2) + i

        def o_copy(j, sl, r0, n):
            return pltpu.make_async_copy(xbuf.at[sl, pl.ds(r0, n)], o_hbm.at[pl.ds(j * G2 + r0, n)], osem.at[sl])

        z0 = zs_ref[0]
        lane = _iota((8, 128), 1) + z0
        sub = _iota((8, 128), 0) + z0
        m0 = (sub & 1) == 0
        m1 = (sub & 2) == 0
        m2 = sub < 4
        lnc = jnp.where(m2, 1.0 / (C * _A), 1.0 / (C * _A * _A))

        def shift_rows(xs, zv):
            for r in range(NR + 2):
                for k in range(6):
                    m = pltpu.bitcast(xbuf[xs, RC[0] - 1 + r, 16 * k:16 * k + 16, :], u32)
                    for q, vs in _shifted(m, lane):
                        for v in range(3):
                            vr_ref[zv, vi(q, k, 3 * r + v)] = vs[v]

        def conv_tile(q, zc, zw, zr):
            st = [None] * NR
            tok = yield None
            for g in range(12):
                w = [dwb_ref[zw, g, t] for t in range(9)]
                acc = [None] * NR
                for r in range(NR + 2):
                    for v in range(3):
                        x = vr_ref[zw, vi(q, g // 2, 3 * r + v)]
                        if v == 2:
                            x = x | tok
                        xf = pltpu.bitcast(x, bf16).astype(f32)[8 * (g % 2):8 * (g % 2) + 8]
                        for n in range(NR):
                            if 0 <= r - n <= 2:
                                t = xf * w[3 * (r - n) + v]
                                acc[n] = t if acc[n] is None else acc[n] + t
                for n in range(NR):
                    cv = acc[n]
                    st[n] = (cv, cv * cv) if st[n] is None else (st[n][0] + cv, st[n][1] + cv * cv)
                    cv_ref[zc, 12 * n + g] = cv
                tok = yield pltpu.bitcast((acc[0] + acc[1]) + acc[2], u32)
            half = lambda i: _merge(_merge(st[0][i], st[1][i], m0, 1), st[2][i] + pltpu.roll(st[2][i], 7, 0), m1, 2)
            f = _merge(half(0), half(1), m2, 4) * lnc
            v = pltpu.roll(f, 4, 0) - f * f
            cv_ref[zr, 36] = lax.rsqrt(jnp.maximum(v, 0.0) + _EPS)
            for n in range(NR):
                rs = cv_ref[zc, 36, n:n + 1, :]
                big_ref[pl.ds(8 + n + zc, 1), :, 128 * q:128 * q + 128] = _pack(
                    cv_ref[zc, 12 * n:12 * n + 12].reshape(C, 128) * rs)
            yield None

        x_copy(0, S0).wait()
        nxt = lambda sl: jnp.where(sl == NB - 1, 0, sl + 1)

        def body(j, xs):
            z = zs_ref[0]
            xs1 = nxt(xs)
            xs3 = nxt(nxt(xs1))

            @pl.when(j + 1 < NG2)
            def _():
                x_copy(j + 1, xs1).wait()

            @pl.when(j >= 2)
            def _():
                o_copy(j - 2, xs3, 0, G2).wait()

            @pl.when(j + 3 < NG2)
            def _():
                x_copy(j + 3, xs3).start()

            tiles = [conv_tile(q, z, zs_ref[2 + q], zs_ref[1]) for q in range(NQ)]
            for t in tiles:
                next(t)
            shift_rows(xs1, z)
            zv = zv_ref[...]
            state = dict(slot=0, piece=0, tok=None)

            def run_pieces(rel):
                res = None
                for _ in range(PLAN[state['slot']]):
                    t = tiles[state['piece'] // 12]
                    val = t.send(rel)
                    res = val if res is None else res | val
                    state['piece'] += 1
                    if state['piece'] % 12 == 0:
                        t.send(None)
                state['slot'] += 1
                state['tok'] = res

            def gate(d):
                if state['tok'] is None:
                    return d
                du = pltpu.bitcast(d[40:48, 384:512], u32) | (state['tok'] & zv)
                last = jnp.concatenate([d[40:48, 0:384], pltpu.bitcast(du, f32)], axis=1)
                return jnp.concatenate([d[0:40], last], axis=0)

            def fin(k, hr):
                for mc in range(2):
                    rs_ = slice(48 * mc, 48 * (mc + 1))
                    o = None
                    for kt in range(3):
                        d = jnp.dot(pltpu.bitcast(w2s_ref[24 * mc:24 * (mc + 1), 128 * kt:128 * kt + 128], bf16),
                                    pltpu.bitcast(hr(kt), bf16), preferred_element_type=f32)
                        rel = pltpu.bitcast(d[0:8, 0:128], u32) & zv
                        d = gate(d)
                        o = d if o is None else o + d
                        if kt == 2:
                            bias = jnp.concatenate([bias_ref[rs_, :]] * NQ, axis=1)
                            xbuf[xs, k, rs_, :] = (o + bias + xbuf[xs, k, rs_, :].astype(f32)).astype(bf16)
                        run_pieces(rel)

            def kept_rows(n, kt):
                return h_ref[j * NST + n, 64 * kt:64 * kt + 64, :]

            def temp_rows(n, kt):
                return jnp.concatenate([big_ref[4 * (n % 2) + z + r // 48, r % 48:r % 48 + 8, :]
                                        for r in range(64 * kt, 64 * kt + 64, 8)], axis=0)

            for op in P2ORD:
                n = int(op[1])
                if op[0] == 'M':
                    assert state['piece'] < 12
                    xn = pltpu.bitcast(big_ref[8 + n + z], bf16)
                    y = jnp.dot(pltpu.bitcast(w1t_ref[...], bf16), xn, preferred_element_type=f32)
                    big_ref[pl.ds(4 * (n % 2) + z, 4)] = _pack(_gelu2(y), 4)
                elif op[0] == 'S':
                    fin(ST[n], functools.partial(kept_rows, n))
                elif op[0] == 'F':
                    fin(RC[n], functools.partial(temp_rows, n))
                else:
                    o_copy(j, xs, n, int(op[2]) - n).start()
            assert state['piece'] == 12 * NQ
            return xs1

        lax.fori_loop(0, NG2, body, jnp.int32(S0))
        for j in range(NG2 - 2, NG2):
            o_copy(j, (j + S0) % NB, 0, G2).wait()

    pl.run_scoped(phase2, pltpu.VMEM((8, 128), u32))


@jax.jit
def pallas_standalone__modern_conv_block_convnext_v2__vision_kernel(x, dw, w1, w2, grn_gamma, grn_beta):
    xt = jnp.transpose(x, (0, 1, 3, 2)).reshape(H, C, W)
    x5 = xt.reshape(H // 2, 2, C // 8, 8, W)
    out = pl.pallas_call(
        _kernel,
        in_specs=[pl.BlockSpec(memory_space=pl.ANY)] * 7,
        out_specs=pl.BlockSpec(memory_space=pl.ANY),
        out_shape=jax.ShapeDtypeStruct((H, C, W), bf16),
        scratch_shapes=[
            pltpu.VMEM((NG2 * NST, E // 2, W), u32),
            pltpu.VMEM((NB, G2, C, W), bf16),
            pltpu.VMEM((8 + NR, C // 2, W), u32),
            pltpu.VMEM((1, NVR, 8, 128), u32),
            pltpu.VMEM((1, 12, 9, 8, 128), f32),
            pltpu.VMEM((1, 40, 8, 128), f32),
            pltpu.VMEM((E // 2, C), u32),
            pltpu.VMEM((C // 2, E), u32),
            pltpu.VMEM((C, 128), f32),
            pltpu.SMEM((6,), i32),
            pltpu.SemaphoreType.DMA((NB,)),
            pltpu.SemaphoreType.DMA((NB,)),
            pltpu.SemaphoreType.DMA((3,)),
            pltpu.SemaphoreType.DMA((5,)),
        ],
        compiler_params=pltpu.CompilerParams(vmem_limit_bytes=128 * 1024 * 1024,
                                             disable_bounds_checks=True),
    )(xt, x5, dw, w1, w2.T, grn_gamma, grn_beta)
    return jnp.transpose(out.reshape(1, H, C, W), (0, 1, 3, 2))
```

```python
import functools
import math

import jax
import jax.numpy as jnp
from jax import lax
import jax.experimental.pallas as pl
import jax.experimental.pallas.tpu as pltpu

H, W, C, E = 512, 512, 96, 384
NQ = W // 128
G2 = 8
NG2 = H // G2
RC = (2, 3, 4)
ST = tuple(k for k in range(G2) if k not in RC)
NST = len(ST)
NR = len(RC)
NVR = NQ * 6 * 3 * (NR + 2)
ACC0 = 2 * 12 * NQ * 3
CL0 = ACC0 + E // 8
NB = 5
S0 = 4
CH = (128, 64, 128, 64)
RD = (2, 1, 2, 1) * 2
NSUB = len(CH)
NP = 2 * NSUB
LN_LAG = 3
P2ORD = 'M0,M1,F0,M2,S0,F1,S1,o04,F2,S2,o46,S3,S4,o68'.split(',')
PLAN = [2, 2] + [1] * 44 + [0, 0]

_C1 = math.sqrt(2.0 / math.pi)
_A = (_C1 * 0.044715) ** (1.0 / 3.0)
_K = _C1 / _A
_GS = 0.5 / _A
_EPS = 1e-5 / (_A * _A)

f32 = jnp.float32
bf16 = jnp.bfloat16
u32 = jnp.uint32
i32 = jnp.int32


def _iota(shape, d):
    return lax.broadcasted_iota(i32, shape, d)


def _pack(y, n=1):
    return pltpu.bitcast(y.reshape(n, y.shape[0] // n, y.shape[1]).astype(bf16), u32)


def _gelu2(y):
    return y * (jnp.tanh(y * (y * y + _K)) + 1.0)


def _rsqrt(v):
    return jnp.exp2((-0.5 / math.log(2.0)) * jnp.log(v))


def _tree_sum(xs):
    xs = list(xs)
    while len(xs) > 1:
        xs = [xs[i] + xs[i + 1] for i in range(0, len(xs) - 1, 2)] + ([xs[-1]] if len(xs) % 2 else [])
    return xs[0]


def _merge(a, b, msk, sh):
    return jnp.where(msk, a, b) + pltpu.roll(jnp.where(msk, b, a), 8 - sh, 0)


def _shifted(m, lane):
    zz = jnp.zeros((8, 128), u32)
    mq = [m[:, 128 * q:128 * q + 128] for q in range(NQ)]
    for q in range(NQ):
        lq = jnp.where(lane == 127, mq[q - 1] if q > 0 else zz, mq[q])
        rq = jnp.where(lane == 0, mq[q + 1] if q + 1 < NQ else zz, mq[q])
        yield q, (pltpu.roll(lq, 1, 1), mq[q], pltpu.roll(rq, 127, 1))


def _kernel(x_hbm, x5_hbm, dw_hbm, w1_hbm, w2t_hbm, g_hbm, b_hbm, o_hbm,
            h_ref, xbuf, big_ref, vr_ref, dwb_ref, cv_ref, w1t_ref, w2s_ref, bias_ref, zs_ref,
            xsem, osem, psem, wsem):

    for i in range(6):
        zs_ref[i] = 0

    def x_copy(j, sl):
        return pltpu.make_async_copy(x_hbm.at[pl.ds(j * G2, G2)], xbuf.at[sl], xsem.at[sl])

    def phase1(gb_ref):
        xn_ref = big_ref
        vi = lambda u, g, q, v: ((u * 12 + g) * NQ + q) * 3 + v
        xp = xbuf.reshape(NB * 4, C // 8, 16, W)

        def rows_copy(u, n, half, i, sem):
            return pltpu.make_async_copy(x5_hbm.at[pl.ds(u - 1 + half, n), 1 - half],
                                         xp.at[pl.ds(i, n), :, pl.ds(8 * half, 8), :], psem.at[sem])

        def start_slot(u, sl, sem, rows=range(8)):
            for i in rows:
                pltpu.make_async_copy(x5_hbm.at[u + i // 2 - 1 + i % 2, 1 - i % 2],
                                      xp.at[4 * sl + i // 2, :, pl.ds(8 * (i % 2), 8), :], psem.at[sem]).start()

        def wait_for(buf, sem):
            pltpu.make_async_copy(buf, buf, psem.at[sem]).wait()

        lane = _iota((8, 128), 1)

        def shift_unit(xu_ref, u):
            for g in range(12):
                for q, vs in _shifted(pltpu.bitcast(xu_ref[g], u32), lane):
                    for v in range(3):
                        vr_ref[0, vi(u, g, q, v)] = vs[v]

        def conv_round(t, q, gs):
            cvs = []
            for g in gs:
                rhs = jnp.concatenate([vr_ref[0, vi(uu & 1, g, q, v)] for uu in (t, t + 1) for v in range(3)], axis=0)
                lhs = pltpu.bitcast(vr_ref[0, CL0 + g, :, 0:C], bf16)
                cvs.append(jnp.dot(lhs, pltpu.bitcast(rhs, bf16), preferred_element_type=f32))
            return cvs

        sub = _iota((8, 128), 0)
        m0 = sub % 2 == 0
        m1 = (sub // 2) % 2 == 0
        lnc = jnp.where(m1, 1.0 / (C * _A), 1.0 / (C * _A * _A))

        def ln_tile(cvs, q, dsts):
            ls = slice(128 * q, 128 * q + 128)
            cs = [[cv[8 * ab:8 * ab + 8] for cv in cvs] for ab in range(2)]
            c1 = _merge(_tree_sum(cs[0]), _tree_sum(cs[1]), m0, 1)
            c2 = _merge(_tree_sum([c * c for c in cs[0]]), _tree_sum([c * c for c in cs[1]]), m0, 1)
            e = _merge(c1, c2, m1, 2)
            f = (e + pltpu.roll(e, 4, 0)) * lnc
            v = pltpu.roll(f, 6, 0) - f * f
            rs = _rsqrt(jnp.maximum(v, 0.0) + _EPS)
            for ab in range(2):
                xn_ref[pl.ds(dsts[ab], 1), :, ls] = _pack(jnp.concatenate(cs[ab], axis=0) * rs[ab:ab + 1, :])

        def setup(dw_ref, g_ref, b_ref):
            w1_ref = xbuf.at[3, 0, :, pl.ds(0, E)]
            w2t_ref = xbuf.at[3, 1, :, pl.ds(0, E)]
            small = [pltpu.make_async_copy(a, b, wsem.at[i]) for i, (a, b) in enumerate(
                [(dw_hbm, dw_ref), (w1_hbm, w1_ref), (w2t_hbm, w2t_ref), (g_hbm, g_ref), (b_hbm, b_ref)])]
            for cp in small[:2]:
                cp.start()
            rows_copy(1, 2, 0, 17, 1).start()
            rows_copy(0, 3, 1, 16, 1).start()
            rows_copy(3, 4, 0, 0, 0).start()
            rows_copy(3, 4, 1, 0, 0).start()
            for cp in small[2:]:
                cp.start()
            small[0].wait()

            vr_ref[0, ACC0:CL0] = jnp.zeros((E // 8, 8, 128), u32)
            dw = dw_ref[...].astype(f32)
            dif = _iota((8, C), 1) - _iota((8, C), 0)
            row = _iota((16, C), 0)
            col = _iota((16, C), 1)
            unit = jnp.where(col >= 48, 1, 0)
            itap = 2 * unit + ((col >> 3) & 1) - (row >> 3)
            tapid = jnp.where((col & 7) == (row & 7), 3 * itap + ((col - 48 * unit) >> 4), -9)
            for g in range(12):
                cl = jnp.zeros((16, C), f32)
                for t in range(9):
                    dwt = jnp.broadcast_to(dw[t // 3, t % 3:t % 3 + 1, :], (8, C))
                    dwc = jnp.sum(jnp.where(dif == 8 * g, dwt, 0.0), axis=1, keepdims=True)
                    dwb_ref[0, g, t] = jnp.broadcast_to(dwc, (8, 128))
                    cb = jnp.broadcast_to(dwc, (8, C))
                    cl = jnp.where(tapid == t, jnp.concatenate([cb, cb], axis=0), cl)
                vr_ref[0, CL0 + g, :, 0:C] = pltpu.bitcast(cl.astype(bf16), u32)

            small[1].wait()
            w1f = w1_ref[...].astype(f32)
            w1c = (w1f - jnp.sum(w1f, axis=0, keepdims=True) * (1.0 / C)).astype(bf16)
            for i in range(3):
                eye = jnp.where(_iota((128, E), 0) + 128 * i == _iota((128, E), 1), 1.0, 0.0).astype(bf16)
                w1t = lax.dot_general(eye, w1c, (((1,), (1,)), ((), ())), preferred_element_type=f32)
                w1t_ref[64 * i:64 * i + 64, :] = pltpu.bitcast(w1t.astype(bf16), u32)

            xp[16, :, 0:8, :] = jnp.zeros((12, 8, W), bf16)
            rows_copy(1, 2, 0, 17, 1).wait()
            rows_copy(0, 3, 1, 16, 1).wait()
            shift_unit(xp.at[16], 0)
            shift_unit(xp.at[17], 1)
            for q in range(NQ):
                ln_tile(conv_round(0, q, range(12)), q, (0, 1))
            shift_unit(xp.at[18], 0)
            for q in range(2):
                ln_tile(conv_round(1, q, range(12)), q, (8, 9))

            for cp in small[2:]:
                cp.wait()
            w2s_ref[...] = pltpu.bitcast(w2t_ref[...], u32)
            gb_ref[0:1, :] = g_ref[...].astype(f32).reshape(1, E)
            gb_ref[1:2, :] = b_ref[...].astype(f32).reshape(1, E)

        pl.run_scoped(setup, pltpu.VMEM((3, 3, C), bf16), pltpu.VMEM((E,), bf16), pltpu.VMEM((E,), bf16))

        nxt = lambda sl: jnp.where(sl == NB - 1, 0, sl + 1)
        NI = H // 32

        def block(g0, slots, prefetch, keep=0):
            z = zs_ref[0]
            z1 = zs_ref[1]
            xslot = lambda k: k + keep if k in RC else k % 8
            pend = []
            cur = []

            def conv_step(p, r):
                for rr in range(12):
                    if not sum(RD[:r]) <= rr < sum(RD[:r + 1]):
                        continue
                    q = (rr // 3 + 2) % 4
                    pair = p + 1 + (rr >= 6)
                    cur.extend(conv_round(pair, q, range(4 * (rr % 3), 4 * (rr % 3) + 4)))
                    if rr % 3 == 2:
                        pend.append((p * NP + r + LN_LAG, list(cur), q, (xslot(2 * pair) + z1, xslot(2 * pair + 1) + z1)))
                        cur.clear()

            npair = 4 * len(slots)
            for p in range(npair):
                for r in range(NP):
                    gr = p * NP + r
                    c = r % NSUB
                    M0, MR = sum(CH[:c]), CH[c]
                    k = 2 * p + r // NSUB
                    last = gr == npair * NP - 1
                    if last:
                        conv_step(p, r)
                    if p % 4 == 0 and r == 1:
                        prefetch(p // 4)
                    while pend and pend[0][0] <= gr:
                        ln_tile(*pend.pop(0)[1:])
                    xn = pltpu.bitcast(xn_ref[xslot(k) + z], bf16)
                    lhs = pltpu.bitcast(w1t_ref[M0 // 2:(M0 + MR) // 2, :], bf16)
                    gl = _gelu2(jnp.dot(lhs, xn, preferred_element_type=f32))
                    if k % G2 in ST:
                        hs = (g0 + k // G2) * NST + ST.index(k % G2)
                        h_ref[pl.ds(hs, 1), M0 // 2:(M0 + MR) // 2, :] = _pack(gl)
                    sq = gl * gl
                    for i in range(MR // 8):
                        ai = ACC0 + M0 // 8 + i
                        sr = [sq[8 * i:8 * i + 8, 128 * q:128 * q + 128] for q in range(NQ)]
                        acc = pltpu.bitcast(vr_ref[0, ai], f32) + ((sr[0] + sr[1]) + (sr[2] + sr[3]))
                        vr_ref[0, ai] = pltpu.bitcast(acc, u32)
                    if not last:
                        conv_step(p, r)
                    if r == NP // 2 - 1:
                        shift_unit(xp.at[4 * slots[p // 4] + p % 4], (p + 3) % 2)
            for e in pend:
                ln_tile(*e[1:])

        def body_a(j, carry):
            wait_for(xp.at[pl.ds(4 * j, 4)], j & 1)

            def prefetch(n):
                @pl.when(j < 3)
                def _():
                    start_slot(7 + 4 * j, j + 1, 1 - (j & 1))
                start_slot(19 + 4 * j, jnp.where(j == 0, 4, j - 1), 2)

            block(j, [j], prefetch, jnp.where(j == 0, 8 - RC[0], 0))
            return carry

        def body_b(jj, s0):
            slots = [s0]
            for _ in range(4):
                slots.append(nxt(slots[-1]))
            sem = 2 * (jj & 1)

            @pl.when(jj < NI - 1)
            def _():
                wait_for(xp.at[pl.ds(0, 16)], sem)

            @pl.when(jj == NI - 1)
            def _():
                wait_for(xp.at[pl.ds(0, 13)], sem)
                wait_for(xp.at[13, :, pl.ds(0, 8), :], sem)
                xp[4 * slots[3] + 1, :, 8:16, :] = jnp.zeros((12, 8, W), bf16)

            def prefetch(n):
                dst = slots[(n + 4) % 5]

                @pl.when(jj < NI - 1)
                def _():
                    start_slot(16 * jj + 19 + 4 * n, dst, 2 - sem, range(3) if n == 3 else range(8))

                if n == 3:
                    @pl.when(jj < NI - 2)
                    def _():
                        start_slot(16 * jj + 19 + 4 * n, dst, 2 - sem, range(3, 8))
                else:
                    @pl.when(jj == NI - 1)
                    def _():
                        x_copy(n, (S0 + n) % NB).start()

            block(4 * jj, slots[:4], prefetch)
            return slots[4]

        lax.fori_loop(0, 4, body_a, 0)
        lax.fori_loop(1, NI, body_b, jnp.int32(4))

        pdif = _iota((8, E), 1) - _iota((8, E), 0) + zs_ref[0]
        parts = []
        for i in range(E // 8):
            col = jnp.sum(pltpu.bitcast(vr_ref[0, ACC0 + i], f32), axis=1, keepdims=True)
            parts.append(jnp.where(pdif == 8 * i, jnp.broadcast_to(col, (8, E)), 0.0))
        ss = jnp.sum(_tree_sum(parts), axis=0, keepdims=True) * (_GS * _GS)
        gx = jnp.sqrt(ss + 1e-6)
        nx = gx / (jnp.sum(gx, axis=1, keepdims=True) * (1.0 / E) + 1e-6)
        s = (gb_ref[0:1, :] * nx + 1.0) * _GS
        w2t = pltpu.bitcast(w2s_ref[...], bf16).astype(f32)
        w2s_ref[...] = pltpu.bitcast((w2t * s).astype(bf16), u32)
        bias_ref[...] = jnp.broadcast_to(jnp.sum(w2t * gb_ref[1:2, :], axis=1, keepdims=True), (C, 128))

    pl.run_scoped(phase1, pltpu.VMEM((8, E), f32))

    def phase2(zv_ref):
        zv_ref[...] = jnp.zeros(zv_ref.shape, u32)
        vi = lambda q, k, i: (q * 6 + k) * 3 * (NR + 2) + i

        def o_copy(j, sl, r0, n):
            return pltpu.make_async_copy(xbuf.at[sl, pl.ds(r0, n)], o_hbm.at[pl.ds(j * G2 + r0, n)], osem.at[sl])

        z0 = zs_ref[0]
        lane = _iota((8, 128), 1) + z0
        sub = _iota((8, 128), 0) + z0
        m0 = (sub & 1) == 0
        m1 = (sub & 2) == 0
        m2 = sub < 4
        lnc = jnp.where(m2, 1.0 / (C * _A), 1.0 / (C * _A * _A))

        def shift_rows(xs, zv):
            for r in range(NR + 2):
                for k in range(6):
                    m = pltpu.bitcast(xbuf[xs, RC[0] - 1 + r, 16 * k:16 * k + 16, :], u32)
                    for q, vs in _shifted(m, lane):
                        for v in range(3):
                            vr_ref[zv, vi(q, k, 3 * r + v)] = vs[v]

        def conv_tile(q, zc, zw, zr):
            st = [None] * NR
            tok = yield None
            for g in range(12):
                w = [dwb_ref[zw, g, t] for t in range(9)]
                acc = [None] * NR
                for r in range(NR + 2):
                    for v in range(3):
                        x = vr_ref[zw, vi(q, g // 2, 3 * r + v)]
                        if v == 2:
                            x = x | tok
                        xf = pltpu.bitcast(x, bf16).astype(f32)[8 * (g % 2):8 * (g % 2) + 8]
                        for n in range(NR):
                            if 0 <= r - n <= 2:
                                t = xf * w[3 * (r - n) + v]
                                acc[n] = t if acc[n] is None else acc[n] + t
                for n in range(NR):
                    cv = acc[n]
                    st[n] = (cv, cv * cv) if st[n] is None else (st[n][0] + cv, st[n][1] + cv * cv)
                    cv_ref[zc, 12 * n + g] = cv
                tok = yield pltpu.bitcast((acc[0] + acc[1]) + acc[2], u32)
            half = lambda i: _merge(_merge(st[0][i], st[1][i], m0, 1), st[2][i] + pltpu.roll(st[2][i], 7, 0), m1, 2)
            f = _merge(half(0), half(1), m2, 4) * lnc
            v = pltpu.roll(f, 4, 0) - f * f
            cv_ref[zr, 36] = lax.rsqrt(jnp.maximum(v, 0.0) + _EPS)
            for n in range(NR):
                rs = cv_ref[zc, 36, n:n + 1, :]
                big_ref[pl.ds(8 + n + zc, 1), :, 128 * q:128 * q + 128] = _pack(
                    cv_ref[zc, 12 * n:12 * n + 12].reshape(C, 128) * rs)
            yield None

        x_copy(0, S0).wait()
        nxt = lambda sl: jnp.where(sl == NB - 1, 0, sl + 1)

        def body(j, xs):
            z = zs_ref[0]
            xs1 = nxt(xs)
            xs3 = nxt(nxt(xs1))

            @pl.when(j + 1 < NG2)
            def _():
                x_copy(j + 1, xs1).wait()

            @pl.when(j >= 2)
            def _():
                o_copy(j - 2, xs3, 0, G2).wait()

            @pl.when(j + 3 < NG2)
            def _():
                x_copy(j + 3, xs3).start()

            tiles = [conv_tile(q, z, zs_ref[2 + q], zs_ref[1]) for q in range(NQ)]
            for t in tiles:
                next(t)
            shift_rows(xs1, z)
            zv = zv_ref[...]
            state = dict(slot=0, piece=0, tok=None)

            def run_pieces(rel):
                res = None
                for _ in range(PLAN[state['slot']]):
                    t = tiles[state['piece'] // 12]
                    val = t.send(rel)
                    res = val if res is None else res | val
                    state['piece'] += 1
                    if state['piece'] % 12 == 0:
                        t.send(None)
                state['slot'] += 1
                state['tok'] = res

            def gate(d):
                if state['tok'] is None:
                    return d
                du = pltpu.bitcast(d[40:48, 384:512], u32) | (state['tok'] & zv)
                last = jnp.concatenate([d[40:48, 0:384], pltpu.bitcast(du, f32)], axis=1)
                return jnp.concatenate([d[0:40], last], axis=0)

            def fin(k, hr):
                for mc in range(2):
                    rs_ = slice(48 * mc, 48 * (mc + 1))
                    o = None
                    for kt in range(3):
                        d = jnp.dot(pltpu.bitcast(w2s_ref[24 * mc:24 * (mc + 1), 128 * kt:128 * kt + 128], bf16),
                                    pltpu.bitcast(hr(kt), bf16), preferred_element_type=f32)
                        rel = pltpu.bitcast(d[0:8, 0:128], u32) & zv
                        d = gate(d)
                        o = d if o is None else o + d
                        if kt == 2:
                            bias = jnp.concatenate([bias_ref[rs_, :]] * NQ, axis=1)
                            xbuf[xs, k, rs_, :] = (o + bias + xbuf[xs, k, rs_, :].astype(f32)).astype(bf16)
                        run_pieces(rel)

            def kept_rows(n, kt):
                return h_ref[j * NST + n, 64 * kt:64 * kt + 64, :]

            def temp_rows(n, kt):
                return jnp.concatenate([big_ref[4 * (n % 2) + z + r // 48, r % 48:r % 48 + 8, :]
                                        for r in range(64 * kt, 64 * kt + 64, 8)], axis=0)

            for op in P2ORD:
                n = int(op[1])
                if op[0] == 'M':
                    assert state['piece'] < 12
                    xn = pltpu.bitcast(big_ref[8 + n + z], bf16)
                    y = jnp.dot(pltpu.bitcast(w1t_ref[...], bf16), xn, preferred_element_type=f32)
                    big_ref[pl.ds(4 * (n % 2) + z, 4)] = _pack(_gelu2(y), 4)
                elif op[0] == 'S':
                    fin(ST[n], functools.partial(kept_rows, n))
                elif op[0] == 'F':
                    fin(RC[n], functools.partial(temp_rows, n))
                else:
                    o_copy(j, xs, n, int(op[2]) - n).start()
            assert state['piece'] == 12 * NQ
            return xs1

        lax.fori_loop(0, NG2, body, jnp.int32(S0))
        for j in range(NG2 - 2, NG2):
            o_copy(j, (j + S0) % NB, 0, G2).wait()

    pl.run_scoped(phase2, pltpu.VMEM((8, 128), u32))


@jax.jit
def pallas_standalone__modern_conv_block_convnext_v2__vision_kernel(x, dw, w1, w2, grn_gamma, grn_beta):
    xt = jnp.transpose(x, (0, 1, 3, 2)).reshape(H, C, W)
    x5 = xt.reshape(H // 2, 2, C // 8, 8, W)
    out = pl.pallas_call(
        _kernel,
        in_specs=[pl.BlockSpec(memory_space=pl.ANY)] * 7,
        out_specs=pl.BlockSpec(memory_space=pl.ANY),
        out_shape=jax.ShapeDtypeStruct((H, C, W), bf16),
        scratch_shapes=[
            pltpu.VMEM((NG2 * NST, E // 2, W), u32),
            pltpu.VMEM((NB, G2, C, W), bf16),
            pltpu.VMEM((8 + NR, C // 2, W), u32),
            pltpu.VMEM((1, NVR, 8, 128), u32),
            pltpu.VMEM((1, 12, 9, 8, 128), f32),
            pltpu.VMEM((1, 40, 8, 128), f32),
            pltpu.VMEM((E // 2, C), u32),
            pltpu.VMEM((C // 2, E), u32),
            pltpu.VMEM((C, 128), f32),
            pltpu.SMEM((6,), i32),
            pltpu.SemaphoreType.DMA((NB,)),
            pltpu.SemaphoreType.DMA((NB,)),
            pltpu.SemaphoreType.DMA((3,)),
            pltpu.SemaphoreType.DMA((5,)),
        ],
        compiler_params=pltpu.CompilerParams(vmem_limit_bytes=128 * 1024 * 1024,
                                             disable_bounds_checks=True),
    )(xt, x5, dw, w1, w2.T, grn_gamma, grn_beta)
    return jnp.transpose(out.reshape(1, H, C, W), (0, 1, 3, 2))
```
